```python
import jax
import jax.numpy as jnp

def _softmax(x, axis=-1):
    return jax.nn.softmax(x, axis=axis)

def _gelu(x):
    return jax.nn.gelu(x, approximate=True)

def _silu(x):
    return jax.nn.silu(x)

def _sigmoid(x):
    return jax.nn.sigmoid(x)

def _layernorm(x, axis=-1, eps=1e-05):
    m = jnp.mean(x, axis=axis, keepdims=True)
    v = jnp.var(x, axis=axis, keepdims=True)
    return (x - m) / jnp.sqrt(v + eps)

def _scatter_add(tgt, idx, src, axis=0):
    return tgt.at[idx].add(src)

def _segment_sum(src, seg, n):
    return jax.ops.segment_sum(src, seg, n)

class _Rng:

    def __init__(self, key):
        self._k = key

    def _next(self):
        self._k, sub = jax.random.split(self._k)
        return sub

    def normal(self, shape):
        return jax.random.normal(self._next(), shape, dtype=jnp.bfloat16)

    def randint(self, lo, hi, shape):
        return jax.random.randint(self._next(), shape, lo, hi, dtype=jnp.int32)

    def uniform(self, shape, lo=0.0, hi=1.0):
        return jax.random.uniform(self._next(), shape, jnp.bfloat16, lo, hi)

    def permutation(self, n):
        return jax.random.permutation(self._next(), n)
kernel_name = 'parallel_sum__memory_aug_infini_attn__moe_arch_mod__prompt'

def setup_inputs():
    _rng = _Rng(jax.random.key(int.from_bytes(__import__("os").urandom(4), "little")))
    _w = lambda a: (lambda t: t.astype(jnp.bfloat16) if jnp.issubdtype(t.dtype, jnp.floating) else t)(jnp.asarray(a))

    def _A_setup():
        B, S, D, H = (1, 2048, 576, 32)
        N = 4
        L = max(1, S // N)
        sc = D ** (-0.5)
        return {'x': _w((lambda *s: _rng.normal(s) * 0.05)(B, N * L, D)), 'wq': _w((lambda *s: _rng.normal(s) * 0.05)(D, D) * sc), 'wk': _w((lambda *s: _rng.normal(s) * 0.05)(D, D) * sc), 'wv': _w((lambda *s: _rng.normal(s) * 0.05)(D, D) * sc), 'wo': _w((lambda *s: _rng.normal(s) * 0.05)(D, D) * sc), 'beta': _w((lambda *s: _rng.normal(s) * 0.05)(H))}
    _A_in = _A_setup()

    def _B_setup():
        B, S, D, F, C = (1, 2048, 576, 4608, 2)
        return {'x': _w((lambda *s: _rng.normal(s) * 0.05)(B, S, D)), 'w_r': _w((lambda *s: _rng.normal(s) * 0.05)(D)), 'w_gate': _w((lambda *s: _rng.normal(s) * 0.05)(D, F)), 'w_up': _w((lambda *s: _rng.normal(s) * 0.05)(D, F)), 'w_down': _w((lambda *s: _rng.normal(s) * 0.05)(F, D))}
    _B_in = _B_setup()
    return {'A_x': _A_in['x'], 'A_wq': _A_in['wq'], 'A_wk': _A_in['wk'], 'A_wv': _A_in['wv'], 'A_wo': _A_in['wo'], 'A_beta': _A_in['beta'], 'B_x': _B_in['x'], 'B_w_r': _B_in['w_r'], 'B_w_gate': _B_in['w_gate'], 'B_w_up': _B_in['w_up'], 'B_w_down': _B_in['w_down']}

def reference(A_x, A_wq, A_wk, A_wv, A_wo, A_beta, B_x, B_w_r, B_w_gate, B_w_up, B_w_down):

    def _A_ref(x, wq, wk, wv, wo, beta):
        B, S, D = x.shape
        H = 32
        Dh = D // H
        N = 4
        L = S // N
        q = (lambda x, *d: x.transpose(*d))((x @ wq).reshape(B, S, H, Dh), 0, 2, 1, 3).reshape(B, H, N, L, Dh)
        k = (lambda x, *d: x.transpose(*d))((x @ wk).reshape(B, S, H, Dh), 0, 2, 1, 3).reshape(B, H, N, L, Dh)
        v = (lambda x, *d: x.transpose(*d))((x @ wv).reshape(B, S, H, Dh), 0, 2, 1, 3).reshape(B, H, N, L, Dh)
        phi = lambda t: jnp.where(t > 0, t + 1.0, jnp.exp(t))
        scale = Dh ** (-0.5)
        ar = jnp.arange(L)
        mask = (lambda x, dt: x.astype(dt))(ar[:, None] < ar[None, :], x.dtype) * -1000000000.0
        g = _sigmoid(beta).reshape(1, H, 1, 1)
        M = jnp.einsum('bhd,bhe->bhde', q[:, :, 0, 0, :] * 0.0, q[:, :, 0, 0, :] * 0.0)
        z = q[:, :, 0, 0, :] * 0.0
        outs = []
        for s in range(N):
            qs, ks, vs = (q[:, :, s].copy(), k[:, :, s].copy(), v[:, :, s].copy())
            logits = jnp.einsum('bhqd,bhkd->bhqk', qs, ks) * scale + mask
            p = _softmax(logits, axis=-1)
            a_dot = jnp.einsum('bhqk,bhkd->bhqd', p, vs)
            pq = phi(qs)
            num = jnp.einsum('bhld,bhde->bhle', pq, M)
            den = jnp.einsum('bhld,bhd->bhl', pq, z)[..., None] + 1e-06
            a_mem = num / den
            o = g * a_mem + (1.0 - g) * a_dot
            outs.append(o)
            pk = phi(ks)
            M = M + jnp.einsum('bhld,bhle->bhde', pk, vs)
            z = z + jnp.einsum('bhld->bhd', pk)
        o = (lambda x, *d: x.transpose(*d))(jnp.stack(outs, 2).reshape(B, H, S, Dh), 0, 2, 1, 3).reshape(B, S, D)
        return o @ wo

    def _B_ref(x, w_r, w_gate, w_up, w_down):
        B, S, D = x.shape
        C = 2
        r = x @ w_r
        idx = jnp.argsort(-r, axis=-1)[:, :C]
        idx_e = jnp.repeat(idx.reshape(B, C, 1), D, axis=2)
        x_sel = jnp.take_along_axis(x, idx_e, axis=1)
        g = _silu(x_sel @ w_gate)
        u = x_sel @ w_up
        y = g * u @ w_down
        r_sel = _sigmoid(jnp.take_along_axis(r, idx, axis=1))
        y = y * r_sel.reshape(B, C, 1)
        b_off = (jnp.arange(B) * S).reshape(B, 1)
        flat_idx = (idx + b_off).reshape(B * C)
        zero = (x * 0.0).reshape(B * S, D)
        upd = _scatter_add(zero, flat_idx, y.reshape(B * C, D), axis=0)
        return x + upd.reshape(B, S, D)
    x = A_x
    xn = _layernorm(x, axis=-1)
    return x + _A_ref(xn, A_wq, A_wk, A_wv, A_wo, A_beta) + _B_ref(xn, B_w_r, B_w_gate, B_w_up, B_w_down)
```

```python
import functools
import math

import jax
import jax.numpy as jnp
from jax import lax
from jax.experimental import pallas as pl
from jax.experimental.pallas import tpu as pltpu

S, D, H, DH = 2048, 576, 32, 18
NSEG, L, F = 4, 512, 4608
T = 128
NT = L // T
NGRP = 5
SLAB = 112
GROUP_FIRST = (0, 7, 13, 19, 25, 32)
MROWS = 144
NCHUNK = F // T

bf16, f32, u32, i32 = jnp.bfloat16, jnp.float32, jnp.uint32, jnp.int32

LOG2E = 1.4426950408889634
QSCALE = (DH ** -0.5) * LOG2E
LN_NORM2 = 2.1 * D
LOGIT_LIMIT = 64.0
VALUE_LIMIT = 2.0 ** 50
NEG_BIG = -1e30


def _group_of(h):
    for g in range(NGRP):
        if GROUP_FIRST[g] <= h < GROUP_FIRST[g + 1]:
            return g
    raise ValueError(h)


def _to_bf16(x):
    return pltpu.bitcast(x, bf16)


def _to_u32(x):
    return pltpu.bitcast(x, u32)


def _round_bf16(x):
    return x.astype(bf16).astype(f32)


def _iota(shape, dim):
    return lax.broadcasted_iota(i32, shape, dim)


def _dot(a, b):
    return jnp.dot(a, b, preferred_element_type=f32)


def _dot_nt(a, b):
    return lax.dot_general(a, b, (((1,), (1,)), ((), ())), preferred_element_type=f32)


def _dot_tn(a, b):
    return lax.dot_general(a, b, (((0,), (0,)), ((), ())), preferred_element_type=f32)


def _phi(t):
    return jnp.where(t > 0, t + 1.0, jnp.exp(t))


def _sigmoid(t):
    return 1.0 / (1.0 + jnp.exp(-t))


def _layernorm_t(xb):
    x = xb.astype(f32)
    mean = jnp.sum(x, axis=0, keepdims=True) / D
    c = x - mean
    var = jnp.sum(c * c, axis=0, keepdims=True) / D
    eps = _round_bf16(jnp.full((1, 1), 1e-5, f32))
    sd = _round_bf16(jnp.sqrt(_round_bf16(_round_bf16(var) + eps)))
    d = _round_bf16(x - _round_bf16(mean))
    return _round_bf16(d * (1.0 / sd))


def _head_of_slab_index(idx, g):
    return ((idx + SLAB * g) * 3641) >> 16


def _cols(s):
    if isinstance(s, int):
        return slice(s * L, (s + 1) * L)
    return pl.ds(pl.multiple_of(s * L, L), L)


def _kernel(x_hbm, wq_hbm, wk_hbm, wv_hbm, wo_hbm, beta_ref, wr_ref, wg_hbm, wu_hbm, wd_hbm,
            out_hbm,
            xt, xn, wstage, wt, wot, wg, wu, wd, qt, vt, kp, num, mt, zt, ot, ao, outb, gb, patch,
            sems):
    def copy(src, dst, i):
        return pltpu.make_async_copy(src, dst, sems.at[i])

    x_copies = [copy(x_hbm.at[:, s * L:(s + 1) * L], xt.at[:, s * L:(s + 1) * L], s) for s in range(NSEG)]
    w_copies = [copy(w, wstage.at[i], 4 + i) for i, w in enumerate((wk_hbm, wq_hbm, wv_hbm, wo_hbm))]
    moe_copies = [copy(wg_hbm, wg, 8), copy(wu_hbm, wu, 9), copy(wd_hbm, wd, 10)]
    out_copies = [copy(outb.at[:, s * L:(s + 1) * L], out_hbm.at[:, s * L:(s + 1) * L], 11 + s)
                  for s in range(NSEG)]

    x_copies[0].start()
    w_copies[0].start()
    w_copies[1].start()
    w_copies[2].start()
    for c in x_copies[1:]:
        c.start()
    w_copies[3].start()
    for c in moe_copies:
        c.start()

    def col_sq_max(w):
        w = w.astype(f32)
        return jnp.max(jnp.sum(w * w, axis=0, keepdims=True))

    x_copies[0].wait()
    xn[:, 0:L] = _layernorm_t(xt[:, 0:L])
    csq = []
    for i in range(3):
        w_copies[i].wait()
        w = wstage[i]
        wt[i * (D // 2):(i + 1) * (D // 2), :] = _to_u32(w.T)
        csq.append(col_sq_max(w))
    for s in range(1, NSEG):
        x_copies[s].wait()
        xn[:, s * L:(s + 1) * L] = _layernorm_t(xt[:, s * L:(s + 1) * L])
    w_copies[3].wait()
    wot[...] = _to_u32(wstage[3].T)

    gb[...] = _sigmoid(jnp.broadcast_to(beta_ref[...].astype(f32).reshape(1, H), (T, H)).T)

    bound2 = (QSCALE * LN_NORM2 * DH) ** 2 * csq[0] * csq[1]
    safe = jnp.logical_and(bound2 <= LOGIT_LIMIT ** 2, LN_NORM2 * csq[2] <= VALUE_LIMIT ** 2)

    def project(s):
        xb = xn[:, _cols(s)].astype(bf16)
        half = D // 2
        kt = _round_bf16(_dot(_to_bf16(wt[0:half, :]), xb))
        q = _dot(_to_bf16(wt[half:2 * half, :]), xb)
        qt[...] = q * QSCALE
        vt[...] = _dot(_to_bf16(wt[2 * half:3 * half, :]), xb)
        for g in range(NGRP):
            kp[g] = _to_u32(kt[SLAB * g:SLAB * g + T, :].astype(bf16).T)
        return kt, _round_bf16(q)

    def memory_read(q):
        pq = _phi(q).astype(bf16)
        for g in range(NGRP):
            num[g] = _dot(mt[g].astype(bf16), pq[SLAB * g:SLAB * g + T, :])

    def memory_update(kt, first):
        pk = _phi(kt).astype(bf16)
        rows = _iota((T, T), 0)
        cols = _iota((T, T), 1)
        for g in range(NGRP):
            ones_row = 0 if g == NGRP - 1 else T - 1
            vs = jnp.where(_iota((T, L), 0) == ones_row, 1.0, vt[SLAB * g:SLAB * g + T, :]).astype(bf16)
            m = _dot_nt(vs, pk[SLAB * g:SLAB * g + T, :])
            hr = _head_of_slab_index(rows, g)
            hc = _head_of_slab_index(cols, g)
            keep = (hr == hc) & (hr >= GROUP_FIRST[g]) & (hr < GROUP_FIRST[g + 1])
            mm = jnp.where(keep, m, 0.0)
            z = m[ones_row:ones_row + 1, :]
            if not first:
                mm = mm + mt[g, 0:T, :]
                z = z + zt[g, 0:1, :]
            mt[g, 0:T, :] = mm
            zt[g, 0:1, :] = z
            zsel = _head_of_slab_index(_iota((16, T), 1), g) == _iota((16, T), 0) + GROUP_FIRST[g]
            mt[g, T:MROWS, :] = jnp.where(zsel, z, 0.0)

    def masked_q(h, j):
        g = _group_of(h)
        f0 = SLAB * g
        r0 = DH * h - f0
        a = (r0 // 16) * 16
        b = -(-(r0 + DH) // 16) * 16
        rows = _iota((b - a, T), 0) + a
        piece = jnp.where((rows >= r0) & (rows < r0 + DH), qt[f0 + a:f0 + b, j * T:(j + 1) * T], 0.0)
        parts = []
        if a > 0:
            parts.append(jnp.zeros((a, T), f32))
        parts.append(piece)
        if b < T:
            parts.append(jnp.zeros((T - b, T), f32))
        return jnp.concatenate(parts, axis=0).astype(bf16)

    def scores(h, use_max):
        g = _group_of(h)
        causal = _iota((T, T), 0) <= _iota((T, T), 1)
        ps = []
        for j in range(NT):
            n = (j + 1) * T
            s = _dot(_to_bf16(kp[g, 0:n // 2, :]), masked_q(h, j))
            if use_max:
                sd = jnp.where(causal, s[n - T:], NEG_BIG)
                m = jnp.max(sd, axis=0, keepdims=True)
                if j > 0:
                    m = jnp.maximum(m, jnp.max(s[:n - T], axis=0, keepdims=True))
                    p = jnp.concatenate([jnp.exp2(s[:n - T] - m), jnp.exp2(sd - m)], axis=0)
                else:
                    p = jnp.exp2(sd - m)
            else:
                pd = jnp.where(causal, jnp.exp2(s[n - T:]), 0.0)
                p = pd if j == 0 else jnp.concatenate([jnp.exp2(s[:n - T]), pd], axis=0)
            ps.append(p.astype(bf16))
        return ps

    def values(h, ps, with_memory):
        g = _group_of(h)
        w0 = min((DH * h // 16) * 16, D - 32)
        off = DH * h - w0
        ones_row = 31 if off < 14 else 0
        vwin = jnp.where(_iota((32, L), 0) == ones_row, 1.0, vt[w0:w0 + 32, :]).astype(bf16)
        gate = gb[h:h + 1, :]
        for j in range(NT):
            n = (j + 1) * T
            cs = slice(j * T, (j + 1) * T)
            acc = _dot(vwin[:, 0:n], ps[j])
            res = acc * ((1.0 - gate) / acc[ones_row:ones_row + 1, :])
            if with_memory:
                m0 = w0 - SLAB * g
                zr = T + h - GROUP_FIRST[g]
                den = num[g, zr:zr + 1, cs] + 1e-6
                res = res + num[g, m0:m0 + 32, cs] * (gate / den)
            ot[DH * h:DH * h + DH, cs] = res[off:off + DH, :]

    def out_project():
        return _dot(_to_bf16(wot[...]), ot[...].astype(bf16))

    def finalize(s, attn):
        cs = _cols(s)
        res = attn + xt[:, cs].astype(f32) + xn[:, cs]
        outb[:, cs] = res.astype(bf16)

    def attention(with_memory, use_max, lag, between=None):
        pending = {}
        for t in range(H + lag):
            if t < H:
                pending[t] = scores(t, use_max)
            if between is not None:
                between(t)
            if t >= lag:
                values(t - lag, pending.pop(t - lag), with_memory)

    def route():
        wcol = jnp.broadcast_to(wr_ref[...].astype(f32).reshape(1, D), (T, D)).T
        parts = []
        for t in range(S // T):
            parts.append(jnp.sum(xn[:, t * T:(t + 1) * T] * wcol, axis=0, keepdims=True))
        r = _round_bf16(jnp.concatenate(parts, axis=1))
        idx = _iota((1, S), 1)
        m1 = jnp.max(r)
        i1 = jnp.min(jnp.where(r == m1, idx, S))
        r2 = jnp.where(idx == i1, -jnp.inf, r)
        m2 = jnp.max(r2)
        i2 = jnp.min(jnp.where(r2 == m2, idx, S))
        i1 = jnp.clip(i1, 0, S - 1)
        i2 = jnp.clip(i2, 0, S - 1)
        return (i1, i2), (m1, m2)

    def tile_of(i):
        return pl.ds(pl.multiple_of((i // T) * T, T), T)

    def one_hot(i, row):
        hit = (_iota((16, T), 0) == row) & (_iota((16, T), 1) == i % T)
        return jnp.where(hit, 1.0, 0.0).astype(bf16)

    def select_tokens(ids):
        sel = None
        for row, i in enumerate(ids):
            part = _dot_nt(one_hot(i, row), xn[:, tile_of(i)].astype(bf16))
            sel = part if sel is None else sel + part
        return sel.astype(bf16)

    def moe_chunk(xsel, c, y):
        cs = slice(c * T, (c + 1) * T)
        gpre = _round_bf16(_dot(xsel, wg[:, cs]))
        gact = _round_bf16(gpre * _sigmoid(gpre))
        up = _round_bf16(_dot(xsel, wu[:, cs]))
        part = _dot_nt((gact * up).astype(bf16), wd[:, cs])
        return part if y is None else y + part

    def moe_patches(ids, scores_sel, y):
        row = _iota((16, D), 0)
        gate = jnp.where(row == 0, scores_sel[0], scores_sel[1])
        y = (_round_bf16(y) * _round_bf16(_sigmoid(gate))).astype(bf16)
        for k, i in enumerate(ids):
            patch[k] = _dot_tn(y, one_hot(i, k))

    def apply_patches(ids):
        for k, i in enumerate(ids):
            cs = tile_of(i)
            ao[:, cs] = ao[:, cs] + patch[k]

    def init_memory():
        mt[...] = jnp.zeros(mt.shape, f32)
        zt[...] = jnp.zeros(zt.shape, f32)

    def finish(ids, sel_scores, y):
        moe_patches(ids, sel_scores, y)
        apply_patches(ids)
        for s in range(NSEG):
            finalize(s, ao[:, s * L:(s + 1) * L])
            out_copies[s].start()

    def fast_path():
        for s in range(NSEG):
            kt, q = project(s)
            if s > 0:
                memory_read(q)
            attention(s > 0, False, 1)
            if s < NSEG - 1:
                memory_update(kt, s == 0)
            ao[:, s * L:(s + 1) * L] = out_project()
        ids, sel_scores = route()
        for c in moe_copies:
            c.wait()
        xsel = select_tokens(ids)
        y = None
        for c in range(NCHUNK):
            y = moe_chunk(xsel, c, y)
        finish(ids, sel_scores, y)

    def slow_path():
        init_memory()

        def seg(s, carry):
            kt, q = project(s)
            memory_read(q)
            attention(True, True, 1)
            memory_update(kt, False)
            ao[:, _cols(s)] = out_project()
            return carry

        lax.fori_loop(0, NSEG, seg, 0)
        ids, sel_scores = route()
        for c in moe_copies:
            c.wait()
        xsel = select_tokens(ids)
        y = None
        for c in range(NCHUNK):
            y = moe_chunk(xsel, c, y)
        finish(ids, sel_scores, y)

    lax.cond(safe, fast_path, slow_path)
    for c in out_copies:
        c.wait()


@jax.jit
def pallas_parallel_sum__memory_aug_infini_attn__moe_arch_mod__prompt_kernel(
    A_x: jax.Array,
    A_wq: jax.Array,
    A_wk: jax.Array,
    A_wv: jax.Array,
    A_wo: jax.Array,
    A_beta: jax.Array,
    B_x: jax.Array,
    B_w_r: jax.Array,
    B_w_gate: jax.Array,
    B_w_up: jax.Array,
    B_w_down: jax.Array,
):
    del B_x
    x_t = jnp.transpose(A_x, (0, 2, 1)).reshape(D, S)
    wd_t = B_w_down.T
    hbm = pl.BlockSpec(memory_space=pl.ANY)
    vmem = pl.BlockSpec(memory_space=pltpu.VMEM)
    out_t = pl.pallas_call(
        _kernel,
        out_shape=jax.ShapeDtypeStruct((D, S), bf16),
        in_specs=[hbm, hbm, hbm, hbm, hbm, vmem, vmem, hbm, hbm, hbm],
        out_specs=hbm,
        scratch_shapes=[
            pltpu.VMEM((D, S), bf16),
            pltpu.VMEM((D, S), f32),
            pltpu.VMEM((4, D, D), bf16),
            pltpu.VMEM((3 * D // 2, D), u32),
            pltpu.VMEM((D // 2, D), u32),
            pltpu.VMEM((D, F), bf16),
            pltpu.VMEM((D, F), bf16),
            pltpu.VMEM((D, F), bf16),
            pltpu.VMEM((D, L), f32),
            pltpu.VMEM((D, L), f32),
            pltpu.VMEM((NGRP, L // 2, T), u32),
            pltpu.VMEM((NGRP, MROWS, L), f32),
            pltpu.VMEM((NGRP, MROWS, T), f32),
            pltpu.VMEM((NGRP, 8, T), f32),
            pltpu.VMEM((D, L), f32),
            pltpu.VMEM((D, S), f32),
            pltpu.VMEM((D, S), bf16),
            pltpu.VMEM((H, T), f32),
            pltpu.VMEM((2, D, T), f32),
            pltpu.SemaphoreType.DMA((15,)),
        ],
        compiler_params=pltpu.CompilerParams(vmem_limit_bytes=100 * 1024 * 1024),
        name="infini_moe",
    )(x_t, A_wq, A_wk, A_wv, A_wo, A_beta, B_w_r, B_w_gate, B_w_up, wd_t)
    return jnp.transpose(out_t.reshape(1, D, S), (0, 2, 1))
```

```python
import contextlib

import jax
import jax.numpy as jnp
from jax import lax
from jax.experimental import pallas as pl
from jax.experimental.pallas import tpu as pltpu

S, D, H, DH = 2048, 576, 32, 18
NSEG, L, F = 4, 512, 4608
T = 128
NT = L // T
NGRP = 5
SLAB = 112
GROUP_FIRST = (0, 7, 13, 19, 25, 32)
MROWS = 144
NCHUNK = F // T

bf16, f32, u32, i32 = jnp.bfloat16, jnp.float32, jnp.uint32, jnp.int32

LOG2E = 1.4426950408889634
QSCALE = (DH ** -0.5) * LOG2E
LN_NORM2 = 2.1 * D
LOGIT_LIMIT = 64.0
VALUE_LIMIT = 2.0 ** 50
NEG_BIG = -1e30


PROFILE_SCOPES = False


def _scope(name):
    return jax.named_scope(name) if PROFILE_SCOPES else contextlib.nullcontext()


def _group_of(h):
    for g in range(NGRP):
        if GROUP_FIRST[g] <= h < GROUP_FIRST[g + 1]:
            return g
    raise ValueError(h)


def _to_bf16(x):
    return pltpu.bitcast(x, bf16)


def _to_u32(x):
    return pltpu.bitcast(x, u32)


def _round_bf16(x):
    return x.astype(bf16).astype(f32)


def _iota(shape, dim):
    return lax.broadcasted_iota(i32, shape, dim)


def _dot(a, b):
    return jnp.dot(a, b, preferred_element_type=f32)


def _dot_nt(a, b):
    return lax.dot_general(a, b, (((1,), (1,)), ((), ())), preferred_element_type=f32)


def _dot_tn(a, b):
    return lax.dot_general(a, b, (((0,), (0,)), ((), ())), preferred_element_type=f32)


def _phi(t):
    return jnp.where(t > 0, t + 1.0, jnp.exp(t))


def _sigmoid(t):
    return 1.0 / (1.0 + jnp.exp(-t))


def _layernorm_t(xb):
    x = xb.astype(f32)
    mean = jnp.sum(x, axis=0, keepdims=True) / D
    c = x - mean
    var = jnp.sum(c * c, axis=0, keepdims=True) / D
    eps = _round_bf16(jnp.full((1, 1), 1e-5, f32))
    sd = _round_bf16(jnp.sqrt(_round_bf16(_round_bf16(var) + eps)))
    d = _round_bf16(x - _round_bf16(mean))
    return _round_bf16(d * (1.0 / sd))


def _head_of_slab_index(idx, g):
    return ((idx + SLAB * g) * 3641) >> 16


def _zero_after(x):
    sign = lax.shift_right_logical(pltpu.bitcast(x, i32), 31)
    return sign.astype(f32) * 0.0


def _kernel(x_hbm, wq_hbm, wk_hbm, wv_hbm, wo_hbm, beta_hbm, wr_hbm, wg_hbm, wu_hbm, wd_hbm,
            out_hbm,
            xt, xn, wstage, wt, wot, wg, wu, wd, beta_ref, wr_ref, qt, vt, kp, num, mt, zt, ot,
            mx, rrow, outb, gb, kall, qall, sems):
    def copy(src, dst, i):
        return pltpu.make_async_copy(src, dst, sems.at[i])

    x0_copy = copy(x_hbm.at[:, 0:L], xt.at[:, 0:L], 0)
    xr_copy = copy(x_hbm.at[:, L:S], xt.at[:, L:S], 1)
    wk_copy, wq_copy, wv_copy, wo_copy = [
        copy(w, wstage.at[i], 2 + i) for i, w in enumerate((wk_hbm, wq_hbm, wv_hbm, wo_hbm))]
    beta_copy = copy(beta_hbm, beta_ref, 6)
    wr_copy = copy(wr_hbm, wr_ref, 7)
    moe_copies = [copy(wg_hbm, wg, 8), copy(wu_hbm, wu, 9), copy(wd_hbm, wd, 10)]

    def out_copy(lo, hi, i):
        return copy(outb.at[:, lo:hi], out_hbm.at[:, lo:hi], 11 + i)

    half = D // 2

    def tile_cols(s, tt):
        return slice(s * L + tt * T, s * L + (tt + 1) * T)

    def local_cols(tt):
        return slice(tt * T, (tt + 1) * T)

    def col_sq_max(i):
        acc = None
        for r in range(0, D, 64):
            w = wstage[i, r:r + 64, :].astype(f32)
            part = jnp.sum((w * w).reshape(8, 8, D), axis=0)
            acc = part if acc is None else acc + part
        return jnp.max(jnp.sum(acc, axis=0, keepdims=True), axis=1, keepdims=True)

    def transpose_weight(i):
        return _to_u32(wstage[i].T)

    def normalize(s, tt):
        cs = tile_cols(s, tt)
        xn[:, cs] = _layernorm_t(xt[:, cs])

    def xn_tile(s, tt):
        return xn[:, tile_cols(s, tt)].astype(bf16)

    def project_k(s, tt):
        kt = _round_bf16(_dot(_to_bf16(wt[0:half, :]), xn_tile(s, tt)))
        for g in range(NGRP):
            kp[s % 2, g, tt * (T // 2):(tt + 1) * (T // 2), :] = _to_u32(
                kt[SLAB * g:SLAB * g + T, :].astype(bf16).T)
        return _phi(kt).astype(bf16)

    def project_q(s, tt, tie=None):
        q = _dot(_to_bf16(wt[half:2 * half, :]), xn_tile(s, tt))
        qt[s % 2, :, local_cols(tt)] = q * (QSCALE if tie is None else QSCALE + tie)
        return _phi(_round_bf16(q)).astype(bf16)

    def project_v(s, tt, tie=None):
        v = _dot(_to_bf16(wt[2 * half:3 * half, :]), xn_tile(s, tt))
        vt[s % 2, :, local_cols(tt)] = v if tie is None else v + tie

    def router_scores(lhs, s, tt):
        row = s * NT + tt
        rrow[row:row + 1, :] = _dot(lhs, xn_tile(s, tt))[0:1, :]

    def memory_read(s, tt, pq):
        for g in range(NGRP):
            num[s % 2, g, :, local_cols(tt)] = _dot(mt[g].astype(bf16), pq[SLAB * g:SLAB * g + T, :])

    def memory_update(s, g, pk):
        ones_row = 0 if g == NGRP - 1 else T - 1
        vs = jnp.where(_iota((T, L), 0) == ones_row, 1.0, vt[s % 2, SLAB * g:SLAB * g + T, :]).astype(bf16)
        m = _dot_nt(vs, jnp.concatenate([p[SLAB * g:SLAB * g + T, :] for p in pk], axis=1))
        hr = _head_of_slab_index(_iota((T, T), 0), g)
        hc = _head_of_slab_index(_iota((T, T), 1), g)
        keep = (hr == hc) & (hr >= GROUP_FIRST[g]) & (hr < GROUP_FIRST[g + 1])
        mm = jnp.where(keep, m, 0.0)
        z = m[ones_row:ones_row + 1, :]
        if s > 0:
            mm = mm + mt[g, 0:T, :]
            z = z + zt[g, 0:1, :]
        mt[g, 0:T, :] = mm
        zt[g, 0:1, :] = z
        zsel = _head_of_slab_index(_iota((16, T), 1), g) == _iota((16, T), 0) + GROUP_FIRST[g]
        mt[g, T:MROWS, :] = jnp.where(zsel, z, 0.0)

    def masked_q(s, h, j):
        g = _group_of(h)
        f0 = SLAB * g
        r0 = DH * h - f0
        a = (r0 // 16) * 16
        b = -(-(r0 + DH) // 16) * 16
        rows = _iota((b - a, T), 0) + a
        piece = jnp.where((rows >= r0) & (rows < r0 + DH), qt[s % 2, f0 + a:f0 + b, local_cols(j)], 0.0)
        parts = []
        if a > 0:
            parts.append(jnp.zeros((a, T), f32))
        parts.append(piece)
        if b < T:
            parts.append(jnp.zeros((T - b, T), f32))
        return jnp.concatenate(parts, axis=0).astype(bf16)

    def scores(s, h, j):
        g = _group_of(h)
        n = (j + 1) * T
        causal = _iota((T, T), 0) <= _iota((T, T), 1)
        logits = _dot(_to_bf16(kp[s % 2, g, 0:n // 2, :]), masked_q(s, h, j))
        e = jnp.exp2(logits - mx[h:h + 1, tile_cols(s, j)])
        pd = jnp.where(causal, e[n - T:], 0.0)
        p = pd if j == 0 else jnp.concatenate([e[:n - T], pd], axis=0)
        return p.astype(bf16)

    def values(s, h, ps):
        g = _group_of(h)
        w0 = min((DH * h // 16) * 16, D - 32)
        off = DH * h - w0
        ones_row = 31 if off < 14 else 0
        vwin = jnp.where(_iota((32, L), 0) == ones_row, 1.0, vt[s % 2, w0:w0 + 32, :]).astype(bf16)
        gate = gb[h:h + 1, :]
        for j in range(NT):
            n = (j + 1) * T
            cs = local_cols(j)
            acc = _dot(vwin[:, 0:n], ps[j])
            res = acc * ((1.0 - gate) / acc[ones_row:ones_row + 1, :])
            if s > 0:
                m0 = w0 - SLAB * g
                zr = T + h - GROUP_FIRST[g]
                den = num[s % 2, g, zr:zr + 1, cs] + 1e-6
                res = res + num[s % 2, g, m0:m0 + 32, cs] * (gate / den)
            ot[s, DH * h:DH * h + DH, cs] = res[off:off + DH, :]

    def route():
        r = _round_bf16(rrow[...])
        idx = _iota((S // T, T), 0) * T + _iota((S // T, T), 1)
        m1 = jnp.max(r)
        i1 = jnp.min(jnp.where(r == m1, idx, S - 1))
        r2 = jnp.where(idx == i1, -jnp.inf, r)
        m2 = jnp.max(r2)
        i2 = jnp.min(jnp.where(r2 == m2, idx, S - 1))
        return (i1, i2), (m1, m2)

    def select_tokens(ids):
        sel = None
        for row, i in enumerate(ids):
            hit = (_iota((16, T), 0) == row) & (_iota((16, T), 1) == i % T)
            cs = pl.ds(pl.multiple_of((i // T) * T, T), T)
            part = _dot_nt(jnp.where(hit, 1.0, 0.0).astype(bf16), xn[:, cs].astype(bf16))
            sel = part if sel is None else sel + part
        return sel.astype(bf16)

    def moe_gate(xsel, c):
        gpre = _round_bf16(_dot(xsel, wg[:, c * T:(c + 1) * T]))
        return _round_bf16(gpre * _sigmoid(gpre))

    def moe_up(xsel, c):
        return _round_bf16(_dot(xsel, wu[:, c * T:(c + 1) * T]))

    def moe_down(hid, c, y):
        part = _dot_nt(hid, wd[:, c * T:(c + 1) * T])
        return part if y is None else y + part

    def out_lhs(ids, sel_scores, y):
        row = _iota((16, D), 0)
        gate = jnp.where(row == 0, sel_scores[0], sel_scores[1])
        y = (_round_bf16(y) * _round_bf16(_sigmoid(gate))).astype(bf16)
        place = (_iota((16, T), 1) == _iota((16, T), 0) + 64) & (_iota((16, T), 0) < 2)
        ycols = _dot_tn(y, jnp.where(place, 1.0, 0.0).astype(bf16))
        last = _to_bf16(wot[:, 4 * T:5 * T]).astype(f32) + ycols
        for s in range(NSEG):
            tok = _iota((64, L), 1) + s * L
            rows = _iota((64, L), 0)
            hit = ((rows == 0) & (tok == ids[0])) | ((rows == 1) & (tok == ids[1]))
            ot[s, D:D + 64, :] = jnp.where(hit, 1.0, 0.0)
        return jnp.concatenate([_to_bf16(wot[:, 0:4 * T]), last.astype(bf16)], axis=1)

    def out_project(lhs, s, tt):
        cs = tile_cols(s, tt)
        attn = _dot(lhs, ot[s, :, local_cols(tt)].astype(bf16))
        outb[:, cs] = (attn + xn[:, cs] + xt[:, cs].astype(f32)).astype(bf16)

    def row_maxima():
        def project_tile(tt, carry):
            cs = pl.ds(pl.multiple_of(tt * T, T), T)
            y = _layernorm_t(xt[:, cs]).astype(bf16)
            kall[:, cs] = _dot(_to_bf16(wt[0:half, :]), y).astype(bf16)
            qall[:, cs] = (_dot(_to_bf16(wt[half:2 * half, :]), y) * QSCALE).astype(bf16)
            return carry

        lax.fori_loop(0, S // T, project_tile, 0)

        def head_tile(i, carry):
            h = i // (S // T)
            tt = i % (S // T)
            cs = pl.ds(pl.multiple_of(tt * T, T), T)
            seg = pl.ds(pl.multiple_of((tt // NT) * L, L), L)
            rows = _iota((D, T), 0)
            qm = jnp.where((rows >= DH * h) & (rows < DH * h + DH), qall[:, cs].astype(f32), 0.0)
            logits = _dot_tn(kall[:, seg], qm.astype(bf16))
            seen = _iota((L, T), 0) <= _iota((L, T), 1) + (tt % NT) * T
            m = jnp.max(jnp.where(seen, logits, NEG_BIG), axis=0, keepdims=True)
            mx[:, cs] = jnp.where(_iota((H, T), 0) == h, m, mx[:, cs])
            return carry

        lax.fori_loop(0, H * (S // T), head_tile, 0)

    x0_copy.start()
    wk_copy.start()
    mx[...] = jnp.zeros(mx.shape, f32)
    wot[:, 4 * T:5 * T] = jnp.zeros((half, T), u32)
    with _scope('p0_wait'):
        x0_copy.wait()
        wk_copy.wait()
    for c in (wq_copy, wv_copy, xr_copy, wo_copy, beta_copy, wr_copy, *moe_copies):
        c.start()
    pk, pq = {}, {}
    with _scope('p1'):
        wt[0:half, :] = transpose_weight(0)
        for tt in range(NT):
            normalize(0, tt)
            pk[0, tt] = project_k(0, tt)
    with _scope('p2_wait'):
        wq_copy.wait()
        wv_copy.wait()
    with _scope('p2'):
        wt[half:2 * half, :] = transpose_weight(1)
        wt[2 * half:3 * half, :] = transpose_weight(2)
        csq = []
        for tt in range(NT):
            tie = None
            if tt > 0:
                csq.append(col_sq_max(tt - 1))
                tie = _zero_after(csq[-1])
            project_q(0, tt, tie)
        for tt in range(NT):
            project_v(0, tt)
        bound2 = (QSCALE * LN_NORM2 * DH) ** 2 * csq[0] * csq[1]
        ok = jnp.logical_and(bound2 <= LOGIT_LIMIT ** 2, LN_NORM2 * csq[2] <= VALUE_LIMIT ** 2)
        unsafe = jnp.max(jnp.where(ok, 0, 1)) > 0
    with _scope('p3_wait'):
        for c in (xr_copy, wo_copy, beta_copy, wr_copy):
            c.wait()

    @pl.when(unsafe)
    def _():
        row_maxima()

    gb[...] = _sigmoid(jnp.broadcast_to(beta_ref[...].astype(f32).reshape(1, H), (T, H)).T)

    slots = {}
    st = {}

    def at(s, t, j, fn):
        slots.setdefault((s, t, j), []).append(fn)

    def wr_lhs():
        if 'wr' not in st:
            w = jnp.broadcast_to(wr_ref[...].astype(f32).reshape(1, D), (16, D))
            st['wr'] = jnp.where(_iota((16, D), 0) == 0, w, 0.0).astype(bf16)
        return st['wr']

    for s in range(NSEG - 1):
        for g in range(NGRP):
            at(s, 1 + g, 3, lambda s=s, g=g: memory_update(s, g, [pk[s, tt] for tt in range(NT)]))
        for tt in range(NT):
            t0 = 7 + 6 * tt
            if s == 0:
                at(s, t0, 1, lambda tt=tt: normalize(1, tt))
            at(s, t0, 3, lambda s=s, tt=tt: pk.__setitem__((s + 1, tt), project_k(s + 1, tt)))
            at(s, t0 + 2, 3, lambda s=s, tt=tt: pq.__setitem__((s + 1, tt), project_q(s + 1, tt)))
            at(s, t0 + 3, 3, lambda s=s, tt=tt: memory_read(s + 1, tt, pq[s + 1, tt]))
            at(s, t0 + 4, 3, lambda s=s, tt=tt: project_v(s + 1, tt))

    order = [(0, tt) for tt in range(NT)] + [(s, tt) for s in (2, 3) for tt in range(NT)]
    for k, (s, tt) in enumerate(order):
        t = 1 + 2 * k
        if s > 0:
            at(0, t, 2, lambda s=s, tt=tt: normalize(s, tt))
        at(0, t, 2, lambda s=s, tt=tt: router_scores(wr_lhs(), s, tt))
    for tt in range(NT):
        at(0, 8 + 6 * tt, 2, lambda tt=tt: router_scores(wr_lhs(), 1, tt))
    at(0, 24, 0, lambda: wot.__setitem__((slice(None), slice(0, D)), transpose_weight(3)))

    at(1, 2, 0, lambda: st.update(zip(('ids', 'sel'), route())))
    at(1, 16, 0, lambda: st.update(xsel=select_tokens(st['ids']), y=None))

    def wait_moe():
        with _scope('moe_wait'):
            for c in moe_copies:
                c.wait()

    at(2, 0, -1, wait_moe)
    hid = {}
    for c in range(NCHUNK):
        t = (c * 30) // NCHUNK
        second = c > 0 and ((c - 1) * 30) // NCHUNK == t
        j0 = 2 if second else 0
        at(2, t, j0, lambda c=c: hid.__setitem__(('g', c), moe_gate(st['xsel'], c)))
        at(2, t, j0 + 1, lambda c=c: hid.__setitem__(('u', c), moe_up(st['xsel'], c)))
        at(2, t + 1, j0, lambda c=c: st.update(y=moe_down(
            (hid.pop(('g', c)) * hid.pop(('u', c))).astype(bf16), c, st['y'])))
    at(3, 0, 0, lambda: st.update(lhs=out_lhs(st['ids'], st['sel'], st['y'])))
    for s in range(NSEG - 1):
        for tt in range(NT):
            at(3, 2 + 2 * (NT * s + tt), 3, lambda s=s, tt=tt: out_project(st['lhs'], s, tt))
        at(3, 2 + 2 * (NT * s + NT - 1) + 1, 0, lambda s=s: out_copy(s * L, (s + 1) * L, s).start())

    stream = [(s, h) for s in range(NSEG) for h in range(H)]
    prev = None
    for s, h in stream:
        with _scope(f'att{s}') if h == 0 else contextlib.nullcontext():
            pass
        for fn in slots.pop((s, h, -1), ()):
            fn()
        ps = []
        for j in range(NT):
            ps.append(scores(s, h, j))
            for fn in slots.pop((s, h, j), ()):
                fn()
        if prev is not None:
            values(*prev)
        prev = (s, h, ps)
    values(*prev)
    assert not slots, slots.keys()
    s = NSEG - 1
    for tt in range(NT):
        out_project(st['lhs'], s, tt)
        out_copy(s * L + tt * T, s * L + (tt + 1) * T, 3 + tt).start()
    with _scope('out_wait'):
        for k in range(NSEG - 1):
            out_copy(k * L, (k + 1) * L, k).wait()
        for tt in range(NT):
            out_copy(s * L + tt * T, s * L + (tt + 1) * T, 3 + tt).wait()


@jax.jit
def pallas_parallel_sum__memory_aug_infini_attn__moe_arch_mod__prompt_kernel(
    A_x: jax.Array,
    A_wq: jax.Array,
    A_wk: jax.Array,
    A_wv: jax.Array,
    A_wo: jax.Array,
    A_beta: jax.Array,
    B_x: jax.Array,
    B_w_r: jax.Array,
    B_w_gate: jax.Array,
    B_w_up: jax.Array,
    B_w_down: jax.Array,
):
    del B_x
    x_t = jnp.transpose(A_x, (0, 2, 1)).reshape(D, S)
    wd_t = B_w_down.T
    hbm = pl.BlockSpec(memory_space=pl.ANY)
    out_t = pl.pallas_call(
        _kernel,
        out_shape=jax.ShapeDtypeStruct((D, S), bf16),
        in_specs=[hbm] * 10,
        out_specs=hbm,
        scratch_shapes=[
            pltpu.VMEM((D, S), bf16),
            pltpu.VMEM((D, S), f32),
            pltpu.VMEM((4, D, D), bf16),
            pltpu.VMEM((3 * D // 2, D), u32),
            pltpu.VMEM((D // 2, 5 * T), u32),
            pltpu.VMEM((D, F), bf16),
            pltpu.VMEM((D, F), bf16),
            pltpu.VMEM((D, F), bf16),
            pltpu.VMEM((H,), bf16),
            pltpu.VMEM((D,), bf16),
            pltpu.VMEM((2, D, L), f32),
            pltpu.VMEM((2, D, L), f32),
            pltpu.VMEM((2, NGRP, L // 2, T), u32),
            pltpu.VMEM((2, NGRP, MROWS, L), f32),
            pltpu.VMEM((NGRP, MROWS, T), f32),
            pltpu.VMEM((NGRP, 8, T), f32),
            pltpu.VMEM((NSEG, 5 * T, L), f32),
            pltpu.VMEM((H, S), f32),
            pltpu.VMEM((S // T, T), f32),
            pltpu.VMEM((D, S), bf16),
            pltpu.VMEM((H, T), f32),
            pltpu.VMEM((D, S), bf16),
            pltpu.VMEM((D, S), bf16),
            pltpu.SemaphoreType.DMA((18,)),
        ],
        compiler_params=pltpu.CompilerParams(vmem_limit_bytes=100 * 1024 * 1024),
        name="infini_moe",
    )(x_t, A_wq, A_wk, A_wv, A_wo, A_beta, B_w_r, B_w_gate, B_w_up, wd_t)
    return jnp.transpose(out_t.reshape(1, D, S), (0, 2, 1))
```

```python
import contextlib
import functools

import jax
import jax.numpy as jnp
from jax import lax
from jax.experimental import pallas as pl
from jax.experimental.pallas import tpu as pltpu

S, D, H, DH = 2048, 576, 32, 18
NSEG, L, F = 4, 512, 4608
T = 128
NT = L // T
NGRP = 5
SLAB = 112
GROUP_FIRST = (0, 7, 13, 19, 25, 32)
MROWS = 144
NCHUNK = F // T
NQUAD = H // 4
QUAD_OFF = (0, 64, 144, 208, 288, 352, 432, 448)
EARLY = 2
SUB = 32

bf16, f32, u32, i32 = jnp.bfloat16, jnp.float32, jnp.uint32, jnp.int32

LOG2E = 1.4426950408889634
QSCALE = (DH ** -0.5) * LOG2E
LN_NORM2 = 2.1 * D
LOGIT_LIMIT = 64.0
VALUE_LIMIT = 2.0 ** 50
NEG_BIG = -1e30


PROFILE_SCOPES = False
CFG = dict(lag=5, rot=0, tie_stats=True, tie_p=3)


def _scope(name):
    return jax.named_scope(name) if PROFILE_SCOPES else contextlib.nullcontext()


def _group_of(h):
    for g in range(NGRP):
        if GROUP_FIRST[g] <= h < GROUP_FIRST[g + 1]:
            return g
    raise ValueError(h)


def _to_bf16(x):
    return pltpu.bitcast(x, bf16)


def _to_u32(x):
    return pltpu.bitcast(x, u32)


def _round_bf16(x):
    return x.astype(bf16).astype(f32)


def _iota(shape, dim):
    return lax.broadcasted_iota(i32, shape, dim)


def _dot(a, b):
    return jnp.dot(a, b, preferred_element_type=f32)


def _dot_nt(a, b):
    return lax.dot_general(a, b, (((1,), (1,)), ((), ())), preferred_element_type=f32)


def _dot_tn(a, b):
    return lax.dot_general(a, b, (((0,), (0,)), ((), ())), preferred_element_type=f32)


def _zero_after_bits(u):
    return lax.shift_right_logical(pltpu.bitcast(u, i32), 31).astype(f32) * 0.0


def _pack_pairs(x):
    lo = jnp.concatenate([x[r:r + 8] for r in range(0, x.shape[0], 16)], axis=0)
    hi = jnp.concatenate([x[r + 8:r + 16] for r in range(0, x.shape[0], 16)], axis=0)
    return pltpu.pack_elementwise([lo, hi], packed_dtype=bf16)


def _unpaired_index(r):
    x = r & 15
    return (r - x) + jnp.where(x < 8, 2 * x, 2 * (x - 8) + 1)


def _phi(t):
    return jnp.where(t > 0, t + 1.0, jnp.exp(t))


def _sigmoid(t):
    return 1.0 / (1.0 + jnp.exp(-t))


def _layernorm_stats(xb):
    x0 = xb[0:1, :].astype(f32)
    acc1, acc2 = [None] * 4, [None] * 4
    for n, r in enumerate(range(0, D, 16)):
        c = xb[r:r + 16, :].astype(f32) - x0
        for part in range(2):
            k = (2 * n + part) % 4
            piece = c[8 * part:8 * part + 8, :]
            acc1[k] = piece if acc1[k] is None else acc1[k] + piece
            acc2[k] = piece * piece if acc2[k] is None else acc2[k] + piece * piece
    s1 = jnp.sum((acc1[0] + acc1[1]) + (acc1[2] + acc1[3]), axis=0, keepdims=True) / D
    s2 = jnp.sum((acc2[0] + acc2[1]) + (acc2[2] + acc2[3]), axis=0, keepdims=True) / D
    var = jnp.maximum(s2 - s1 * s1, 0.0)
    eps = _round_bf16(jnp.full((1, 1), 1e-5, f32))
    sd = _round_bf16(jnp.sqrt(_round_bf16(_round_bf16(var) + eps)))
    return _round_bf16(x0 + s1), 1.0 / sd


def _layernorm_apply(xb, stats):
    mean, inv = stats
    return _round_bf16(xb.astype(f32) - mean) * inv


def _block_transpose(xs):
    lane = _iota(next(x for x in xs if x is not None).shape, 1)

    def exchange(u, v, low, shift):
        def pick(p, q):
            if p is None and q is None:
                return None
            return jnp.where(low, 0.0 if p is None else p, 0.0 if q is None else q)
        ru = None if u is None else pltpu.roll(u, T - shift, 1)
        rv = None if v is None else pltpu.roll(v, shift, 1)
        return pick(u, rv), pick(ru, v)

    y0, y2 = exchange(xs[0], xs[2], lane < 64, 64)
    y1, y3 = exchange(xs[1], xs[3], lane < 64, 64)
    low = (lane & 32) == 0
    z0, z1 = exchange(y0, y1, low, 32)
    z2, z3 = exchange(y2, y3, low, 32)
    return [z0, z1, z2, z3]


def _head_of_slab_index(idx, g):
    return ((idx + SLAB * g) * 3641) >> 16


def _zero_after(x):
    sign = lax.shift_right_logical(pltpu.bitcast(x, i32), 31)
    return sign.astype(f32) * 0.0


def _kernel(x_hbm, wq_hbm, wk_hbm, wv_hbm, wo_hbm, beta_hbm, wr_hbm, wg_hbm, wu_hbm, wd_hbm,
            out_hbm,
            xt, xn, wstage, wt, wot, wg, wu, wd, beta_ref, wr_ref, qt, vt, kp, num, mt, zt, ot,
            mx, mxp, rrow, ao, outb, gb, kall, qall, sems):
    def copy(src, dst, i):
        return pltpu.make_async_copy(src, dst, sems.at[i])

    x0_copy = copy(x_hbm.at[:, 0:L], xt.at[:, 0:L], 0)
    xr_copy = copy(x_hbm.at[:, L:S], xt.at[:, L:S], 1)
    wk_copy, wq_copy, wv_copy, wo_copy = [
        copy(w, wstage.at[i], 2 + i) for i, w in enumerate((wk_hbm, wq_hbm, wv_hbm, wo_hbm))]
    beta_copy = copy(beta_hbm, beta_ref, 6)
    wr_copy = copy(wr_hbm, wr_ref, 7)
    moe_copies = [copy(wg_hbm, wg, 8), copy(wu_hbm, wu, 9), copy(wd_hbm, wd, 10)]

    def out_copy(lo, hi, i):
        return copy(outb.at[:, lo:hi], out_hbm.at[:, lo:hi], 11 + i)

    half = D // 2
    ties = []

    def tile_cols(s, tt):
        return slice(s * L + tt * T, s * L + (tt + 1) * T)

    def local_cols(tt):
        return slice(tt * T, (tt + 1) * T)

    def col_sq_max(i):
        acc = None
        for r in range(0, D, 64):
            w = wstage[i, r:r + 64, :].astype(f32)
            part = jnp.sum((w * w).reshape(8, 8, D), axis=0)
            acc = part if acc is None else acc + part
        return jnp.max(jnp.sum(acc, axis=0, keepdims=True), axis=1, keepdims=True)

    def transpose_weight(i):
        return _to_u32(wstage[i].T)

    def ln_stats(s, tt):
        return _layernorm_stats(xt[:, tile_cols(s, tt)])

    def normalize(s, tt, stats):
        cs = tile_cols(s, tt)
        xn[:, cs] = _layernorm_apply(xt[:, cs], stats)

    def xn_tile(s, tt):
        return xn[:, tile_cols(s, tt)].astype(bf16)

    def project_k(s, tt):
        kt = _round_bf16(_dot(_to_bf16(wt[0:half, :]), xn_tile(s, tt)))
        shuffled = jnp.take_along_axis(kt, _unpaired_index(_iota((D, T), 1)), axis=1)
        for b in range(NQUAD):
            kp[s % 2, b, tt * (T // 2):(tt + 1) * (T // 2), :] = _to_u32(
                shuffled[QUAD_OFF[b]:QUAD_OFF[b] + T, :].astype(bf16).T)
        return _phi(kt).astype(bf16)

    def project_q(s, tt, tie=None):
        q = _dot(_to_bf16(wt[half:2 * half, :]), xn_tile(s, tt))
        qt[s % 2, :, local_cols(tt)] = q * (QSCALE if tie is None else QSCALE + tie)
        return _phi(_round_bf16(q)).astype(bf16)

    def project_v(s, tt, tie=None):
        v = _dot(_to_bf16(wt[2 * half:3 * half, :]), xn_tile(s, tt))
        vt[s % 2, :, local_cols(tt)] = v if tie is None else v + tie

    def router_scores(lhs, s, tt):
        row = s * NT + tt
        rrow[row:row + 1, :] = _dot(lhs, xn_tile(s, tt))[0:1, :]

    def memory_read(s, tt, pq):
        for g in range(NGRP):
            num[s % 2, g, :, local_cols(tt)] = _dot(mt[g].astype(bf16), pq[SLAB * g:SLAB * g + T, :])

    def memory_update(s, g, pk):
        ones_row = 0 if g == NGRP - 1 else T - 1
        vs = jnp.where(_iota((T, L), 0) == ones_row, 1.0, vt[s % 2, SLAB * g:SLAB * g + T, :]).astype(bf16)
        m = _dot_nt(vs, jnp.concatenate([p[SLAB * g:SLAB * g + T, :] for p in pk], axis=1))
        hr = _head_of_slab_index(_iota((T, T), 0), g)
        hc = _head_of_slab_index(_iota((T, T), 1), g)
        keep = (hr == hc) & (hr >= GROUP_FIRST[g]) & (hr < GROUP_FIRST[g + 1])
        mm = jnp.where(keep, m, 0.0)
        z = m[ones_row:ones_row + 1, :]
        if s > 0:
            mm = mm + mt[g, 0:T, :]
            z = z + zt[g, 0:1, :]
        mt[g, 0:T, :] = mm
        zt[g, 0:1, :] = z
        zsel = _head_of_slab_index(_iota((16, T), 1), g) == _iota((16, T), 0) + GROUP_FIRST[g]
        mt[g, T:MROWS, :] = jnp.where(zsel, z, 0.0)

    def assemble_rows(pieces):
        groups = []
        for r in range(0, T, 8):
            hit = [x[r - r0:r - r0 + 8, :] for r0, x in pieces if r0 <= r < r0 + x.shape[0]]
            groups.append(functools.reduce(lambda u, v: u + v, hit) if hit else None)
        out, r = [], 0
        while r < len(groups):
            if groups[r] is None:
                n = 1
                while r + n < len(groups) and groups[r + n] is None:
                    n += 1
                out.append(jnp.zeros((8 * n, T), f32))
                r += n
            else:
                out.append(groups[r])
                r += 1
        return jnp.concatenate(out, axis=0)

    def quad_queries(s, b, j):
        f0 = QUAD_OFF[b]
        wide, packed = [], [[] for _ in range(4)]
        for a in range(4):
            r0 = DH * (4 * b + a) - f0
            lo = (r0 // 8) * 8
            hi = -(-(r0 + DH) // 8) * 8
            rows = _iota((hi - lo, T), 0) + lo
            mine = (rows >= r0) & (rows < r0 + DH)
            q = qt[s % 2, f0 + lo:f0 + hi, local_cols(j)]
            wide.append(assemble_rows([(lo, jnp.where(mine, q, 0.0))]))
            here = mine & (_iota((hi - lo, T), 1) // SUB == a)
            for i in range(4):
                shift = (SUB * (a - i)) % T
                moved = q if shift == 0 else pltpu.roll(q, shift, 1)
                packed[i].append((lo, jnp.where(here, moved, 0.0)))
        return wide, [assemble_rows(p).astype(bf16) for p in packed]

    def scores(s, b, j):
        wide, packed = quad_queries(s, b, j)
        tie = None
        unit = (s * NQUAD + b) * NT + j
        due = [z for when, z in ties if when <= unit]
        ties[:] = [(when, z) for when, z in ties if when > unit]
        if due:
            tie = functools.reduce(lambda u, v: u + v, due)
        tile = s * NT + j
        k0 = j * (T // 2)
        off = None
        if j > 0:
            logits = _dot(_to_bf16(kp[s % 2, b, 0:k0, :]), jnp.concatenate(wide, axis=1).astype(bf16))
            shift = jnp.concatenate([mx[4 * b + a:4 * b + a + 1, tile_cols(s, j)] for a in range(4)], axis=1)
            off = jnp.exp2(logits - shift)
        causal = _unpaired_index(_iota((SUB, T), 0)) <= (_iota((SUB, T), 1) & (SUB - 1))
        diag = [None] * 4
        for i in [(k + CFG['rot'] * j) % 4 for k in range(4)]:
            n = SUB * (i + 1)
            logits = _dot(_to_bf16(kp[s % 2, b, k0:k0 + n // 2, :]), packed[i])
            shift = mxp[tile, 4 * b + i:4 * b + i + 1, :]
            if tie is not None and i == 3:
                shift = shift + tie
            e = jnp.exp2(logits - shift)
            blocks = [e[r * SUB:(r + 1) * SUB, :] for r in range(i)]
            blocks.append(jnp.where(causal, e[i * SUB:, :], 0.0))
            diag[i] = blocks
        per_head = [[] for _ in range(4)]
        for r in range(4):
            outs = _block_transpose([diag[i][r] if i >= r else None for i in range(4)])
            for a in range(4):
                per_head[a].append(outs[a])
        ps = []
        for a in range(4):
            parts = ([off[:, a * T:(a + 1) * T]] if j > 0 else []) + per_head[a]
            ps.append(_pack_pairs(jnp.concatenate(parts, axis=0)))
        if CFG['tie_p'] is not None:
            rows = [u[r:r + 8] for u in ps for r in range(0, u.shape[0], 8)]
            while len(rows) > 1:
                rows = [rows[i] | rows[i + 1] for i in range(0, len(rows) - 1, 2)] + rows[len(rows) & ~1:]
            ties.append((unit + CFG['tie_p'], _zero_after_bits(rows[0])[0:1, :]))
        return [_to_bf16(u) for u in ps]

    def values(s, h, j, p):
        g = _group_of(h)
        w0 = min((DH * h // 16) * 16, D - 32)
        off = DH * h - w0
        ones_row = 31 if off < 14 else 0
        n = (j + 1) * T
        cs = local_cols(j)
        vwin = jnp.where(_iota((32, n), 0) == ones_row, 1.0, vt[s % 2, w0:w0 + 32, 0:n]).astype(bf16)
        gate = gb[h:h + 1, :]
        acc = _dot(vwin, p)
        res = acc * ((1.0 - gate) / acc[ones_row:ones_row + 1, :])
        if s > 0:
            m0 = w0 - SLAB * g
            zr = T + h - GROUP_FIRST[g]
            den = num[s % 2, g, zr:zr + 1, cs] + 1e-6
            res = res + num[s % 2, g, m0:m0 + 32, cs] * (gate / den)
        else:
            ties.append((0, _zero_after((res[0:8] + res[8:16]) + (res[16:24] + res[24:32]))[0:1, :]))
        ot[s, DH * h:DH * h + DH, cs] = res[off:off + DH, :]

    def route():
        r = _round_bf16(rrow[...])
        idx = _iota((S // T, T), 0) * T + _iota((S // T, T), 1)
        m1 = jnp.max(r)
        i1 = jnp.min(jnp.where(r == m1, idx, S - 1))
        r2 = jnp.where(idx == i1, -jnp.inf, r)
        m2 = jnp.max(r2)
        i2 = jnp.min(jnp.where(r2 == m2, idx, S - 1))
        return (i1, i2), (m1, m2)

    def select_tokens(ids):
        sel = None
        for row, i in enumerate(ids):
            hit = (_iota((16, T), 0) == row) & (_iota((16, T), 1) == i % T)
            cs = pl.ds(pl.multiple_of((i // T) * T, T), T)
            part = _dot_nt(jnp.where(hit, 1.0, 0.0).astype(bf16), xn[:, cs].astype(bf16))
            sel = part if sel is None else sel + part
        return sel.astype(bf16)

    def moe_gate(xsel, c):
        gpre = _round_bf16(_dot(xsel, wg[:, c * T:(c + 1) * T]))
        return _round_bf16(gpre * _sigmoid(gpre))

    def moe_up(xsel, c):
        return _round_bf16(_dot(xsel, wu[:, c * T:(c + 1) * T]))

    def moe_down(hid, c, y):
        part = _dot_nt(hid, wd[:, c * T:(c + 1) * T])
        return part if y is None else y + part

    def moe_result(sel_scores, y):
        row = _iota((16, D), 0)
        gate = jnp.where(row == 0, sel_scores[0], sel_scores[1])
        return (_round_bf16(y) * _round_bf16(_sigmoid(gate))).astype(bf16)

    def patch_early(ids, y):
        for k, i in enumerate(ids):
            hit = (_iota((16, T), 0) == k) & (_iota((16, T), 1) == i % T) & (i < EARLY * L)
            cs = pl.ds(pl.multiple_of((jnp.minimum(i, EARLY * L - 1) // T) * T, T), T)
            ao[:, cs] = ao[:, cs] + _dot_tn(y, jnp.where(hit, 1.0, 0.0).astype(bf16))

    def out_lhs(ids, y):
        place = (_iota((16, T), 1) == _iota((16, T), 0) + 64) & (_iota((16, T), 0) < 2)
        ycols = _dot_tn(y, jnp.where(place, 1.0, 0.0).astype(bf16))
        last = _to_bf16(wot[:, 4 * T:5 * T]).astype(f32) + ycols
        for s in range(EARLY, NSEG):
            tok = _iota((64, L), 1) + s * L
            rows = _iota((64, L), 0)
            hit = ((rows == 0) & (tok == ids[0])) | ((rows == 1) & (tok == ids[1]))
            ot[s, D:D + 64, :] = jnp.where(hit, 1.0, 0.0)
        return jnp.concatenate([_to_bf16(wot[:, 0:4 * T]), last.astype(bf16)], axis=1)

    def out_project_early(s, tt):
        cs = tile_cols(s, tt)
        attn = _dot(_to_bf16(wot[:, 0:D]), ot[s, 0:D, local_cols(tt)].astype(bf16))
        ao[:, cs] = attn + xn[:, cs] + xt[:, cs].astype(f32)

    def flush_early(s, tt):
        cs = tile_cols(s, tt)
        outb[:, cs] = ao[:, cs].astype(bf16)

    def out_project(lhs, s, tt):
        cs = tile_cols(s, tt)
        attn = _dot(lhs, ot[s, :, local_cols(tt)].astype(bf16))
        outb[:, cs] = (attn + xn[:, cs] + xt[:, cs].astype(f32)).astype(bf16)

    def row_maxima():
        def project_tile(tt, carry):
            cs = pl.ds(pl.multiple_of(tt * T, T), T)
            y = _layernorm_apply(xt[:, cs], _layernorm_stats(xt[:, cs])).astype(bf16)
            kall[:, cs] = _dot(_to_bf16(wt[0:half, :]), y).astype(bf16)
            qall[:, cs] = (_dot(_to_bf16(wt[half:2 * half, :]), y) * QSCALE).astype(bf16)
            return carry

        lax.fori_loop(0, S // T, project_tile, 0)

        def head_tile(i, carry):
            h = i // (S // T)
            tt = i % (S // T)
            cs = pl.ds(pl.multiple_of(tt * T, T), T)
            seg = pl.ds(pl.multiple_of((tt // NT) * L, L), L)
            rows = _iota((D, T), 0)
            qm = jnp.where((rows >= DH * h) & (rows < DH * h + DH), qall[:, cs].astype(f32), 0.0)
            logits = _dot_tn(kall[:, seg], qm.astype(bf16))
            seen = _iota((L, T), 0) <= _iota((L, T), 1) + (tt % NT) * T
            m = jnp.max(jnp.where(seen, logits, NEG_BIG), axis=0, keepdims=True)
            mx[:, cs] = jnp.where(_iota((H, T), 0) == h, m, mx[:, cs])
            return carry

        lax.fori_loop(0, H * (S // T), head_tile, 0)

        def pack_tile(tt, carry):
            cs = pl.ds(pl.multiple_of(tt * T, T), T)
            m = mx[:, cs]
            block = _iota((1, T), 1) // SUB
            for b in range(NQUAD):
                for i in range(4):
                    row = jnp.zeros((1, T), f32)
                    for a in range(4):
                        src = m[4 * b + a:4 * b + a + 1, :]
                        shift = (SUB * (a - i)) % T
                        row = jnp.where(block == a, src if shift == 0 else pltpu.roll(src, shift, 1), row)
                    mxp[tt, 4 * b + i:4 * b + i + 1, :] = row
            return carry

        lax.fori_loop(0, S // T, pack_tile, 0)

    x0_copy.start()
    wk_copy.start()
    mx[...] = jnp.zeros(mx.shape, f32)
    mxp[...] = jnp.zeros(mxp.shape, f32)
    wot[:, 4 * T:5 * T] = jnp.zeros((half, T), u32)
    with _scope('p0_wait'):
        x0_copy.wait()
        wk_copy.wait()
    for c in (wq_copy, wv_copy, xr_copy, wo_copy, beta_copy, wr_copy, *moe_copies):
        c.start()
    pk, pq = {}, {}
    with _scope('p1'):
        wt[0:half, :] = transpose_weight(0)
        for tt in range(NT):
            normalize(0, tt, ln_stats(0, tt))
            pk[0, tt] = project_k(0, tt)
    with _scope('p2_wait'):
        wq_copy.wait()
        wv_copy.wait()
    with _scope('p2'):
        wt[half:2 * half, :] = transpose_weight(1)
        wt[2 * half:3 * half, :] = transpose_weight(2)
        csq = []
        for tt in range(NT):
            tie = None
            if tt > 0:
                csq.append(col_sq_max(tt - 1))
                tie = _zero_after(csq[-1])
            project_q(0, tt, tie)
        for tt in range(NT):
            project_v(0, tt)
        bound2 = (QSCALE * LN_NORM2 * DH) ** 2 * csq[0] * csq[1]
        ok = jnp.logical_and(bound2 <= LOGIT_LIMIT ** 2, LN_NORM2 * csq[2] <= VALUE_LIMIT ** 2)
        unsafe = jnp.max(jnp.where(ok, 0, 1)) > 0
    with _scope('p3_wait'):
        for c in (xr_copy, wo_copy, beta_copy, wr_copy):
            c.wait()

    @pl.when(unsafe)
    def _():
        row_maxima()

    gb[...] = _sigmoid(jnp.broadcast_to(beta_ref[...].astype(f32).reshape(1, H), (T, H)).T)

    slots = {}
    st = {}

    def at(s, b, j, fn):
        slots.setdefault((s, b, j), []).append(fn)

    def at_pos(s, pos, fn):
        at(s, pos // NT, pos % NT, fn)

    def wr_lhs():
        if 'wr' not in st:
            w = jnp.broadcast_to(wr_ref[...].astype(f32).reshape(1, D), (16, D))
            st['wr'] = jnp.where(_iota((16, D), 0) == 0, w, 0.0).astype(bf16)
        return st['wr']

    stats = {}

    def stats_task(s, tt):
        def fn():
            stats[s, tt] = ln_stats(s, tt)
            if CFG['tie_stats']:
                ties.append((0, _zero_after(stats[s, tt][1])))
        return fn

    def norm_task(s, tt):
        return lambda: normalize(s, tt, stats[s, tt])

    def score_task(s, tt):
        return lambda: router_scores(wr_lhs(), s, tt)

    for s in range(NSEG - 1):
        for g in range(NGRP):
            at_pos(s, 2 * g, lambda s=s, g=g: memory_update(s, g, [pk[s, tt] for tt in range(NT)]))
        if s == 0:
            at_pos(0, 3, stats_task(1, 0))
            at_pos(0, 5, norm_task(1, 0))
        for tt in range(NT):
            p0 = 9 + 6 * tt
            if s == 0:
                at_pos(s, p0, stats_task(2, tt))
                if tt > 0:
                    at_pos(s, p0, norm_task(3, tt - 1))
            at_pos(s, p0, lambda s=s, tt=tt: pk.__setitem__((s + 1, tt), project_k(s + 1, tt)))
            if s == 0:
                if tt > 0:
                    at_pos(s, p0, score_task(3, tt - 1))
                at_pos(s, p0 + 2, norm_task(2, tt))
                if tt + 1 < NT:
                    at_pos(s, p0 + 2, stats_task(1, tt + 1))
            at_pos(s, p0 + 2, lambda s=s, tt=tt: pq.__setitem__((s + 1, tt), project_q(s + 1, tt)))
            if s == 0:
                at_pos(s, p0 + 2, score_task(2, tt))
            at_pos(s, p0 + 3, lambda s=s, tt=tt: memory_read(s + 1, tt, pq[s + 1, tt]))
            if s == 0:
                if tt + 1 < NT:
                    at_pos(s, p0 + 4, norm_task(1, tt + 1))
                at_pos(s, p0 + 4, stats_task(3, tt))
            at_pos(s, p0 + 4, lambda s=s, tt=tt: project_v(s + 1, tt))
    at_pos(1, 0, norm_task(3, NT - 1))
    for s in range(EARLY):
        for tt in range(NT):
            at_pos(s + 1, 1 + 2 * tt if s > 0 else 8 + 6 * tt, lambda s=s, tt=tt: out_project_early(s, tt))
    at_pos(1, 1, score_task(3, NT - 1))
    for tt in range(NT):
        at_pos(0, 1 + 2 * tt, score_task(0, tt))
        at_pos(0, 10 + 6 * tt, score_task(1, tt))
    at_pos(0, 22, lambda: wot.__setitem__((slice(None), slice(0, D)), transpose_weight(3)))

    at_pos(1, 2, lambda: st.update(zip(('ids', 'sel'), route())))
    at_pos(1, 16, lambda: st.update(xsel=select_tokens(st['ids']), y=None))

    def wait_moe():
        with _scope('moe_wait'):
            for c in moe_copies:
                c.wait()

    at(2, 0, -1, wait_moe)
    hid = {}
    for c in range(NCHUNK):
        pos = (c * 30) // NCHUNK
        at_pos(2, pos, lambda c=c: hid.__setitem__(('g', c), moe_gate(st['xsel'], c)))
        at_pos(2, pos, lambda c=c: hid.__setitem__(('u', c), moe_up(st['xsel'], c)))
        at_pos(2, pos + 1, lambda c=c: st.update(y=moe_down(
            (hid.pop(('g', c)) * hid.pop(('u', c))).astype(bf16), c, st['y'])))

    def finish_moe():
        y = moe_result(st['sel'], st['y'])
        patch_early(st['ids'], y)
        st['lhs'] = out_lhs(st['ids'], y)

    at_pos(3, 0, finish_moe)
    for tt in range(NT):
        at_pos(3, 4 + 3 * tt, lambda tt=tt: out_project(st['lhs'], 2, tt))
    at_pos(3, 14, lambda: out_copy(2 * L, 3 * L, 2).start())
    for s in range(EARLY):
        for tt in range(NT):
            at_pos(3, 15 + NT * s + tt, lambda s=s, tt=tt: flush_early(s, tt))
        at_pos(3, 15 + NT * s + NT, lambda s=s: out_copy(s * L, (s + 1) * L, s).start())

    def quad_values(s, b, j, ps):
        for a in range(4):
            values(s, 4 * b + a, j, ps[a])

    pending = []
    for s in range(NSEG):
        for b in range(NQUAD):
            for fn in slots.pop((s, b, -1), ()):
                fn()
            for j in range(NT):
                pending.append((s, b, j, scores(s, b, j)))
                for fn in slots.pop((s, b, j), ()):
                    fn()
                if len(pending) > CFG['lag']:
                    quad_values(*pending.pop(0))
    for unit in pending:
        quad_values(*unit)
    assert not slots, slots.keys()
    s = NSEG - 1
    for tt in range(NT):
        out_project(st['lhs'], s, tt)
        out_copy(s * L + tt * T, s * L + (tt + 1) * T, 3 + tt).start()
    with _scope('out_wait'):
        for k in range(NSEG - 1):
            out_copy(k * L, (k + 1) * L, k).wait()
        for tt in range(NT):
            out_copy(s * L + tt * T, s * L + (tt + 1) * T, 3 + tt).wait()


@jax.jit
def pallas_parallel_sum__memory_aug_infini_attn__moe_arch_mod__prompt_kernel(
    A_x: jax.Array,
    A_wq: jax.Array,
    A_wk: jax.Array,
    A_wv: jax.Array,
    A_wo: jax.Array,
    A_beta: jax.Array,
    B_x: jax.Array,
    B_w_r: jax.Array,
    B_w_gate: jax.Array,
    B_w_up: jax.Array,
    B_w_down: jax.Array,
):
    del B_x
    x_t = jnp.transpose(A_x, (0, 2, 1)).reshape(D, S)
    wd_t = B_w_down.T
    hbm = pl.BlockSpec(memory_space=pl.ANY)
    out_t = pl.pallas_call(
        _kernel,
        out_shape=jax.ShapeDtypeStruct((D, S), bf16),
        in_specs=[hbm] * 10,
        out_specs=hbm,
        scratch_shapes=[
            pltpu.VMEM((D, S), bf16),
            pltpu.VMEM((D, S), f32),
            pltpu.VMEM((4, D, D), bf16),
            pltpu.VMEM((3 * D // 2, D), u32),
            pltpu.VMEM((D // 2, 5 * T), u32),
            pltpu.VMEM((D, F), bf16),
            pltpu.VMEM((D, F), bf16),
            pltpu.VMEM((D, F), bf16),
            pltpu.VMEM((H,), bf16),
            pltpu.VMEM((D,), bf16),
            pltpu.VMEM((2, D, L), f32),
            pltpu.VMEM((2, D, L), f32),
            pltpu.VMEM((2, NQUAD, L // 2, T), u32),
            pltpu.VMEM((2, NGRP, MROWS, L), f32),
            pltpu.VMEM((NGRP, MROWS, T), f32),
            pltpu.VMEM((NGRP, 8, T), f32),
            pltpu.VMEM((NSEG, 5 * T, L), f32),
            pltpu.VMEM((H, S), f32),
            pltpu.VMEM((S // T, H, T), f32),
            pltpu.VMEM((S // T, T), f32),
            pltpu.VMEM((D, EARLY * L), f32),
            pltpu.VMEM((D, S), bf16),
            pltpu.VMEM((H, T), f32),
            pltpu.VMEM((D, S), bf16),
            pltpu.VMEM((D, S), bf16),
            pltpu.SemaphoreType.DMA((18,)),
        ],
        compiler_params=pltpu.CompilerParams(vmem_limit_bytes=100 * 1024 * 1024),
        name="infini_moe",
    )(x_t, A_wq, A_wk, A_wv, A_wo, A_beta, B_w_r, B_w_gate, B_w_up, wd_t)
    return jnp.transpose(out_t.reshape(1, D, S), (0, 2, 1))
```

```python
import contextlib
import functools

import jax
import jax.numpy as jnp
from jax import lax
from jax.experimental import pallas as pl
from jax.experimental.pallas import tpu as pltpu

S, D, H, DH = 2048, 576, 32, 18
NSEG, L, F = 4, 512, 4608
T = 128
NT = L // T
NGRP = 5
SLAB = 112
GROUP_FIRST = (0, 7, 13, 19, 25, 32)
MROWS = 144
NCHUNK = F // T
NQUAD = H // 4
QUAD_OFF = (0, 64, 144, 208, 288, 352, 432, 448)
EARLY = 2
SUB = 32

bf16, f32, u32, i32 = jnp.bfloat16, jnp.float32, jnp.uint32, jnp.int32

LOG2E = 1.4426950408889634
QSCALE = (DH ** -0.5) * LOG2E
LN_NORM2 = 2.1 * D
LOGIT_LIMIT = 64.0
VALUE_LIMIT = 2.0 ** 50
NEG_BIG = -1e30


PROFILE_SCOPES = False
CFG = dict(lag=5, rot=0, tie_stats=True, tie_p=3, fill_proj=12, fill_qk=10, select_pos=7, moe_quad=5)


def _scope(name):
    return jax.named_scope(name) if PROFILE_SCOPES else contextlib.nullcontext()


def _group_of(h):
    for g in range(NGRP):
        if GROUP_FIRST[g] <= h < GROUP_FIRST[g + 1]:
            return g
    raise ValueError(h)


def _to_bf16(x):
    return pltpu.bitcast(x, bf16)


def _to_u32(x):
    return pltpu.bitcast(x, u32)


def _round_bf16(x):
    return x.astype(bf16).astype(f32)


def _iota(shape, dim):
    return lax.broadcasted_iota(i32, shape, dim)


def _dot(a, b):
    return jnp.dot(a, b, preferred_element_type=f32)


def _dot_nt(a, b):
    return lax.dot_general(a, b, (((1,), (1,)), ((), ())), preferred_element_type=f32)


def _dot_tn(a, b):
    return lax.dot_general(a, b, (((0,), (0,)), ((), ())), preferred_element_type=f32)


def _zero_after_bits(u):
    return lax.shift_right_logical(pltpu.bitcast(u, i32), 31).astype(f32) * 0.0


def _pack_pairs(x):
    lo = jnp.concatenate([x[r:r + 8] for r in range(0, x.shape[0], 16)], axis=0)
    hi = jnp.concatenate([x[r + 8:r + 16] for r in range(0, x.shape[0], 16)], axis=0)
    return pltpu.pack_elementwise([lo, hi], packed_dtype=bf16)


def _unpaired_index(r):
    x = r & 15
    return (r - x) + jnp.where(x < 8, 2 * x, 2 * (x - 8) + 1)


def _phi(t):
    return jnp.where(t > 0, t + 1.0, jnp.exp(t))


def _sigmoid(t):
    return 1.0 / (1.0 + jnp.exp(-t))


def _layernorm_stats(xb):
    x0 = xb[0:1, :].astype(f32)
    acc1, acc2 = [None] * 4, [None] * 4
    for n, r in enumerate(range(0, D, 16)):
        c = xb[r:r + 16, :].astype(f32) - x0
        for part in range(2):
            k = (2 * n + part) % 4
            piece = c[8 * part:8 * part + 8, :]
            acc1[k] = piece if acc1[k] is None else acc1[k] + piece
            acc2[k] = piece * piece if acc2[k] is None else acc2[k] + piece * piece
    s1 = jnp.sum((acc1[0] + acc1[1]) + (acc1[2] + acc1[3]), axis=0, keepdims=True) / D
    s2 = jnp.sum((acc2[0] + acc2[1]) + (acc2[2] + acc2[3]), axis=0, keepdims=True) / D
    var = jnp.maximum(s2 - s1 * s1, 0.0)
    eps = _round_bf16(jnp.full((1, 1), 1e-5, f32))
    sd = _round_bf16(jnp.sqrt(_round_bf16(_round_bf16(var) + eps)))
    return _round_bf16(x0 + s1), 1.0 / sd


def _layernorm_apply(xb, stats):
    mean, inv = stats
    return _round_bf16(xb.astype(f32) - mean) * inv


def _block_transpose(xs):
    lane = _iota(next(x for x in xs if x is not None).shape, 1)

    def exchange(u, v, low, shift):
        def pick(p, q):
            if p is None and q is None:
                return None
            return jnp.where(low, 0.0 if p is None else p, 0.0 if q is None else q)
        ru = None if u is None else pltpu.roll(u, T - shift, 1)
        rv = None if v is None else pltpu.roll(v, shift, 1)
        return pick(u, rv), pick(ru, v)

    y0, y2 = exchange(xs[0], xs[2], lane < 64, 64)
    y1, y3 = exchange(xs[1], xs[3], lane < 64, 64)
    low = (lane & 32) == 0
    z0, z1 = exchange(y0, y1, low, 32)
    z2, z3 = exchange(y2, y3, low, 32)
    return [z0, z1, z2, z3]


def _head_of_slab_index(idx, g):
    return ((idx + SLAB * g) * 3641) >> 16


def _zero_after(x):
    sign = lax.shift_right_logical(pltpu.bitcast(x, i32), 31)
    return sign.astype(f32) * 0.0


def _kernel(x_hbm, wq_hbm, wk_hbm, wv_hbm, wo_hbm, beta_hbm, wr_hbm, wg_hbm, wu_hbm, wd_hbm,
            out_hbm,
            xt, xn, wstage, wt, wot, wg, wu, wd, beta_ref, wr_ref, qt, vt, kp, num, mt, zt, ot,
            mx, mxp, rrow, ao, outb, gb, kall, qall, sems):
    def copy(src, dst, i):
        return pltpu.make_async_copy(src, dst, sems.at[i])

    x0_copy = copy(x_hbm.at[:, 0:L], xt.at[:, 0:L], 0)
    xr_copy = copy(x_hbm.at[:, L:S], xt.at[:, L:S], 1)
    wk_copy, wq_copy, wv_copy, wo_copy = [
        copy(w, wstage.at[i], 2 + i) for i, w in enumerate((wk_hbm, wq_hbm, wv_hbm, wo_hbm))]
    beta_copy = copy(beta_hbm, beta_ref, 6)
    wr_copy = copy(wr_hbm, wr_ref, 7)
    moe_copies = [copy(wg_hbm, wg, 8), copy(wu_hbm, wu, 9), copy(wd_hbm, wd, 10)]

    def out_copy(lo, hi, i):
        return copy(outb.at[:, lo:hi], out_hbm.at[:, lo:hi], 11 + i)

    half = D // 2
    emitted = set()

    def produced(*key):
        emitted.add(key)

    def require(*key):
        assert key in emitted, key

    def require_heads(s, j):
        for h in range(H):
            require('ot', s, h, j)

    fillers = []

    def fill(n):
        for _ in range(min(n, len(fillers))):
            fillers.pop(0)()

    ties = []

    def tile_cols(s, tt):
        return slice(s * L + tt * T, s * L + (tt + 1) * T)

    def local_cols(tt):
        return slice(tt * T, (tt + 1) * T)

    def col_sq_part(i, lo, hi):
        acc = None
        for r in range(lo, hi, 16):
            w = wstage[i, r:r + 16, :].astype(f32)
            w = w * w
            part = w[0:8] + w[8:16]
            acc = part if acc is None else acc + part
        return acc

    def col_sq_max(parts):
        acc = functools.reduce(lambda u, v: u + v, parts)
        return jnp.max(jnp.sum(acc, axis=0, keepdims=True), axis=1, keepdims=True)

    def tie_of(part):
        folded = functools.reduce(lambda u, v: u + v, [part[:, c:c + T] for c in range(0, 4 * T, T)])
        return _zero_after(folded[0:1, 0:1] + part[0:1, 4 * T:4 * T + 1])

    def transpose_weight(i):
        return _to_u32(wstage[i].T)

    def ln_stats(s, tt):
        return _layernorm_stats(xt[:, tile_cols(s, tt)])

    def normalize(s, tt, stats):
        cs = tile_cols(s, tt)
        xn[:, cs] = _layernorm_apply(xt[:, cs], stats)
        produced('xn', s, tt)

    def xn_tile(s, tt):
        require('xn', s, tt)
        return xn[:, tile_cols(s, tt)].astype(bf16)

    def keys_raw(s, tt):
        kt = _dot(_to_bf16(wt[0:half, :]), xn_tile(s, tt))
        fill(CFG['fill_proj'])
        return kt

    def keys_finish(s, tt, kt, tie=None):
        kt = _round_bf16(kt if tie is None else kt + tie)
        shuffled = jnp.take_along_axis(kt, _unpaired_index(_iota((D, T), 1)), axis=1)
        for b in range(NQUAD):
            kp[s % 2, b, tt * (T // 2):(tt + 1) * (T // 2), :] = _to_u32(
                shuffled[QUAD_OFF[b]:QUAD_OFF[b] + T, :].astype(bf16).T)
        produced('k', s, tt)
        return _phi(kt).astype(bf16)

    def project_k(s, tt):
        return keys_finish(s, tt, keys_raw(s, tt))

    def project_q(s, tt, tie=None):
        q = _dot(_to_bf16(wt[half:2 * half, :]), xn_tile(s, tt))
        fill(CFG['fill_proj'])
        qt[s % 2, :, local_cols(tt)] = q * (QSCALE if tie is None else QSCALE + tie)
        produced('q', s, tt)
        return _phi(_round_bf16(q)).astype(bf16)

    def require_segment_done(s):
        if s >= 0:
            for j in range(NT):
                require_heads(s, j)

    def project_v(s, tt, tie=None):
        require_segment_done(s - 2)
        v = _dot(_to_bf16(wt[2 * half:3 * half, :]), xn_tile(s, tt))
        fill(CFG['fill_proj'])
        vt[s % 2, :, local_cols(tt)] = v if tie is None else v + tie
        produced('v', s, tt)

    def router_scores(lhs, s, tt):
        row = s * NT + tt
        rrow[row:row + 1, :] = _dot(lhs, xn_tile(s, tt))[0:1, :]
        produced('r', s, tt)

    def memory_read(s, tt, pq):
        require_segment_done(s - 2)
        for g in range(NGRP):
            require('mt', s - 1, g)
        for g in range(NGRP):
            num[s % 2, g, :, local_cols(tt)] = _dot(mt[g].astype(bf16), pq[SLAB * g:SLAB * g + T, :])
        produced('num', s, tt)

    def memory_update(s, g, pk):
        ones_row = 0 if g == NGRP - 1 else T - 1
        vs = jnp.where(_iota((T, L), 0) == ones_row, 1.0, vt[s % 2, SLAB * g:SLAB * g + T, :]).astype(bf16)
        m = _dot_nt(vs, jnp.concatenate([p[SLAB * g:SLAB * g + T, :] for p in pk], axis=1))
        hr = _head_of_slab_index(_iota((T, T), 0), g)
        hc = _head_of_slab_index(_iota((T, T), 1), g)
        keep = (hr == hc) & (hr >= GROUP_FIRST[g]) & (hr < GROUP_FIRST[g + 1])
        mm = jnp.where(keep, m, 0.0)
        z = m[ones_row:ones_row + 1, :]
        if s > 0:
            mm = mm + mt[g, 0:T, :]
            z = z + zt[g, 0:1, :]
        mt[g, 0:T, :] = mm
        zt[g, 0:1, :] = z
        zsel = _head_of_slab_index(_iota((16, T), 1), g) == _iota((16, T), 0) + GROUP_FIRST[g]
        mt[g, T:MROWS, :] = jnp.where(zsel, z, 0.0)
        produced('mt', s, g)

    def assemble_rows(pieces):
        groups = []
        for r in range(0, T, 8):
            hit = [x[r - r0:r - r0 + 8, :] for r0, x in pieces if r0 <= r < r0 + x.shape[0]]
            groups.append(functools.reduce(lambda u, v: u + v, hit) if hit else None)
        out, r = [], 0
        while r < len(groups):
            if groups[r] is None:
                n = 1
                while r + n < len(groups) and groups[r + n] is None:
                    n += 1
                out.append(jnp.zeros((8 * n, T), f32))
                r += n
            else:
                out.append(groups[r])
                r += 1
        return jnp.concatenate(out, axis=0)

    def quad_queries(s, b, j):
        f0 = QUAD_OFF[b]
        wide, packed = [], [[] for _ in range(4)]
        for a in range(4):
            r0 = DH * (4 * b + a) - f0
            lo = (r0 // 8) * 8
            hi = -(-(r0 + DH) // 8) * 8
            rows = _iota((hi - lo, T), 0) + lo
            mine = (rows >= r0) & (rows < r0 + DH)
            q = qt[s % 2, f0 + lo:f0 + hi, local_cols(j)]
            wide.append(assemble_rows([(lo, jnp.where(mine, q, 0.0))]))
            here = mine & (_iota((hi - lo, T), 1) // SUB == a)
            for i in range(4):
                shift = (SUB * (a - i)) % T
                moved = q if shift == 0 else pltpu.roll(q, shift, 1)
                packed[i].append((lo, jnp.where(here, moved, 0.0)))
        return wide, [assemble_rows(p).astype(bf16) for p in packed]

    def scores(s, b, j):
        require('q', s, j)
        for tt in range(j + 1):
            require('k', s, tt)
        wide, packed = quad_queries(s, b, j)
        tie = None
        unit = (s * NQUAD + b) * NT + j
        due = [z for when, z in ties if when <= unit]
        ties[:] = [(when, z) for when, z in ties if when > unit]
        if due:
            tie = functools.reduce(lambda u, v: u + v, due)
        tile = s * NT + j
        k0 = j * (T // 2)
        off = None
        if j > 0:
            logits = _dot(_to_bf16(kp[s % 2, b, 0:k0, :]), jnp.concatenate(wide, axis=1).astype(bf16))
            fill(CFG['fill_qk'])
            shift = jnp.concatenate([mx[4 * b + a:4 * b + a + 1, tile_cols(s, j)] for a in range(4)], axis=1)
            off = jnp.exp2(logits - shift)
        causal = _unpaired_index(_iota((SUB, T), 0)) <= (_iota((SUB, T), 1) & (SUB - 1))
        diag = [None] * 4
        for i in [(k + CFG['rot'] * j) % 4 for k in range(4)]:
            n = SUB * (i + 1)
            logits = _dot(_to_bf16(kp[s % 2, b, k0:k0 + n // 2, :]), packed[i])
            shift = mxp[tile, 4 * b + i:4 * b + i + 1, :]
            if tie is not None and i == 3:
                shift = shift + tie
            e = jnp.exp2(logits - shift)
            blocks = [e[r * SUB:(r + 1) * SUB, :] for r in range(i)]
            blocks.append(jnp.where(causal, e[i * SUB:, :], 0.0))
            diag[i] = blocks
        per_head = [[] for _ in range(4)]
        for r in range(4):
            outs = _block_transpose([diag[i][r] if i >= r else None for i in range(4)])
            for a in range(4):
                per_head[a].append(outs[a])
        ps = []
        for a in range(4):
            parts = ([off[:, a * T:(a + 1) * T]] if j > 0 else []) + per_head[a]
            ps.append(_pack_pairs(jnp.concatenate(parts, axis=0)))
        if CFG['tie_p'] is not None:
            rows = [u[r:r + 8] for u in ps for r in range(0, u.shape[0], 8)]
            while len(rows) > 1:
                rows = [rows[i] | rows[i + 1] for i in range(0, len(rows) - 1, 2)] + rows[len(rows) & ~1:]
            ties.append((unit + CFG['tie_p'], _zero_after_bits(rows[0])[0:1, :]))
        return [_to_bf16(u) for u in ps]

    def values(s, h, j, p):
        g = _group_of(h)
        w0 = min((DH * h // 16) * 16, D - 32)
        off = DH * h - w0
        ones_row = 31 if off < 14 else 0
        n = (j + 1) * T
        cs = local_cols(j)
        for tt in range(j + 1):
            require('v', s, tt)
        if s > 0:
            require('num', s, j)
        vwin = jnp.where(_iota((32, n), 0) == ones_row, 1.0, vt[s % 2, w0:w0 + 32, 0:n]).astype(bf16)
        gate = gb[h:h + 1, :]
        acc = _dot(vwin, p)
        res = acc * ((1.0 - gate) / acc[ones_row:ones_row + 1, :])
        if s > 0:
            m0 = w0 - SLAB * g
            zr = T + h - GROUP_FIRST[g]
            den = num[s % 2, g, zr:zr + 1, cs] + 1e-6
            res = res + num[s % 2, g, m0:m0 + 32, cs] * (gate / den)
        else:
            ties.append((0, _zero_after((res[0:8] + res[8:16]) + (res[16:24] + res[24:32]))[0:1, :]))
        ot[s, DH * h:DH * h + DH, cs] = res[off:off + DH, :]
        produced('ot', s, h, j)

    def route():
        for s in range(NSEG):
            for tt in range(NT):
                require('r', s, tt)
        r = _round_bf16(rrow[...])
        idx = _iota((S // T, T), 0) * T + _iota((S // T, T), 1)
        m1 = jnp.max(r)
        i1 = jnp.min(jnp.where(r == m1, idx, S - 1))
        r2 = jnp.where(idx == i1, -jnp.inf, r)
        m2 = jnp.max(r2)
        i2 = jnp.min(jnp.where(r2 == m2, idx, S - 1))
        return (i1, i2), (m1, m2)

    def select_tokens(ids):
        sel = None
        for row, i in enumerate(ids):
            hit = (_iota((16, T), 0) == row) & (_iota((16, T), 1) == i % T)
            cs = pl.ds(pl.multiple_of((i // T) * T, T), T)
            part = _dot_nt(jnp.where(hit, 1.0, 0.0).astype(bf16), xn[:, cs].astype(bf16))
            sel = part if sel is None else sel + part
        return sel.astype(bf16)

    def queue_moe(xsel, state):
        ktiles = [(k, min(k + T, D)) for k in range(0, D, T)]
        pre, hid = {}, {}
        ycols = state['ycols'] = [None] * len(ktiles)

        def first(w, name, c, lo, hi):
            def fn():
                part = _dot(xsel[:, lo:hi], w[lo:hi, c * T:(c + 1) * T])
                pre[name, c] = part if lo == 0 else pre[name, c] + part
            return fn

        def down(c, n, lo, hi):
            def fn():
                if c not in hid:
                    gpre = _round_bf16(pre.pop(('g', c)))
                    gact = _round_bf16(gpre * _sigmoid(gpre))
                    hid[c] = (gact * _round_bf16(pre.pop(('u', c)))).astype(bf16)
                part = _dot_nt(hid[c], wd[lo:hi, c * T:(c + 1) * T])
                ycols[n] = part if ycols[n] is None else ycols[n] + part
            return fn

        for c in range(NCHUNK + 2):
            if c < NCHUNK:
                for lo, hi in ktiles:
                    fillers.append(first(wg, 'g', c, lo, hi))
                    fillers.append(first(wu, 'u', c, lo, hi))
            if c >= 2:
                for n, (lo, hi) in enumerate(ktiles):
                    fillers.append(down(c - 2, n, lo, hi))

    def moe_result(sel_scores, y):
        row = _iota((16, D), 0)
        gate = jnp.where(row == 0, sel_scores[0], sel_scores[1])
        return (_round_bf16(y) * _round_bf16(_sigmoid(gate))).astype(bf16)

    def patch_early(ids, y):
        for k, i in enumerate(ids):
            hit = (_iota((16, T), 0) == k) & (_iota((16, T), 1) == i % T) & (i < EARLY * L)
            cs = pl.ds(pl.multiple_of((jnp.minimum(i, EARLY * L - 1) // T) * T, T), T)
            ao[:, cs] = ao[:, cs] + _dot_tn(y, jnp.where(hit, 1.0, 0.0).astype(bf16))

    def out_lhs(ids, y):
        place = (_iota((16, T), 1) == _iota((16, T), 0) + 64) & (_iota((16, T), 0) < 2)
        ycols = _dot_tn(y, jnp.where(place, 1.0, 0.0).astype(bf16))
        last = _to_bf16(wot[:, 4 * T:5 * T]).astype(f32) + ycols
        for s in range(EARLY, NSEG):
            tok = _iota((64, L), 1) + s * L
            rows = _iota((64, L), 0)
            hit = ((rows == 0) & (tok == ids[0])) | ((rows == 1) & (tok == ids[1]))
            ot[s, D:D + 64, :] = jnp.where(hit, 1.0, 0.0)
        return jnp.concatenate([_to_bf16(wot[:, 0:4 * T]), last.astype(bf16)], axis=1)

    def out_project_early(s, tt):
        require_heads(s, tt)
        require('wot')
        cs = tile_cols(s, tt)
        attn = _dot(_to_bf16(wot[:, 0:D]), ot[s, 0:D, local_cols(tt)].astype(bf16))
        fill(CFG['fill_proj'])
        ao[:, cs] = attn + xn[:, cs] + xt[:, cs].astype(f32)

    def flush_early(s, tt):
        cs = tile_cols(s, tt)
        outb[:, cs] = ao[:, cs].astype(bf16)

    def out_project(lhs, s, tt):
        require_heads(s, tt)
        cs = tile_cols(s, tt)
        attn = _dot(lhs, ot[s, :, local_cols(tt)].astype(bf16))
        outb[:, cs] = (attn + xn[:, cs] + xt[:, cs].astype(f32)).astype(bf16)

    def row_maxima():
        def project_tile(tt, carry):
            cs = pl.ds(pl.multiple_of(tt * T, T), T)
            y = _layernorm_apply(xt[:, cs], _layernorm_stats(xt[:, cs])).astype(bf16)
            kall[:, cs] = _dot(_to_bf16(wt[0:half, :]), y).astype(bf16)
            qall[:, cs] = (_dot(_to_bf16(wt[half:2 * half, :]), y) * QSCALE).astype(bf16)
            return carry

        lax.fori_loop(0, S // T, project_tile, 0)

        def head_tile(i, carry):
            h = i // (S // T)
            tt = i % (S // T)
            cs = pl.ds(pl.multiple_of(tt * T, T), T)
            seg = pl.ds(pl.multiple_of((tt // NT) * L, L), L)
            rows = _iota((D, T), 0)
            qm = jnp.where((rows >= DH * h) & (rows < DH * h + DH), qall[:, cs].astype(f32), 0.0)
            logits = _dot_tn(kall[:, seg], qm.astype(bf16))
            seen = _iota((L, T), 0) <= _iota((L, T), 1) + (tt % NT) * T
            m = jnp.max(jnp.where(seen, logits, NEG_BIG), axis=0, keepdims=True)
            mx[:, cs] = jnp.where(_iota((H, T), 0) == h, m, mx[:, cs])
            return carry

        lax.fori_loop(0, H * (S // T), head_tile, 0)

        def pack_tile(tt, carry):
            cs = pl.ds(pl.multiple_of(tt * T, T), T)
            m = mx[:, cs]
            block = _iota((1, T), 1) // SUB
            for b in range(NQUAD):
                for i in range(4):
                    row = jnp.zeros((1, T), f32)
                    for a in range(4):
                        src = m[4 * b + a:4 * b + a + 1, :]
                        shift = (SUB * (a - i)) % T
                        row = jnp.where(block == a, src if shift == 0 else pltpu.roll(src, shift, 1), row)
                    mxp[tt, 4 * b + i:4 * b + i + 1, :] = row
            return carry

        lax.fori_loop(0, S // T, pack_tile, 0)

    for c in (x0_copy, wk_copy, wq_copy, wv_copy, xr_copy, wo_copy, beta_copy, wr_copy, *moe_copies):
        c.start()
    mx[...] = jnp.zeros(mx.shape, f32)
    mxp[...] = jnp.zeros(mxp.shape, f32)
    wot[:, 4 * T:5 * T] = jnp.zeros((half, T), u32)
    pk, pq = {}, {}
    sq = [[], [], []]

    def sq_tie(i, n, parts):
        rows = -(-D // (16 * parts)) * 16
        part = col_sq_part(i, n * rows, min(D, (n + 1) * rows))
        sq[i].append(part)
        return tie_of(part)

    with _scope('p0_wait'):
        x0_copy.wait()
    with _scope('p0'):
        for tt in range(NT):
            normalize(0, tt, ln_stats(0, tt))
    with _scope('p1_wait'):
        wk_copy.wait()
    with _scope('p1'):
        wt[0:half, :] = transpose_weight(0)
        k0 = keys_raw(0, 0)
        k1 = keys_raw(0, 1)
        pk[0, 0] = keys_finish(0, 0, k0, sq_tie(0, 0, 2))
        k2 = keys_raw(0, 2)
        pk[0, 1] = keys_finish(0, 1, k1, sq_tie(0, 1, 2))
    with _scope('p2_wait'):
        wq_copy.wait()
        wv_copy.wait()
    with _scope('p2'):
        k3 = keys_raw(0, 3)
        wt[half:2 * half, :] = transpose_weight(1)
        wt[2 * half:3 * half, :] = transpose_weight(2)
        pk[0, 2] = keys_finish(0, 2, k2)
        project_q(0, 0, sq_tie(1, 0, 4))
        pk[0, 3] = keys_finish(0, 3, k3)
        for tt in range(1, NT):
            project_q(0, tt, sq_tie(1, tt, 4))
        for tt in range(NT):
            project_v(0, tt, sq_tie(2, tt, 3) if tt < 3 else None)
        csq = [col_sq_max(parts) for parts in sq]
        bound2 = (QSCALE * LN_NORM2 * DH) ** 2 * csq[0] * csq[1]
        ok = jnp.logical_and(bound2 <= LOGIT_LIMIT ** 2, LN_NORM2 * csq[2] <= VALUE_LIMIT ** 2)
        unsafe = jnp.max(jnp.where(ok, 0, 1)) > 0
    with _scope('p4_wait'):
        for c in (xr_copy, wo_copy, beta_copy, wr_copy):
            c.wait()

    @pl.when(unsafe)
    def _():
        row_maxima()

    gb[...] = _sigmoid(jnp.broadcast_to(beta_ref[...].astype(f32).reshape(1, H), (T, H)).T)

    slots = {}
    st = {}

    def at(s, b, j, fn):
        slots.setdefault((s, b, j), []).append(fn)

    def at_pos(s, pos, fn):
        at(s, pos // NT, pos % NT, fn)

    def wr_lhs():
        if 'wr' not in st:
            w = jnp.broadcast_to(wr_ref[...].astype(f32).reshape(1, D), (16, D))
            st['wr'] = jnp.where(_iota((16, D), 0) == 0, w, 0.0).astype(bf16)
        return st['wr']

    stats = {}

    def stats_task(s, tt):
        def fn():
            stats[s, tt] = ln_stats(s, tt)
            if CFG['tie_stats']:
                ties.append((0, _zero_after(stats[s, tt][1])))
        return fn

    def norm_task(s, tt):
        return lambda: normalize(s, tt, stats[s, tt])

    def score_task(s, tt):
        return lambda: router_scores(wr_lhs(), s, tt)

    for s in range(NSEG - 1):
        for g in range(NGRP):
            at_pos(s, 2 * g, lambda s=s, g=g: memory_update(s, g, [pk[s, tt] for tt in range(NT)]))
        if s == 0:
            at_pos(0, 3, stats_task(1, 0))
            at_pos(0, 5, norm_task(1, 0))
        for tt in range(NT):
            p0 = 9 + 6 * tt
            if s == 0:
                at_pos(s, p0, stats_task(2, tt))
                if tt > 0:
                    at_pos(s, p0, norm_task(3, tt - 1))
            at_pos(s, p0, lambda s=s, tt=tt: pk.__setitem__((s + 1, tt), project_k(s + 1, tt)))
            if s == 0:
                if tt > 0:
                    at_pos(s, p0, score_task(3, tt - 1))
                at_pos(s, p0 + 2, norm_task(2, tt))
                if tt + 1 < NT:
                    at_pos(s, p0 + 2, stats_task(1, tt + 1))
            at_pos(s, p0 + 2, lambda s=s, tt=tt: pq.__setitem__((s + 1, tt), project_q(s + 1, tt)))
            if s == 0:
                at_pos(s, p0 + 2, score_task(2, tt))
            at_pos(s, p0 + 3, lambda s=s, tt=tt: memory_read(s + 1, tt, pq[s + 1, tt]))
            if s == 0:
                if tt + 1 < NT:
                    at_pos(s, p0 + 4, norm_task(1, tt + 1))
                at_pos(s, p0 + 4, stats_task(3, tt))
            at_pos(s, p0 + 4, lambda s=s, tt=tt: project_v(s + 1, tt))
    at_pos(1, 0, norm_task(3, NT - 1))
    for s in range(EARLY):
        for tt in range(NT):
            at_pos(s + 1, 3 + 2 * tt if s > 0 else 8 + 6 * tt, lambda s=s, tt=tt: out_project_early(s, tt))
    at_pos(1, 1, score_task(3, NT - 1))
    for tt in range(NT):
        at_pos(0, 1 + 2 * tt, score_task(0, tt))
        at_pos(0, 10 + 6 * tt, score_task(1, tt))
    def set_out_weight():
        wot[:, 0:D] = transpose_weight(3)
        produced('wot')

    at_pos(0, 22, set_out_weight)

    at_pos(1, 2, lambda: st.update(zip(('ids', 'sel'), route())))
    at_pos(1, CFG['select_pos'], lambda: st.update(xsel=select_tokens(st['ids'])))

    def start_moe():
        with _scope('moe_wait'):
            for c in moe_copies:
                c.wait()
        queue_moe(st['xsel'], st)

    at(1, CFG['moe_quad'], -1, start_moe)

    def finish_moe():
        fill(len(fillers))
        y = moe_result(st['sel'], jnp.concatenate(st['ycols'], axis=1))
        patch_early(st['ids'], y)
        st['lhs'] = out_lhs(st['ids'], y)

    at_pos(3, 0, finish_moe)
    for tt in range(NT):
        at_pos(3, 4 + 3 * tt, lambda tt=tt: out_project(st['lhs'], 2, tt))
    at_pos(3, 14, lambda: out_copy(2 * L, 3 * L, 2).start())
    for s in range(EARLY):
        for tt in range(NT):
            at_pos(3, 15 + NT * s + tt, lambda s=s, tt=tt: flush_early(s, tt))
        at_pos(3, 15 + NT * s + NT, lambda s=s: out_copy(s * L, (s + 1) * L, s).start())

    def quad_values(s, b, j, ps):
        for a in range(4):
            values(s, 4 * b + a, j, ps[a])

    pending = []
    for s in range(NSEG):
        for b in range(NQUAD):
            for fn in slots.pop((s, b, -1), ()):
                fn()
            for j in range(NT):
                pending.append((s, b, j, scores(s, b, j)))
                for fn in slots.pop((s, b, j), ()):
                    fn()
                if len(pending) > CFG['lag']:
                    quad_values(*pending.pop(0))
    for unit in pending:
        quad_values(*unit)
    assert not slots, slots.keys()
    s = NSEG - 1
    for tt in range(NT):
        out_project(st['lhs'], s, tt)
        out_copy(s * L + tt * T, s * L + (tt + 1) * T, 3 + tt).start()
    with _scope('out_wait'):
        for k in range(NSEG - 1):
            out_copy(k * L, (k + 1) * L, k).wait()
        for tt in range(NT):
            out_copy(s * L + tt * T, s * L + (tt + 1) * T, 3 + tt).wait()


@jax.jit
def pallas_parallel_sum__memory_aug_infini_attn__moe_arch_mod__prompt_kernel(
    A_x: jax.Array,
    A_wq: jax.Array,
    A_wk: jax.Array,
    A_wv: jax.Array,
    A_wo: jax.Array,
    A_beta: jax.Array,
    B_x: jax.Array,
    B_w_r: jax.Array,
    B_w_gate: jax.Array,
    B_w_up: jax.Array,
    B_w_down: jax.Array,
):
    del B_x
    x_t = jnp.transpose(A_x, (0, 2, 1)).reshape(D, S)
    wd_t = B_w_down.T
    hbm = pl.BlockSpec(memory_space=pl.ANY)
    out_t = pl.pallas_call(
        _kernel,
        out_shape=jax.ShapeDtypeStruct((D, S), bf16),
        in_specs=[hbm] * 10,
        out_specs=hbm,
        scratch_shapes=[
            pltpu.VMEM((D, S), bf16),
            pltpu.VMEM((D, S), f32),
            pltpu.VMEM((4, D, D), bf16),
            pltpu.VMEM((3 * D // 2, D), u32),
            pltpu.VMEM((D // 2, 5 * T), u32),
            pltpu.VMEM((D, F), bf16),
            pltpu.VMEM((D, F), bf16),
            pltpu.VMEM((D, F), bf16),
            pltpu.VMEM((H,), bf16),
            pltpu.VMEM((D,), bf16),
            pltpu.VMEM((2, D, L), f32),
            pltpu.VMEM((2, D, L), f32),
            pltpu.VMEM((2, NQUAD, L // 2, T), u32),
            pltpu.VMEM((2, NGRP, MROWS, L), f32),
            pltpu.VMEM((NGRP, MROWS, T), f32),
            pltpu.VMEM((NGRP, 8, T), f32),
            pltpu.VMEM((NSEG, 5 * T, L), f32),
            pltpu.VMEM((H, S), f32),
            pltpu.VMEM((S // T, H, T), f32),
            pltpu.VMEM((S // T, T), f32),
            pltpu.VMEM((D, EARLY * L), f32),
            pltpu.VMEM((D, S), bf16),
            pltpu.VMEM((H, T), f32),
            pltpu.VMEM((D, S), bf16),
            pltpu.VMEM((D, S), bf16),
            pltpu.SemaphoreType.DMA((18,)),
        ],
        compiler_params=pltpu.CompilerParams(vmem_limit_bytes=100 * 1024 * 1024),
        name="infini_moe",
    )(x_t, A_wq, A_wk, A_wv, A_wo, A_beta, B_w_r, B_w_gate, B_w_up, wd_t)
    return jnp.transpose(out_t.reshape(1, D, S), (0, 2, 1))
```

```python
import contextlib
import functools

import jax
import jax.numpy as jnp
from jax import lax
from jax.experimental import pallas as pl
from jax.experimental.pallas import tpu as pltpu

S, D, H, DH = 2048, 576, 32, 18
NSEG, L, F = 4, 512, 4608
T = 128
NT = L // T
NGRP = 5
SLAB = 112
GROUP_FIRST = (0, 7, 13, 19, 25, 32)
MROWS = 144
NCHUNK = F // T
NQUAD = H // 4
QUAD_OFF = (0, 64, 144, 208, 288, 352, 432, 448)
EARLY = 2
SUB = 32

bf16, f32, u32, i32 = jnp.bfloat16, jnp.float32, jnp.uint32, jnp.int32

LOG2E = 1.4426950408889634
QSCALE = (DH ** -0.5) * LOG2E
LN_NORM2 = 2.1 * D
LOGIT_LIMIT = 64.0
VALUE_LIMIT = 2.0 ** 50
NEG_BIG = -1e30


PROFILE_SCOPES = False
CFG = dict(lag=5, rot=0, tie_stats=True, tie_p=3, fill_proj=10, fill_qk=8, select_pos=7, moe_quad=5, moe_end=8, op_gap=3)


def _scope(name):
    return jax.named_scope(name) if PROFILE_SCOPES else contextlib.nullcontext()


def _group_of(h):
    for g in range(NGRP):
        if GROUP_FIRST[g] <= h < GROUP_FIRST[g + 1]:
            return g
    raise ValueError(h)


def _to_bf16(x):
    return pltpu.bitcast(x, bf16)


def _to_u32(x):
    return pltpu.bitcast(x, u32)


def _round_bf16(x):
    return x.astype(bf16).astype(f32)


def _iota(shape, dim):
    return lax.broadcasted_iota(i32, shape, dim)


def _dot(a, b):
    return jnp.dot(a, b, preferred_element_type=f32)


def _dot_nt(a, b):
    return lax.dot_general(a, b, (((1,), (1,)), ((), ())), preferred_element_type=f32)


def _dot_tn(a, b):
    return lax.dot_general(a, b, (((0,), (0,)), ((), ())), preferred_element_type=f32)


def _zero_after_bits(u):
    return lax.shift_right_logical(pltpu.bitcast(u, i32), 31).astype(f32) * 0.0


def _pack_pairs(x):
    lo = jnp.concatenate([x[r:r + 8] for r in range(0, x.shape[0], 16)], axis=0)
    hi = jnp.concatenate([x[r + 8:r + 16] for r in range(0, x.shape[0], 16)], axis=0)
    return pltpu.pack_elementwise([lo, hi], packed_dtype=bf16)


def _unpaired_index(r):
    x = r & 15
    return (r - x) + jnp.where(x < 8, 2 * x, 2 * (x - 8) + 1)


def _phi(t):
    return jnp.where(t > 0, t + 1.0, jnp.exp(t))


def _sigmoid(t):
    return 1.0 / (1.0 + jnp.exp(-t))


def _layernorm_stats(xb):
    x0 = xb[0:1, :].astype(f32)
    acc1, acc2 = [None] * 4, [None] * 4
    for n, r in enumerate(range(0, D, 16)):
        c = xb[r:r + 16, :].astype(f32) - x0
        for part in range(2):
            k = (2 * n + part) % 4
            piece = c[8 * part:8 * part + 8, :]
            acc1[k] = piece if acc1[k] is None else acc1[k] + piece
            acc2[k] = piece * piece if acc2[k] is None else acc2[k] + piece * piece
    s1 = jnp.sum((acc1[0] + acc1[1]) + (acc1[2] + acc1[3]), axis=0, keepdims=True) / D
    s2 = jnp.sum((acc2[0] + acc2[1]) + (acc2[2] + acc2[3]), axis=0, keepdims=True) / D
    var = jnp.maximum(s2 - s1 * s1, 0.0)
    eps = _round_bf16(jnp.full((1, 1), 1e-5, f32))
    sd = _round_bf16(jnp.sqrt(_round_bf16(_round_bf16(var) + eps)))
    return _round_bf16(x0 + s1), 1.0 / sd


def _layernorm_apply(xb, stats):
    mean, inv = stats
    return _round_bf16(xb.astype(f32) - mean) * inv


def _block_transpose(xs):
    lane = _iota(next(x for x in xs if x is not None).shape, 1)

    def exchange(u, v, low, shift):
        def pick(p, q):
            if p is None and q is None:
                return None
            return jnp.where(low, 0.0 if p is None else p, 0.0 if q is None else q)
        ru = None if u is None else pltpu.roll(u, T - shift, 1)
        rv = None if v is None else pltpu.roll(v, shift, 1)
        return pick(u, rv), pick(ru, v)

    y0, y2 = exchange(xs[0], xs[2], lane < 64, 64)
    y1, y3 = exchange(xs[1], xs[3], lane < 64, 64)
    low = (lane & 32) == 0
    z0, z1 = exchange(y0, y1, low, 32)
    z2, z3 = exchange(y2, y3, low, 32)
    return [z0, z1, z2, z3]


def _head_of_slab_index(idx, g):
    return ((idx + SLAB * g) * 3641) >> 16


def _zero_after(x):
    sign = lax.shift_right_logical(pltpu.bitcast(x, i32), 31)
    return sign.astype(f32) * 0.0


def _kernel(x_hbm, wq_hbm, wk_hbm, wv_hbm, wo_hbm, beta_hbm, wr_hbm, wg_hbm, wu_hbm, wd_hbm,
            out_hbm,
            xt, xn, wstage, wt, wot, wg, wu, wd, beta_ref, wr_ref, qt, vt, kp, num, mt, zt, ot,
            mx, mxp, rrow, outb, gb, kall, qall, sems):
    def copy(src, dst, i):
        return pltpu.make_async_copy(src, dst, sems.at[i])

    xa_copy = copy(x_hbm.at[:, 0:T], xt.at[:, 0:T], 0)
    xb_copy = copy(x_hbm.at[:, T:L], xt.at[:, T:L], 18)
    xr_copy = copy(x_hbm.at[:, L:S], xt.at[:, L:S], 1)
    wk_copy, wq_copy, wv_copy, wo_copy = [
        copy(w, wstage.at[i], 2 + i) for i, w in enumerate((wk_hbm, wq_hbm, wv_hbm, wo_hbm))]
    beta_copy = copy(beta_hbm, beta_ref, 6)
    wr_copy = copy(wr_hbm, wr_ref, 7)
    moe_copies = [copy(wg_hbm, wg, 8), copy(wu_hbm, wu, 9), copy(wd_hbm, wd, 10)]

    def out_copy(lo, hi, i):
        return copy(outb.at[:, lo:hi], out_hbm.at[:, lo:hi], 11 + i)

    half = D // 2
    emitted = set()

    def produced(*key):
        emitted.add(key)

    def require(*key):
        assert key in emitted, key

    def require_heads(s, j):
        for h in range(H):
            require('ot', s, h, j)

    fillers = []

    def fill(n):
        for _ in range(min(n, len(fillers))):
            fillers.pop(0)()

    ties = []

    def tile_cols(s, tt):
        return slice(s * L + tt * T, s * L + (tt + 1) * T)

    def local_cols(tt):
        return slice(tt * T, (tt + 1) * T)

    def col_sq_part(i, lo, hi):
        acc = None
        for r in range(lo, hi, 16):
            w = wstage[i, r:r + 16, :].astype(f32)
            w = w * w
            part = w[0:8] + w[8:16]
            acc = part if acc is None else acc + part
        return acc

    def col_sq_max(parts):
        acc = functools.reduce(lambda u, v: u + v, parts)
        return jnp.max(jnp.sum(acc, axis=0, keepdims=True), axis=1, keepdims=True)

    def tie_of(part):
        folded = functools.reduce(lambda u, v: u + v, [part[:, c:c + T] for c in range(0, 4 * T, T)])
        return _zero_after(folded[0:1, 0:1] + part[0:1, 4 * T:4 * T + 1])

    def transpose_weight(i):
        return _to_u32(wstage[i].T)

    def ln_stats(s, tt):
        return _layernorm_stats(xt[:, tile_cols(s, tt)])

    def normalize(s, tt, stats):
        cs = tile_cols(s, tt)
        xn[:, cs] = _layernorm_apply(xt[:, cs], stats)
        produced('xn', s, tt)

    def xn_tile(s, tt):
        require('xn', s, tt)
        return xn[:, tile_cols(s, tt)].astype(bf16)

    def keys_raw(s, tt, lo=0, hi=D):
        kt = _dot(_to_bf16(wt[lo // 2:hi // 2, :]), xn_tile(s, tt))
        fill(CFG['fill_proj'])
        return kt

    def keys_finish(s, tt, kt, tie=None):
        kt = _round_bf16(kt if tie is None else kt + tie)
        shuffled = jnp.take_along_axis(kt, _unpaired_index(_iota((D, T), 1)), axis=1)
        for b in range(NQUAD):
            kp[s % 2, b, tt * (T // 2):(tt + 1) * (T // 2), :] = _to_u32(
                shuffled[QUAD_OFF[b]:QUAD_OFF[b] + T, :].astype(bf16).T)
        produced('k', s, tt)
        return _phi(kt).astype(bf16)

    def project_k(s, tt):
        return keys_finish(s, tt, keys_raw(s, tt))

    def project_q(s, tt, tie=None):
        q = _dot(_to_bf16(wt[half:2 * half, :]), xn_tile(s, tt))
        fill(CFG['fill_proj'])
        qt[s % 2, :, local_cols(tt)] = q * (QSCALE if tie is None else QSCALE + tie)
        produced('q', s, tt)
        return _phi(_round_bf16(q)).astype(bf16)

    def require_segment_done(s):
        if s >= 0:
            for j in range(NT):
                require_heads(s, j)

    def project_v(s, tt, tie=None):
        require_segment_done(s - 2)
        v = _dot(_to_bf16(wt[2 * half:3 * half, :]), xn_tile(s, tt))
        fill(CFG['fill_proj'])
        vt[s % 2, :, local_cols(tt)] = v if tie is None else v + tie
        produced('v', s, tt)

    def router_scores(lhs, s, tt):
        row = s * NT + tt
        rrow[row:row + 1, :] = _dot(lhs, xn_tile(s, tt))[0:1, :]
        produced('r', s, tt)

    def memory_read(s, tt, pq):
        require_segment_done(s - 2)
        for g in range(NGRP):
            require('mt', s - 1, g)
        for g in range(NGRP):
            num[s % 2, g, :, local_cols(tt)] = _dot(mt[g].astype(bf16), pq[SLAB * g:SLAB * g + T, :])
        produced('num', s, tt)

    def memory_update(s, g, pk):
        ones_row = 0 if g == NGRP - 1 else T - 1
        vs = jnp.where(_iota((T, L), 0) == ones_row, 1.0, vt[s % 2, SLAB * g:SLAB * g + T, :]).astype(bf16)
        m = _dot_nt(vs, jnp.concatenate([p[SLAB * g:SLAB * g + T, :] for p in pk], axis=1))
        hr = _head_of_slab_index(_iota((T, T), 0), g)
        hc = _head_of_slab_index(_iota((T, T), 1), g)
        keep = (hr == hc) & (hr >= GROUP_FIRST[g]) & (hr < GROUP_FIRST[g + 1])
        mm = jnp.where(keep, m, 0.0)
        z = m[ones_row:ones_row + 1, :]
        if s > 0:
            mm = mm + mt[g, 0:T, :]
            z = z + zt[g, 0:1, :]
        mt[g, 0:T, :] = mm
        zt[g, 0:1, :] = z
        zsel = _head_of_slab_index(_iota((16, T), 1), g) == _iota((16, T), 0) + GROUP_FIRST[g]
        mt[g, T:MROWS, :] = jnp.where(zsel, z, 0.0)
        produced('mt', s, g)

    def assemble_rows(pieces):
        groups = []
        for r in range(0, T, 8):
            hit = [x[r - r0:r - r0 + 8, :] for r0, x in pieces if r0 <= r < r0 + x.shape[0]]
            groups.append(functools.reduce(lambda u, v: u + v, hit) if hit else None)
        out, r = [], 0
        while r < len(groups):
            if groups[r] is None:
                n = 1
                while r + n < len(groups) and groups[r + n] is None:
                    n += 1
                out.append(jnp.zeros((8 * n, T), f32))
                r += n
            else:
                out.append(groups[r])
                r += 1
        return jnp.concatenate(out, axis=0)

    def quad_queries(s, b, j):
        f0 = QUAD_OFF[b]
        wide, packed = [], [[] for _ in range(4)]
        for a in range(4):
            r0 = DH * (4 * b + a) - f0
            lo = (r0 // 8) * 8
            hi = -(-(r0 + DH) // 8) * 8
            rows = _iota((hi - lo, T), 0) + lo
            mine = (rows >= r0) & (rows < r0 + DH)
            q = qt[s % 2, f0 + lo:f0 + hi, local_cols(j)]
            wide.append(assemble_rows([(lo, jnp.where(mine, q, 0.0))]))
            here = mine & (_iota((hi - lo, T), 1) // SUB == a)
            for i in range(4):
                shift = (SUB * (a - i)) % T
                moved = q if shift == 0 else pltpu.roll(q, shift, 1)
                packed[i].append((lo, jnp.where(here, moved, 0.0)))
        return wide, [assemble_rows(p).astype(bf16) for p in packed]

    def scores(s, b, j):
        require('q', s, j)
        for tt in range(j + 1):
            require('k', s, tt)
        wide, packed = quad_queries(s, b, j)
        tie = None
        unit = (s * NQUAD + b) * NT + j
        due = [z for when, z in ties if when <= unit]
        ties[:] = [(when, z) for when, z in ties if when > unit]
        if due:
            tie = functools.reduce(lambda u, v: u + v, due)
        tile = s * NT + j
        k0 = j * (T // 2)
        off = None
        if j > 0:
            logits = _dot(_to_bf16(kp[s % 2, b, 0:k0, :]), jnp.concatenate(wide, axis=1).astype(bf16))
            fill(CFG['fill_qk'])
            shift = jnp.concatenate([mx[4 * b + a:4 * b + a + 1, tile_cols(s, j)] for a in range(4)], axis=1)
            off = jnp.exp2(logits - shift)
        causal = _unpaired_index(_iota((SUB, T), 0)) <= (_iota((SUB, T), 1) & (SUB - 1))
        diag = [None] * 4
        for i in [(k + CFG['rot'] * j) % 4 for k in range(4)]:
            n = SUB * (i + 1)
            logits = _dot(_to_bf16(kp[s % 2, b, k0:k0 + n // 2, :]), packed[i])
            shift = mxp[tile, 4 * b + i:4 * b + i + 1, :]
            if tie is not None and i == 3:
                shift = shift + tie
            e = jnp.exp2(logits - shift)
            blocks = [e[r * SUB:(r + 1) * SUB, :] for r in range(i)]
            blocks.append(jnp.where(causal, e[i * SUB:, :], 0.0))
            diag[i] = blocks
        per_head = [[] for _ in range(4)]
        for r in range(4):
            outs = _block_transpose([diag[i][r] if i >= r else None for i in range(4)])
            for a in range(4):
                per_head[a].append(outs[a])
        ps = []
        for a in range(4):
            parts = ([off[:, a * T:(a + 1) * T]] if j > 0 else []) + per_head[a]
            ps.append(_pack_pairs(jnp.concatenate(parts, axis=0)))
        if CFG['tie_p'] is not None:
            rows = [u[r:r + 8] for u in ps for r in range(0, u.shape[0], 8)]
            while len(rows) > 1:
                rows = [rows[i] | rows[i + 1] for i in range(0, len(rows) - 1, 2)] + rows[len(rows) & ~1:]
            ties.append((unit + CFG['tie_p'], _zero_after_bits(rows[0])[0:1, :]))
        return [_to_bf16(u) for u in ps]

    def values(s, h, j, p):
        g = _group_of(h)
        w0 = min((DH * h // 16) * 16, D - 32)
        off = DH * h - w0
        ones_row = 31 if off < 14 else 0
        n = (j + 1) * T
        cs = local_cols(j)
        for tt in range(j + 1):
            require('v', s, tt)
        if s > 0:
            require('num', s, j)
        vwin = jnp.where(_iota((32, n), 0) == ones_row, 1.0, vt[s % 2, w0:w0 + 32, 0:n]).astype(bf16)
        gate = gb[h:h + 1, :]
        acc = _dot(vwin, p)
        res = acc * ((1.0 - gate) / acc[ones_row:ones_row + 1, :])
        if s > 0:
            m0 = w0 - SLAB * g
            zr = T + h - GROUP_FIRST[g]
            den = num[s % 2, g, zr:zr + 1, cs] + 1e-6
            res = res + num[s % 2, g, m0:m0 + 32, cs] * (gate / den)
        else:
            ties.append((0, _zero_after((res[0:8] + res[8:16]) + (res[16:24] + res[24:32]))[0:1, :]))
        ot[s, DH * h:DH * h + DH, cs] = res[off:off + DH, :]
        produced('ot', s, h, j)

    def route():
        for s in range(NSEG):
            for tt in range(NT):
                require('r', s, tt)
        r = _round_bf16(rrow[...])
        idx = _iota((S // T, T), 0) * T + _iota((S // T, T), 1)
        m1 = jnp.max(r)
        i1 = jnp.min(jnp.where(r == m1, idx, S - 1))
        r2 = jnp.where(idx == i1, -jnp.inf, r)
        m2 = jnp.max(r2)
        i2 = jnp.min(jnp.where(r2 == m2, idx, S - 1))
        return (i1, i2), (m1, m2)

    def select_tokens(ids):
        sel = None
        for row, i in enumerate(ids):
            hit = (_iota((16, T), 0) == row) & (_iota((16, T), 1) == i % T)
            cs = pl.ds(pl.multiple_of((i // T) * T, T), T)
            part = _dot_nt(jnp.where(hit, 1.0, 0.0).astype(bf16), xn[:, cs].astype(bf16))
            sel = part if sel is None else sel + part
        return sel.astype(bf16)

    def queue_moe(xsel, state):
        ktiles = [(k, min(k + T, D)) for k in range(0, D, T)]
        pre, hid = {}, {}
        ycols = state['ycols'] = [None] * len(ktiles)

        def first(w, name, c, lo, hi):
            def fn():
                part = _dot(xsel[:, lo:hi], w[lo:hi, c * T:(c + 1) * T])
                pre[name, c] = part if lo == 0 else pre[name, c] + part
            return fn

        def down(c, n, lo, hi):
            def fn():
                if c not in hid:
                    gpre = _round_bf16(pre.pop(('g', c)))
                    gact = _round_bf16(gpre * _sigmoid(gpre))
                    hid[c] = (gact * _round_bf16(pre.pop(('u', c)))).astype(bf16)
                part = _dot_nt(hid[c], wd[lo:hi, c * T:(c + 1) * T])
                ycols[n] = part if ycols[n] is None else ycols[n] + part
            return fn

        for c in range(NCHUNK + 2):
            if c < NCHUNK:
                for lo, hi in ktiles:
                    fillers.append(first(wg, 'g', c, lo, hi))
                    fillers.append(first(wu, 'u', c, lo, hi))
            if c >= 2:
                for n, (lo, hi) in enumerate(ktiles):
                    fillers.append(down(c - 2, n, lo, hi))

    def moe_result(sel_scores, y):
        row = _iota((16, D), 0)
        gate = jnp.where(row == 0, sel_scores[0], sel_scores[1])
        return (_round_bf16(y) * _round_bf16(_sigmoid(gate))).astype(bf16)

    def patch_early(ids, y):
        for k, i in enumerate(ids):
            hit = (_iota((16, T), 0) == k) & (_iota((16, T), 1) == i % T) & (i < EARLY * L)
            cs = pl.ds(pl.multiple_of((jnp.minimum(i, EARLY * L - 1) // T) * T, T), T)
            patch = _dot_tn(y, jnp.where(hit, 1.0, 0.0).astype(bf16))
            outb[:, cs] = (outb[:, cs].astype(f32) + patch).astype(bf16)

    def out_lhs(ids, y):
        place = (_iota((16, T), 1) == _iota((16, T), 0) + 64) & (_iota((16, T), 0) < 2)
        ycols = _dot_tn(y, jnp.where(place, 1.0, 0.0).astype(bf16))
        last = _to_bf16(wot[:, 4 * T:5 * T]).astype(f32) + ycols
        for s in range(EARLY, NSEG):
            tok = _iota((64, L), 1) + s * L
            rows = _iota((64, L), 0)
            hit = ((rows == 0) & (tok == ids[0])) | ((rows == 1) & (tok == ids[1]))
            ot[s, D:D + 64, :] = jnp.where(hit, 1.0, 0.0)
        return jnp.concatenate([_to_bf16(wot[:, 0:4 * T]), last.astype(bf16)], axis=1)

    def out_project_early(s, tt):
        require_heads(s, tt)
        require('wot')
        cs = tile_cols(s, tt)
        attn = _dot(_to_bf16(wot[:, 0:D]), ot[s, 0:D, local_cols(tt)].astype(bf16))
        fill(CFG['fill_proj'])
        outb[:, cs] = (attn + xn[:, cs] + xt[:, cs].astype(f32)).astype(bf16)

    def out_project(lhs, s, tt):
        require_heads(s, tt)
        cs = tile_cols(s, tt)
        attn = _dot(lhs, ot[s, :, local_cols(tt)].astype(bf16))
        outb[:, cs] = (attn + xn[:, cs] + xt[:, cs].astype(f32)).astype(bf16)

    def row_maxima():
        def project_tile(tt, carry):
            cs = pl.ds(pl.multiple_of(tt * T, T), T)
            y = _layernorm_apply(xt[:, cs], _layernorm_stats(xt[:, cs])).astype(bf16)
            kall[:, cs] = _dot(_to_bf16(wt[0:half, :]), y).astype(bf16)
            qall[:, cs] = (_dot(_to_bf16(wt[half:2 * half, :]), y) * QSCALE).astype(bf16)
            return carry

        lax.fori_loop(0, S // T, project_tile, 0)

        def head_tile(i, carry):
            h = i // (S // T)
            tt = i % (S // T)
            cs = pl.ds(pl.multiple_of(tt * T, T), T)
            seg = pl.ds(pl.multiple_of((tt // NT) * L, L), L)
            rows = _iota((D, T), 0)
            qm = jnp.where((rows >= DH * h) & (rows < DH * h + DH), qall[:, cs].astype(f32), 0.0)
            logits = _dot_tn(kall[:, seg], qm.astype(bf16))
            seen = _iota((L, T), 0) <= _iota((L, T), 1) + (tt % NT) * T
            m = jnp.max(jnp.where(seen, logits, NEG_BIG), axis=0, keepdims=True)
            mx[:, cs] = jnp.where(_iota((H, T), 0) == h, m, mx[:, cs])
            return carry

        lax.fori_loop(0, H * (S // T), head_tile, 0)

        def pack_tile(tt, carry):
            cs = pl.ds(pl.multiple_of(tt * T, T), T)
            m = mx[:, cs]
            block = _iota((1, T), 1) // SUB
            for b in range(NQUAD):
                for i in range(4):
                    row = jnp.zeros((1, T), f32)
                    for a in range(4):
                        src = m[4 * b + a:4 * b + a + 1, :]
                        shift = (SUB * (a - i)) % T
                        row = jnp.where(block == a, src if shift == 0 else pltpu.roll(src, shift, 1), row)
                    mxp[tt, 4 * b + i:4 * b + i + 1, :] = row
            return carry

        lax.fori_loop(0, S // T, pack_tile, 0)

    for c in (xa_copy, wk_copy, xb_copy, wq_copy, wv_copy, xr_copy, wo_copy, beta_copy, wr_copy,
              *moe_copies):
        c.start()
    mx[...] = jnp.zeros(mx.shape, f32)
    mxp[...] = jnp.zeros(mxp.shape, f32)
    wot[:, 4 * T:5 * T] = jnp.zeros((half, T), u32)
    pk, pq = {}, {}
    sq = [[], [], []]

    def sq_tie(i, n, parts):
        rows = -(-D // (16 * parts)) * 16
        part = col_sq_part(i, n * rows, min(D, (n + 1) * rows))
        sq[i].append(part)
        return tie_of(part)

    with _scope('p0_wait'):
        xa_copy.wait()
    with _scope('p0'):
        normalize(0, 0, ln_stats(0, 0))
    with _scope('p1_wait'):
        wk_copy.wait()
    with _scope('p1'):
        wt[0:half, :] = transpose_weight(0)
        k0a = keys_raw(0, 0, 0, half)
    with _scope('p1b_wait'):
        xb_copy.wait()
    with _scope('p1b'):
        st1 = ln_stats(0, 1)
        k0 = jnp.concatenate([k0a, keys_raw(0, 0, half, D)], axis=0)
        normalize(0, 1, st1)
        st2 = ln_stats(0, 2)
        k1 = keys_raw(0, 1)
        pk[0, 0] = keys_finish(0, 0, k0, sq_tie(0, 0, 2) + _zero_after(st2[1]))
        normalize(0, 2, st2)
        st3 = ln_stats(0, 3)
        k2 = keys_raw(0, 2)
        pk[0, 1] = keys_finish(0, 1, k1, sq_tie(0, 1, 2) + _zero_after(st3[1]))
        normalize(0, 3, st3)
        k3a = keys_raw(0, 3, 0, half)
    with _scope('p2_wait'):
        wq_copy.wait()
        wv_copy.wait()
    with _scope('p2'):
        k3 = jnp.concatenate([k3a, keys_raw(0, 3, half, D)], axis=0)
        wt[half:2 * half, :] = transpose_weight(1)
        wt[2 * half:3 * half, :] = transpose_weight(2)
        pk[0, 2] = keys_finish(0, 2, k2)
        project_q(0, 0, sq_tie(1, 0, 4))
        pk[0, 3] = keys_finish(0, 3, k3)
        for tt in range(1, NT):
            project_q(0, tt, sq_tie(1, tt, 4))
        for tt in range(NT - 1):
            project_v(0, tt, sq_tie(2, tt, 2) if tt < 2 else None)
        csq = [col_sq_max(parts) for parts in sq]
        bound2 = (QSCALE * LN_NORM2 * DH) ** 2 * csq[0] * csq[1]
        ok = jnp.logical_and(bound2 <= LOGIT_LIMIT ** 2, LN_NORM2 * csq[2] <= VALUE_LIMIT ** 2)
        unsafe = jnp.max(jnp.where(ok, 0, 1)) > 0
    with _scope('p4_wait'):
        for c in (xr_copy, wo_copy, beta_copy, wr_copy):
            c.wait()

    @pl.when(unsafe)
    def _():
        row_maxima()

    project_v(0, NT - 1)
    gb[...] = _sigmoid(jnp.broadcast_to(beta_ref[...].astype(f32).reshape(1, H), (T, H)).T)

    slots = {}
    st = {}

    def at(s, b, j, fn):
        slots.setdefault((s, b, j), []).append(fn)

    def at_pos(s, pos, fn):
        at(s, pos // NT, pos % NT, fn)

    def wr_lhs():
        if 'wr' not in st:
            w = jnp.broadcast_to(wr_ref[...].astype(f32).reshape(1, D), (16, D))
            st['wr'] = jnp.where(_iota((16, D), 0) == 0, w, 0.0).astype(bf16)
        return st['wr']

    stats = {}

    def stats_task(s, tt):
        def fn():
            stats[s, tt] = ln_stats(s, tt)
            if CFG['tie_stats']:
                ties.append((0, _zero_after(stats[s, tt][1])))
        return fn

    def norm_task(s, tt):
        return lambda: normalize(s, tt, stats[s, tt])

    def score_task(s, tt):
        return lambda: router_scores(wr_lhs(), s, tt)

    for s in range(NSEG - 1):
        for g in range(NGRP):
            at_pos(s, 2 * g, lambda s=s, g=g: memory_update(s, g, [pk[s, tt] for tt in range(NT)]))
        if s == 0:
            at_pos(0, 3, stats_task(1, 0))
            at_pos(0, 5, norm_task(1, 0))
        for tt in range(NT):
            p0 = 9 + 6 * tt
            if s == 0:
                at_pos(s, p0, stats_task(2, tt))
                if tt > 0:
                    at_pos(s, p0, norm_task(3, tt - 1))
            at_pos(s, p0, lambda s=s, tt=tt: pk.__setitem__((s + 1, tt), project_k(s + 1, tt)))
            if s == 0:
                if tt > 0:
                    at_pos(s, p0, score_task(3, tt - 1))
                at_pos(s, p0 + 2, norm_task(2, tt))
                if tt + 1 < NT:
                    at_pos(s, p0 + 2, stats_task(1, tt + 1))
            at_pos(s, p0 + 2, lambda s=s, tt=tt: pq.__setitem__((s + 1, tt), project_q(s + 1, tt)))
            if s == 0:
                at_pos(s, p0 + 2, score_task(2, tt))
            at_pos(s, p0 + 3, lambda s=s, tt=tt: memory_read(s + 1, tt, pq[s + 1, tt]))
            if s == 0:
                if tt + 1 < NT:
                    at_pos(s, p0 + 4, norm_task(1, tt + 1))
                at_pos(s, p0 + 4, stats_task(3, tt))
            at_pos(s, p0 + 4, lambda s=s, tt=tt: project_v(s + 1, tt))
    at_pos(1, 0, norm_task(3, NT - 1))
    for s in range(EARLY):
        for tt in range(NT):
            at_pos(s + 1, 3 + 2 * tt if s > 0 else 8 + 6 * tt, lambda s=s, tt=tt: out_project_early(s, tt))
    at_pos(1, 1, score_task(3, NT - 1))
    for tt in range(NT):
        at_pos(0, 1 + 2 * tt, score_task(0, tt))
        at_pos(0, 10 + 6 * tt, score_task(1, tt))
    def set_out_weight():
        wot[:, 0:D] = transpose_weight(3)
        produced('wot')

    at_pos(0, 22, set_out_weight)

    at_pos(1, 2, lambda: st.update(zip(('ids', 'sel'), route())))
    at_pos(1, CFG['select_pos'], lambda: st.update(xsel=select_tokens(st['ids'])))

    def start_moe():
        with _scope('moe_wait'):
            for c in moe_copies:
                c.wait()
        queue_moe(st['xsel'], st)

    at(1, CFG['moe_quad'], -1, start_moe)

    def finish_moe():
        fill(len(fillers))
        y = moe_result(st['sel'], jnp.concatenate(st['ycols'], axis=1))
        patch_early(st['ids'], y)
        st['lhs'] = out_lhs(st['ids'], y)

    e0 = CFG['moe_end']
    at_pos(3, e0, finish_moe)
    for s in range(EARLY):
        at_pos(3, e0 + 1 + s, lambda s=s: out_copy(s * L, (s + 1) * L, s).start())
    for tt in range(NT):
        at_pos(3, e0 + 2 + CFG['op_gap'] * tt, lambda tt=tt: out_project(st['lhs'], 2, tt))
    at_pos(3, e0 + 3 + CFG['op_gap'] * (NT - 1), lambda: out_copy(2 * L, 3 * L, 2).start())

    def quad_values(s, b, j, ps):
        for a in range(4):
            values(s, 4 * b + a, j, ps[a])

    pending = []
    for s in range(NSEG):
        for b in range(NQUAD):
            for fn in slots.pop((s, b, -1), ()):
                fn()
            for j in range(NT):
                pending.append((s, b, j, scores(s, b, j)))
                for fn in slots.pop((s, b, j), ()):
                    fn()
                if len(pending) > CFG['lag']:
                    quad_values(*pending.pop(0))
    tail = [unit for unit in pending]
    assert not slots, slots.keys()
    s = NSEG - 1

    def last_tile(tt):
        out_project(st['lhs'], s, tt)
        out_copy(s * L + tt * T, s * L + (tt + 1) * T, 3 + tt).start()

    done = 0
    for unit in tail:
        quad_values(*unit)
        while done < NT and unit[1] == NQUAD - 1 and done < unit[2]:
            last_tile(done)
            done += 1
    while done < NT:
        last_tile(done)
        done += 1
    with _scope('out_wait'):
        for k in range(NSEG - 1):
            out_copy(k * L, (k + 1) * L, k).wait()
        for tt in range(NT):
            out_copy(s * L + tt * T, s * L + (tt + 1) * T, 3 + tt).wait()


@jax.jit
def pallas_parallel_sum__memory_aug_infini_attn__moe_arch_mod__prompt_kernel(
    A_x: jax.Array,
    A_wq: jax.Array,
    A_wk: jax.Array,
    A_wv: jax.Array,
    A_wo: jax.Array,
    A_beta: jax.Array,
    B_x: jax.Array,
    B_w_r: jax.Array,
    B_w_gate: jax.Array,
    B_w_up: jax.Array,
    B_w_down: jax.Array,
):
    del B_x
    x_t = jnp.transpose(A_x, (0, 2, 1)).reshape(D, S)
    wd_t = B_w_down.T
    hbm = pl.BlockSpec(memory_space=pl.ANY)
    out_t = pl.pallas_call(
        _kernel,
        out_shape=jax.ShapeDtypeStruct((D, S), bf16),
        in_specs=[hbm] * 10,
        out_specs=hbm,
        scratch_shapes=[
            pltpu.VMEM((D, S), bf16),
            pltpu.VMEM((D, S), f32),
            pltpu.VMEM((4, D, D), bf16),
            pltpu.VMEM((3 * D // 2, D), u32),
            pltpu.VMEM((D // 2, 5 * T), u32),
            pltpu.VMEM((D, F), bf16),
            pltpu.VMEM((D, F), bf16),
            pltpu.VMEM((D, F), bf16),
            pltpu.VMEM((H,), bf16),
            pltpu.VMEM((D,), bf16),
            pltpu.VMEM((2, D, L), f32),
            pltpu.VMEM((2, D, L), f32),
            pltpu.VMEM((2, NQUAD, L // 2, T), u32),
            pltpu.VMEM((2, NGRP, MROWS, L), f32),
            pltpu.VMEM((NGRP, MROWS, T), f32),
            pltpu.VMEM((NGRP, 8, T), f32),
            pltpu.VMEM((NSEG, 5 * T, L), f32),
            pltpu.VMEM((H, S), f32),
            pltpu.VMEM((S // T, H, T), f32),
            pltpu.VMEM((S // T, T), f32),
            pltpu.VMEM((D, S), bf16),
            pltpu.VMEM((H, T), f32),
            pltpu.VMEM((D, S), bf16),
            pltpu.VMEM((D, S), bf16),
            pltpu.SemaphoreType.DMA((19,)),
        ],
        compiler_params=pltpu.CompilerParams(vmem_limit_bytes=100 * 1024 * 1024),
        name="infini_moe",
    )(x_t, A_wq, A_wk, A_wv, A_wo, A_beta, B_w_r, B_w_gate, B_w_up, wd_t)
    return jnp.transpose(out_t.reshape(1, D, S), (0, 2, 1))
```

```python
import contextlib
import functools

import jax
import jax.numpy as jnp
from jax import lax
from jax.experimental import pallas as pl
from jax.experimental.pallas import tpu as pltpu

S, D, H, DH = 2048, 576, 32, 18
NSEG, L, F = 4, 512, 4608
T = 128
NT = L // T
NGRP = 5
SLAB = 112
GROUP_FIRST = (0, 7, 13, 19, 25, 32)
MROWS = 144
NCHUNK = F // T
NQUAD = H // 4
QUAD_OFF = (0, 64, 144, 208, 288, 352, 432, 448)
EARLY = 2
SUB = 32

bf16, f32, u32, i32 = jnp.bfloat16, jnp.float32, jnp.uint32, jnp.int32

LOG2E = 1.4426950408889634
QSCALE = (DH ** -0.5) * LOG2E
LN_NORM2 = 2.1 * D
LOGIT_LIMIT = 50.0
NEG_BIG = -1e30


PROFILE_SCOPES = False
CFG = dict(lag=5, rot=0, tie_stats=True, tie_p=3, fill_proj=10, fill_qk=8, select_pos=7, moe_quad=5, moe_end=8, op_gap=3, read_off=4)


def _scope(name):
    return jax.named_scope(name) if PROFILE_SCOPES else contextlib.nullcontext()


def _group_of(h):
    for g in range(NGRP):
        if GROUP_FIRST[g] <= h < GROUP_FIRST[g + 1]:
            return g
    raise ValueError(h)


def _to_bf16(x):
    return pltpu.bitcast(x, bf16)


def _to_u32(x):
    return pltpu.bitcast(x, u32)


def _round_bf16(x):
    return x.astype(bf16).astype(f32)


def _iota(shape, dim):
    return lax.broadcasted_iota(i32, shape, dim)


def _dot(a, b):
    return jnp.dot(a, b, preferred_element_type=f32)


def _dot_nt(a, b):
    return lax.dot_general(a, b, (((1,), (1,)), ((), ())), preferred_element_type=f32)


def _dot_tn(a, b):
    return lax.dot_general(a, b, (((0,), (0,)), ((), ())), preferred_element_type=f32)


def _zero_after_bits(u):
    return lax.shift_right_logical(pltpu.bitcast(u, i32), 31).astype(f32) * 0.0


def _pack_pairs(x):
    lo = jnp.concatenate([x[r:r + 8] for r in range(0, x.shape[0], 16)], axis=0)
    hi = jnp.concatenate([x[r + 8:r + 16] for r in range(0, x.shape[0], 16)], axis=0)
    return pltpu.pack_elementwise([lo, hi], packed_dtype=bf16)


def _unpaired_index(r):
    x = r & 15
    return (r - x) + jnp.where(x < 8, 2 * x, 2 * (x - 8) + 1)


def _phi(t):
    return jnp.where(t > 0, t + 1.0, jnp.exp(t))


def _sigmoid(t):
    return 1.0 / (1.0 + jnp.exp(-t))


def _layernorm_stats(xb):
    x0 = xb[0:1, :].astype(f32)
    acc1, acc2 = [None] * 4, [None] * 4
    for n, r in enumerate(range(0, D, 16)):
        c = xb[r:r + 16, :].astype(f32) - x0
        for part in range(2):
            k = (2 * n + part) % 4
            piece = c[8 * part:8 * part + 8, :]
            acc1[k] = piece if acc1[k] is None else acc1[k] + piece
            acc2[k] = piece * piece if acc2[k] is None else acc2[k] + piece * piece
    s1 = jnp.sum((acc1[0] + acc1[1]) + (acc1[2] + acc1[3]), axis=0, keepdims=True) / D
    s2 = jnp.sum((acc2[0] + acc2[1]) + (acc2[2] + acc2[3]), axis=0, keepdims=True) / D
    var = jnp.maximum(s2 - s1 * s1, 0.0)
    eps = _round_bf16(jnp.full((1, 1), 1e-5, f32))
    sd = _round_bf16(jnp.sqrt(_round_bf16(_round_bf16(var) + eps)))
    return _round_bf16(x0 + s1), 1.0 / sd


def _layernorm_apply(xb, stats):
    mean, inv = stats
    return _round_bf16(xb.astype(f32) - mean) * inv


def _block_transpose(xs):
    lane = _iota(next(x for x in xs if x is not None).shape, 1)

    def exchange(u, v, low, shift):
        def pick(p, q):
            if p is None and q is None:
                return None
            return jnp.where(low, 0.0 if p is None else p, 0.0 if q is None else q)
        ru = None if u is None else pltpu.roll(u, T - shift, 1)
        rv = None if v is None else pltpu.roll(v, shift, 1)
        return pick(u, rv), pick(ru, v)

    y0, y2 = exchange(xs[0], xs[2], lane < 64, 64)
    y1, y3 = exchange(xs[1], xs[3], lane < 64, 64)
    low = (lane & 32) == 0
    z0, z1 = exchange(y0, y1, low, 32)
    z2, z3 = exchange(y2, y3, low, 32)
    return [z0, z1, z2, z3]


def _head_of_slab_index(idx, g):
    return ((idx + SLAB * g) * 3641) >> 16


def _zero_after(x):
    sign = lax.shift_right_logical(pltpu.bitcast(x, i32), 31)
    return sign.astype(f32) * 0.0


def _kernel(x_hbm, wq_hbm, wk_hbm, wv_hbm, wo_hbm, beta_hbm, wr_hbm, wg_hbm, wu_hbm, wd_hbm,
            out_hbm,
            xt, xn, wstage, wt, wot, wg, wu, wd, beta_ref, wr_ref, qt, vt, kp, num, mt, zt, ot,
            mx, mxp, rrow, outb, gb, kall, qall, sems):
    def copy(src, dst, i):
        return pltpu.make_async_copy(src, dst, sems.at[i])

    xa_copy = copy(x_hbm.at[:, 0:T], xt.at[:, 0:T], 0)
    xb_copy = copy(x_hbm.at[:, T:L], xt.at[:, T:L], 18)
    xr_copy = copy(x_hbm.at[:, L:S], xt.at[:, L:S], 1)
    wk_copy, wq_copy, wv_copy, wo_copy = [
        copy(w, wstage.at[i], 2 + i) for i, w in enumerate((wk_hbm, wq_hbm, wv_hbm, wo_hbm))]
    beta_copy = copy(beta_hbm, beta_ref, 6)
    wr_copy = copy(wr_hbm, wr_ref, 7)
    moe_copies = [copy(wg_hbm, wg, 8), copy(wu_hbm, wu, 9), copy(wd_hbm, wd, 10)]

    def out_copy(lo, hi, i):
        return copy(outb.at[:, lo:hi], out_hbm.at[:, lo:hi], 11 + i)

    half = D // 2
    emitted = set()

    def produced(*key):
        emitted.add(key)

    def require(*key):
        assert key in emitted, key

    def require_heads(s, j):
        for h in range(H):
            require('ot', s, h, j)

    fillers = []

    def fill(n):
        for _ in range(min(n, len(fillers))):
            fillers.pop(0)()

    ties = []

    def tile_cols(s, tt):
        return slice(s * L + tt * T, s * L + (tt + 1) * T)

    def local_cols(tt):
        return slice(tt * T, (tt + 1) * T)

    def col_sq_part(i, lo, hi):
        acc = None
        for r in range(lo, hi, 16):
            w = wstage[i, r:r + 16, :].astype(f32)
            w = w * w
            part = w[0:8] + w[8:16]
            acc = part if acc is None else acc + part
        return acc

    def col_sq_max(parts):
        acc = functools.reduce(lambda u, v: u + v, parts)
        return jnp.max(jnp.sum(acc, axis=0, keepdims=True), axis=1, keepdims=True)

    def tie_of(part):
        folded = functools.reduce(lambda u, v: u + v, [part[:, c:c + T] for c in range(0, 4 * T, T)])
        return _zero_after(folded[0:1, 0:1] + part[0:1, 4 * T:4 * T + 1])

    def transpose_weight(i):
        return _to_u32(wstage[i].T)

    def ln_stats(s, tt):
        return _layernorm_stats(xt[:, tile_cols(s, tt)])

    def normalize(s, tt, stats):
        cs = tile_cols(s, tt)
        xn[:, cs] = _layernorm_apply(xt[:, cs], stats)
        produced('xn', s, tt)

    def xn_tile(s, tt):
        require('xn', s, tt)
        return xn[:, tile_cols(s, tt)].astype(bf16)

    def keys_raw(s, tt, lo=0, hi=D):
        kt = _dot(_to_bf16(wt[lo // 2:hi // 2, :]), xn_tile(s, tt))
        fill(CFG['fill_proj'])
        return kt

    def keys_finish(s, tt, kt, tie=None):
        kt = _round_bf16(kt if tie is None else kt + tie)
        shuffled = jnp.take_along_axis(kt, _unpaired_index(_iota((D, T), 1)), axis=1)
        for b in range(NQUAD):
            kp[s % 2, b, tt * (T // 2):(tt + 1) * (T // 2), :] = _to_u32(
                shuffled[QUAD_OFF[b]:QUAD_OFF[b] + T, :].astype(bf16).T)
        produced('k', s, tt)
        return _phi(kt).astype(bf16)

    def project_k(s, tt):
        return keys_finish(s, tt, keys_raw(s, tt))

    def project_q(s, tt, tie=None):
        q = _dot(_to_bf16(wt[half:2 * half, :]), xn_tile(s, tt))
        fill(CFG['fill_proj'])
        qt[s % 2, :, local_cols(tt)] = q * (QSCALE if tie is None else QSCALE + tie)
        produced('q', s, tt)
        return _phi(_round_bf16(q)).astype(bf16)

    def require_segment_done(s):
        if s >= 0:
            for j in range(NT):
                require_heads(s, j)

    def project_v(s, tt, tie=None):
        require_segment_done(s - 2)
        v = _dot(_to_bf16(wt[2 * half:3 * half, :]), xn_tile(s, tt))
        fill(CFG['fill_proj'])
        vt[s % 2, :, local_cols(tt)] = v if tie is None else v + tie
        produced('v', s, tt)

    def router_scores(lhs, s, tt):
        row = s * NT + tt
        rrow[row:row + 1, :] = _dot(lhs, xn_tile(s, tt))[0:1, :]
        produced('r', s, tt)

    def memory_read(s, tt, pq):
        require_segment_done(s - 2)
        for g in range(NGRP):
            require('mt', s - 1, g)
        for g in range(NGRP):
            num[s % 2, g, :, local_cols(tt)] = _dot(mt[g].astype(bf16), pq[SLAB * g:SLAB * g + T, :])
        produced('num', s, tt)

    def memory_update(s, g, pk):
        ones_row = 0 if g == NGRP - 1 else T - 1
        vs = jnp.where(_iota((T, L), 0) == ones_row, 1.0, vt[s % 2, SLAB * g:SLAB * g + T, :]).astype(bf16)
        m = _dot_nt(vs, jnp.concatenate([p[SLAB * g:SLAB * g + T, :] for p in pk], axis=1))
        hr = _head_of_slab_index(_iota((T, T), 0), g)
        hc = _head_of_slab_index(_iota((T, T), 1), g)
        keep = (hr == hc) & (hr >= GROUP_FIRST[g]) & (hr < GROUP_FIRST[g + 1])
        mm = jnp.where(keep, m, 0.0)
        z = m[ones_row:ones_row + 1, :]
        if s > 0:
            mm = mm + mt[g, 0:T, :]
            z = z + zt[g, 0:1, :]
        mt[g, 0:T, :] = mm
        zt[g, 0:1, :] = z
        zsel = _head_of_slab_index(_iota((16, T), 1), g) == _iota((16, T), 0) + GROUP_FIRST[g]
        mt[g, T:MROWS, :] = jnp.where(zsel, z, 0.0)
        produced('mt', s, g)

    def assemble_rows(pieces):
        groups = []
        for r in range(0, T, 8):
            hit = [x[r - r0:r - r0 + 8, :] for r0, x in pieces if r0 <= r < r0 + x.shape[0]]
            groups.append(functools.reduce(lambda u, v: u + v, hit) if hit else None)
        out, r = [], 0
        while r < len(groups):
            if groups[r] is None:
                n = 1
                while r + n < len(groups) and groups[r + n] is None:
                    n += 1
                out.append(jnp.zeros((8 * n, T), f32))
                r += n
            else:
                out.append(groups[r])
                r += 1
        return jnp.concatenate(out, axis=0)

    def quad_queries(s, b, j):
        f0 = QUAD_OFF[b]
        wide, packed = [], [[] for _ in range(4)]
        for a in range(4):
            r0 = DH * (4 * b + a) - f0
            lo = (r0 // 8) * 8
            hi = -(-(r0 + DH) // 8) * 8
            rows = _iota((hi - lo, T), 0) + lo
            mine = (rows >= r0) & (rows < r0 + DH)
            q = qt[s % 2, f0 + lo:f0 + hi, local_cols(j)]
            wide.append(assemble_rows([(lo, jnp.where(mine, q, 0.0))]))
            here = mine & (_iota((hi - lo, T), 1) // SUB == a)
            for i in range(4):
                shift = (SUB * (a - i)) % T
                moved = q if shift == 0 else pltpu.roll(q, shift, 1)
                packed[i].append((lo, jnp.where(here, moved, 0.0)))
        return wide, [assemble_rows(p).astype(bf16) for p in packed]

    def scores(s, b, j):
        require('q', s, j)
        for tt in range(j + 1):
            require('k', s, tt)
        wide, packed = quad_queries(s, b, j)
        tie = None
        unit = (s * NQUAD + b) * NT + j
        due = [z for when, z in ties if when <= unit]
        ties[:] = [(when, z) for when, z in ties if when > unit]
        if due:
            tie = functools.reduce(lambda u, v: u + v, due)
        tile = s * NT + j
        k0 = j * (T // 2)
        off = None
        if j > 0:
            logits = _dot(_to_bf16(kp[s % 2, b, 0:k0, :]), jnp.concatenate(wide, axis=1).astype(bf16))
            fill(CFG['fill_qk'])
            shift = jnp.concatenate([mx[4 * b + a:4 * b + a + 1, tile_cols(s, j)] for a in range(4)], axis=1)
            off = jnp.exp2(logits - shift)
        causal = _unpaired_index(_iota((SUB, T), 0)) <= (_iota((SUB, T), 1) & (SUB - 1))
        diag = [None] * 4
        for i in [(k + CFG['rot'] * j) % 4 for k in range(4)]:
            n = SUB * (i + 1)
            logits = _dot(_to_bf16(kp[s % 2, b, k0:k0 + n // 2, :]), packed[i])
            shift = mxp[tile, 4 * b + i:4 * b + i + 1, :]
            if tie is not None and i == 3:
                shift = shift + tie
            e = jnp.exp2(logits - shift)
            blocks = [e[r * SUB:(r + 1) * SUB, :] for r in range(i)]
            blocks.append(jnp.where(causal, e[i * SUB:, :], 0.0))
            diag[i] = blocks
        per_head = [[] for _ in range(4)]
        for r in range(4):
            outs = _block_transpose([diag[i][r] if i >= r else None for i in range(4)])
            for a in range(4):
                per_head[a].append(outs[a])
        ps = []
        for a in range(4):
            parts = ([off[:, a * T:(a + 1) * T]] if j > 0 else []) + per_head[a]
            ps.append(_pack_pairs(jnp.concatenate(parts, axis=0)))
        if CFG['tie_p'] is not None:
            rows = [u[r:r + 8] for u in ps for r in range(0, u.shape[0], 8)]
            while len(rows) > 1:
                rows = [rows[i] | rows[i + 1] for i in range(0, len(rows) - 1, 2)] + rows[len(rows) & ~1:]
            ties.append((unit + CFG['tie_p'], _zero_after_bits(rows[0])[0:1, :]))
        return [_to_bf16(u) for u in ps]

    def values(s, h, j, p):
        g = _group_of(h)
        w0 = min((DH * h // 16) * 16, D - 32)
        off = DH * h - w0
        ones_row = 31 if off < 14 else 0
        n = (j + 1) * T
        cs = local_cols(j)
        for tt in range(j + 1):
            require('v', s, tt)
        if s > 0:
            require('num', s, j)
        vwin = jnp.where(_iota((32, n), 0) == ones_row, 1.0, vt[s % 2, w0:w0 + 32, 0:n]).astype(bf16)
        gate = gb[h:h + 1, :]
        acc = _dot(vwin, p)
        res = acc * ((1.0 - gate) / acc[ones_row:ones_row + 1, :])
        if s > 0:
            m0 = w0 - SLAB * g
            zr = T + h - GROUP_FIRST[g]
            den = num[s % 2, g, zr:zr + 1, cs] + 1e-6
            res = res + num[s % 2, g, m0:m0 + 32, cs] * (gate / den)
        else:
            ties.append((0, _zero_after((res[0:8] + res[8:16]) + (res[16:24] + res[24:32]))[0:1, :]))
        ot[s, DH * h:DH * h + DH, cs] = res[off:off + DH, :]
        produced('ot', s, h, j)

    def route():
        for s in range(NSEG):
            for tt in range(NT):
                require('r', s, tt)
        r = _round_bf16(rrow[...])
        idx = _iota((S // T, T), 0) * T + _iota((S // T, T), 1)
        m1 = jnp.max(r)
        i1 = jnp.min(jnp.where(r == m1, idx, S - 1))
        r2 = jnp.where(idx == i1, -jnp.inf, r)
        m2 = jnp.max(r2)
        i2 = jnp.min(jnp.where(r2 == m2, idx, S - 1))
        return (i1, i2), (m1, m2)

    def select_tokens(ids):
        sel = None
        for row, i in enumerate(ids):
            hit = (_iota((16, T), 0) == row) & (_iota((16, T), 1) == i % T)
            cs = pl.ds(pl.multiple_of((i // T) * T, T), T)
            part = _dot_nt(jnp.where(hit, 1.0, 0.0).astype(bf16), xn[:, cs].astype(bf16))
            sel = part if sel is None else sel + part
        return sel.astype(bf16)

    def queue_moe(xsel, state):
        ktiles = [(k, min(k + T, D)) for k in range(0, D, T)]
        pre, hid = {}, {}
        ycols = state['ycols'] = [None] * len(ktiles)

        def first(w, name, c, lo, hi):
            def fn():
                part = _dot(xsel[:, lo:hi], w[lo:hi, c * T:(c + 1) * T])
                pre[name, c] = part if lo == 0 else pre[name, c] + part
            return fn

        def down(c, n, lo, hi):
            def fn():
                if c not in hid:
                    gpre = _round_bf16(pre.pop(('g', c)))
                    gact = _round_bf16(gpre * _sigmoid(gpre))
                    hid[c] = (gact * _round_bf16(pre.pop(('u', c)))).astype(bf16)
                part = _dot_nt(hid[c], wd[lo:hi, c * T:(c + 1) * T])
                ycols[n] = part if ycols[n] is None else ycols[n] + part
            return fn

        for c in range(NCHUNK + 2):
            if c < NCHUNK:
                for lo, hi in ktiles:
                    fillers.append(first(wg, 'g', c, lo, hi))
                    fillers.append(first(wu, 'u', c, lo, hi))
            if c >= 2:
                for n, (lo, hi) in enumerate(ktiles):
                    fillers.append(down(c - 2, n, lo, hi))

    def moe_result(sel_scores, y):
        row = _iota((16, D), 0)
        gate = jnp.where(row == 0, sel_scores[0], sel_scores[1])
        return (_round_bf16(y) * _round_bf16(_sigmoid(gate))).astype(bf16)

    def patch_early(ids, y):
        for k, i in enumerate(ids):
            hit = (_iota((16, T), 0) == k) & (_iota((16, T), 1) == i % T) & (i < EARLY * L)
            cs = pl.ds(pl.multiple_of((jnp.minimum(i, EARLY * L - 1) // T) * T, T), T)
            patch = _dot_tn(y, jnp.where(hit, 1.0, 0.0).astype(bf16))
            outb[:, cs] = (outb[:, cs].astype(f32) + patch).astype(bf16)

    def out_lhs(ids, y):
        place = (_iota((16, T), 1) == _iota((16, T), 0) + 64) & (_iota((16, T), 0) < 2)
        ycols = _dot_tn(y, jnp.where(place, 1.0, 0.0).astype(bf16))
        last = _to_bf16(wot[:, 4 * T:5 * T]).astype(f32) + ycols
        for s in range(EARLY, NSEG):
            tok = _iota((64, L), 1) + s * L
            rows = _iota((64, L), 0)
            hit = ((rows == 0) & (tok == ids[0])) | ((rows == 1) & (tok == ids[1]))
            ot[s, D:D + 64, :] = jnp.where(hit, 1.0, 0.0)
        return jnp.concatenate([_to_bf16(wot[:, 0:4 * T]), last.astype(bf16)], axis=1)

    def out_project_early(s, tt):
        require_heads(s, tt)
        require('wot')
        cs = tile_cols(s, tt)
        attn = _dot(_to_bf16(wot[:, 0:D]), ot[s, 0:D, local_cols(tt)].astype(bf16))
        fill(CFG['fill_proj'])
        outb[:, cs] = (attn + xn[:, cs] + xt[:, cs].astype(f32)).astype(bf16)

    def out_project(lhs, s, tt):
        require_heads(s, tt)
        cs = tile_cols(s, tt)
        attn = _dot(lhs, ot[s, :, local_cols(tt)].astype(bf16))
        outb[:, cs] = (attn + xn[:, cs] + xt[:, cs].astype(f32)).astype(bf16)

    def row_maxima():
        def project_tile(tt, carry):
            cs = pl.ds(pl.multiple_of(tt * T, T), T)
            y = _layernorm_apply(xt[:, cs], _layernorm_stats(xt[:, cs])).astype(bf16)
            kall[:, cs] = _dot(_to_bf16(wt[0:half, :]), y).astype(bf16)
            qall[:, cs] = (_dot(_to_bf16(wt[half:2 * half, :]), y) * QSCALE).astype(bf16)
            return carry

        lax.fori_loop(0, S // T, project_tile, 0)

        def head_tile(i, carry):
            h = i // (S // T)
            tt = i % (S // T)
            cs = pl.ds(pl.multiple_of(tt * T, T), T)
            seg = pl.ds(pl.multiple_of((tt // NT) * L, L), L)
            rows = _iota((D, T), 0)
            qm = jnp.where((rows >= DH * h) & (rows < DH * h + DH), qall[:, cs].astype(f32), 0.0)
            logits = _dot_tn(kall[:, seg], qm.astype(bf16))
            seen = _iota((L, T), 0) <= _iota((L, T), 1) + (tt % NT) * T
            m = jnp.max(jnp.where(seen, logits, NEG_BIG), axis=0, keepdims=True)
            mx[:, cs] = jnp.where(_iota((H, T), 0) == h, m, mx[:, cs])
            return carry

        lax.fori_loop(0, H * (S // T), head_tile, 0)

        def pack_tile(tt, carry):
            cs = pl.ds(pl.multiple_of(tt * T, T), T)
            m = mx[:, cs]
            block = _iota((1, T), 1) // SUB
            for b in range(NQUAD):
                for i in range(4):
                    row = jnp.zeros((1, T), f32)
                    for a in range(4):
                        src = m[4 * b + a:4 * b + a + 1, :]
                        shift = (SUB * (a - i)) % T
                        row = jnp.where(block == a, src if shift == 0 else pltpu.roll(src, shift, 1), row)
                    mxp[tt, 4 * b + i:4 * b + i + 1, :] = row
            return carry

        lax.fori_loop(0, S // T, pack_tile, 0)

    for c in (xa_copy, wk_copy, xb_copy, wq_copy, wv_copy):
        c.start()
    wot[:, 4 * T:5 * T] = jnp.zeros((half, T), u32)
    pk, pq = {}, {}
    sq = [[], []]

    def sq_tie(i, n, parts):
        rows = -(-D // (16 * parts)) * 16
        part = col_sq_part(i, n * rows, min(D, (n + 1) * rows))
        sq[i].append(part)
        return tie_of(part)

    with _scope('p0_wait'):
        xa_copy.wait()
    with _scope('p0'):
        normalize(0, 0, ln_stats(0, 0))
    with _scope('p1_wait'):
        wk_copy.wait()
    with _scope('p1'):
        wt[0:half, :] = transpose_weight(0)
        k0a = keys_raw(0, 0, 0, half)
    with _scope('p1b_wait'):
        xb_copy.wait()
    with _scope('p1b'):
        st1 = ln_stats(0, 1)
        k0 = jnp.concatenate([k0a, keys_raw(0, 0, half, D)], axis=0)
        normalize(0, 1, st1)
        st2 = ln_stats(0, 2)
        k1 = keys_raw(0, 1)
        pk[0, 0] = keys_finish(0, 0, k0, sq_tie(0, 0, 2) + _zero_after(st2[1]))
        normalize(0, 2, st2)
        st3 = ln_stats(0, 3)
        k2 = keys_raw(0, 2)
        pk[0, 1] = keys_finish(0, 1, k1, sq_tie(0, 1, 2) + _zero_after(st3[1]))
        normalize(0, 3, st3)
        k3a = keys_raw(0, 3, 0, half)
    with _scope('p2_wait'):
        wq_copy.wait()
        wv_copy.wait()
    for c in (xr_copy, wo_copy, beta_copy, wr_copy):
        c.start()
    with _scope('p2'):
        k3 = jnp.concatenate([k3a, keys_raw(0, 3, half, D)], axis=0)
        wt[half:2 * half, :] = transpose_weight(1)
        wt[2 * half:3 * half, :] = transpose_weight(2)
        pk[0, 2] = keys_finish(0, 2, k2)
        project_q(0, 0, sq_tie(1, 0, 4))
        pk[0, 3] = keys_finish(0, 3, k3)
        for tt in range(1, NT):
            project_q(0, tt, sq_tie(1, tt, 4))
        for tt in range(NT - 1):
            project_v(0, tt)
        csq = [col_sq_max(parts) for parts in sq]
        bound = (QSCALE * LN_NORM2 * DH) * jnp.sqrt(csq[0] * csq[1])
        mx[...] = jnp.broadcast_to(bound, mx.shape)
        mxp[...] = jnp.broadcast_to(bound, mxp.shape[1:])[None] + jnp.zeros(mxp.shape, f32)
        unsafe = jnp.max(jnp.where(bound <= LOGIT_LIMIT, 0, 1)) > 0
    with _scope('p4_wait'):
        for c in (xr_copy, wo_copy, beta_copy, wr_copy):
            c.wait()
    for c in moe_copies:
        c.start()

    @pl.when(unsafe)
    def _():
        row_maxima()

    project_v(0, NT - 1)
    gb[...] = _sigmoid(jnp.broadcast_to(beta_ref[...].astype(f32).reshape(1, H), (T, H)).T)

    slots = {}
    st = {}

    def at(s, b, j, fn):
        slots.setdefault((s, b, j), []).append(fn)

    def at_pos(s, pos, fn):
        at(s, pos // NT, pos % NT, fn)

    def wr_lhs():
        if 'wr' not in st:
            w = jnp.broadcast_to(wr_ref[...].astype(f32).reshape(1, D), (16, D))
            st['wr'] = jnp.where(_iota((16, D), 0) == 0, w, 0.0).astype(bf16)
        return st['wr']

    stats = {}

    def stats_task(s, tt):
        def fn():
            stats[s, tt] = ln_stats(s, tt)
            if CFG['tie_stats']:
                ties.append((0, _zero_after(stats[s, tt][1])))
        return fn

    def norm_task(s, tt):
        return lambda: normalize(s, tt, stats[s, tt])

    def score_task(s, tt):
        return lambda: router_scores(wr_lhs(), s, tt)

    for s in range(NSEG - 1):
        for g in range(NGRP):
            at_pos(s, 2 * g, lambda s=s, g=g: memory_update(s, g, [pk[s, tt] for tt in range(NT)]))
        if s == 0:
            at_pos(0, 3, stats_task(1, 0))
            at_pos(0, 5, norm_task(1, 0))
        for tt in range(NT):
            p0 = 9 + 6 * tt
            if s == 0:
                at_pos(s, p0, stats_task(2, tt))
                if tt > 0:
                    at_pos(s, p0, norm_task(3, tt - 1))
            at_pos(s, p0, lambda s=s, tt=tt: pk.__setitem__((s + 1, tt), project_k(s + 1, tt)))
            if s == 0:
                if tt > 0:
                    at_pos(s, p0, score_task(3, tt - 1))
                at_pos(s, p0 + 2, norm_task(2, tt))
                if tt + 1 < NT:
                    at_pos(s, p0 + 2, stats_task(1, tt + 1))
            at_pos(s, p0 + 2, lambda s=s, tt=tt: pq.__setitem__((s + 1, tt), project_q(s + 1, tt)))
            if s == 0:
                at_pos(s, p0 + 2, score_task(2, tt))
            if s == 0:
                if tt + 1 < NT:
                    at_pos(s, p0 + 4, norm_task(1, tt + 1))
                at_pos(s, p0 + 4, stats_task(3, tt))
            at_pos(s, p0 + 4, lambda s=s, tt=tt: project_v(s + 1, tt))
            at_pos(s, p0 + CFG['read_off'], lambda s=s, tt=tt: memory_read(s + 1, tt, pq[s + 1, tt]))
    at_pos(1, 0, norm_task(3, NT - 1))
    for s in range(EARLY):
        for tt in range(NT):
            at_pos(s + 1, 3 + 2 * tt if s > 0 else 8 + 6 * tt, lambda s=s, tt=tt: out_project_early(s, tt))
    at_pos(1, 1, score_task(3, NT - 1))
    for tt in range(NT):
        at_pos(0, 1 + 2 * tt, score_task(0, tt))
        at_pos(0, 10 + 6 * tt, score_task(1, tt))
    def set_out_weight():
        wot[:, 0:D] = transpose_weight(3)
        produced('wot')

    at_pos(0, 22, set_out_weight)

    at_pos(1, 2, lambda: st.update(zip(('ids', 'sel'), route())))
    at_pos(1, CFG['select_pos'], lambda: st.update(xsel=select_tokens(st['ids'])))

    def start_moe():
        with _scope('moe_wait'):
            for c in moe_copies:
                c.wait()
        queue_moe(st['xsel'], st)

    at(1, CFG['moe_quad'], -1, start_moe)

    def finish_moe():
        fill(len(fillers))
        y = moe_result(st['sel'], jnp.concatenate(st['ycols'], axis=1))
        patch_early(st['ids'], y)
        st['lhs'] = out_lhs(st['ids'], y)

    e0 = CFG['moe_end']
    at_pos(3, e0, finish_moe)
    for s in range(EARLY):
        at_pos(3, e0 + 1 + s, lambda s=s: out_copy(s * L, (s + 1) * L, s).start())
    for tt in range(NT):
        at_pos(3, e0 + 2 + CFG['op_gap'] * tt, lambda tt=tt: out_project(st['lhs'], 2, tt))
    at_pos(3, e0 + 3 + CFG['op_gap'] * (NT - 1), lambda: out_copy(2 * L, 3 * L, 2).start())

    def quad_values(s, b, j, ps):
        for a in range(4):
            values(s, 4 * b + a, j, ps[a])

    pending = []
    for s in range(NSEG):
        for b in range(NQUAD):
            for fn in slots.pop((s, b, -1), ()):
                fn()
            for j in range(NT):
                pending.append((s, b, j, scores(s, b, j)))
                for fn in slots.pop((s, b, j), ()):
                    fn()
                if len(pending) > CFG['lag']:
                    quad_values(*pending.pop(0))
    tail = [unit for unit in pending]
    assert not slots, slots.keys()
    s = NSEG - 1

    def last_tile(tt):
        out_project(st['lhs'], s, tt)
        out_copy(s * L + tt * T, s * L + (tt + 1) * T, 3 + tt).start()

    done = 0
    for unit in tail:
        quad_values(*unit)
        while done < NT and unit[1] == NQUAD - 1 and done < unit[2]:
            last_tile(done)
            done += 1
    while done < NT:
        last_tile(done)
        done += 1
    with _scope('out_wait'):
        for k in range(NSEG - 1):
            out_copy(k * L, (k + 1) * L, k).wait()
        for tt in range(NT):
            out_copy(s * L + tt * T, s * L + (tt + 1) * T, 3 + tt).wait()


@jax.jit
def pallas_parallel_sum__memory_aug_infini_attn__moe_arch_mod__prompt_kernel(
    A_x: jax.Array,
    A_wq: jax.Array,
    A_wk: jax.Array,
    A_wv: jax.Array,
    A_wo: jax.Array,
    A_beta: jax.Array,
    B_x: jax.Array,
    B_w_r: jax.Array,
    B_w_gate: jax.Array,
    B_w_up: jax.Array,
    B_w_down: jax.Array,
):
    del B_x
    x_t = jnp.transpose(A_x, (0, 2, 1)).reshape(D, S)
    wd_t = B_w_down.T
    hbm = pl.BlockSpec(memory_space=pl.ANY)
    out_t = pl.pallas_call(
        _kernel,
        out_shape=jax.ShapeDtypeStruct((D, S), bf16),
        in_specs=[hbm] * 10,
        out_specs=hbm,
        scratch_shapes=[
            pltpu.VMEM((D, S), bf16),
            pltpu.VMEM((D, S), f32),
            pltpu.VMEM((4, D, D), bf16),
            pltpu.VMEM((3 * D // 2, D), u32),
            pltpu.VMEM((D // 2, 5 * T), u32),
            pltpu.VMEM((D, F), bf16),
            pltpu.VMEM((D, F), bf16),
            pltpu.VMEM((D, F), bf16),
            pltpu.VMEM((H,), bf16),
            pltpu.VMEM((D,), bf16),
            pltpu.VMEM((2, D, L), f32),
            pltpu.VMEM((2, D, L), f32),
            pltpu.VMEM((2, NQUAD, L // 2, T), u32),
            pltpu.VMEM((2, NGRP, MROWS, L), f32),
            pltpu.VMEM((NGRP, MROWS, T), f32),
            pltpu.VMEM((NGRP, 8, T), f32),
            pltpu.VMEM((NSEG, 5 * T, L), f32),
            pltpu.VMEM((H, S), f32),
            pltpu.VMEM((S // T, H, T), f32),
            pltpu.VMEM((S // T, T), f32),
            pltpu.VMEM((D, S), bf16),
            pltpu.VMEM((H, T), f32),
            pltpu.VMEM((D, S), bf16),
            pltpu.VMEM((D, S), bf16),
            pltpu.SemaphoreType.DMA((19,)),
        ],
        compiler_params=pltpu.CompilerParams(vmem_limit_bytes=100 * 1024 * 1024),
        name="infini_moe",
    )(x_t, A_wq, A_wk, A_wv, A_wo, A_beta, B_w_r, B_w_gate, B_w_up, wd_t)
    return jnp.transpose(out_t.reshape(1, D, S), (0, 2, 1))
```

```python
import contextlib
import functools

import jax
import jax.numpy as jnp
from jax import lax
from jax.experimental import pallas as pl
from jax.experimental.pallas import tpu as pltpu

S, D, H, DH = 2048, 576, 32, 18
NSEG, L, F = 4, 512, 4608
T = 128
NT = L // T
NGRP = 5
SLAB = 112
GROUP_FIRST = (0, 7, 13, 19, 25, 32)
MROWS = 144
NCHUNK = F // T
NQUAD = H // 4
QUAD_OFF = (0, 64, 144, 208, 288, 352, 432, 448)
EARLY = 2
SUB = 32

bf16, f32, u32, i32 = jnp.bfloat16, jnp.float32, jnp.uint32, jnp.int32

LOG2E = 1.4426950408889634
QSCALE = (DH ** -0.5) * LOG2E
LN_NORM2 = 2.1 * D
LOGIT_LIMIT = 50.0
NEG_BIG = -1e30


PROFILE_SCOPES = False
CFG = dict(lag=5, rot=0, tie_stats=True, tie_p=3, fill_proj=10, fill_qk=8, select_pos=7, moe_quad=5, moe_end=8, op_gap=3, read_off=4)


def _scope(name):
    return jax.named_scope(name) if PROFILE_SCOPES else contextlib.nullcontext()


def _group_of(h):
    for g in range(NGRP):
        if GROUP_FIRST[g] <= h < GROUP_FIRST[g + 1]:
            return g
    raise ValueError(h)


def _to_bf16(x):
    return pltpu.bitcast(x, bf16)


def _to_u32(x):
    return pltpu.bitcast(x, u32)


def _round_bf16(x):
    return x.astype(bf16).astype(f32)


def _iota(shape, dim):
    return lax.broadcasted_iota(i32, shape, dim)


def _dot(a, b):
    return jnp.dot(a, b, preferred_element_type=f32)


def _dot_nt(a, b):
    return lax.dot_general(a, b, (((1,), (1,)), ((), ())), preferred_element_type=f32)


def _dot_tn(a, b):
    return lax.dot_general(a, b, (((0,), (0,)), ((), ())), preferred_element_type=f32)


def _zero_after_bits(u):
    return lax.shift_right_logical(pltpu.bitcast(u, i32), 31).astype(f32) * 0.0


def _pack_pairs(x):
    lo = jnp.concatenate([x[r:r + 8] for r in range(0, x.shape[0], 16)], axis=0)
    hi = jnp.concatenate([x[r + 8:r + 16] for r in range(0, x.shape[0], 16)], axis=0)
    return pltpu.pack_elementwise([lo, hi], packed_dtype=bf16)


def _unpaired_index(r):
    x = r & 15
    return (r - x) + jnp.where(x < 8, 2 * x, 2 * (x - 8) + 1)


def _zero_bits_after(u):
    sixteen = jnp.full(u.shape, 16, u32)
    return lax.shift_right_logical(lax.shift_right_logical(u, sixteen), sixteen)


def _pair_mask(first, lo, hi, keep_lane=None):
    f = _iota((8, T), 0) + first
    low = (f >= lo) & (f < hi)
    high = (f + 8 >= lo) & (f + 8 < hi)
    if keep_lane is not None:
        low, high = low & keep_lane, high & keep_lane
    return jnp.where(low, jnp.uint32(0xFFFF), jnp.uint32(0)) | jnp.where(high, jnp.uint32(0xFFFF0000), jnp.uint32(0))


def _bf16_bits(x):
    return pltpu.bitcast(_round_bf16(x), u32)


def _shift_words(m, low_half):
    first = _round_bf16(-m)
    second = _round_bf16(-m - first)
    third = -m - first - second
    row = _iota((8, T), 0)
    val = jnp.where(row == 5, first, jnp.where(row == 6, second, jnp.where(row == 7, third, 0.0)))
    bits = _bf16_bits(val)
    return lax.shift_right_logical(bits, jnp.full(bits.shape, 16, u32)) if low_half else bits


def _phi(t):
    return jnp.where(t > 0, t + 1.0, jnp.exp(t))


def _sigmoid(t):
    return 1.0 / (1.0 + jnp.exp(-t))


def _layernorm_stats(xb):
    x0 = xb[0:1, :].astype(f32)
    acc1, acc2 = [None] * 4, [None] * 4
    for n, r in enumerate(range(0, D, 16)):
        c = xb[r:r + 16, :].astype(f32) - x0
        for part in range(2):
            k = (2 * n + part) % 4
            piece = c[8 * part:8 * part + 8, :]
            acc1[k] = piece if acc1[k] is None else acc1[k] + piece
            acc2[k] = piece * piece if acc2[k] is None else acc2[k] + piece * piece
    s1 = jnp.sum((acc1[0] + acc1[1]) + (acc1[2] + acc1[3]), axis=0, keepdims=True) / D
    s2 = jnp.sum((acc2[0] + acc2[1]) + (acc2[2] + acc2[3]), axis=0, keepdims=True) / D
    var = jnp.maximum(s2 - s1 * s1, 0.0)
    eps = _round_bf16(jnp.full((1, 1), 1e-5, f32))
    sd = _round_bf16(jnp.sqrt(_round_bf16(_round_bf16(var) + eps)))
    return _round_bf16(x0 + s1), 1.0 / sd


def _layernorm_apply(xb, stats):
    mean, inv = stats
    return _round_bf16(xb.astype(f32) - mean) * inv


def _block_transpose(xs):
    lane = _iota(next(x for x in xs if x is not None).shape, 1)

    def exchange(u, v, low, shift):
        def pick(p, q):
            if p is None and q is None:
                return None
            return jnp.where(low, 0.0 if p is None else p, 0.0 if q is None else q)
        ru = None if u is None else pltpu.roll(u, T - shift, 1)
        rv = None if v is None else pltpu.roll(v, shift, 1)
        return pick(u, rv), pick(ru, v)

    y0, y2 = exchange(xs[0], xs[2], lane < 64, 64)
    y1, y3 = exchange(xs[1], xs[3], lane < 64, 64)
    low = (lane & 32) == 0
    z0, z1 = exchange(y0, y1, low, 32)
    z2, z3 = exchange(y2, y3, low, 32)
    return [z0, z1, z2, z3]


def _head_of_slab_index(idx, g):
    return ((idx + SLAB * g) * 3641) >> 16


def _zero_after(x):
    sign = lax.shift_right_logical(pltpu.bitcast(x, i32), 31)
    return sign.astype(f32) * 0.0


def _kernel(x_hbm, wq_hbm, wk_hbm, wv_hbm, wo_hbm, beta_hbm, wr_hbm, wg_hbm, wu_hbm, wd_hbm,
            out_hbm,
            xt, xn, wstage, wt, wot, wg, wu, wd, beta_ref, wr_ref, qt, vt, kp, num, mt, zt, ot,
            mx, mxp, mrow, qmask, rrow, outb, gb, kall, qall, sems):
    def copy(src, dst, i):
        return pltpu.make_async_copy(src, dst, sems.at[i])

    xa_copy = copy(x_hbm.at[:, 0:T], xt.at[:, 0:T], 0)
    xb_copy = copy(x_hbm.at[:, T:L], xt.at[:, T:L], 18)
    xr_copy = copy(x_hbm.at[:, L:S], xt.at[:, L:S], 1)
    wk_copy, wq_copy, wv_copy, wo_copy = [
        copy(w, wstage.at[i], 2 + i) for i, w in enumerate((wk_hbm, wq_hbm, wv_hbm, wo_hbm))]
    beta_copy = copy(beta_hbm, beta_ref, 6)
    wr_copy = copy(wr_hbm, wr_ref, 7)
    moe_copies = [copy(wg_hbm, wg, 8), copy(wu_hbm, wu, 9), copy(wd_hbm, wd, 10)]

    def out_copy(lo, hi, i):
        return copy(outb.at[:, lo:hi], out_hbm.at[:, lo:hi], 11 + i)

    half = D // 2
    emitted = set()

    def produced(*key):
        emitted.add(key)

    def require(*key):
        assert key in emitted, key

    def require_heads(s, j):
        for h in range(H):
            require('ot', s, h, j)

    fillers = []

    def fill(n):
        for _ in range(min(n, len(fillers))):
            fillers.pop(0)()

    ties = []

    def tile_cols(s, tt):
        return slice(s * L + tt * T, s * L + (tt + 1) * T)

    def local_cols(tt):
        return slice(tt * T, (tt + 1) * T)

    def col_sq_part(i, lo, hi):
        acc = None
        for r in range(lo, hi, 16):
            w = wstage[i, r:r + 16, :].astype(f32)
            w = w * w
            part = w[0:8] + w[8:16]
            acc = part if acc is None else acc + part
        return acc

    def col_sq_max(parts):
        acc = functools.reduce(lambda u, v: u + v, parts)
        return jnp.max(jnp.sum(acc, axis=0, keepdims=True), axis=1, keepdims=True)

    def tie_of(part):
        folded = functools.reduce(lambda u, v: u + v, [part[:, c:c + T] for c in range(0, 4 * T, T)])
        return _zero_after(folded[0:1, 0:1] + part[0:1, 4 * T:4 * T + 1])

    def transpose_weight(i):
        return _to_u32(wstage[i].T)

    def ln_stats(s, tt):
        return _layernorm_stats(xt[:, tile_cols(s, tt)])

    def normalize(s, tt, stats):
        cs = tile_cols(s, tt)
        xn[:, cs] = _layernorm_apply(xt[:, cs], stats)
        produced('xn', s, tt)

    def xn_tile(s, tt):
        require('xn', s, tt)
        return xn[:, tile_cols(s, tt)].astype(bf16)

    def keys_raw(s, tt, lo=0, hi=D):
        kt = _dot(_to_bf16(wt[lo // 2:hi // 2, :]), xn_tile(s, tt))
        fill(CFG['fill_proj'])
        return kt

    def keys_finish(s, tt, kt, tie=None):
        if tie is not None:
            kt = kt + tie
        words = jnp.take_along_axis(_pack_pairs(kt), _unpaired_index(_iota((half, T), 1)), axis=1)
        shift_rows = _iota((8, T), 0) >= 5
        for b in range(NQUAD):
            slab = words[QUAD_OFF[b] // 2:QUAD_OFF[b] // 2 + T // 2, :]
            if b == NQUAD - 1:
                ones = jnp.where(shift_rows, (slab[0:8] & jnp.uint32(0xFFFF0000)) | jnp.uint32(0x3F80), slab[0:8])
                slab = jnp.concatenate([ones, slab[8:]], axis=0)
            else:
                ones = jnp.where(shift_rows, (slab[56:64] & jnp.uint32(0xFFFF)) | jnp.uint32(0x3F800000), slab[56:64])
                slab = jnp.concatenate([slab[:56], ones], axis=0)
            kp[s % 2, b, tt * (T // 2):(tt + 1) * (T // 2), :] = _to_u32(_to_bf16(slab).T)
        produced('k', s, tt)
        return _phi(kt).astype(bf16)

    def project_k(s, tt):
        return keys_finish(s, tt, keys_raw(s, tt))

    def project_q(s, tt, tie=None):
        q = _dot(_to_bf16(wt[half:2 * half, :]), xn_tile(s, tt))
        fill(CFG['fill_proj'])
        qt[s % 2, :, local_cols(tt)] = _pack_pairs(q * (QSCALE if tie is None else QSCALE + tie))
        produced('q', s, tt)
        return _phi(q).astype(bf16)

    def require_segment_done(s):
        if s >= 0:
            for j in range(NT):
                require_heads(s, j)

    def project_v(s, tt, tie=None):
        require_segment_done(s - 2)
        v = _dot(_to_bf16(wt[2 * half:3 * half, :]), xn_tile(s, tt))
        fill(CFG['fill_proj'])
        vt[s % 2, :, local_cols(tt)] = v if tie is None else v + tie
        produced('v', s, tt)

    def router_scores(lhs, s, tt):
        row = s * NT + tt
        rrow[row:row + 1, :] = _dot(lhs, xn_tile(s, tt))[0:1, :]
        produced('r', s, tt)

    def memory_read(s, tt, pq):
        require_segment_done(s - 2)
        for g in range(NGRP):
            require('mt', s - 1, g)
        for g in range(NGRP):
            num[s % 2, g, :, local_cols(tt)] = _dot(mt[g].astype(bf16), pq[SLAB * g:SLAB * g + T, :])
        produced('num', s, tt)

    def memory_update(s, g, pk):
        ones_row = 0 if g == NGRP - 1 else T - 1
        vs = jnp.where(_iota((T, L), 0) == ones_row, 1.0, vt[s % 2, SLAB * g:SLAB * g + T, :]).astype(bf16)
        m = _dot_nt(vs, jnp.concatenate([p[SLAB * g:SLAB * g + T, :] for p in pk], axis=1))
        hr = _head_of_slab_index(_iota((T, T), 0), g)
        hc = _head_of_slab_index(_iota((T, T), 1), g)
        keep = (hr == hc) & (hr >= GROUP_FIRST[g]) & (hr < GROUP_FIRST[g + 1])
        mm = jnp.where(keep, m, 0.0)
        z = m[ones_row:ones_row + 1, :]
        if s > 0:
            mm = mm + mt[g, 0:T, :]
            z = z + zt[g, 0:1, :]
        mt[g, 0:T, :] = mm
        zt[g, 0:1, :] = z
        zsel = _head_of_slab_index(_iota((16, T), 1), g) == _iota((16, T), 0) + GROUP_FIRST[g]
        mt[g, T:MROWS, :] = jnp.where(zsel, z, 0.0)
        produced('mt', s, g)

    def head_groups(b, a):
        f = DH * (4 * b + a) - QUAD_OFF[b]
        return f, (f // 16, f // 16 + 1)

    def build_query_masks():
        block = _iota((8, T), 1) // SUB
        for b in range(NQUAD):
            for a in range(4):
                f, groups = head_groups(b, a)
                for n, g in enumerate(groups):
                    qmask[b, 4 * a + 2 * n] = _pair_mask(16 * g, f, f + DH)
                    qmask[b, 4 * a + 2 * n + 1] = _pair_mask(16 * g, f, f + DH, block == a)

    def stack_groups(groups):
        return _to_bf16(jnp.concatenate(
            [groups.get(g, jnp.zeros((8, T), u32)) for g in range(T // 16)], axis=0))

    def quad_queries(s, b, j, tie):
        tile = s * NT + j
        last = b == NQUAD - 1
        shift_group = 0 if last else T // 16 - 1
        base = QUAD_OFF[b] // 2
        words = {}

        def group(g):
            if g not in words:
                words[g] = qt[s % 2, base + 8 * g:base + 8 * g + 8, local_cols(j)]
            return words[g]

        wide = []
        for a in range(4):
            _, groups = head_groups(b, a)
            parts = {g: group(g) & qmask[b, 4 * a + 2 * n] for n, g in enumerate(groups)}
            if j > 0:
                parts[shift_group] = mx[int(last) + shift_sel * (2 - int(last) + (4 * b + a) * (S // T) + tile)]
                wide.append(stack_groups(parts))
        packed = []
        for i in range(4):
            parts = {}
            for a in range(4):
                _, groups = head_groups(b, a)
                shift = (SUB * (a - i)) % T
                for n, g in enumerate(groups):
                    moved = group(g) if shift == 0 else pltpu.roll(group(g), shift, 1)
                    piece = moved & qmask[b, 4 * a + 2 * n + 1]
                    parts[g] = piece if g not in parts else parts[g] | piece
            rows = mxp[int(last) + shift_sel * (2 - int(last) + tile * H + 4 * b + i)]
            if tie is not None and i == 3:
                rows = rows | tie
            parts[shift_group] = rows
            packed.append(stack_groups(parts))
        return wide, packed

    def scores(s, b, j):
        require('q', s, j)
        for tt in range(j + 1):
            require('k', s, tt)
        tie = None
        unit = (s * NQUAD + b) * NT + j
        due = [z for when, z in ties if when <= unit]
        ties[:] = [(when, z) for when, z in ties if when > unit]
        if due:
            tie = functools.reduce(lambda u, v: u | v, due)
        wide, packed = quad_queries(s, b, j, tie)
        k0 = j * (T // 2)
        off = None
        if j > 0:
            logits = _dot(_to_bf16(kp[s % 2, b, 0:k0, :]), jnp.concatenate(wide, axis=1))
            fill(CFG['fill_qk'])
            off = jnp.exp2(logits)
        causal = _unpaired_index(_iota((SUB, T), 0)) <= (_iota((SUB, T), 1) & (SUB - 1))
        diag = [None] * 4
        for i in range(4):
            n = SUB * (i + 1)
            e = jnp.exp2(_dot(_to_bf16(kp[s % 2, b, k0:k0 + n // 2, :]), packed[i]))
            blocks = [e[r * SUB:(r + 1) * SUB, :] for r in range(i)]
            blocks.append(jnp.where(causal, e[i * SUB:, :], 0.0))
            diag[i] = blocks
        per_head = [[] for _ in range(4)]
        for r in range(4):
            outs = _block_transpose([diag[i][r] if i >= r else None for i in range(4)])
            for a in range(4):
                per_head[a].append(outs[a])
        ps = []
        for a in range(4):
            parts = ([off[:, a * T:(a + 1) * T]] if j > 0 else []) + per_head[a]
            ps.append(_pack_pairs(jnp.concatenate(parts, axis=0)))
        if CFG['tie_p'] is not None:
            rows = [u[r:r + 8] for u in ps for r in range(0, u.shape[0], 8)]
            while len(rows) > 1:
                rows = [rows[i] | rows[i + 1] for i in range(0, len(rows) - 1, 2)] + rows[len(rows) & ~1:]
            ties.append((unit + CFG['tie_p'], _zero_bits_after(rows[0])))
        return [_to_bf16(u) for u in ps]

    def values(s, h, j, p):
        g = _group_of(h)
        w0 = min((DH * h // 16) * 16, D - 32)
        off = DH * h - w0
        ones_row = 31 if off < 14 else 0
        n = (j + 1) * T
        cs = local_cols(j)
        for tt in range(j + 1):
            require('v', s, tt)
        if s > 0:
            require('num', s, j)
        g0 = (ones_row // 8) * 8
        marked = jnp.where(_iota((8, n), 0) == ones_row - g0, 1.0, vt[s % 2, w0 + g0:w0 + g0 + 8, 0:n])
        rest = vt[s % 2, w0 + 8:w0 + 32, 0:n] if g0 == 0 else vt[s % 2, w0:w0 + 24, 0:n]
        vwin = jnp.concatenate([marked, rest] if g0 == 0 else [rest, marked], axis=0).astype(bf16)
        gate = gb[h:h + 1, :]
        acc = _dot(vwin, p)
        res = acc * ((1.0 - gate) / acc[ones_row:ones_row + 1, :])
        if s > 0:
            m0 = w0 - SLAB * g
            zr = T + h - GROUP_FIRST[g]
            den = num[s % 2, g, zr:zr + 1, cs] + 1e-6
            res = res + num[s % 2, g, m0:m0 + 32, cs] * (gate / den)
        else:
            ties.append((0, _zero_bits_after(_to_u32((res[0:8] + res[8:16]) + (res[16:24] + res[24:32])))))
        ot[s, DH * h:DH * h + DH, cs] = res[off:off + DH, :]
        produced('ot', s, h, j)

    def route():
        for s in range(NSEG):
            for tt in range(NT):
                require('r', s, tt)
        r = _round_bf16(rrow[...])
        idx = _iota((S // T, T), 0) * T + _iota((S // T, T), 1)
        m1 = jnp.max(r)
        i1 = jnp.min(jnp.where(r == m1, idx, S - 1))
        r2 = jnp.where(idx == i1, -jnp.inf, r)
        m2 = jnp.max(r2)
        i2 = jnp.min(jnp.where(r2 == m2, idx, S - 1))
        return (i1, i2), (m1, m2)

    def select_tokens(ids):
        sel = None
        for row, i in enumerate(ids):
            hit = (_iota((16, T), 0) == row) & (_iota((16, T), 1) == i % T)
            cs = pl.ds(pl.multiple_of((i // T) * T, T), T)
            part = _dot_nt(jnp.where(hit, 1.0, 0.0).astype(bf16), xn[:, cs].astype(bf16))
            sel = part if sel is None else sel + part
        return sel.astype(bf16)

    def queue_moe(xsel, state):
        ktiles = [(k, min(k + T, D)) for k in range(0, D, T)]
        pre, hid = {}, {}
        ycols = state['ycols'] = [None] * len(ktiles)

        def first(w, name, c, lo, hi):
            def fn():
                part = _dot(xsel[:, lo:hi], w[lo:hi, c * T:(c + 1) * T])
                pre[name, c] = part if lo == 0 else pre[name, c] + part
            return fn

        def down(c, n, lo, hi):
            def fn():
                if c not in hid:
                    gpre = _round_bf16(pre.pop(('g', c)))
                    gact = _round_bf16(gpre * _sigmoid(gpre))
                    hid[c] = (gact * _round_bf16(pre.pop(('u', c)))).astype(bf16)
                part = _dot_nt(hid[c], wd[lo:hi, c * T:(c + 1) * T])
                ycols[n] = part if ycols[n] is None else ycols[n] + part
            return fn

        for c in range(NCHUNK + 2):
            if c < NCHUNK:
                for lo, hi in ktiles:
                    fillers.append(first(wg, 'g', c, lo, hi))
                    fillers.append(first(wu, 'u', c, lo, hi))
            if c >= 2:
                for n, (lo, hi) in enumerate(ktiles):
                    fillers.append(down(c - 2, n, lo, hi))

    def moe_result(sel_scores, y):
        row = _iota((16, D), 0)
        gate = jnp.where(row == 0, sel_scores[0], sel_scores[1])
        return (_round_bf16(y) * _round_bf16(_sigmoid(gate))).astype(bf16)

    def patch_early(ids, y):
        for k, i in enumerate(ids):
            hit = (_iota((16, T), 0) == k) & (_iota((16, T), 1) == i % T) & (i < EARLY * L)
            cs = pl.ds(pl.multiple_of((jnp.minimum(i, EARLY * L - 1) // T) * T, T), T)
            patch = _dot_tn(y, jnp.where(hit, 1.0, 0.0).astype(bf16))
            outb[:, cs] = (outb[:, cs].astype(f32) + patch).astype(bf16)

    def out_lhs(ids, y):
        place = (_iota((16, T), 1) == _iota((16, T), 0) + 64) & (_iota((16, T), 0) < 2)
        ycols = _dot_tn(y, jnp.where(place, 1.0, 0.0).astype(bf16))
        last = _to_bf16(wot[:, 4 * T:5 * T]).astype(f32) + ycols
        for s in range(EARLY, NSEG):
            tok = _iota((64, L), 1) + s * L
            rows = _iota((64, L), 0)
            hit = ((rows == 0) & (tok == ids[0])) | ((rows == 1) & (tok == ids[1]))
            ot[s, D:D + 64, :] = jnp.where(hit, 1.0, 0.0)
        return jnp.concatenate([_to_bf16(wot[:, 0:4 * T]), last.astype(bf16)], axis=1)

    def out_project_early(s, tt):
        require_heads(s, tt)
        require('wot')
        cs = tile_cols(s, tt)
        attn = _dot(_to_bf16(wot[:, 0:D]), ot[s, 0:D, local_cols(tt)].astype(bf16))
        fill(CFG['fill_proj'])
        outb[:, cs] = (attn + xn[:, cs] + xt[:, cs].astype(f32)).astype(bf16)

    def out_project(lhs, s, tt):
        require_heads(s, tt)
        cs = tile_cols(s, tt)
        attn = _dot(lhs, ot[s, :, local_cols(tt)].astype(bf16))
        outb[:, cs] = (attn + xn[:, cs] + xt[:, cs].astype(f32)).astype(bf16)

    def row_maxima():
        def project_tile(tt, carry):
            cs = pl.ds(pl.multiple_of(tt * T, T), T)
            y = _layernorm_apply(xt[:, cs], _layernorm_stats(xt[:, cs])).astype(bf16)
            kall[:, cs] = _dot(_to_bf16(wt[0:half, :]), y).astype(bf16)
            qall[:, cs] = (_dot(_to_bf16(wt[half:2 * half, :]), y) * QSCALE).astype(bf16)
            return carry

        lax.fori_loop(0, S // T, project_tile, 0)

        def head_tile(i, carry):
            h = i // (S // T)
            tt = i % (S // T)
            cs = pl.ds(pl.multiple_of(tt * T, T), T)
            seg = pl.ds(pl.multiple_of((tt // NT) * L, L), L)
            rows = _iota((D, T), 0)
            qm = jnp.where((rows >= DH * h) & (rows < DH * h + DH), qall[:, cs].astype(f32), 0.0)
            logits = _dot_tn(kall[:, seg], qm.astype(bf16))
            seen = _iota((L, T), 0) <= _iota((L, T), 1) + (tt % NT) * T
            m = jnp.max(jnp.where(seen, logits, NEG_BIG), axis=0, keepdims=True)
            mrow[:, cs] = jnp.where(_iota((H, T), 0) == h, m, mrow[:, cs])
            wide_m = jnp.broadcast_to(m, (8, T))
            mx[2 + i] = jnp.where(h >= H - 4, _shift_words(wide_m, True), _shift_words(wide_m, False))
            return carry

        mrow[...] = jnp.zeros(mrow.shape, f32)
        lax.fori_loop(0, H * (S // T), head_tile, 0)

        def pack_tile(tt, carry):
            cs = pl.ds(pl.multiple_of(tt * T, T), T)
            m = mrow[:, cs]
            block = _iota((1, T), 1) // SUB
            for b in range(NQUAD):
                for i in range(4):
                    row = jnp.zeros((1, T), f32)
                    for a in range(4):
                        src = m[4 * b + a:4 * b + a + 1, :]
                        shift = (SUB * (a - i)) % T
                        row = jnp.where(block == a, src if shift == 0 else pltpu.roll(src, shift, 1), row)
                    mxp[2 + tt * H + 4 * b + i] = _shift_words(jnp.broadcast_to(row, (8, T)), b == NQUAD - 1)
            return carry

        lax.fori_loop(0, S // T, pack_tile, 0)

    for c in (xa_copy, wk_copy, xb_copy, wq_copy, wv_copy):
        c.start()
    wot[:, 4 * T:5 * T] = jnp.zeros((half, T), u32)
    pk, pq = {}, {}
    sq = [[], []]

    def sq_tie(i, n, parts):
        rows = -(-D // (16 * parts)) * 16
        part = col_sq_part(i, n * rows, min(D, (n + 1) * rows))
        sq[i].append(part)
        return tie_of(part)

    build_query_masks()
    with _scope('p0_wait'):
        xa_copy.wait()
    with _scope('p0'):
        normalize(0, 0, ln_stats(0, 0))
    with _scope('p1_wait'):
        wk_copy.wait()
    with _scope('p1'):
        wt[0:half, :] = transpose_weight(0)
        k0a = keys_raw(0, 0, 0, half)
    with _scope('p1b_wait'):
        xb_copy.wait()
    with _scope('p1b'):
        st1 = ln_stats(0, 1)
        k0 = jnp.concatenate([k0a, keys_raw(0, 0, half, D)], axis=0)
        normalize(0, 1, st1)
        st2 = ln_stats(0, 2)
        k1 = keys_raw(0, 1)
        pk[0, 0] = keys_finish(0, 0, k0, sq_tie(0, 0, 2) + _zero_after(st2[1]))
        normalize(0, 2, st2)
        st3 = ln_stats(0, 3)
        k2 = keys_raw(0, 2)
        pk[0, 1] = keys_finish(0, 1, k1, sq_tie(0, 1, 2) + _zero_after(st3[1]))
        normalize(0, 3, st3)
        k3a = keys_raw(0, 3, 0, half)
    with _scope('p2_wait'):
        wq_copy.wait()
        wv_copy.wait()
    for c in (xr_copy, wo_copy, beta_copy, wr_copy):
        c.start()
    with _scope('p2'):
        k3 = jnp.concatenate([k3a, keys_raw(0, 3, half, D)], axis=0)
        wt[half:2 * half, :] = transpose_weight(1)
        wt[2 * half:3 * half, :] = transpose_weight(2)
        pk[0, 2] = keys_finish(0, 2, k2)
        project_q(0, 0, sq_tie(1, 0, 4))
        pk[0, 3] = keys_finish(0, 3, k3)
        for tt in range(1, NT):
            project_q(0, tt, sq_tie(1, tt, 4))
        for tt in range(NT - 1):
            project_v(0, tt)
        csq = [col_sq_max(parts) for parts in sq]
        bound = (QSCALE * LN_NORM2 * DH) * jnp.sqrt(csq[0] * csq[1])
        for low in range(2):
            words = _shift_words(jnp.broadcast_to(bound, (8, T)), low == 1)
            mx[low] = words
            mxp[low] = words
        shift_sel = jnp.max(jnp.where(bound <= LOGIT_LIMIT, 0, 1))
        unsafe = shift_sel > 0
    with _scope('p4_wait'):
        for c in (xr_copy, wo_copy, beta_copy, wr_copy):
            c.wait()
    for c in moe_copies:
        c.start()

    @pl.when(unsafe)
    def _():
        row_maxima()

    project_v(0, NT - 1)
    gb[...] = _sigmoid(jnp.broadcast_to(beta_ref[...].astype(f32).reshape(1, H), (T, H)).T)

    slots = {}
    st = {}

    def at(s, b, j, fn):
        slots.setdefault((s, b, j), []).append(fn)

    def at_pos(s, pos, fn):
        at(s, pos // NT, pos % NT, fn)

    def wr_lhs():
        if 'wr' not in st:
            w = jnp.broadcast_to(wr_ref[...].astype(f32).reshape(1, D), (16, D))
            st['wr'] = jnp.where(_iota((16, D), 0) == 0, w, 0.0).astype(bf16)
        return st['wr']

    stats = {}

    def stats_task(s, tt):
        def fn():
            stats[s, tt] = ln_stats(s, tt)
            if CFG['tie_stats']:
                ties.append((0, _zero_bits_after(_to_u32(jnp.broadcast_to(stats[s, tt][1], (8, T))))))
        return fn

    def norm_task(s, tt):
        return lambda: normalize(s, tt, stats[s, tt])

    def score_task(s, tt):
        return lambda: router_scores(wr_lhs(), s, tt)

    for s in range(NSEG - 1):
        for g in range(NGRP):
            at_pos(s, 2 * g, lambda s=s, g=g: memory_update(s, g, [pk[s, tt] for tt in range(NT)]))
        if s == 0:
            at_pos(0, 3, stats_task(1, 0))
            at_pos(0, 5, norm_task(1, 0))
        for tt in range(NT):
            p0 = 9 + 6 * tt
            if s == 0:
                at_pos(s, p0, stats_task(2, tt))
                if tt > 0:
                    at_pos(s, p0, norm_task(3, tt - 1))
            at_pos(s, p0, lambda s=s, tt=tt: pk.__setitem__((s + 1, tt), project_k(s + 1, tt)))
            if s == 0:
                if tt > 0:
                    at_pos(s, p0, score_task(3, tt - 1))
                at_pos(s, p0 + 2, norm_task(2, tt))
                if tt + 1 < NT:
                    at_pos(s, p0 + 2, stats_task(1, tt + 1))
            at_pos(s, p0 + 2, lambda s=s, tt=tt: pq.__setitem__((s + 1, tt), project_q(s + 1, tt)))
            if s == 0:
                at_pos(s, p0 + 2, score_task(2, tt))
            if s == 0:
                if tt + 1 < NT:
                    at_pos(s, p0 + 4, norm_task(1, tt + 1))
                at_pos(s, p0 + 4, stats_task(3, tt))
            at_pos(s, p0 + 4, lambda s=s, tt=tt: project_v(s + 1, tt))
            at_pos(s, p0 + CFG['read_off'], lambda s=s, tt=tt: memory_read(s + 1, tt, pq[s + 1, tt]))
    at_pos(1, 0, norm_task(3, NT - 1))
    for s in range(EARLY):
        for tt in range(NT):
            at_pos(s + 1, 3 + 2 * tt if s > 0 else 8 + 6 * tt, lambda s=s, tt=tt: out_project_early(s, tt))
    at_pos(1, 1, score_task(3, NT - 1))
    for tt in range(NT):
        at_pos(0, 1 + 2 * tt, score_task(0, tt))
        at_pos(0, 10 + 6 * tt, score_task(1, tt))
    def set_out_weight():
        wot[:, 0:D] = transpose_weight(3)
        produced('wot')

    at_pos(0, 22, set_out_weight)

    at_pos(1, 2, lambda: st.update(zip(('ids', 'sel'), route())))
    at_pos(1, CFG['select_pos'], lambda: st.update(xsel=select_tokens(st['ids'])))

    def start_moe():
        with _scope('moe_wait'):
            for c in moe_copies:
                c.wait()
        queue_moe(st['xsel'], st)

    at(1, CFG['moe_quad'], -1, start_moe)

    def finish_moe():
        fill(len(fillers))
        y = moe_result(st['sel'], jnp.concatenate(st['ycols'], axis=1))
        patch_early(st['ids'], y)
        st['lhs'] = out_lhs(st['ids'], y)

    e0 = CFG['moe_end']
    at_pos(3, e0, finish_moe)
    for s in range(EARLY):
        at_pos(3, e0 + 1 + s, lambda s=s: out_copy(s * L, (s + 1) * L, s).start())
    for tt in range(NT):
        at_pos(3, e0 + 2 + CFG['op_gap'] * tt, lambda tt=tt: out_project(st['lhs'], 2, tt))
    at_pos(3, e0 + 3 + CFG['op_gap'] * (NT - 1), lambda: out_copy(2 * L, 3 * L, 2).start())

    def quad_values(s, b, j, ps):
        for a in range(4):
            values(s, 4 * b + a, j, ps[a])

    pending = []
    for s in range(NSEG):
        for b in range(NQUAD):
            for fn in slots.pop((s, b, -1), ()):
                fn()
            for j in range(NT):
                pending.append((s, b, j, scores(s, b, j)))
                for fn in slots.pop((s, b, j), ()):
                    fn()
                if len(pending) > CFG['lag']:
                    quad_values(*pending.pop(0))
    tail = [unit for unit in pending]
    assert not slots, slots.keys()
    s = NSEG - 1

    def last_tile(tt):
        out_project(st['lhs'], s, tt)
        out_copy(s * L + tt * T, s * L + (tt + 1) * T, 3 + tt).start()

    done = 0
    for unit in tail:
        quad_values(*unit)
        while done < NT and unit[1] == NQUAD - 1 and done < unit[2]:
            last_tile(done)
            done += 1
    while done < NT:
        last_tile(done)
        done += 1
    with _scope('out_wait'):
        for k in range(NSEG - 1):
            out_copy(k * L, (k + 1) * L, k).wait()
        for tt in range(NT):
            out_copy(s * L + tt * T, s * L + (tt + 1) * T, 3 + tt).wait()


@jax.jit
def pallas_parallel_sum__memory_aug_infini_attn__moe_arch_mod__prompt_kernel(
    A_x: jax.Array,
    A_wq: jax.Array,
    A_wk: jax.Array,
    A_wv: jax.Array,
    A_wo: jax.Array,
    A_beta: jax.Array,
    B_x: jax.Array,
    B_w_r: jax.Array,
    B_w_gate: jax.Array,
    B_w_up: jax.Array,
    B_w_down: jax.Array,
):
    del B_x
    x_t = jnp.transpose(A_x, (0, 2, 1)).reshape(D, S)
    wd_t = B_w_down.T
    hbm = pl.BlockSpec(memory_space=pl.ANY)
    out_t = pl.pallas_call(
        _kernel,
        out_shape=jax.ShapeDtypeStruct((D, S), bf16),
        in_specs=[hbm] * 10,
        out_specs=hbm,
        scratch_shapes=[
            pltpu.VMEM((D, S), bf16),
            pltpu.VMEM((D, S), f32),
            pltpu.VMEM((4, D, D), bf16),
            pltpu.VMEM((3 * D // 2, D), u32),
            pltpu.VMEM((D // 2, 5 * T), u32),
            pltpu.VMEM((D, F), bf16),
            pltpu.VMEM((D, F), bf16),
            pltpu.VMEM((D, F), bf16),
            pltpu.VMEM((H,), bf16),
            pltpu.VMEM((D,), bf16),
            pltpu.VMEM((2, D // 2, L), u32),
            pltpu.VMEM((2, D, L), f32),
            pltpu.VMEM((2, NQUAD, L // 2, T), u32),
            pltpu.VMEM((2, NGRP, MROWS, L), f32),
            pltpu.VMEM((NGRP, MROWS, T), f32),
            pltpu.VMEM((NGRP, 8, T), f32),
            pltpu.VMEM((NSEG, 5 * T, L), f32),
            pltpu.VMEM((2 + H * S // T, 8, T), u32),
            pltpu.VMEM((2 + H * S // T, 8, T), u32),
            pltpu.VMEM((H, S), f32),
            pltpu.VMEM((NQUAD, 16, 8, T), u32),
            pltpu.VMEM((S // T, T), f32),
            pltpu.VMEM((D, S), bf16),
            pltpu.VMEM((H, T), f32),
            pltpu.VMEM((D, S), bf16),
            pltpu.VMEM((D, S), bf16),
            pltpu.SemaphoreType.DMA((19,)),
        ],
        compiler_params=pltpu.CompilerParams(vmem_limit_bytes=100 * 1024 * 1024),
        name="infini_moe",
    )(x_t, A_wq, A_wk, A_wv, A_wo, A_beta, B_w_r, B_w_gate, B_w_up, wd_t)
    return jnp.transpose(out_t.reshape(1, D, S), (0, 2, 1))
```

```python
import contextlib
import functools

import jax
import jax.numpy as jnp
from jax import lax
from jax.experimental import pallas as pl
from jax.experimental.pallas import tpu as pltpu

S, D, H, DH = 2048, 576, 32, 18
NSEG, L, F = 4, 512, 4608
T = 128
NT = L // T
NGRP = 5
SLAB = 112
GROUP_FIRST = (0, 7, 13, 19, 25, 32)
MROWS = 144
NCHUNK = F // T
NQUAD = H // 4
QUAD_OFF = (0, 64, 144, 208, 288, 352, 432, 448)
EARLY = 2
SUB = 32

bf16, f32, u32, i32 = jnp.bfloat16, jnp.float32, jnp.uint32, jnp.int32

LOG2E = 1.4426950408889634
QSCALE = (DH ** -0.5) * LOG2E
LN_NORM2 = 2.1 * D
LOGIT_LIMIT = 50.0
NEG_BIG = -1e30


PROFILE_SCOPES = False
CFG = dict(lag=5, rot=0, tie_stats=True, tie_p=3, fill_proj=10, fill_qk=8, select_pos=7, moe_quad=5, moe_end=8, op_gap=3, read_off=4, tie_res=3, tie_ln=1)


def _scope(name):
    return jax.named_scope(name) if PROFILE_SCOPES else contextlib.nullcontext()


def _group_of(h):
    for g in range(NGRP):
        if GROUP_FIRST[g] <= h < GROUP_FIRST[g + 1]:
            return g
    raise ValueError(h)


def _to_bf16(x):
    return pltpu.bitcast(x, bf16)


def _to_u32(x):
    return pltpu.bitcast(x, u32)


def _round_bf16(x):
    return x.astype(bf16).astype(f32)


def _iota(shape, dim):
    return lax.broadcasted_iota(i32, shape, dim)


def _dot(a, b):
    return jnp.dot(a, b, preferred_element_type=f32)


def _dot_nt(a, b):
    return lax.dot_general(a, b, (((1,), (1,)), ((), ())), preferred_element_type=f32)


def _dot_tn(a, b):
    return lax.dot_general(a, b, (((0,), (0,)), ((), ())), preferred_element_type=f32)


def _zero_after_bits(u):
    return lax.shift_right_logical(pltpu.bitcast(u, i32), 31).astype(f32) * 0.0


def _pack_pairs(x):
    lo = jnp.concatenate([x[r:r + 8] for r in range(0, x.shape[0], 16)], axis=0)
    hi = jnp.concatenate([x[r + 8:r + 16] for r in range(0, x.shape[0], 16)], axis=0)
    return pltpu.pack_elementwise([lo, hi], packed_dtype=bf16)


def _unpaired_index(r):
    x = r & 15
    return (r - x) + jnp.where(x < 8, 2 * x, 2 * (x - 8) + 1)


def _zero_bits_after(u):
    sixteen = jnp.full(u.shape, 16, u32)
    return lax.shift_right_logical(lax.shift_right_logical(u, sixteen), sixteen)


def _pair_mask(first, lo, hi, keep_lane=None):
    f = _iota((8, T), 0) + first
    low = (f >= lo) & (f < hi)
    high = (f + 8 >= lo) & (f + 8 < hi)
    if keep_lane is not None:
        low, high = low & keep_lane, high & keep_lane
    return jnp.where(low, jnp.uint32(0xFFFF), jnp.uint32(0)) | jnp.where(high, jnp.uint32(0xFFFF0000), jnp.uint32(0))


def _bf16_bits(x):
    return pltpu.bitcast(_round_bf16(x), u32)


def _shift_words(m, low_half):
    first = _round_bf16(-m)
    second = _round_bf16(-m - first)
    third = -m - first - second
    row = _iota((8, T), 0)
    val = jnp.where(row == 5, first, jnp.where(row == 6, second, jnp.where(row == 7, third, 0.0)))
    bits = _bf16_bits(val)
    return lax.shift_right_logical(bits, jnp.full(bits.shape, 16, u32)) if low_half else bits


def _phi(t):
    return jnp.where(t > 0, t + 1.0, jnp.exp(t))


def _sigmoid(t):
    return 1.0 / (1.0 + jnp.exp(-t))


def _layernorm_stats(xb):
    x0 = xb[0:1, :].astype(f32)
    acc1, acc2 = [None] * 4, [None] * 4
    for n, r in enumerate(range(0, D, 16)):
        c = xb[r:r + 16, :].astype(f32) - x0
        for part in range(2):
            k = (2 * n + part) % 4
            piece = c[8 * part:8 * part + 8, :]
            acc1[k] = piece if acc1[k] is None else acc1[k] + piece
            acc2[k] = piece * piece if acc2[k] is None else acc2[k] + piece * piece
    s1 = jnp.sum((acc1[0] + acc1[1]) + (acc1[2] + acc1[3]), axis=0, keepdims=True) / D
    s2 = jnp.sum((acc2[0] + acc2[1]) + (acc2[2] + acc2[3]), axis=0, keepdims=True) / D
    var = jnp.maximum(s2 - s1 * s1, 0.0)
    eps = _round_bf16(jnp.full((1, 1), 1e-5, f32))
    sd = _round_bf16(jnp.sqrt(_round_bf16(_round_bf16(var) + eps)))
    return _round_bf16(x0 + s1), 1.0 / sd


def _layernorm_apply(xb, stats):
    mean, inv = stats
    return _round_bf16(xb.astype(f32) - mean) * inv


def _block_transpose(xs):
    lane = _iota(next(x for x in xs if x is not None).shape, 1)

    def exchange(u, v, low, shift):
        def pick(p, q):
            if p is None and q is None:
                return None
            return jnp.where(low, 0.0 if p is None else p, 0.0 if q is None else q)
        ru = None if u is None else pltpu.roll(u, T - shift, 1)
        rv = None if v is None else pltpu.roll(v, shift, 1)
        return pick(u, rv), pick(ru, v)

    y0, y2 = exchange(xs[0], xs[2], lane < 64, 64)
    y1, y3 = exchange(xs[1], xs[3], lane < 64, 64)
    low = (lane & 32) == 0
    z0, z1 = exchange(y0, y1, low, 32)
    z2, z3 = exchange(y2, y3, low, 32)
    return [z0, z1, z2, z3]


def _head_of_slab_index(idx, g):
    return ((idx + SLAB * g) * 3641) >> 16


def _zero_after(x):
    sign = lax.shift_right_logical(pltpu.bitcast(x, i32), 31)
    return sign.astype(f32) * 0.0


def _kernel(x_hbm, wq_hbm, wk_hbm, wv_hbm, wo_hbm, beta_hbm, wr_hbm, wg_hbm, wu_hbm, wd_hbm,
            out_hbm,
            xt, xn, wstage, wt, wot, wg, wu, wd, beta_ref, wr_ref, qt, vt, kp, num, mt, zt, ot,
            mx, mxp, mrow, qmask, rrow, outb, gb, kall, qall, sems):
    def copy(src, dst, i):
        return pltpu.make_async_copy(src, dst, sems.at[i])

    xa_copy = copy(x_hbm.at[:, 0:T], xt.at[:, 0:T], 0)
    xb_copy = copy(x_hbm.at[:, T:L], xt.at[:, T:L], 18)
    xr_copy = copy(x_hbm.at[:, L:S], xt.at[:, L:S], 1)
    wk_copy, wq_copy, wv_copy, wo_copy = [
        copy(w, wstage.at[i], 2 + i) for i, w in enumerate((wk_hbm, wq_hbm, wv_hbm, wo_hbm))]
    beta_copy = copy(beta_hbm, beta_ref, 6)
    wr_copy = copy(wr_hbm, wr_ref, 7)
    moe_copies = [copy(wg_hbm, wg, 8), copy(wu_hbm, wu, 9), copy(wd_hbm, wd, 10)]

    def out_copy(lo, hi, i):
        return copy(outb.at[:, lo:hi], out_hbm.at[:, lo:hi], 11 + i)

    half = D // 2
    emitted = set()

    def produced(*key):
        emitted.add(key)

    def require(*key):
        assert key in emitted, key

    def require_heads(s, j):
        for h in range(H):
            require('ot', s, h, j)

    fillers = []

    def fill(n):
        for _ in range(min(n, len(fillers))):
            fillers.pop(0)()

    clock = [0]
    ties = []

    def tile_cols(s, tt):
        return slice(s * L + tt * T, s * L + (tt + 1) * T)

    def local_cols(tt):
        return slice(tt * T, (tt + 1) * T)

    def col_sq_part(i, lo, hi):
        acc = None
        for r in range(lo, hi, 16):
            w = wstage[i, r:r + 16, :].astype(f32)
            w = w * w
            part = w[0:8] + w[8:16]
            acc = part if acc is None else acc + part
        return acc

    def col_sq_max(parts):
        acc = functools.reduce(lambda u, v: u + v, parts)
        return jnp.max(jnp.sum(acc, axis=0, keepdims=True), axis=1, keepdims=True)

    def tie_of(part):
        folded = functools.reduce(lambda u, v: u + v, [part[:, c:c + T] for c in range(0, 4 * T, T)])
        return _zero_after(folded[0:1, 0:1] + part[0:1, 4 * T:4 * T + 1])

    def transpose_weight(i):
        return _to_u32(wstage[i].T)

    def ln_stats(s, tt):
        return _layernorm_stats(xt[:, tile_cols(s, tt)])

    def normalize(s, tt, stats):
        cs = tile_cols(s, tt)
        xn[:, cs] = _layernorm_apply(xt[:, cs], stats)
        produced('xn', s, tt)

    def xn_tile(s, tt):
        require('xn', s, tt)
        return xn[:, tile_cols(s, tt)].astype(bf16)

    def keys_raw(s, tt, lo=0, hi=D):
        kt = _dot(_to_bf16(wt[lo // 2:hi // 2, :]), xn_tile(s, tt))
        fill(CFG['fill_proj'])
        return kt

    def keys_finish(s, tt, kt, tie=None):
        if tie is not None:
            kt = kt + tie
        words = jnp.take_along_axis(_pack_pairs(kt), _unpaired_index(_iota((half, T), 1)), axis=1)
        shift_rows = _iota((8, T), 0) >= 5
        for b in range(NQUAD):
            slab = words[QUAD_OFF[b] // 2:QUAD_OFF[b] // 2 + T // 2, :]
            if b == NQUAD - 1:
                ones = jnp.where(shift_rows, (slab[0:8] & jnp.uint32(0xFFFF0000)) | jnp.uint32(0x3F80), slab[0:8])
                slab = jnp.concatenate([ones, slab[8:]], axis=0)
            else:
                ones = jnp.where(shift_rows, (slab[56:64] & jnp.uint32(0xFFFF)) | jnp.uint32(0x3F800000), slab[56:64])
                slab = jnp.concatenate([slab[:56], ones], axis=0)
            kp[s % 2, b, tt * (T // 2):(tt + 1) * (T // 2), :] = _to_u32(_to_bf16(slab).T)
        produced('k', s, tt)
        return _phi(kt).astype(bf16)

    def project_k(s, tt):
        return keys_finish(s, tt, keys_raw(s, tt))

    def project_q(s, tt, tie=None):
        q = _dot(_to_bf16(wt[half:2 * half, :]), xn_tile(s, tt))
        fill(CFG['fill_proj'])
        qt[s % 2, :, local_cols(tt)] = _pack_pairs(q * (QSCALE if tie is None else QSCALE + tie))
        produced('q', s, tt)
        return _phi(q).astype(bf16)

    def require_segment_done(s):
        if s >= 0:
            for j in range(NT):
                require_heads(s, j)

    def project_v(s, tt, tie=None):
        require_segment_done(s - 2)
        v = _dot(_to_bf16(wt[2 * half:3 * half, :]), xn_tile(s, tt))
        fill(CFG['fill_proj'])
        vt[s % 2, :, local_cols(tt)] = v if tie is None else v + tie
        produced('v', s, tt)

    def router_scores(lhs, s, tt):
        row = s * NT + tt
        rrow[row:row + 1, :] = _dot(lhs, xn_tile(s, tt))[0:1, :]
        produced('r', s, tt)

    def memory_read(s, tt, pq):
        require_segment_done(s - 2)
        for g in range(NGRP):
            require('mt', s - 1, g)
        for g in range(NGRP):
            num[s % 2, g, :, local_cols(tt)] = _dot(mt[g].astype(bf16), pq[SLAB * g:SLAB * g + T, :])
        produced('num', s, tt)

    def memory_update(s, g, pk):
        ones_row = 0 if g == NGRP - 1 else T - 1
        vs = jnp.where(_iota((T, L), 0) == ones_row, 1.0, vt[s % 2, SLAB * g:SLAB * g + T, :]).astype(bf16)
        m = _dot_nt(vs, jnp.concatenate([p[SLAB * g:SLAB * g + T, :] for p in pk], axis=1))
        hr = _head_of_slab_index(_iota((T, T), 0), g)
        hc = _head_of_slab_index(_iota((T, T), 1), g)
        keep = (hr == hc) & (hr >= GROUP_FIRST[g]) & (hr < GROUP_FIRST[g + 1])
        mm = jnp.where(keep, m, 0.0)
        z = m[ones_row:ones_row + 1, :]
        if s > 0:
            mm = mm + mt[g, 0:T, :]
            z = z + zt[g, 0:1, :]
        mt[g, 0:T, :] = mm
        zt[g, 0:1, :] = z
        zsel = _head_of_slab_index(_iota((16, T), 1), g) == _iota((16, T), 0) + GROUP_FIRST[g]
        mt[g, T:MROWS, :] = jnp.where(zsel, z, 0.0)
        produced('mt', s, g)

    def head_groups(b, a):
        f = DH * (4 * b + a) - QUAD_OFF[b]
        return f, (f // 16, f // 16 + 1)

    def build_query_masks():
        block = _iota((8, T), 1) // SUB
        for b in range(NQUAD):
            for a in range(4):
                f, groups = head_groups(b, a)
                for n, g in enumerate(groups):
                    qmask[b, 4 * a + 2 * n] = _pair_mask(16 * g, f, f + DH)
                    qmask[b, 4 * a + 2 * n + 1] = _pair_mask(16 * g, f, f + DH, block == a)

    def stack_groups(groups):
        return _to_bf16(jnp.concatenate(
            [groups.get(g, jnp.zeros((8, T), u32)) for g in range(T // 16)], axis=0))

    def quad_queries(s, b, j, tie):
        tile = s * NT + j
        last = b == NQUAD - 1
        shift_group = 0 if last else T // 16 - 1
        base = QUAD_OFF[b] // 2
        words = {}

        def group(g):
            if g not in words:
                words[g] = qt[s % 2, base + 8 * g:base + 8 * g + 8, local_cols(j)]
            return words[g]

        wide = []
        for a in range(4):
            _, groups = head_groups(b, a)
            parts = {g: group(g) & qmask[b, 4 * a + 2 * n] for n, g in enumerate(groups)}
            if j > 0:
                parts[shift_group] = mx[int(last) + shift_sel * (2 - int(last) + (4 * b + a) * (S // T) + tile)]
                wide.append(stack_groups(parts))
        packed = []
        for i in range(4):
            parts = {}
            for a in range(4):
                _, groups = head_groups(b, a)
                shift = (SUB * (a - i)) % T
                for n, g in enumerate(groups):
                    moved = group(g) if shift == 0 else pltpu.roll(group(g), shift, 1)
                    piece = moved & qmask[b, 4 * a + 2 * n + 1]
                    parts[g] = piece if g not in parts else parts[g] | piece
            rows = mxp[int(last) + shift_sel * (2 - int(last) + tile * H + 4 * b + i)]
            if tie is not None and i == 3:
                rows = rows | tie
            parts[shift_group] = rows
            packed.append(stack_groups(parts))
        return wide, packed

    def scores(s, b, j):
        require('q', s, j)
        for tt in range(j + 1):
            require('k', s, tt)
        tie = None
        unit = clock[0] = (s * NQUAD + b) * NT + j
        due = [z for when, z in ties if when <= unit]
        ties[:] = [(when, z) for when, z in ties if when > unit]
        if due:
            tie = functools.reduce(lambda u, v: u | v, due)
        wide, packed = quad_queries(s, b, j, tie)
        k0 = j * (T // 2)
        off = None
        if j > 0:
            logits = _dot(_to_bf16(kp[s % 2, b, 0:k0, :]), jnp.concatenate(wide, axis=1))
            fill(CFG['fill_qk'])
            off = jnp.exp2(logits)
        causal = _unpaired_index(_iota((SUB, T), 0)) <= (_iota((SUB, T), 1) & (SUB - 1))
        diag = [None] * 4
        for i in range(4):
            n = SUB * (i + 1)
            e = jnp.exp2(_dot(_to_bf16(kp[s % 2, b, k0:k0 + n // 2, :]), packed[i]))
            blocks = [e[r * SUB:(r + 1) * SUB, :] for r in range(i)]
            blocks.append(jnp.where(causal, e[i * SUB:, :], 0.0))
            diag[i] = blocks
        per_head = [[] for _ in range(4)]
        for r in range(4):
            outs = _block_transpose([diag[i][r] if i >= r else None for i in range(4)])
            for a in range(4):
                per_head[a].append(outs[a])
        ps = []
        for a in range(4):
            parts = ([off[:, a * T:(a + 1) * T]] if j > 0 else []) + per_head[a]
            ps.append(_pack_pairs(jnp.concatenate(parts, axis=0)))
        if CFG['tie_p'] is not None:
            rows = [u[r:r + 8] for u in ps for r in range(0, u.shape[0], 8)]
            while len(rows) > 1:
                rows = [rows[i] | rows[i + 1] for i in range(0, len(rows) - 1, 2)] + rows[len(rows) & ~1:]
            ties.append((unit + CFG['tie_p'], _zero_bits_after(rows[0])))
        return [_to_bf16(u) for u in ps]

    def values(s, h, j, p):
        g = _group_of(h)
        w0 = min((DH * h // 16) * 16, D - 32)
        off = DH * h - w0
        ones_row = 31 if off < 14 else 0
        n = (j + 1) * T
        cs = local_cols(j)
        for tt in range(j + 1):
            require('v', s, tt)
        if s > 0:
            require('num', s, j)
        g0 = (ones_row // 8) * 8
        marked = jnp.where(_iota((8, n), 0) == ones_row - g0, 1.0, vt[s % 2, w0 + g0:w0 + g0 + 8, 0:n])
        rest = vt[s % 2, w0 + 8:w0 + 32, 0:n] if g0 == 0 else vt[s % 2, w0:w0 + 24, 0:n]
        vwin = jnp.concatenate([marked, rest] if g0 == 0 else [rest, marked], axis=0).astype(bf16)
        gate = gb[h:h + 1, :]
        acc = _dot(vwin, p)
        res = acc * ((1.0 - gate) / acc[ones_row:ones_row + 1, :])
        if s > 0:
            m0 = w0 - SLAB * g
            zr = T + h - GROUP_FIRST[g]
            den = num[s % 2, g, zr:zr + 1, cs] + 1e-6
            res = res + num[s % 2, g, m0:m0 + 32, cs] * (gate / den)
        else:
            ties.append((clock[0] + CFG['tie_res'], _zero_bits_after(_to_u32((res[0:8] + res[8:16]) + (res[16:24] + res[24:32])))))
        ot[s, DH * h:DH * h + DH, cs] = res[off:off + DH, :]
        produced('ot', s, h, j)

    def route():
        for s in range(NSEG):
            for tt in range(NT):
                require('r', s, tt)
        r = _round_bf16(rrow[...])
        idx = _iota((S // T, T), 0) * T + _iota((S // T, T), 1)
        m1 = jnp.max(r)
        i1 = jnp.min(jnp.where(r == m1, idx, S - 1))
        r2 = jnp.where(idx == i1, -jnp.inf, r)
        m2 = jnp.max(r2)
        i2 = jnp.min(jnp.where(r2 == m2, idx, S - 1))
        return (i1, i2), (m1, m2)

    def select_tokens(ids):
        sel = None
        for row, i in enumerate(ids):
            hit = (_iota((16, T), 0) == row) & (_iota((16, T), 1) == i % T)
            cs = pl.ds(pl.multiple_of((i // T) * T, T), T)
            part = _dot_nt(jnp.where(hit, 1.0, 0.0).astype(bf16), xn[:, cs].astype(bf16))
            sel = part if sel is None else sel + part
        return sel.astype(bf16)

    def queue_moe(xsel, state):
        ktiles = [(k, min(k + T, D)) for k in range(0, D, T)]
        pre, hid = {}, {}
        ycols = state['ycols'] = [None] * len(ktiles)

        def first(w, name, c, lo, hi):
            def fn():
                part = _dot(xsel[:, lo:hi], w[lo:hi, c * T:(c + 1) * T])
                pre[name, c] = part if lo == 0 else pre[name, c] + part
            return fn

        def down(c, n, lo, hi):
            def fn():
                if c not in hid:
                    gpre = _round_bf16(pre.pop(('g', c)))
                    gact = _round_bf16(gpre * _sigmoid(gpre))
                    hid[c] = (gact * _round_bf16(pre.pop(('u', c)))).astype(bf16)
                part = _dot_nt(hid[c], wd[lo:hi, c * T:(c + 1) * T])
                ycols[n] = part if ycols[n] is None else ycols[n] + part
            return fn

        for c in range(NCHUNK + 2):
            if c < NCHUNK:
                for lo, hi in ktiles:
                    fillers.append(first(wg, 'g', c, lo, hi))
                    fillers.append(first(wu, 'u', c, lo, hi))
            if c >= 2:
                for n, (lo, hi) in enumerate(ktiles):
                    fillers.append(down(c - 2, n, lo, hi))

    def moe_result(sel_scores, y):
        row = _iota((16, D), 0)
        gate = jnp.where(row == 0, sel_scores[0], sel_scores[1])
        return (_round_bf16(y) * _round_bf16(_sigmoid(gate))).astype(bf16)

    def patch_early(ids, y):
        for k, i in enumerate(ids):
            hit = (_iota((16, T), 0) == k) & (_iota((16, T), 1) == i % T) & (i < EARLY * L)
            cs = pl.ds(pl.multiple_of((jnp.minimum(i, EARLY * L - 1) // T) * T, T), T)
            patch = _dot_tn(y, jnp.where(hit, 1.0, 0.0).astype(bf16))
            outb[:, cs] = (outb[:, cs].astype(f32) + patch).astype(bf16)

    def out_lhs(ids, y):
        place = (_iota((16, T), 1) == _iota((16, T), 0) + 64) & (_iota((16, T), 0) < 2)
        ycols = _dot_tn(y, jnp.where(place, 1.0, 0.0).astype(bf16))
        last = _to_bf16(wot[:, 4 * T:5 * T]).astype(f32) + ycols
        for s in range(EARLY, NSEG):
            tok = _iota((64, L), 1) + s * L
            rows = _iota((64, L), 0)
            hit = ((rows == 0) & (tok == ids[0])) | ((rows == 1) & (tok == ids[1]))
            ot[s, D:D + 64, :] = jnp.where(hit, 1.0, 0.0)
        return jnp.concatenate([_to_bf16(wot[:, 0:4 * T]), last.astype(bf16)], axis=1)

    def out_project_early(s, tt):
        require_heads(s, tt)
        require('wot')
        cs = tile_cols(s, tt)
        attn = _dot(_to_bf16(wot[:, 0:D]), ot[s, 0:D, local_cols(tt)].astype(bf16))
        fill(CFG['fill_proj'])
        outb[:, cs] = (attn + xn[:, cs] + xt[:, cs].astype(f32)).astype(bf16)

    def out_project(lhs, s, tt):
        require_heads(s, tt)
        cs = tile_cols(s, tt)
        attn = _dot(lhs, ot[s, :, local_cols(tt)].astype(bf16))
        outb[:, cs] = (attn + xn[:, cs] + xt[:, cs].astype(f32)).astype(bf16)

    def row_maxima():
        def project_tile(tt, carry):
            cs = pl.ds(pl.multiple_of(tt * T, T), T)
            y = _layernorm_apply(xt[:, cs], _layernorm_stats(xt[:, cs])).astype(bf16)
            kall[:, cs] = _dot(_to_bf16(wt[0:half, :]), y).astype(bf16)
            qall[:, cs] = (_dot(_to_bf16(wt[half:2 * half, :]), y) * QSCALE).astype(bf16)
            return carry

        lax.fori_loop(0, S // T, project_tile, 0)

        def head_tile(i, carry):
            h = i // (S // T)
            tt = i % (S // T)
            cs = pl.ds(pl.multiple_of(tt * T, T), T)
            seg = pl.ds(pl.multiple_of((tt // NT) * L, L), L)
            rows = _iota((D, T), 0)
            qm = jnp.where((rows >= DH * h) & (rows < DH * h + DH), qall[:, cs].astype(f32), 0.0)
            logits = _dot_tn(kall[:, seg], qm.astype(bf16))
            seen = _iota((L, T), 0) <= _iota((L, T), 1) + (tt % NT) * T
            m = jnp.max(jnp.where(seen, logits, NEG_BIG), axis=0, keepdims=True)
            mrow[:, cs] = jnp.where(_iota((H, T), 0) == h, m, mrow[:, cs])
            wide_m = jnp.broadcast_to(m, (8, T))
            mx[2 + i] = jnp.where(h >= H - 4, _shift_words(wide_m, True), _shift_words(wide_m, False))
            return carry

        mrow[...] = jnp.zeros(mrow.shape, f32)
        lax.fori_loop(0, H * (S // T), head_tile, 0)

        def pack_tile(tt, carry):
            cs = pl.ds(pl.multiple_of(tt * T, T), T)
            m = mrow[:, cs]
            block = _iota((1, T), 1) // SUB
            for b in range(NQUAD):
                for i in range(4):
                    row = jnp.zeros((1, T), f32)
                    for a in range(4):
                        src = m[4 * b + a:4 * b + a + 1, :]
                        shift = (SUB * (a - i)) % T
                        row = jnp.where(block == a, src if shift == 0 else pltpu.roll(src, shift, 1), row)
                    mxp[2 + tt * H + 4 * b + i] = _shift_words(jnp.broadcast_to(row, (8, T)), b == NQUAD - 1)
            return carry

        lax.fori_loop(0, S // T, pack_tile, 0)

    for c in (xa_copy, wk_copy, xb_copy, wq_copy, wv_copy):
        c.start()
    wot[:, 4 * T:5 * T] = jnp.zeros((half, T), u32)
    pk, pq = {}, {}
    sq = [[], []]

    def sq_tie(i, n, parts):
        rows = -(-D // (16 * parts)) * 16
        part = col_sq_part(i, n * rows, min(D, (n + 1) * rows))
        sq[i].append(part)
        return tie_of(part)

    build_query_masks()
    with _scope('p0_wait'):
        xa_copy.wait()
    with _scope('p0'):
        normalize(0, 0, ln_stats(0, 0))
    with _scope('p1_wait'):
        wk_copy.wait()
    with _scope('p1'):
        wt[0:half, :] = transpose_weight(0)
        k0a = keys_raw(0, 0, 0, half)
    with _scope('p1b_wait'):
        xb_copy.wait()
    with _scope('p1b'):
        st1 = ln_stats(0, 1)
        k0 = jnp.concatenate([k0a, keys_raw(0, 0, half, D)], axis=0)
        normalize(0, 1, st1)
        st2 = ln_stats(0, 2)
        k1 = keys_raw(0, 1)
        pk[0, 0] = keys_finish(0, 0, k0, sq_tie(0, 0, 2) + _zero_after(st2[1]))
        normalize(0, 2, st2)
        st3 = ln_stats(0, 3)
        k2 = keys_raw(0, 2)
        pk[0, 1] = keys_finish(0, 1, k1, sq_tie(0, 1, 2) + _zero_after(st3[1]))
        normalize(0, 3, st3)
        k3a = keys_raw(0, 3, 0, half)
    with _scope('p2_wait'):
        wq_copy.wait()
        wv_copy.wait()
    for c in (xr_copy, wo_copy, beta_copy, wr_copy):
        c.start()
    with _scope('p2'):
        k3 = jnp.concatenate([k3a, keys_raw(0, 3, half, D)], axis=0)
        wt[half:2 * half, :] = transpose_weight(1)
        wt[2 * half:3 * half, :] = transpose_weight(2)
        pk[0, 2] = keys_finish(0, 2, k2)
        project_q(0, 0, sq_tie(1, 0, 4))
        pk[0, 3] = keys_finish(0, 3, k3)
        for tt in range(1, NT):
            project_q(0, tt, sq_tie(1, tt, 4))
        for tt in range(NT - 1):
            project_v(0, tt)
        csq = [col_sq_max(parts) for parts in sq]
        bound = (QSCALE * LN_NORM2 * DH) * jnp.sqrt(csq[0] * csq[1])
        for low in range(2):
            words = _shift_words(jnp.broadcast_to(bound, (8, T)), low == 1)
            mx[low] = words
            mxp[low] = words
        shift_sel = jnp.max(jnp.where(bound <= LOGIT_LIMIT, 0, 1))
        unsafe = shift_sel > 0
    with _scope('p4_wait'):
        for c in (xr_copy, wo_copy, beta_copy, wr_copy):
            c.wait()
    for c in moe_copies:
        c.start()

    @pl.when(unsafe)
    def _():
        row_maxima()

    project_v(0, NT - 1)
    gb[...] = _sigmoid(jnp.broadcast_to(beta_ref[...].astype(f32).reshape(1, H), (T, H)).T)

    slots = {}
    st = {}

    def at(s, b, j, fn):
        slots.setdefault((s, b, j), []).append(fn)

    def at_pos(s, pos, fn):
        at(s, pos // NT, pos % NT, fn)

    def wr_lhs():
        if 'wr' not in st:
            w = jnp.broadcast_to(wr_ref[...].astype(f32).reshape(1, D), (16, D))
            st['wr'] = jnp.where(_iota((16, D), 0) == 0, w, 0.0).astype(bf16)
        return st['wr']

    stats = {}

    def stats_task(s, tt):
        def fn():
            stats[s, tt] = ln_stats(s, tt)
            if CFG['tie_stats']:
                ties.append((clock[0] + CFG['tie_ln'], _zero_bits_after(_to_u32(jnp.broadcast_to(stats[s, tt][1], (8, T))))))
        return fn

    def norm_task(s, tt):
        return lambda: normalize(s, tt, stats[s, tt])

    def score_task(s, tt):
        return lambda: router_scores(wr_lhs(), s, tt)

    for s in range(NSEG - 1):
        for g in range(NGRP):
            at_pos(s, 2 * g, lambda s=s, g=g: memory_update(s, g, [pk[s, tt] for tt in range(NT)]))
        if s == 0:
            at_pos(0, 3, stats_task(1, 0))
            at_pos(0, 5, norm_task(1, 0))
        for tt in range(NT):
            p0 = 9 + 6 * tt
            if s == 0:
                at_pos(s, p0, stats_task(2, tt))
                if tt > 0:
                    at_pos(s, p0, norm_task(3, tt - 1))
            at_pos(s, p0, lambda s=s, tt=tt: pk.__setitem__((s + 1, tt), project_k(s + 1, tt)))
            if s == 0:
                if tt > 0:
                    at_pos(s, p0, score_task(3, tt - 1))
                at_pos(s, p0 + 2, norm_task(2, tt))
                if tt + 1 < NT:
                    at_pos(s, p0 + 2, stats_task(1, tt + 1))
            at_pos(s, p0 + 2, lambda s=s, tt=tt: pq.__setitem__((s + 1, tt), project_q(s + 1, tt)))
            if s == 0:
                at_pos(s, p0 + 2, score_task(2, tt))
            if s == 0:
                if tt + 1 < NT:
                    at_pos(s, p0 + 4, norm_task(1, tt + 1))
                at_pos(s, p0 + 4, stats_task(3, tt))
            at_pos(s, p0 + 4, lambda s=s, tt=tt: project_v(s + 1, tt))
            at_pos(s, p0 + CFG['read_off'], lambda s=s, tt=tt: memory_read(s + 1, tt, pq[s + 1, tt]))
    at_pos(1, 0, norm_task(3, NT - 1))
    for s in range(EARLY):
        for tt in range(NT):
            at_pos(s + 1, 3 + 2 * tt if s > 0 else 8 + 6 * tt, lambda s=s, tt=tt: out_project_early(s, tt))
    at_pos(1, 1, score_task(3, NT - 1))
    for tt in range(NT):
        at_pos(0, 1 + 2 * tt, score_task(0, tt))
        at_pos(0, 10 + 6 * tt, score_task(1, tt))
    def set_out_weight():
        wot[:, 0:D] = transpose_weight(3)
        produced('wot')

    at_pos(0, 22, set_out_weight)

    at_pos(1, 2, lambda: st.update(zip(('ids', 'sel'), route())))
    at_pos(1, CFG['select_pos'], lambda: st.update(xsel=select_tokens(st['ids'])))

    def start_moe():
        with _scope('moe_wait'):
            for c in moe_copies:
                c.wait()
        queue_moe(st['xsel'], st)

    at(1, CFG['moe_quad'], -1, start_moe)

    def finish_moe():
        fill(len(fillers))
        y = moe_result(st['sel'], jnp.concatenate(st['ycols'], axis=1))
        patch_early(st['ids'], y)
        st['lhs'] = out_lhs(st['ids'], y)

    e0 = CFG['moe_end']
    at_pos(3, e0, finish_moe)
    for s in range(EARLY):
        at_pos(3, e0 + 1 + s, lambda s=s: out_copy(s * L, (s + 1) * L, s).start())
    for tt in range(NT):
        at_pos(3, e0 + 2 + CFG['op_gap'] * tt, lambda tt=tt: out_project(st['lhs'], 2, tt))
    at_pos(3, e0 + 3 + CFG['op_gap'] * (NT - 1), lambda: out_copy(2 * L, 3 * L, 2).start())

    def quad_values(s, b, j, ps):
        for a in range(4):
            values(s, 4 * b + a, j, ps[a])

    pending = []
    for s in range(NSEG):
        for b in range(NQUAD):
            for fn in slots.pop((s, b, -1), ()):
                fn()
            for j in range(NT):
                pending.append((s, b, j, scores(s, b, j)))
                for fn in slots.pop((s, b, j), ()):
                    fn()
                if len(pending) > CFG['lag']:
                    quad_values(*pending.pop(0))
    tail = [unit for unit in pending]
    assert not slots, slots.keys()
    s = NSEG - 1

    def last_tile(tt):
        out_project(st['lhs'], s, tt)
        out_copy(s * L + tt * T, s * L + (tt + 1) * T, 3 + tt).start()

    done = 0
    for unit in tail:
        quad_values(*unit)
        while done < NT and unit[1] == NQUAD - 1 and done < unit[2]:
            last_tile(done)
            done += 1
    while done < NT:
        last_tile(done)
        done += 1
    with _scope('out_wait'):
        for k in range(NSEG - 1):
            out_copy(k * L, (k + 1) * L, k).wait()
        for tt in range(NT):
            out_copy(s * L + tt * T, s * L + (tt + 1) * T, 3 + tt).wait()


@jax.jit
def pallas_parallel_sum__memory_aug_infini_attn__moe_arch_mod__prompt_kernel(
    A_x: jax.Array,
    A_wq: jax.Array,
    A_wk: jax.Array,
    A_wv: jax.Array,
    A_wo: jax.Array,
    A_beta: jax.Array,
    B_x: jax.Array,
    B_w_r: jax.Array,
    B_w_gate: jax.Array,
    B_w_up: jax.Array,
    B_w_down: jax.Array,
):
    del B_x
    x_t = jnp.transpose(A_x, (0, 2, 1)).reshape(D, S)
    wd_t = B_w_down.T
    hbm = pl.BlockSpec(memory_space=pl.ANY)
    out_t = pl.pallas_call(
        _kernel,
        out_shape=jax.ShapeDtypeStruct((D, S), bf16),
        in_specs=[hbm] * 10,
        out_specs=hbm,
        scratch_shapes=[
            pltpu.VMEM((D, S), bf16),
            pltpu.VMEM((D, S), f32),
            pltpu.VMEM((4, D, D), bf16),
            pltpu.VMEM((3 * D // 2, D), u32),
            pltpu.VMEM((D // 2, 5 * T), u32),
            pltpu.VMEM((D, F), bf16),
            pltpu.VMEM((D, F), bf16),
            pltpu.VMEM((D, F), bf16),
            pltpu.VMEM((H,), bf16),
            pltpu.VMEM((D,), bf16),
            pltpu.VMEM((2, D // 2, L), u32),
            pltpu.VMEM((2, D, L), f32),
            pltpu.VMEM((2, NQUAD, L // 2, T), u32),
            pltpu.VMEM((2, NGRP, MROWS, L), f32),
            pltpu.VMEM((NGRP, MROWS, T), f32),
            pltpu.VMEM((NGRP, 8, T), f32),
            pltpu.VMEM((NSEG, 5 * T, L), f32),
            pltpu.VMEM((2 + H * S // T, 8, T), u32),
            pltpu.VMEM((2 + H * S // T, 8, T), u32),
            pltpu.VMEM((H, S), f32),
            pltpu.VMEM((NQUAD, 16, 8, T), u32),
            pltpu.VMEM((S // T, T), f32),
            pltpu.VMEM((D, S), bf16),
            pltpu.VMEM((H, T), f32),
            pltpu.VMEM((D, S), bf16),
            pltpu.VMEM((D, S), bf16),
            pltpu.SemaphoreType.DMA((19,)),
        ],
        compiler_params=pltpu.CompilerParams(vmem_limit_bytes=100 * 1024 * 1024),
        name="infini_moe",
    )(x_t, A_wq, A_wk, A_wv, A_wo, A_beta, B_w_r, B_w_gate, B_w_up, wd_t)
    return jnp.transpose(out_t.reshape(1, D, S), (0, 2, 1))
```

```python
import contextlib
import functools

import jax
import jax.numpy as jnp
from jax import lax
from jax.experimental import pallas as pl
from jax.experimental.pallas import tpu as pltpu

S, D, H, DH = 2048, 576, 32, 18
NSEG, L, F = 4, 512, 4608
T = 128
NT = L // T
NGRP = 5
SLAB = 112
GROUP_FIRST = (0, 7, 13, 19, 25, 32)
MROWS = 144
NCHUNK = F // T
NQUAD = H // 4
QUAD_OFF = (0, 64, 144, 208, 288, 352, 432, 448)
EARLY = 2
KSPLIT = 256
SUB = 32

bf16, f32, u32, i32 = jnp.bfloat16, jnp.float32, jnp.uint32, jnp.int32

LOG2E = 1.4426950408889634
QSCALE = (DH ** -0.5) * LOG2E
LN_NORM2 = 2.1 * D
LOGIT_LIMIT = 50.0
NEG_BIG = -1e30


PROFILE_SCOPES = False
CFG = dict(lag=5, rot=0, tie_stats=True, tie_p=3, fill_proj=10, fill_qk=8, select_pos=7, moe_quad=5, moe_end=8, op_gap=3, read_off=4, tie_res=3, tie_ln=1)


def _scope(name):
    return jax.named_scope(name) if PROFILE_SCOPES else contextlib.nullcontext()


def _group_of(h):
    for g in range(NGRP):
        if GROUP_FIRST[g] <= h < GROUP_FIRST[g + 1]:
            return g
    raise ValueError(h)


def _to_bf16(x):
    return pltpu.bitcast(x, bf16)


def _to_u32(x):
    return pltpu.bitcast(x, u32)


def _round_bf16(x):
    return x.astype(bf16).astype(f32)


def _iota(shape, dim):
    return lax.broadcasted_iota(i32, shape, dim)


def _dot(a, b):
    return jnp.dot(a, b, preferred_element_type=f32)


def _dot_nt(a, b):
    return lax.dot_general(a, b, (((1,), (1,)), ((), ())), preferred_element_type=f32)


def _dot_tn(a, b):
    return lax.dot_general(a, b, (((0,), (0,)), ((), ())), preferred_element_type=f32)


def _zero_after_bits(u):
    return lax.shift_right_logical(pltpu.bitcast(u, i32), 31).astype(f32) * 0.0


def _pack_pairs(x):
    lo = jnp.concatenate([x[r:r + 8] for r in range(0, x.shape[0], 16)], axis=0)
    hi = jnp.concatenate([x[r + 8:r + 16] for r in range(0, x.shape[0], 16)], axis=0)
    return pltpu.pack_elementwise([lo, hi], packed_dtype=bf16)


def _unpaired_index(r):
    x = r & 15
    return (r - x) + jnp.where(x < 8, 2 * x, 2 * (x - 8) + 1)


def _zero_bits_after(u):
    sixteen = jnp.full(u.shape, 16, u32)
    return lax.shift_right_logical(lax.shift_right_logical(u, sixteen), sixteen)


def _pair_mask(first, lo, hi, keep_lane=None):
    f = _iota((8, T), 0) + first
    low = (f >= lo) & (f < hi)
    high = (f + 8 >= lo) & (f + 8 < hi)
    if keep_lane is not None:
        low, high = low & keep_lane, high & keep_lane
    return jnp.where(low, jnp.uint32(0xFFFF), jnp.uint32(0)) | jnp.where(high, jnp.uint32(0xFFFF0000), jnp.uint32(0))


def _bf16_bits(x):
    return pltpu.bitcast(_round_bf16(x), u32)


def _shift_words(m, low_half):
    first = _round_bf16(-m)
    second = _round_bf16(-m - first)
    third = -m - first - second
    row = _iota((8, T), 0)
    val = jnp.where(row == 5, first, jnp.where(row == 6, second, jnp.where(row == 7, third, 0.0)))
    bits = _bf16_bits(val)
    return lax.shift_right_logical(bits, jnp.full(bits.shape, 16, u32)) if low_half else bits


def _phi(t):
    return jnp.where(t > 0, t + 1.0, jnp.exp(t))


def _sigmoid(t):
    return 1.0 / (1.0 + jnp.exp(-t))


def _layernorm_stats(xb):
    x0 = xb[0:1, :].astype(f32)
    acc1, acc2 = [None] * 4, [None] * 4
    for n, r in enumerate(range(0, D, 16)):
        c = xb[r:r + 16, :].astype(f32) - x0
        for part in range(2):
            k = (2 * n + part) % 4
            piece = c[8 * part:8 * part + 8, :]
            acc1[k] = piece if acc1[k] is None else acc1[k] + piece
            acc2[k] = piece * piece if acc2[k] is None else acc2[k] + piece * piece
    s1 = jnp.sum((acc1[0] + acc1[1]) + (acc1[2] + acc1[3]), axis=0, keepdims=True) / D
    s2 = jnp.sum((acc2[0] + acc2[1]) + (acc2[2] + acc2[3]), axis=0, keepdims=True) / D
    var = jnp.maximum(s2 - s1 * s1, 0.0)
    eps = _round_bf16(jnp.full((1, 1), 1e-5, f32))
    sd = _round_bf16(jnp.sqrt(_round_bf16(_round_bf16(var) + eps)))
    return _round_bf16(x0 + s1), 1.0 / sd


def _layernorm_apply(xb, stats):
    mean, inv = stats
    return _round_bf16(xb.astype(f32) - mean) * inv


def _block_transpose(xs):
    lane = _iota(next(x for x in xs if x is not None).shape, 1)

    def exchange(u, v, low, shift):
        def pick(p, q):
            if p is None and q is None:
                return None
            return jnp.where(low, 0.0 if p is None else p, 0.0 if q is None else q)
        ru = None if u is None else pltpu.roll(u, T - shift, 1)
        rv = None if v is None else pltpu.roll(v, shift, 1)
        return pick(u, rv), pick(ru, v)

    y0, y2 = exchange(xs[0], xs[2], lane < 64, 64)
    y1, y3 = exchange(xs[1], xs[3], lane < 64, 64)
    low = (lane & 32) == 0
    z0, z1 = exchange(y0, y1, low, 32)
    z2, z3 = exchange(y2, y3, low, 32)
    return [z0, z1, z2, z3]


def _head_of_slab_index(idx, g):
    return ((idx + SLAB * g) * 3641) >> 16


def _zero_after(x):
    sign = lax.shift_right_logical(pltpu.bitcast(x, i32), 31)
    return sign.astype(f32) * 0.0


def _kernel(x_hbm, wq_hbm, wk_hbm, wv_hbm, wo_hbm, beta_hbm, wr_hbm, wg_hbm, wu_hbm, wd_hbm,
            out_hbm,
            xt, xn, wstage, wt, wot, wg, wu, wd, beta_ref, wr_ref, qt, vt, kp, num, mt, zt, ot,
            mx, mxp, mrow, qmask, rrow, outb, gb, kall, qall, sems):
    def copy(src, dst, i):
        return pltpu.make_async_copy(src, dst, sems.at[i])

    xa_copy = copy(x_hbm.at[:, 0:T], xt.at[:, 0:T], 0)
    xb_copy = copy(x_hbm.at[:, T:L], xt.at[:, T:L], 18)
    xr_copy = copy(x_hbm.at[:, L:S], xt.at[:, L:S], 1)
    wq_copy, wv_copy, wo_copy = [
        copy(w, wstage.at[i], 2 + i) for i, w in ((1, wq_hbm), (2, wv_hbm), (3, wo_hbm))]
    wka_copy = copy(wk_hbm.at[:, 0:KSPLIT], wstage.at[0, :, 0:KSPLIT], 2)
    wkb_copy = copy(wk_hbm.at[:, KSPLIT:D], wstage.at[0, :, KSPLIT:D], 19)
    beta_copy = copy(beta_hbm, beta_ref, 6)
    wr_copy = copy(wr_hbm, wr_ref, 7)
    moe_copies = [copy(wg_hbm, wg, 8), copy(wu_hbm, wu, 9), copy(wd_hbm, wd, 10)]

    def out_copy(lo, hi, i):
        return copy(outb.at[:, lo:hi], out_hbm.at[:, lo:hi], 11 + i)

    half = D // 2
    emitted = set()

    def produced(*key):
        emitted.add(key)

    def require(*key):
        assert key in emitted, key

    def require_heads(s, j):
        for h in range(H):
            require('ot', s, h, j)

    fillers = []

    def fill(n):
        for _ in range(min(n, len(fillers))):
            fillers.pop(0)()

    clock = [0]
    ties = []

    def tile_cols(s, tt):
        return slice(s * L + tt * T, s * L + (tt + 1) * T)

    def local_cols(tt):
        return slice(tt * T, (tt + 1) * T)

    def col_sq_part(i, lo, hi):
        acc = None
        for r in range(lo, hi, 16):
            w = wstage[i, r:r + 16, :].astype(f32)
            w = w * w
            part = w[0:8] + w[8:16]
            acc = part if acc is None else acc + part
        return acc

    def col_sq_max(parts):
        acc = functools.reduce(lambda u, v: u + v, parts)
        return jnp.max(jnp.sum(acc, axis=0, keepdims=True), axis=1, keepdims=True)

    def tie_of(part):
        folded = functools.reduce(lambda u, v: u + v, [part[:, c:c + T] for c in range(0, 4 * T, T)])
        return _zero_after(folded[0:1, 0:1] + part[0:1, 4 * T:4 * T + 1])

    def transpose_weight(i):
        return _to_u32(wstage[i].T)

    def ln_stats(s, tt):
        return _layernorm_stats(xt[:, tile_cols(s, tt)])

    def normalize(s, tt, stats):
        cs = tile_cols(s, tt)
        xn[:, cs] = _layernorm_apply(xt[:, cs], stats)
        produced('xn', s, tt)

    def xn_tile(s, tt):
        require('xn', s, tt)
        return xn[:, tile_cols(s, tt)].astype(bf16)

    def keys_raw(s, tt, lo=0, hi=D):
        kt = _dot(_to_bf16(wt[lo // 2:hi // 2, :]), xn_tile(s, tt))
        fill(CFG['fill_proj'])
        return kt

    def keys_finish(s, tt, kt, tie=None):
        if tie is not None:
            kt = kt + tie
        words = jnp.take_along_axis(_pack_pairs(kt), _unpaired_index(_iota((half, T), 1)), axis=1)
        shift_rows = _iota((8, T), 0) >= 5
        for b in range(NQUAD):
            slab = words[QUAD_OFF[b] // 2:QUAD_OFF[b] // 2 + T // 2, :]
            if b == NQUAD - 1:
                ones = jnp.where(shift_rows, (slab[0:8] & jnp.uint32(0xFFFF0000)) | jnp.uint32(0x3F80), slab[0:8])
                slab = jnp.concatenate([ones, slab[8:]], axis=0)
            else:
                ones = jnp.where(shift_rows, (slab[56:64] & jnp.uint32(0xFFFF)) | jnp.uint32(0x3F800000), slab[56:64])
                slab = jnp.concatenate([slab[:56], ones], axis=0)
            kp[s % 2, b, tt * (T // 2):(tt + 1) * (T // 2), :] = _to_u32(_to_bf16(slab).T)
        produced('k', s, tt)
        return _phi(kt).astype(bf16)

    def project_k(s, tt):
        return keys_finish(s, tt, keys_raw(s, tt))

    def project_q(s, tt, tie=None):
        q = _dot(_to_bf16(wt[half:2 * half, :]), xn_tile(s, tt))
        fill(CFG['fill_proj'])
        qt[s % 2, :, local_cols(tt)] = _pack_pairs(q * (QSCALE if tie is None else QSCALE + tie))
        produced('q', s, tt)
        return _phi(q).astype(bf16)

    def require_segment_done(s):
        if s >= 0:
            for j in range(NT):
                require_heads(s, j)

    def project_v(s, tt, tie=None):
        require_segment_done(s - 2)
        v = _dot(_to_bf16(wt[2 * half:3 * half, :]), xn_tile(s, tt))
        fill(CFG['fill_proj'])
        vt[s % 2, :, local_cols(tt)] = v if tie is None else v + tie
        produced('v', s, tt)

    def router_scores(lhs, s, tt):
        row = s * NT + tt
        rrow[row:row + 1, :] = _dot(lhs, xn_tile(s, tt))[0:1, :]
        produced('r', s, tt)

    def memory_read(s, tt, pq):
        require_segment_done(s - 2)
        for g in range(NGRP):
            require('mt', s - 1, g)
        for g in range(NGRP):
            num[s % 2, g, :, local_cols(tt)] = _dot(mt[g].astype(bf16), pq[SLAB * g:SLAB * g + T, :])
        produced('num', s, tt)

    def memory_update(s, g, pk):
        ones_row = 0 if g == NGRP - 1 else T - 1
        vs = jnp.where(_iota((T, L), 0) == ones_row, 1.0, vt[s % 2, SLAB * g:SLAB * g + T, :]).astype(bf16)
        m = _dot_nt(vs, jnp.concatenate([p[SLAB * g:SLAB * g + T, :] for p in pk], axis=1))
        hr = _head_of_slab_index(_iota((T, T), 0), g)
        hc = _head_of_slab_index(_iota((T, T), 1), g)
        keep = (hr == hc) & (hr >= GROUP_FIRST[g]) & (hr < GROUP_FIRST[g + 1])
        mm = jnp.where(keep, m, 0.0)
        z = m[ones_row:ones_row + 1, :]
        if s > 0:
            mm = mm + mt[g, 0:T, :]
            z = z + zt[g, 0:1, :]
        mt[g, 0:T, :] = mm
        zt[g, 0:1, :] = z
        zsel = _head_of_slab_index(_iota((16, T), 1), g) == _iota((16, T), 0) + GROUP_FIRST[g]
        mt[g, T:MROWS, :] = jnp.where(zsel, z, 0.0)
        produced('mt', s, g)

    def head_groups(b, a):
        f = DH * (4 * b + a) - QUAD_OFF[b]
        return f, (f // 16, f // 16 + 1)

    def build_query_masks():
        block = _iota((8, T), 1) // SUB
        for b in range(NQUAD):
            for a in range(4):
                f, groups = head_groups(b, a)
                for n, g in enumerate(groups):
                    qmask[b, 4 * a + 2 * n] = _pair_mask(16 * g, f, f + DH)
                    qmask[b, 4 * a + 2 * n + 1] = _pair_mask(16 * g, f, f + DH, block == a)

    def stack_groups(groups):
        return _to_bf16(jnp.concatenate(
            [groups.get(g, jnp.zeros((8, T), u32)) for g in range(T // 16)], axis=0))

    def quad_queries(s, b, j, tie):
        tile = s * NT + j
        last = b == NQUAD - 1
        shift_group = 0 if last else T // 16 - 1
        base = QUAD_OFF[b] // 2
        words = {}

        def group(g):
            if g not in words:
                words[g] = qt[s % 2, base + 8 * g:base + 8 * g + 8, local_cols(j)]
            return words[g]

        wide = []
        for a in range(4):
            _, groups = head_groups(b, a)
            parts = {g: group(g) & qmask[b, 4 * a + 2 * n] for n, g in enumerate(groups)}
            if j > 0:
                parts[shift_group] = mx[int(last) + shift_sel * (2 - int(last) + (4 * b + a) * (S // T) + tile)]
                wide.append(stack_groups(parts))
        packed = []
        for i in range(4):
            parts = {}
            for a in range(4):
                _, groups = head_groups(b, a)
                shift = (SUB * (a - i)) % T
                for n, g in enumerate(groups):
                    moved = group(g) if shift == 0 else pltpu.roll(group(g), shift, 1)
                    piece = moved & qmask[b, 4 * a + 2 * n + 1]
                    parts[g] = piece if g not in parts else parts[g] | piece
            rows = mxp[int(last) + shift_sel * (2 - int(last) + tile * H + 4 * b + i)]
            if tie is not None and i == 3:
                rows = rows | tie
            parts[shift_group] = rows
            packed.append(stack_groups(parts))
        return wide, packed

    def scores(s, b, j):
        require('q', s, j)
        for tt in range(j + 1):
            require('k', s, tt)
        tie = None
        unit = clock[0] = (s * NQUAD + b) * NT + j
        due = [z for when, z in ties if when <= unit]
        ties[:] = [(when, z) for when, z in ties if when > unit]
        if due:
            tie = functools.reduce(lambda u, v: u | v, due)
        wide, packed = quad_queries(s, b, j, tie)
        k0 = j * (T // 2)
        off = None
        if j > 0:
            logits = _dot(_to_bf16(kp[s % 2, b, 0:k0, :]), jnp.concatenate(wide, axis=1))
            fill(CFG['fill_qk'])
            off = jnp.exp2(logits)
        causal = _unpaired_index(_iota((SUB, T), 0)) <= (_iota((SUB, T), 1) & (SUB - 1))
        diag = [None] * 4
        for i in range(4):
            n = SUB * (i + 1)
            e = jnp.exp2(_dot(_to_bf16(kp[s % 2, b, k0:k0 + n // 2, :]), packed[i]))
            blocks = [e[r * SUB:(r + 1) * SUB, :] for r in range(i)]
            blocks.append(jnp.where(causal, e[i * SUB:, :], 0.0))
            diag[i] = blocks
        per_head = [[] for _ in range(4)]
        for r in range(4):
            outs = _block_transpose([diag[i][r] if i >= r else None for i in range(4)])
            for a in range(4):
                per_head[a].append(outs[a])
        ps = []
        for a in range(4):
            parts = ([off[:, a * T:(a + 1) * T]] if j > 0 else []) + per_head[a]
            ps.append(_pack_pairs(jnp.concatenate(parts, axis=0)))
        if CFG['tie_p'] is not None:
            rows = [u[r:r + 8] for u in ps for r in range(0, u.shape[0], 8)]
            while len(rows) > 1:
                rows = [rows[i] | rows[i + 1] for i in range(0, len(rows) - 1, 2)] + rows[len(rows) & ~1:]
            ties.append((unit + CFG['tie_p'], _zero_bits_after(rows[0])))
        return [_to_bf16(u) for u in ps]

    def values(s, h, j, p):
        g = _group_of(h)
        w0 = min((DH * h // 16) * 16, D - 32)
        off = DH * h - w0
        ones_row = 31 if off < 14 else 0
        n = (j + 1) * T
        cs = local_cols(j)
        for tt in range(j + 1):
            require('v', s, tt)
        if s > 0:
            require('num', s, j)
        g0 = (ones_row // 8) * 8
        marked = jnp.where(_iota((8, n), 0) == ones_row - g0, 1.0, vt[s % 2, w0 + g0:w0 + g0 + 8, 0:n])
        rest = vt[s % 2, w0 + 8:w0 + 32, 0:n] if g0 == 0 else vt[s % 2, w0:w0 + 24, 0:n]
        vwin = jnp.concatenate([marked, rest] if g0 == 0 else [rest, marked], axis=0).astype(bf16)
        gate = gb[h:h + 1, :]
        acc = _dot(vwin, p)
        res = acc * ((1.0 - gate) / acc[ones_row:ones_row + 1, :])
        if s > 0:
            m0 = w0 - SLAB * g
            zr = T + h - GROUP_FIRST[g]
            den = num[s % 2, g, zr:zr + 1, cs] + 1e-6
            res = res + num[s % 2, g, m0:m0 + 32, cs] * (gate / den)
        else:
            ties.append((clock[0] + CFG['tie_res'], _zero_bits_after(_to_u32((res[0:8] + res[8:16]) + (res[16:24] + res[24:32])))))
        ot[s, DH * h:DH * h + DH, cs] = res[off:off + DH, :]
        produced('ot', s, h, j)

    def route():
        for s in range(NSEG):
            for tt in range(NT):
                require('r', s, tt)
        r = _round_bf16(rrow[...])
        idx = _iota((S // T, T), 0) * T + _iota((S // T, T), 1)
        m1 = jnp.max(r)
        i1 = jnp.min(jnp.where(r == m1, idx, S - 1))
        r2 = jnp.where(idx == i1, -jnp.inf, r)
        m2 = jnp.max(r2)
        i2 = jnp.min(jnp.where(r2 == m2, idx, S - 1))
        return (i1, i2), (m1, m2)

    def select_tokens(ids):
        sel = None
        for row, i in enumerate(ids):
            hit = (_iota((16, T), 0) == row) & (_iota((16, T), 1) == i % T)
            cs = pl.ds(pl.multiple_of((i // T) * T, T), T)
            part = _dot_nt(jnp.where(hit, 1.0, 0.0).astype(bf16), xn[:, cs].astype(bf16))
            sel = part if sel is None else sel + part
        return sel.astype(bf16)

    def queue_moe(xsel, state):
        ktiles = [(k, min(k + T, D)) for k in range(0, D, T)]
        pre, hid = {}, {}
        ycols = state['ycols'] = [None] * len(ktiles)

        def first(w, name, c, lo, hi):
            def fn():
                part = _dot(xsel[:, lo:hi], w[lo:hi, c * T:(c + 1) * T])
                pre[name, c] = part if lo == 0 else pre[name, c] + part
            return fn

        def down(c, n, lo, hi):
            def fn():
                if c not in hid:
                    gpre = _round_bf16(pre.pop(('g', c)))
                    gact = _round_bf16(gpre * _sigmoid(gpre))
                    hid[c] = (gact * _round_bf16(pre.pop(('u', c)))).astype(bf16)
                part = _dot_nt(hid[c], wd[lo:hi, c * T:(c + 1) * T])
                ycols[n] = part if ycols[n] is None else ycols[n] + part
            return fn

        for c in range(NCHUNK + 2):
            if c < NCHUNK:
                for lo, hi in ktiles:
                    fillers.append(first(wg, 'g', c, lo, hi))
                    fillers.append(first(wu, 'u', c, lo, hi))
            if c >= 2:
                for n, (lo, hi) in enumerate(ktiles):
                    fillers.append(down(c - 2, n, lo, hi))

    def moe_result(sel_scores, y):
        row = _iota((16, D), 0)
        gate = jnp.where(row == 0, sel_scores[0], sel_scores[1])
        return (_round_bf16(y) * _round_bf16(_sigmoid(gate))).astype(bf16)

    def patch_early(ids, y):
        for k, i in enumerate(ids):
            hit = (_iota((16, T), 0) == k) & (_iota((16, T), 1) == i % T) & (i < EARLY * L)
            cs = pl.ds(pl.multiple_of((jnp.minimum(i, EARLY * L - 1) // T) * T, T), T)
            patch = _dot_tn(y, jnp.where(hit, 1.0, 0.0).astype(bf16))
            outb[:, cs] = (outb[:, cs].astype(f32) + patch).astype(bf16)

    def out_lhs(ids, y):
        place = (_iota((16, T), 1) == _iota((16, T), 0) + 64) & (_iota((16, T), 0) < 2)
        ycols = _dot_tn(y, jnp.where(place, 1.0, 0.0).astype(bf16))
        last = _to_bf16(wot[:, 4 * T:5 * T]).astype(f32) + ycols
        for s in range(EARLY, NSEG):
            tok = _iota((64, L), 1) + s * L
            rows = _iota((64, L), 0)
            hit = ((rows == 0) & (tok == ids[0])) | ((rows == 1) & (tok == ids[1]))
            ot[s, D:D + 64, :] = jnp.where(hit, 1.0, 0.0)
        return jnp.concatenate([_to_bf16(wot[:, 0:4 * T]), last.astype(bf16)], axis=1)

    def out_project_early(s, tt):
        require_heads(s, tt)
        require('wot')
        cs = tile_cols(s, tt)
        attn = _dot(_to_bf16(wot[:, 0:D]), ot[s, 0:D, local_cols(tt)].astype(bf16))
        fill(CFG['fill_proj'])
        outb[:, cs] = (attn + xn[:, cs] + xt[:, cs].astype(f32)).astype(bf16)

    def out_project(lhs, s, tt):
        require_heads(s, tt)
        cs = tile_cols(s, tt)
        attn = _dot(lhs, ot[s, :, local_cols(tt)].astype(bf16))
        outb[:, cs] = (attn + xn[:, cs] + xt[:, cs].astype(f32)).astype(bf16)

    def row_maxima():
        def project_tile(tt, carry):
            cs = pl.ds(pl.multiple_of(tt * T, T), T)
            y = _layernorm_apply(xt[:, cs], _layernorm_stats(xt[:, cs])).astype(bf16)
            kall[:, cs] = _dot(_to_bf16(wt[0:half, :]), y).astype(bf16)
            qall[:, cs] = (_dot(_to_bf16(wt[half:2 * half, :]), y) * QSCALE).astype(bf16)
            return carry

        lax.fori_loop(0, S // T, project_tile, 0)

        def head_tile(i, carry):
            h = i // (S // T)
            tt = i % (S // T)
            cs = pl.ds(pl.multiple_of(tt * T, T), T)
            seg = pl.ds(pl.multiple_of((tt // NT) * L, L), L)
            rows = _iota((D, T), 0)
            qm = jnp.where((rows >= DH * h) & (rows < DH * h + DH), qall[:, cs].astype(f32), 0.0)
            logits = _dot_tn(kall[:, seg], qm.astype(bf16))
            seen = _iota((L, T), 0) <= _iota((L, T), 1) + (tt % NT) * T
            m = jnp.max(jnp.where(seen, logits, NEG_BIG), axis=0, keepdims=True)
            mrow[:, cs] = jnp.where(_iota((H, T), 0) == h, m, mrow[:, cs])
            wide_m = jnp.broadcast_to(m, (8, T))
            mx[2 + i] = jnp.where(h >= H - 4, _shift_words(wide_m, True), _shift_words(wide_m, False))
            return carry

        mrow[...] = jnp.zeros(mrow.shape, f32)
        lax.fori_loop(0, H * (S // T), head_tile, 0)

        def pack_tile(tt, carry):
            cs = pl.ds(pl.multiple_of(tt * T, T), T)
            m = mrow[:, cs]
            block = _iota((1, T), 1) // SUB
            for b in range(NQUAD):
                for i in range(4):
                    row = jnp.zeros((1, T), f32)
                    for a in range(4):
                        src = m[4 * b + a:4 * b + a + 1, :]
                        shift = (SUB * (a - i)) % T
                        row = jnp.where(block == a, src if shift == 0 else pltpu.roll(src, shift, 1), row)
                    mxp[2 + tt * H + 4 * b + i] = _shift_words(jnp.broadcast_to(row, (8, T)), b == NQUAD - 1)
            return carry

        lax.fori_loop(0, S // T, pack_tile, 0)

    for c in (xa_copy, wka_copy, xb_copy, wkb_copy, wq_copy, wv_copy):
        c.start()
    wot[:, 4 * T:5 * T] = jnp.zeros((half, T), u32)
    pk, pq = {}, {}
    sq = [[], []]

    def sq_tie(i, n, parts):
        rows = -(-D // (16 * parts)) * 16
        part = col_sq_part(i, n * rows, min(D, (n + 1) * rows))
        sq[i].append(part)
        return tie_of(part)

    build_query_masks()
    with _scope('p0_wait'):
        xa_copy.wait()
    with _scope('p0'):
        normalize(0, 0, ln_stats(0, 0))
    with _scope('p1_wait'):
        wka_copy.wait()
    with _scope('p1'):
        wt[0:KSPLIT // 2, :] = _to_u32(wstage[0, :, 0:KSPLIT].T)
        ka = [keys_raw(0, 0, 0, KSPLIT)]
    with _scope('p1b_wait'):
        xb_copy.wait()
    with _scope('p1b'):
        for tt in range(1, NT):
            normalize(0, tt, ln_stats(0, tt))
            if tt < NT - 1:
                ka.append(keys_raw(0, tt, 0, KSPLIT))
    with _scope('p1c_wait'):
        wkb_copy.wait()
    with _scope('p1c'):
        ka.append(keys_raw(0, NT - 1, 0, KSPLIT))
        wt[KSPLIT // 2:half, :] = _to_u32(wstage[0, :, KSPLIT:D].T)
        kb = []
        for tt in range(NT - 1):
            kb.append(keys_raw(0, tt, KSPLIT, D))
            if tt > 0:
                pk[0, tt - 1] = keys_finish(0, tt - 1, jnp.concatenate([ka[tt - 1], kb[tt - 1]], axis=0),
                                            sq_tie(0, tt - 1, 2))
    with _scope('p2_wait'):
        wq_copy.wait()
    for c in (xr_copy, beta_copy, wr_copy, wo_copy):
        c.start()
    with _scope('p2'):
        k2 = jnp.concatenate([ka[2], kb[2]], axis=0)
        k3 = jnp.concatenate([ka[3], keys_raw(0, 3, KSPLIT, D)], axis=0)
        wt[half:2 * half, :] = transpose_weight(1)
        pk[0, 2] = keys_finish(0, 2, k2)
        project_q(0, 0, sq_tie(1, 0, 3))
        pk[0, 3] = keys_finish(0, 3, k3)
        for tt in range(1, NT - 1):
            project_q(0, tt, sq_tie(1, tt, 3))
    with _scope('p3_wait'):
        wv_copy.wait()
    with _scope('p3'):
        wt[2 * half:3 * half, :] = transpose_weight(2)
        project_q(0, NT - 1)
        for tt in range(NT - 1):
            project_v(0, tt)
        csq = [col_sq_max(parts) for parts in sq]
        bound = (QSCALE * LN_NORM2 * DH) * jnp.sqrt(csq[0] * csq[1])
        for low in range(2):
            words = _shift_words(jnp.broadcast_to(bound, (8, T)), low == 1)
            mx[low] = words
            mxp[low] = words
        shift_sel = jnp.max(jnp.where(bound <= LOGIT_LIMIT, 0, 1))
        unsafe = shift_sel > 0
    with _scope('p4_wait'):
        for c in (xr_copy, beta_copy, wr_copy, wo_copy):
            c.wait()
    for c in moe_copies:
        c.start()

    @pl.when(unsafe)
    def _():
        row_maxima()

    project_v(0, NT - 1)
    gb[...] = _sigmoid(jnp.broadcast_to(beta_ref[...].astype(f32).reshape(1, H), (T, H)).T)

    slots = {}
    st = {}

    def at(s, b, j, fn):
        slots.setdefault((s, b, j), []).append(fn)

    def at_pos(s, pos, fn):
        at(s, pos // NT, pos % NT, fn)

    def wr_lhs():
        if 'wr' not in st:
            w = jnp.broadcast_to(wr_ref[...].astype(f32).reshape(1, D), (16, D))
            st['wr'] = jnp.where(_iota((16, D), 0) == 0, w, 0.0).astype(bf16)
        return st['wr']

    stats = {}

    def stats_task(s, tt):
        def fn():
            stats[s, tt] = ln_stats(s, tt)
            if CFG['tie_stats']:
                ties.append((clock[0] + CFG['tie_ln'], _zero_bits_after(_to_u32(jnp.broadcast_to(stats[s, tt][1], (8, T))))))
        return fn

    def norm_task(s, tt):
        return lambda: normalize(s, tt, stats[s, tt])

    def score_task(s, tt):
        return lambda: router_scores(wr_lhs(), s, tt)

    for s in range(NSEG - 1):
        for g in range(NGRP):
            at_pos(s, 2 * g, lambda s=s, g=g: memory_update(s, g, [pk[s, tt] for tt in range(NT)]))
        if s == 0:
            at_pos(0, 3, stats_task(1, 0))
            at_pos(0, 5, norm_task(1, 0))
        for tt in range(NT):
            p0 = 9 + 6 * tt
            if s == 0:
                at_pos(s, p0, stats_task(2, tt))
                if tt > 0:
                    at_pos(s, p0, norm_task(3, tt - 1))
            at_pos(s, p0, lambda s=s, tt=tt: pk.__setitem__((s + 1, tt), project_k(s + 1, tt)))
            if s == 0:
                if tt > 0:
                    at_pos(s, p0, score_task(3, tt - 1))
                at_pos(s, p0 + 2, norm_task(2, tt))
                if tt + 1 < NT:
                    at_pos(s, p0 + 2, stats_task(1, tt + 1))
            at_pos(s, p0 + 2, lambda s=s, tt=tt: pq.__setitem__((s + 1, tt), project_q(s + 1, tt)))
            if s == 0:
                at_pos(s, p0 + 2, score_task(2, tt))
            if s == 0:
                if tt + 1 < NT:
                    at_pos(s, p0 + 4, norm_task(1, tt + 1))
                at_pos(s, p0 + 4, stats_task(3, tt))
            at_pos(s, p0 + 4, lambda s=s, tt=tt: project_v(s + 1, tt))
            at_pos(s, p0 + CFG['read_off'], lambda s=s, tt=tt: memory_read(s + 1, tt, pq[s + 1, tt]))
    at_pos(1, 0, norm_task(3, NT - 1))
    for s in range(EARLY):
        for tt in range(NT):
            at_pos(s + 1, 3 + 2 * tt if s > 0 else 8 + 6 * tt, lambda s=s, tt=tt: out_project_early(s, tt))
    at_pos(1, 1, score_task(3, NT - 1))
    for tt in range(NT):
        at_pos(0, 1 + 2 * tt, score_task(0, tt))
        at_pos(0, 10 + 6 * tt, score_task(1, tt))
    def set_out_weight():
        wot[:, 0:D] = transpose_weight(3)
        produced('wot')

    at_pos(0, 22, set_out_weight)

    at_pos(1, 2, lambda: st.update(zip(('ids', 'sel'), route())))
    at_pos(1, CFG['select_pos'], lambda: st.update(xsel=select_tokens(st['ids'])))

    def start_moe():
        with _scope('moe_wait'):
            for c in moe_copies:
                c.wait()
        queue_moe(st['xsel'], st)

    at(1, CFG['moe_quad'], -1, start_moe)

    def finish_moe():
        fill(len(fillers))
        y = moe_result(st['sel'], jnp.concatenate(st['ycols'], axis=1))
        patch_early(st['ids'], y)
        st['lhs'] = out_lhs(st['ids'], y)

    e0 = CFG['moe_end']
    at_pos(3, e0, finish_moe)
    for s in range(EARLY):
        at_pos(3, e0 + 1 + s, lambda s=s: out_copy(s * L, (s + 1) * L, s).start())
    for tt in range(NT):
        at_pos(3, e0 + 2 + CFG['op_gap'] * tt, lambda tt=tt: out_project(st['lhs'], 2, tt))
    at_pos(3, e0 + 3 + CFG['op_gap'] * (NT - 1), lambda: out_copy(2 * L, 3 * L, 2).start())

    def quad_values(s, b, j, ps):
        for a in range(4):
            values(s, 4 * b + a, j, ps[a])

    pending = []
    for s in range(NSEG):
        for b in range(NQUAD):
            for fn in slots.pop((s, b, -1), ()):
                fn()
            for j in range(NT):
                pending.append((s, b, j, scores(s, b, j)))
                for fn in slots.pop((s, b, j), ()):
                    fn()
                if len(pending) > CFG['lag']:
                    quad_values(*pending.pop(0))
    tail = [unit for unit in pending]
    assert not slots, slots.keys()
    s = NSEG - 1

    def last_tile(tt):
        out_project(st['lhs'], s, tt)
        out_copy(s * L + tt * T, s * L + (tt + 1) * T, 3 + tt).start()

    done = 0
    for unit in tail:
        quad_values(*unit)
        while done < NT and unit[1] == NQUAD - 1 and done < unit[2]:
            last_tile(done)
            done += 1
    while done < NT:
        last_tile(done)
        done += 1
    with _scope('out_wait'):
        for k in range(NSEG - 1):
            out_copy(k * L, (k + 1) * L, k).wait()
        for tt in range(NT):
            out_copy(s * L + tt * T, s * L + (tt + 1) * T, 3 + tt).wait()


@jax.jit
def pallas_parallel_sum__memory_aug_infini_attn__moe_arch_mod__prompt_kernel(
    A_x: jax.Array,
    A_wq: jax.Array,
    A_wk: jax.Array,
    A_wv: jax.Array,
    A_wo: jax.Array,
    A_beta: jax.Array,
    B_x: jax.Array,
    B_w_r: jax.Array,
    B_w_gate: jax.Array,
    B_w_up: jax.Array,
    B_w_down: jax.Array,
):
    del B_x
    x_t = jnp.transpose(A_x, (0, 2, 1)).reshape(D, S)
    wd_t = B_w_down.T
    hbm = pl.BlockSpec(memory_space=pl.ANY)
    out_t = pl.pallas_call(
        _kernel,
        out_shape=jax.ShapeDtypeStruct((D, S), bf16),
        in_specs=[hbm] * 10,
        out_specs=hbm,
        scratch_shapes=[
            pltpu.VMEM((D, S), bf16),
            pltpu.VMEM((D, S), f32),
            pltpu.VMEM((4, D, D), bf16),
            pltpu.VMEM((3 * D // 2, D), u32),
            pltpu.VMEM((D // 2, 5 * T), u32),
            pltpu.VMEM((D, F), bf16),
            pltpu.VMEM((D, F), bf16),
            pltpu.VMEM((D, F), bf16),
            pltpu.VMEM((H,), bf16),
            pltpu.VMEM((D,), bf16),
            pltpu.VMEM((2, D // 2, L), u32),
            pltpu.VMEM((2, D, L), f32),
            pltpu.VMEM((2, NQUAD, L // 2, T), u32),
            pltpu.VMEM((2, NGRP, MROWS, L), f32),
            pltpu.VMEM((NGRP, MROWS, T), f32),
            pltpu.VMEM((NGRP, 8, T), f32),
            pltpu.VMEM((NSEG, 5 * T, L), f32),
            pltpu.VMEM((2 + H * S // T, 8, T), u32),
            pltpu.VMEM((2 + H * S // T, 8, T), u32),
            pltpu.VMEM((H, S), f32),
            pltpu.VMEM((NQUAD, 16, 8, T), u32),
            pltpu.VMEM((S // T, T), f32),
            pltpu.VMEM((D, S), bf16),
            pltpu.VMEM((H, T), f32),
            pltpu.VMEM((D, S), bf16),
            pltpu.VMEM((D, S), bf16),
            pltpu.SemaphoreType.DMA((20,)),
        ],
        compiler_params=pltpu.CompilerParams(vmem_limit_bytes=100 * 1024 * 1024),
        name="infini_moe",
    )(x_t, A_wq, A_wk, A_wv, A_wo, A_beta, B_w_r, B_w_gate, B_w_up, wd_t)
    return jnp.transpose(out_t.reshape(1, D, S), (0, 2, 1))
```

```python
import contextlib
import functools

import jax
import jax.numpy as jnp
from jax import lax
from jax.experimental import pallas as pl
from jax.experimental.pallas import tpu as pltpu

S, D, H, DH = 2048, 576, 32, 18
NSEG, L, F = 4, 512, 4608
T = 128
NT = L // T
NGRP = 5
SLAB = 112
GROUP_FIRST = (0, 7, 13, 19, 25, 32)
MROWS = 144
NCHUNK = F // T
NQUAD = H // 4
QUAD_OFF = (0, 64, 144, 208, 288, 352, 432, 448)
EARLY = 2
KSPLIT = 256
SUB = 32

bf16, f32, u32, i32 = jnp.bfloat16, jnp.float32, jnp.uint32, jnp.int32

LOG2E = 1.4426950408889634
QSCALE = (DH ** -0.5) * LOG2E
LN_NORM2 = 2.1 * D
LOGIT_LIMIT = 50.0
NEG_BIG = -1e30


PROFILE_SCOPES = False
CFG = dict(
    lag=5,
    tie_p=3,
    tie_res=3,
    tie_ln=1,
    fill_proj=10,
    fill_qk=8,
    select_pos=7,
    moe_quad=5,
    moe_end=8,
    op_gap=3,
    read_off=4,
)


def _scope(name):
    return jax.named_scope(name) if PROFILE_SCOPES else contextlib.nullcontext()


def _group_of(h):
    for g in range(NGRP):
        if GROUP_FIRST[g] <= h < GROUP_FIRST[g + 1]:
            return g
    raise ValueError(h)


def _to_bf16(x):
    return pltpu.bitcast(x, bf16)


def _to_u32(x):
    return pltpu.bitcast(x, u32)


def _round_bf16(x):
    return x.astype(bf16).astype(f32)


def _iota(shape, dim):
    return lax.broadcasted_iota(i32, shape, dim)


def _dot(a, b):
    return jnp.dot(a, b, preferred_element_type=f32)


def _dot_nt(a, b):
    return lax.dot_general(a, b, (((1,), (1,)), ((), ())), preferred_element_type=f32)


def _dot_tn(a, b):
    return lax.dot_general(a, b, (((0,), (0,)), ((), ())), preferred_element_type=f32)


def _pack_pairs(x):
    lo = jnp.concatenate([x[r:r + 8] for r in range(0, x.shape[0], 16)], axis=0)
    hi = jnp.concatenate([x[r + 8:r + 16] for r in range(0, x.shape[0], 16)], axis=0)
    return pltpu.pack_elementwise([lo, hi], packed_dtype=bf16)


def _unpaired_index(r):
    x = r & 15
    return (r - x) + jnp.where(x < 8, 2 * x, 2 * (x - 8) + 1)


def _zero_bits_after(u):
    sixteen = jnp.full(u.shape, 16, u32)
    return lax.shift_right_logical(lax.shift_right_logical(u, sixteen), sixteen)


def _pair_mask(first, lo, hi, keep_lane=None):
    f = _iota((8, T), 0) + first
    low = (f >= lo) & (f < hi)
    high = (f + 8 >= lo) & (f + 8 < hi)
    if keep_lane is not None:
        low, high = low & keep_lane, high & keep_lane
    return jnp.where(low, jnp.uint32(0xFFFF), jnp.uint32(0)) | jnp.where(high, jnp.uint32(0xFFFF0000), jnp.uint32(0))


def _bf16_bits(x):
    return pltpu.bitcast(_round_bf16(x), u32)


def _shift_words(m, low_half):
    first = _round_bf16(-m)
    second = _round_bf16(-m - first)
    third = -m - first - second
    row = _iota((8, T), 0)
    val = jnp.where(row == 5, first, jnp.where(row == 6, second, jnp.where(row == 7, third, 0.0)))
    bits = _bf16_bits(val)
    return lax.shift_right_logical(bits, jnp.full(bits.shape, 16, u32)) if low_half else bits


def _phi(t):
    return jnp.where(t > 0, t + 1.0, jnp.exp(t))


def _sigmoid(t):
    return 1.0 / (1.0 + jnp.exp(-t))


def _layernorm_stats(xb):
    x0 = xb[0:1, :].astype(f32)
    acc1, acc2 = [None] * 4, [None] * 4
    for n, r in enumerate(range(0, D, 16)):
        c = xb[r:r + 16, :].astype(f32) - x0
        for part in range(2):
            k = (2 * n + part) % 4
            piece = c[8 * part:8 * part + 8, :]
            acc1[k] = piece if acc1[k] is None else acc1[k] + piece
            acc2[k] = piece * piece if acc2[k] is None else acc2[k] + piece * piece
    s1 = jnp.sum((acc1[0] + acc1[1]) + (acc1[2] + acc1[3]), axis=0, keepdims=True) / D
    s2 = jnp.sum((acc2[0] + acc2[1]) + (acc2[2] + acc2[3]), axis=0, keepdims=True) / D
    var = jnp.maximum(s2 - s1 * s1, 0.0)
    eps = _round_bf16(jnp.full((1, 1), 1e-5, f32))
    sd = _round_bf16(jnp.sqrt(_round_bf16(_round_bf16(var) + eps)))
    return _round_bf16(x0 + s1), 1.0 / sd


def _layernorm_apply(xb, stats):
    mean, inv = stats
    return _round_bf16(xb.astype(f32) - mean) * inv


def _block_transpose(xs):
    lane = _iota(next(x for x in xs if x is not None).shape, 1)

    def exchange(u, v, low, shift):
        def pick(p, q):
            if p is None and q is None:
                return None
            return jnp.where(low, 0.0 if p is None else p, 0.0 if q is None else q)
        ru = None if u is None else pltpu.roll(u, T - shift, 1)
        rv = None if v is None else pltpu.roll(v, shift, 1)
        return pick(u, rv), pick(ru, v)

    y0, y2 = exchange(xs[0], xs[2], lane < 64, 64)
    y1, y3 = exchange(xs[1], xs[3], lane < 64, 64)
    low = (lane & 32) == 0
    z0, z1 = exchange(y0, y1, low, 32)
    z2, z3 = exchange(y2, y3, low, 32)
    return [z0, z1, z2, z3]


def _head_of_slab_index(idx, g):
    return ((idx + SLAB * g) * 3641) >> 16


def _zero_after(x):
    sign = lax.shift_right_logical(pltpu.bitcast(x, i32), 31)
    return sign.astype(f32) * 0.0


def _kernel(x_hbm, wq_hbm, wk_hbm, wv_hbm, wo_hbm, beta_hbm, wr_hbm, wg_hbm, wu_hbm, wd_hbm,
            out_hbm,
            xt, xn, wstage, wt, wot, wg, wu, wd, beta_ref, wr_ref, qt, vt, kp, num, mt, zt, ot,
            mx, mxp, mrow, qmask, rrow, outb, gb, kall, qall, sems):
    def copy(src, dst, i):
        return pltpu.make_async_copy(src, dst, sems.at[i])

    xa_copy = copy(x_hbm.at[:, 0:T], xt.at[:, 0:T], 0)
    xb_copy = copy(x_hbm.at[:, T:L], xt.at[:, T:L], 18)
    xr_copy = copy(x_hbm.at[:, L:S], xt.at[:, L:S], 1)
    wq_copy, wv_copy, wo_copy = [
        copy(w, wstage.at[i], 2 + i) for i, w in ((1, wq_hbm), (2, wv_hbm), (3, wo_hbm))]
    wka_copy = copy(wk_hbm.at[:, 0:KSPLIT], wstage.at[0, :, 0:KSPLIT], 2)
    wkb_copy = copy(wk_hbm.at[:, KSPLIT:D], wstage.at[0, :, KSPLIT:D], 19)
    beta_copy = copy(beta_hbm, beta_ref, 6)
    wr_copy = copy(wr_hbm, wr_ref, 7)
    moe_copies = [copy(wg_hbm, wg, 8), copy(wu_hbm, wu, 9), copy(wd_hbm, wd, 10)]

    def out_copy(lo, hi, i):
        return copy(outb.at[:, lo:hi], out_hbm.at[:, lo:hi], 11 + i)

    half = D // 2
    emitted = set()

    def produced(*key):
        emitted.add(key)

    def require(*key):
        assert key in emitted, key

    def require_heads(s, j):
        for h in range(H):
            require('ot', s, h, j)

    fillers = []

    def fill(n):
        for _ in range(min(n, len(fillers))):
            fillers.pop(0)()

    clock = [0]
    ties = []

    def tile_cols(s, tt):
        return slice(s * L + tt * T, s * L + (tt + 1) * T)

    def local_cols(tt):
        return slice(tt * T, (tt + 1) * T)

    def col_sq_part(i, lo, hi):
        acc = None
        for r in range(lo, hi, 16):
            w = wstage[i, r:r + 16, :].astype(f32)
            w = w * w
            part = w[0:8] + w[8:16]
            acc = part if acc is None else acc + part
        return acc

    def col_sq_max(parts):
        acc = functools.reduce(lambda u, v: u + v, parts)
        return jnp.max(jnp.sum(acc, axis=0, keepdims=True), axis=1, keepdims=True)

    def tie_of(part):
        folded = functools.reduce(lambda u, v: u + v, [part[:, c:c + T] for c in range(0, 4 * T, T)])
        return _zero_after(folded[0:1, 0:1] + part[0:1, 4 * T:4 * T + 1])

    def transpose_weight(i):
        return _to_u32(wstage[i].T)

    def ln_stats(s, tt):
        return _layernorm_stats(xt[:, tile_cols(s, tt)])

    def normalize(s, tt, stats):
        cs = tile_cols(s, tt)
        xn[:, cs] = _layernorm_apply(xt[:, cs], stats)
        produced('xn', s, tt)

    def xn_tile(s, tt):
        require('xn', s, tt)
        return xn[:, tile_cols(s, tt)].astype(bf16)

    def keys_raw(s, tt, lo=0, hi=D):
        kt = _dot(_to_bf16(wt[lo // 2:hi // 2, :]), xn_tile(s, tt))
        fill(CFG['fill_proj'])
        return kt

    def keys_finish(s, tt, kt, tie=None):
        if tie is not None:
            kt = kt + tie
        words = jnp.take_along_axis(_pack_pairs(kt), _unpaired_index(_iota((half, T), 1)), axis=1)
        shift_rows = _iota((8, T), 0) >= 5
        for b in range(NQUAD):
            slab = words[QUAD_OFF[b] // 2:QUAD_OFF[b] // 2 + T // 2, :]
            if b == NQUAD - 1:
                ones = jnp.where(shift_rows, (slab[0:8] & jnp.uint32(0xFFFF0000)) | jnp.uint32(0x3F80), slab[0:8])
                slab = jnp.concatenate([ones, slab[8:]], axis=0)
            else:
                ones = jnp.where(shift_rows, (slab[56:64] & jnp.uint32(0xFFFF)) | jnp.uint32(0x3F800000), slab[56:64])
                slab = jnp.concatenate([slab[:56], ones], axis=0)
            kp[s % 2, b, tt * (T // 2):(tt + 1) * (T // 2), :] = _to_u32(_to_bf16(slab).T)
        produced('k', s, tt)
        return _phi(kt).astype(bf16)

    def project_k(s, tt):
        return keys_finish(s, tt, keys_raw(s, tt))

    def project_q(s, tt, tie=None):
        q = _dot(_to_bf16(wt[half:2 * half, :]), xn_tile(s, tt))
        fill(CFG['fill_proj'])
        qt[s % 2, :, local_cols(tt)] = _pack_pairs(q * (QSCALE if tie is None else QSCALE + tie))
        produced('q', s, tt)
        return _phi(q).astype(bf16)

    def require_segment_done(s):
        if s >= 0:
            for j in range(NT):
                require_heads(s, j)

    def project_v(s, tt):
        require_segment_done(s - 2)
        v = _dot(_to_bf16(wt[2 * half:3 * half, :]), xn_tile(s, tt))
        fill(CFG['fill_proj'])
        vt[s % 2, :, local_cols(tt)] = v
        produced('v', s, tt)

    def router_scores(lhs, s, tt):
        row = s * NT + tt
        rrow[row:row + 1, :] = _dot(lhs, xn_tile(s, tt))[0:1, :]
        produced('r', s, tt)

    def memory_read(s, tt, pq):
        require_segment_done(s - 2)
        for g in range(NGRP):
            require('mt', s - 1, g)
        for g in range(NGRP):
            num[s % 2, g, :, local_cols(tt)] = _dot(mt[g].astype(bf16), pq[SLAB * g:SLAB * g + T, :])
        produced('num', s, tt)

    def memory_update(s, g, pk):
        ones_row = 0 if g == NGRP - 1 else T - 1
        vs = jnp.where(_iota((T, L), 0) == ones_row, 1.0, vt[s % 2, SLAB * g:SLAB * g + T, :]).astype(bf16)
        m = _dot_nt(vs, jnp.concatenate([p[SLAB * g:SLAB * g + T, :] for p in pk], axis=1))
        hr = _head_of_slab_index(_iota((T, T), 0), g)
        hc = _head_of_slab_index(_iota((T, T), 1), g)
        keep = (hr == hc) & (hr >= GROUP_FIRST[g]) & (hr < GROUP_FIRST[g + 1])
        mm = jnp.where(keep, m, 0.0)
        z = m[ones_row:ones_row + 1, :]
        if s > 0:
            mm = mm + mt[g, 0:T, :]
            z = z + zt[g, 0:1, :]
        mt[g, 0:T, :] = mm
        zt[g, 0:1, :] = z
        zsel = _head_of_slab_index(_iota((16, T), 1), g) == _iota((16, T), 0) + GROUP_FIRST[g]
        mt[g, T:MROWS, :] = jnp.where(zsel, z, 0.0)
        produced('mt', s, g)

    def head_groups(b, a):
        f = DH * (4 * b + a) - QUAD_OFF[b]
        return f, (f // 16, f // 16 + 1)

    def build_query_masks():
        block = _iota((8, T), 1) // SUB
        for b in range(NQUAD):
            for a in range(4):
                f, groups = head_groups(b, a)
                for n, g in enumerate(groups):
                    qmask[b, 4 * a + 2 * n] = _pair_mask(16 * g, f, f + DH)
                    qmask[b, 4 * a + 2 * n + 1] = _pair_mask(16 * g, f, f + DH, block == a)

    def stack_groups(groups):
        return _to_bf16(jnp.concatenate(
            [groups.get(g, jnp.zeros((8, T), u32)) for g in range(T // 16)], axis=0))

    def quad_queries(s, b, j, tie):
        tile = s * NT + j
        last = b == NQUAD - 1
        shift_group = 0 if last else T // 16 - 1
        base = QUAD_OFF[b] // 2
        words = {}

        def group(g):
            if g not in words:
                words[g] = qt[s % 2, base + 8 * g:base + 8 * g + 8, local_cols(j)]
            return words[g]

        wide = []
        for a in range(4):
            _, groups = head_groups(b, a)
            parts = {g: group(g) & qmask[b, 4 * a + 2 * n] for n, g in enumerate(groups)}
            if j > 0:
                parts[shift_group] = mx[int(last) + shift_sel * (2 - int(last) + (4 * b + a) * (S // T) + tile)]
                wide.append(stack_groups(parts))
        packed = []
        for i in range(4):
            parts = {}
            for a in range(4):
                _, groups = head_groups(b, a)
                shift = (SUB * (a - i)) % T
                for n, g in enumerate(groups):
                    moved = group(g) if shift == 0 else pltpu.roll(group(g), shift, 1)
                    piece = moved & qmask[b, 4 * a + 2 * n + 1]
                    parts[g] = piece if g not in parts else parts[g] | piece
            rows = mxp[int(last) + shift_sel * (2 - int(last) + tile * H + 4 * b + i)]
            if tie is not None and i == 3:
                rows = rows | tie
            parts[shift_group] = rows
            packed.append(stack_groups(parts))
        return wide, packed

    def scores(s, b, j):
        require('q', s, j)
        for tt in range(j + 1):
            require('k', s, tt)
        tie = None
        unit = clock[0] = (s * NQUAD + b) * NT + j
        due = [z for when, z in ties if when <= unit]
        ties[:] = [(when, z) for when, z in ties if when > unit]
        if due:
            tie = functools.reduce(lambda u, v: u | v, due)
        wide, packed = quad_queries(s, b, j, tie)
        k0 = j * (T // 2)
        off = None
        if j > 0:
            logits = _dot(_to_bf16(kp[s % 2, b, 0:k0, :]), jnp.concatenate(wide, axis=1))
            fill(CFG['fill_qk'])
            off = jnp.exp2(logits)
        causal = _unpaired_index(_iota((SUB, T), 0)) <= (_iota((SUB, T), 1) & (SUB - 1))
        diag = [None] * 4
        for i in range(4):
            n = SUB * (i + 1)
            e = jnp.exp2(_dot(_to_bf16(kp[s % 2, b, k0:k0 + n // 2, :]), packed[i]))
            blocks = [e[r * SUB:(r + 1) * SUB, :] for r in range(i)]
            blocks.append(jnp.where(causal, e[i * SUB:, :], 0.0))
            diag[i] = blocks
        per_head = [[] for _ in range(4)]
        for r in range(4):
            outs = _block_transpose([diag[i][r] if i >= r else None for i in range(4)])
            for a in range(4):
                per_head[a].append(outs[a])
        ps = []
        for a in range(4):
            parts = ([off[:, a * T:(a + 1) * T]] if j > 0 else []) + per_head[a]
            ps.append(_pack_pairs(jnp.concatenate(parts, axis=0)))
        rows = [u[r:r + 8] for u in ps for r in range(0, u.shape[0], 8)]
        while len(rows) > 1:
            rows = [rows[i] | rows[i + 1] for i in range(0, len(rows) - 1, 2)] + rows[len(rows) & ~1:]
        ties.append((unit + CFG['tie_p'], _zero_bits_after(rows[0])))
        return [_to_bf16(u) for u in ps]

    def values(s, h, j, p):
        g = _group_of(h)
        w0 = min((DH * h // 16) * 16, D - 32)
        off = DH * h - w0
        ones_row = 31 if off < 14 else 0
        n = (j + 1) * T
        cs = local_cols(j)
        for tt in range(j + 1):
            require('v', s, tt)
        if s > 0:
            require('num', s, j)
        g0 = (ones_row // 8) * 8
        marked = jnp.where(_iota((8, n), 0) == ones_row - g0, 1.0, vt[s % 2, w0 + g0:w0 + g0 + 8, 0:n])
        rest = vt[s % 2, w0 + 8:w0 + 32, 0:n] if g0 == 0 else vt[s % 2, w0:w0 + 24, 0:n]
        vwin = jnp.concatenate([marked, rest] if g0 == 0 else [rest, marked], axis=0).astype(bf16)
        gate = gb[h:h + 1, :]
        acc = _dot(vwin, p)
        res = acc * ((1.0 - gate) / acc[ones_row:ones_row + 1, :])
        if s > 0:
            m0 = w0 - SLAB * g
            zr = T + h - GROUP_FIRST[g]
            den = num[s % 2, g, zr:zr + 1, cs] + 1e-6
            res = res + num[s % 2, g, m0:m0 + 32, cs] * (gate / den)
        else:
            folded = (res[0:8] + res[8:16]) + (res[16:24] + res[24:32])
            ties.append((clock[0] + CFG['tie_res'], _zero_bits_after(_to_u32(folded))))
        ot[s, DH * h:DH * h + DH, cs] = res[off:off + DH, :]
        produced('ot', s, h, j)

    def route():
        for s in range(NSEG):
            for tt in range(NT):
                require('r', s, tt)
        r = _round_bf16(rrow[...])
        idx = _iota((S // T, T), 0) * T + _iota((S // T, T), 1)
        m1 = jnp.max(r)
        i1 = jnp.min(jnp.where(r == m1, idx, S - 1))
        r2 = jnp.where(idx == i1, -jnp.inf, r)
        m2 = jnp.max(r2)
        i2 = jnp.min(jnp.where(r2 == m2, idx, S - 1))
        return (i1, i2), (m1, m2)

    def select_tokens(ids):
        sel = None
        for row, i in enumerate(ids):
            hit = (_iota((16, T), 0) == row) & (_iota((16, T), 1) == i % T)
            cs = pl.ds(pl.multiple_of((i // T) * T, T), T)
            part = _dot_nt(jnp.where(hit, 1.0, 0.0).astype(bf16), xn[:, cs].astype(bf16))
            sel = part if sel is None else sel + part
        return sel.astype(bf16)

    def queue_moe(xsel, state):
        ktiles = [(k, min(k + T, D)) for k in range(0, D, T)]
        pre, hid = {}, {}
        ycols = state['ycols'] = [None] * len(ktiles)

        def first(w, name, c, lo, hi):
            def fn():
                part = _dot(xsel[:, lo:hi], w[lo:hi, c * T:(c + 1) * T])
                pre[name, c] = part if lo == 0 else pre[name, c] + part
            return fn

        def down(c, n, lo, hi):
            def fn():
                if c not in hid:
                    gpre = _round_bf16(pre.pop(('g', c)))
                    gact = _round_bf16(gpre * _sigmoid(gpre))
                    hid[c] = (gact * _round_bf16(pre.pop(('u', c)))).astype(bf16)
                part = _dot_nt(hid[c], wd[lo:hi, c * T:(c + 1) * T])
                ycols[n] = part if ycols[n] is None else ycols[n] + part
            return fn

        for c in range(NCHUNK + 2):
            if c < NCHUNK:
                for lo, hi in ktiles:
                    fillers.append(first(wg, 'g', c, lo, hi))
                    fillers.append(first(wu, 'u', c, lo, hi))
            if c >= 2:
                for n, (lo, hi) in enumerate(ktiles):
                    fillers.append(down(c - 2, n, lo, hi))

    def moe_result(sel_scores, y):
        row = _iota((16, D), 0)
        gate = jnp.where(row == 0, sel_scores[0], sel_scores[1])
        return (_round_bf16(y) * _round_bf16(_sigmoid(gate))).astype(bf16)

    def patch_early(ids, y):
        for k, i in enumerate(ids):
            hit = (_iota((16, T), 0) == k) & (_iota((16, T), 1) == i % T) & (i < EARLY * L)
            cs = pl.ds(pl.multiple_of((jnp.minimum(i, EARLY * L - 1) // T) * T, T), T)
            patch = _dot_tn(y, jnp.where(hit, 1.0, 0.0).astype(bf16))
            outb[:, cs] = (outb[:, cs].astype(f32) + patch).astype(bf16)

    def out_lhs(ids, y):
        place = (_iota((16, T), 1) == _iota((16, T), 0) + 64) & (_iota((16, T), 0) < 2)
        ycols = _dot_tn(y, jnp.where(place, 1.0, 0.0).astype(bf16))
        last = _to_bf16(wot[:, 4 * T:5 * T]).astype(f32) + ycols
        for s in range(EARLY, NSEG):
            tok = _iota((64, L), 1) + s * L
            rows = _iota((64, L), 0)
            hit = ((rows == 0) & (tok == ids[0])) | ((rows == 1) & (tok == ids[1]))
            ot[s, D:D + 64, :] = jnp.where(hit, 1.0, 0.0)
        return jnp.concatenate([_to_bf16(wot[:, 0:4 * T]), last.astype(bf16)], axis=1)

    def out_project_early(s, tt):
        require_heads(s, tt)
        require('wot')
        cs = tile_cols(s, tt)
        attn = _dot(_to_bf16(wot[:, 0:D]), ot[s, 0:D, local_cols(tt)].astype(bf16))
        fill(CFG['fill_proj'])
        outb[:, cs] = (attn + xn[:, cs] + xt[:, cs].astype(f32)).astype(bf16)

    def out_project(lhs, s, tt):
        require_heads(s, tt)
        cs = tile_cols(s, tt)
        attn = _dot(lhs, ot[s, :, local_cols(tt)].astype(bf16))
        outb[:, cs] = (attn + xn[:, cs] + xt[:, cs].astype(f32)).astype(bf16)

    def row_maxima():
        def project_tile(tt, carry):
            cs = pl.ds(pl.multiple_of(tt * T, T), T)
            y = _layernorm_apply(xt[:, cs], _layernorm_stats(xt[:, cs])).astype(bf16)
            kall[:, cs] = _dot(_to_bf16(wt[0:half, :]), y).astype(bf16)
            qall[:, cs] = (_dot(_to_bf16(wt[half:2 * half, :]), y) * QSCALE).astype(bf16)
            return carry

        lax.fori_loop(0, S // T, project_tile, 0)

        def head_tile(i, carry):
            h = i // (S // T)
            tt = i % (S // T)
            cs = pl.ds(pl.multiple_of(tt * T, T), T)
            seg = pl.ds(pl.multiple_of((tt // NT) * L, L), L)
            rows = _iota((D, T), 0)
            qm = jnp.where((rows >= DH * h) & (rows < DH * h + DH), qall[:, cs].astype(f32), 0.0)
            logits = _dot_tn(kall[:, seg], qm.astype(bf16))
            seen = _iota((L, T), 0) <= _iota((L, T), 1) + (tt % NT) * T
            m = jnp.max(jnp.where(seen, logits, NEG_BIG), axis=0, keepdims=True)
            mrow[:, cs] = jnp.where(_iota((H, T), 0) == h, m, mrow[:, cs])
            wide_m = jnp.broadcast_to(m, (8, T))
            mx[2 + i] = jnp.where(h >= H - 4, _shift_words(wide_m, True), _shift_words(wide_m, False))
            return carry

        mrow[...] = jnp.zeros(mrow.shape, f32)
        lax.fori_loop(0, H * (S // T), head_tile, 0)

        def pack_tile(tt, carry):
            cs = pl.ds(pl.multiple_of(tt * T, T), T)
            m = mrow[:, cs]
            block = _iota((1, T), 1) // SUB
            for b in range(NQUAD):
                for i in range(4):
                    row = jnp.zeros((1, T), f32)
                    for a in range(4):
                        src = m[4 * b + a:4 * b + a + 1, :]
                        shift = (SUB * (a - i)) % T
                        row = jnp.where(block == a, src if shift == 0 else pltpu.roll(src, shift, 1), row)
                    mxp[2 + tt * H + 4 * b + i] = _shift_words(jnp.broadcast_to(row, (8, T)), b == NQUAD - 1)
            return carry

        lax.fori_loop(0, S // T, pack_tile, 0)

    for c in (xa_copy, wka_copy, xb_copy, wkb_copy, wq_copy, wv_copy):
        c.start()
    wot[:, 4 * T:5 * T] = jnp.zeros((half, T), u32)
    pk, pq = {}, {}
    sq = [[], []]

    def sq_tie(i, n, parts):
        rows = -(-D // (16 * parts)) * 16
        part = col_sq_part(i, n * rows, min(D, (n + 1) * rows))
        sq[i].append(part)
        return tie_of(part)

    build_query_masks()
    with _scope('p0_wait'):
        xa_copy.wait()
    with _scope('p0'):
        normalize(0, 0, ln_stats(0, 0))
    with _scope('p1_wait'):
        wka_copy.wait()
    with _scope('p1'):
        wt[0:KSPLIT // 2, :] = _to_u32(wstage[0, :, 0:KSPLIT].T)
        ka = [keys_raw(0, 0, 0, KSPLIT)]
    with _scope('p1b_wait'):
        xb_copy.wait()
    with _scope('p1b'):
        for tt in range(1, NT):
            normalize(0, tt, ln_stats(0, tt))
            if tt < NT - 1:
                ka.append(keys_raw(0, tt, 0, KSPLIT))
    with _scope('p1c_wait'):
        wkb_copy.wait()
    with _scope('p1c'):
        ka.append(keys_raw(0, NT - 1, 0, KSPLIT))
        wt[KSPLIT // 2:half, :] = _to_u32(wstage[0, :, KSPLIT:D].T)
        kb = []
        for tt in range(NT - 1):
            kb.append(keys_raw(0, tt, KSPLIT, D))
            if tt > 0:
                pk[0, tt - 1] = keys_finish(0, tt - 1, jnp.concatenate([ka[tt - 1], kb[tt - 1]], axis=0),
                                            sq_tie(0, tt - 1, 2))
    with _scope('p2_wait'):
        wq_copy.wait()
    for c in (xr_copy, beta_copy, wr_copy, wo_copy):
        c.start()
    with _scope('p2'):
        k2 = jnp.concatenate([ka[2], kb[2]], axis=0)
        k3 = jnp.concatenate([ka[3], keys_raw(0, 3, KSPLIT, D)], axis=0)
        wt[half:2 * half, :] = transpose_weight(1)
        pk[0, 2] = keys_finish(0, 2, k2)
        project_q(0, 0, sq_tie(1, 0, 3))
        pk[0, 3] = keys_finish(0, 3, k3)
        for tt in range(1, NT - 1):
            project_q(0, tt, sq_tie(1, tt, 3))
    with _scope('p3_wait'):
        wv_copy.wait()
    with _scope('p3'):
        wt[2 * half:3 * half, :] = transpose_weight(2)
        project_q(0, NT - 1)
        for tt in range(NT - 1):
            project_v(0, tt)
        csq = [col_sq_max(parts) for parts in sq]
        bound = (QSCALE * LN_NORM2 * DH) * jnp.sqrt(csq[0] * csq[1])
        for low in range(2):
            words = _shift_words(jnp.broadcast_to(bound, (8, T)), low == 1)
            mx[low] = words
            mxp[low] = words
        shift_sel = jnp.max(jnp.where(bound <= LOGIT_LIMIT, 0, 1))
        unsafe = shift_sel > 0
    for c in moe_copies:
        c.start()
    with _scope('p4_wait'):
        for c in (xr_copy, beta_copy, wr_copy, wo_copy):
            c.wait()

    @pl.when(unsafe)
    def _():
        row_maxima()

    project_v(0, NT - 1)
    gb[...] = _sigmoid(jnp.broadcast_to(beta_ref[...].astype(f32).reshape(1, H), (T, H)).T)

    slots = {}
    st = {}

    def at(s, b, j, fn):
        slots.setdefault((s, b, j), []).append(fn)

    def at_pos(s, pos, fn):
        at(s, pos // NT, pos % NT, fn)

    def wr_lhs():
        if 'wr' not in st:
            w = jnp.broadcast_to(wr_ref[...].astype(f32).reshape(1, D), (16, D))
            st['wr'] = jnp.where(_iota((16, D), 0) == 0, w, 0.0).astype(bf16)
        return st['wr']

    stats = {}

    def stats_task(s, tt):
        def fn():
            stats[s, tt] = ln_stats(s, tt)
            inv = jnp.broadcast_to(stats[s, tt][1], (8, T))
            ties.append((clock[0] + CFG['tie_ln'], _zero_bits_after(_to_u32(inv))))
        return fn

    def norm_task(s, tt):
        return lambda: normalize(s, tt, stats[s, tt])

    def score_task(s, tt):
        return lambda: router_scores(wr_lhs(), s, tt)

    for s in range(NSEG - 1):
        for g in range(NGRP):
            at_pos(s, 2 * g, lambda s=s, g=g: memory_update(s, g, [pk[s, tt] for tt in range(NT)]))
        if s == 0:
            at_pos(0, 3, stats_task(1, 0))
            at_pos(0, 5, norm_task(1, 0))
        for tt in range(NT):
            p0 = 9 + 6 * tt
            if s == 0:
                at_pos(s, p0, stats_task(2, tt))
                if tt > 0:
                    at_pos(s, p0, norm_task(3, tt - 1))
            at_pos(s, p0, lambda s=s, tt=tt: pk.__setitem__((s + 1, tt), project_k(s + 1, tt)))
            if s == 0:
                if tt > 0:
                    at_pos(s, p0, score_task(3, tt - 1))
                at_pos(s, p0 + 2, norm_task(2, tt))
                if tt + 1 < NT:
                    at_pos(s, p0 + 2, stats_task(1, tt + 1))
            at_pos(s, p0 + 2, lambda s=s, tt=tt: pq.__setitem__((s + 1, tt), project_q(s + 1, tt)))
            if s == 0:
                at_pos(s, p0 + 2, score_task(2, tt))
                if tt + 1 < NT:
                    at_pos(s, p0 + 4, norm_task(1, tt + 1))
                at_pos(s, p0 + 4, stats_task(3, tt))
            at_pos(s, p0 + 4, lambda s=s, tt=tt: project_v(s + 1, tt))
            at_pos(s, p0 + CFG['read_off'], lambda s=s, tt=tt: memory_read(s + 1, tt, pq[s + 1, tt]))
    at_pos(1, 0, norm_task(3, NT - 1))
    for s in range(EARLY):
        for tt in range(NT):
            at_pos(s + 1, 3 + 2 * tt if s > 0 else 8 + 6 * tt, lambda s=s, tt=tt: out_project_early(s, tt))
    at_pos(1, 1, score_task(3, NT - 1))
    for tt in range(NT):
        at_pos(0, 1 + 2 * tt, score_task(0, tt))
        at_pos(0, 10 + 6 * tt, score_task(1, tt))

    def set_out_weight():
        wot[:, 0:D] = transpose_weight(3)
        produced('wot')

    at_pos(0, 22, set_out_weight)

    at_pos(1, 2, lambda: st.update(zip(('ids', 'sel'), route())))
    at_pos(1, CFG['select_pos'], lambda: st.update(xsel=select_tokens(st['ids'])))

    def start_moe():
        with _scope('moe_wait'):
            for c in moe_copies:
                c.wait()
        queue_moe(st['xsel'], st)

    at(1, CFG['moe_quad'], -1, start_moe)

    def finish_moe():
        fill(len(fillers))
        y = moe_result(st['sel'], jnp.concatenate(st['ycols'], axis=1))
        patch_early(st['ids'], y)
        st['lhs'] = out_lhs(st['ids'], y)

    e0 = CFG['moe_end']
    at_pos(3, e0, finish_moe)
    for s in range(EARLY):
        at_pos(3, e0 + 1 + s, lambda s=s: out_copy(s * L, (s + 1) * L, s).start())
    for tt in range(NT):
        at_pos(3, e0 + 2 + CFG['op_gap'] * tt, lambda tt=tt: out_project(st['lhs'], 2, tt))
    at_pos(3, e0 + 3 + CFG['op_gap'] * (NT - 1), lambda: out_copy(2 * L, 3 * L, 2).start())

    def quad_values(s, b, j, ps):
        for a in range(4):
            values(s, 4 * b + a, j, ps[a])

    pending = []
    for s in range(NSEG):
        for b in range(NQUAD):
            for fn in slots.pop((s, b, -1), ()):
                fn()
            for j in range(NT):
                pending.append((s, b, j, scores(s, b, j)))
                for fn in slots.pop((s, b, j), ()):
                    fn()
                if len(pending) > CFG['lag']:
                    quad_values(*pending.pop(0))
    assert not slots, slots.keys()
    s = NSEG - 1

    def last_tile(tt):
        out_project(st['lhs'], s, tt)
        out_copy(s * L + tt * T, s * L + (tt + 1) * T, 3 + tt).start()

    done = 0
    for unit in pending:
        quad_values(*unit)
        while done < NT and unit[1] == NQUAD - 1 and done < unit[2]:
            last_tile(done)
            done += 1
    while done < NT:
        last_tile(done)
        done += 1
    with _scope('out_wait'):
        for k in range(NSEG - 1):
            out_copy(k * L, (k + 1) * L, k).wait()
        for tt in range(NT):
            out_copy(s * L + tt * T, s * L + (tt + 1) * T, 3 + tt).wait()


@jax.jit
def pallas_parallel_sum__memory_aug_infini_attn__moe_arch_mod__prompt_kernel(
    A_x: jax.Array,
    A_wq: jax.Array,
    A_wk: jax.Array,
    A_wv: jax.Array,
    A_wo: jax.Array,
    A_beta: jax.Array,
    B_x: jax.Array,
    B_w_r: jax.Array,
    B_w_gate: jax.Array,
    B_w_up: jax.Array,
    B_w_down: jax.Array,
):
    del B_x
    x_t = jnp.transpose(A_x, (0, 2, 1)).reshape(D, S)
    wd_t = B_w_down.T
    hbm = pl.BlockSpec(memory_space=pl.ANY)
    out_t = pl.pallas_call(
        _kernel,
        out_shape=jax.ShapeDtypeStruct((D, S), bf16),
        in_specs=[hbm] * 10,
        out_specs=hbm,
        scratch_shapes=[
            pltpu.VMEM((D, S), bf16),
            pltpu.VMEM((D, S), f32),
            pltpu.VMEM((4, D, D), bf16),
            pltpu.VMEM((3 * D // 2, D), u32),
            pltpu.VMEM((D // 2, 5 * T), u32),
            pltpu.VMEM((D, F), bf16),
            pltpu.VMEM((D, F), bf16),
            pltpu.VMEM((D, F), bf16),
            pltpu.VMEM((H,), bf16),
            pltpu.VMEM((D,), bf16),
            pltpu.VMEM((2, D // 2, L), u32),
            pltpu.VMEM((2, D, L), f32),
            pltpu.VMEM((2, NQUAD, L // 2, T), u32),
            pltpu.VMEM((2, NGRP, MROWS, L), f32),
            pltpu.VMEM((NGRP, MROWS, T), f32),
            pltpu.VMEM((NGRP, 8, T), f32),
            pltpu.VMEM((NSEG, 5 * T, L), f32),
            pltpu.VMEM((2 + H * S // T, 8, T), u32),
            pltpu.VMEM((2 + H * S // T, 8, T), u32),
            pltpu.VMEM((H, S), f32),
            pltpu.VMEM((NQUAD, 16, 8, T), u32),
            pltpu.VMEM((S // T, T), f32),
            pltpu.VMEM((D, S), bf16),
            pltpu.VMEM((H, T), f32),
            pltpu.VMEM((D, S), bf16),
            pltpu.VMEM((D, S), bf16),
            pltpu.SemaphoreType.DMA((20,)),
        ],
        compiler_params=pltpu.CompilerParams(vmem_limit_bytes=100 * 1024 * 1024),
        name="infini_moe",
    )(x_t, A_wq, A_wk, A_wv, A_wo, A_beta, B_w_r, B_w_gate, B_w_up, wd_t)
    return jnp.transpose(out_t.reshape(1, D, S), (0, 2, 1))
```

```python
import contextlib
import functools

import jax
import jax.numpy as jnp
from jax import lax
from jax.experimental import pallas as pl
from jax.experimental.pallas import tpu as pltpu

S, D, H, DH = 2048, 576, 32, 18
NSEG, L, F = 4, 512, 4608
T = 128
NT = L // T
NGRP = 5
SLAB = 112
GROUP_FIRST = (0, 7, 13, 19, 25, 32)
MROWS = 144
NCHUNK = F // T
NQUAD = H // 4
QUAD_OFF = (0, 64, 144, 208, 288, 352, 432, 448)
EARLY = 2
KSPLIT = 256
SUB = 32

bf16, f32, u32, i32 = jnp.bfloat16, jnp.float32, jnp.uint32, jnp.int32

LOG2E = 1.4426950408889634
QSCALE = (DH ** -0.5) * LOG2E
LN_NORM2 = 2.1 * D
LOGIT_LIMIT = 50.0
NEG_BIG = -1e30


PROFILE_SCOPES = False
CFG = dict(
    lag=5,
    tie_p=3,
    tie_res=3,
    tie_ln=1,
    fill_proj=10,
    fill_qk=8,
    select_pos=7,
    moe_quad=5,
    moe_end=8,
    op_gap=3,
    read_off=4,
    upd_pos=(0, 2, 4, 6, 8),
    early_pos=((8, 14, 20, 26), (3, 5, 7, 9)),
    moe_delay=2,
)


def _scope(name):
    return jax.named_scope(name) if PROFILE_SCOPES else contextlib.nullcontext()


def _group_of(h):
    for g in range(NGRP):
        if GROUP_FIRST[g] <= h < GROUP_FIRST[g + 1]:
            return g
    raise ValueError(h)


def _to_bf16(x):
    return pltpu.bitcast(x, bf16)


def _to_u32(x):
    return pltpu.bitcast(x, u32)


def _round_bf16(x):
    return x.astype(bf16).astype(f32)


def _iota(shape, dim):
    return lax.broadcasted_iota(i32, shape, dim)


def _dot(a, b):
    return jnp.dot(a, b, preferred_element_type=f32)


def _dot_nt(a, b):
    return lax.dot_general(a, b, (((1,), (1,)), ((), ())), preferred_element_type=f32)


def _dot_tn(a, b):
    return lax.dot_general(a, b, (((0,), (0,)), ((), ())), preferred_element_type=f32)


def _pack_pairs(x):
    lo = jnp.concatenate([x[r:r + 8] for r in range(0, x.shape[0], 16)], axis=0)
    hi = jnp.concatenate([x[r + 8:r + 16] for r in range(0, x.shape[0], 16)], axis=0)
    return pltpu.pack_elementwise([lo, hi], packed_dtype=bf16)


def _unpaired_index(r):
    x = r & 15
    return (r - x) + jnp.where(x < 8, 2 * x, 2 * (x - 8) + 1)


def _zero_bits_after(u):
    sixteen = jnp.full(u.shape, 16, u32)
    return lax.shift_right_logical(lax.shift_right_logical(u, sixteen), sixteen)


def _pair_mask(first, lo, hi, keep_lane=None):
    f = _iota((8, T), 0) + first
    low = (f >= lo) & (f < hi)
    high = (f + 8 >= lo) & (f + 8 < hi)
    if keep_lane is not None:
        low, high = low & keep_lane, high & keep_lane
    return jnp.where(low, jnp.uint32(0xFFFF), jnp.uint32(0)) | jnp.where(high, jnp.uint32(0xFFFF0000), jnp.uint32(0))


def _bf16_bits(x):
    return pltpu.bitcast(_round_bf16(x), u32)


def _shift_words(m, low_half):
    first = _round_bf16(-m)
    second = _round_bf16(-m - first)
    third = -m - first - second
    row = _iota((8, T), 0)
    val = jnp.where(row == 5, first, jnp.where(row == 6, second, jnp.where(row == 7, third, 0.0)))
    bits = _bf16_bits(val)
    return lax.shift_right_logical(bits, jnp.full(bits.shape, 16, u32)) if low_half else bits


def _phi(t):
    return jnp.where(t > 0, t + 1.0, jnp.exp(t))


def _sigmoid(t):
    return _round_bf16(1.0 / _round_bf16(1.0 + _round_bf16(jnp.exp(-t))))


def _layernorm_stats(xb):
    x0 = xb[0:1, :].astype(f32)
    acc1, acc2 = [None] * 4, [None] * 4
    for n, r in enumerate(range(0, D, 16)):
        c = xb[r:r + 16, :].astype(f32) - x0
        for part in range(2):
            k = (2 * n + part) % 4
            piece = c[8 * part:8 * part + 8, :]
            acc1[k] = piece if acc1[k] is None else acc1[k] + piece
            acc2[k] = piece * piece if acc2[k] is None else acc2[k] + piece * piece
    s1 = jnp.sum((acc1[0] + acc1[1]) + (acc1[2] + acc1[3]), axis=0, keepdims=True) / D
    s2 = jnp.sum((acc2[0] + acc2[1]) + (acc2[2] + acc2[3]), axis=0, keepdims=True) / D
    var = jnp.maximum(s2 - s1 * s1, 0.0)
    eps = _round_bf16(jnp.full((1, 1), 1e-5, f32))
    sd = _round_bf16(jnp.sqrt(_round_bf16(_round_bf16(var) + eps)))
    return _round_bf16(x0 + s1), 1.0 / sd


def _layernorm_apply(xb, stats):
    mean, inv = stats
    return _round_bf16(xb.astype(f32) - mean) * inv


def _block_transpose(xs):
    lane = _iota(next(x for x in xs if x is not None).shape, 1)

    def exchange(u, v, low, shift):
        def pick(p, q):
            if p is None and q is None:
                return None
            return jnp.where(low, 0.0 if p is None else p, 0.0 if q is None else q)
        ru = None if u is None else pltpu.roll(u, T - shift, 1)
        rv = None if v is None else pltpu.roll(v, shift, 1)
        return pick(u, rv), pick(ru, v)

    y0, y2 = exchange(xs[0], xs[2], lane < 64, 64)
    y1, y3 = exchange(xs[1], xs[3], lane < 64, 64)
    low = (lane & 32) == 0
    z0, z1 = exchange(y0, y1, low, 32)
    z2, z3 = exchange(y2, y3, low, 32)
    return [z0, z1, z2, z3]


def _head_of_slab_index(idx, g):
    return ((idx + SLAB * g) * 3641) >> 16


def _zero_after(x):
    sign = lax.shift_right_logical(pltpu.bitcast(x, i32), 31)
    return sign.astype(f32) * 0.0


def _kernel(x_hbm, wq_hbm, wk_hbm, wv_hbm, wo_hbm, beta_hbm, wr_hbm, wg_hbm, wu_hbm, wd_hbm,
            out_hbm,
            xt, xn, wstage, wt, wot, wg, wu, wd, beta_ref, wr_ref, qt, vt, kp, num, mt, zt, ot,
            mx, mxp, mrow, qmask, rrow, outb, gb, kall, qall, sems):
    def copy(src, dst, i):
        return pltpu.make_async_copy(src, dst, sems.at[i])

    xa_copy = copy(x_hbm.at[:, 0:T], xt.at[:, 0:T], 0)
    xb_copy = copy(x_hbm.at[:, T:L], xt.at[:, T:L], 18)
    xr_copy = copy(x_hbm.at[:, L:S], xt.at[:, L:S], 1)
    wq_copy, wv_copy, wo_copy = [
        copy(w, wstage.at[i], 2 + i) for i, w in ((1, wq_hbm), (2, wv_hbm), (3, wo_hbm))]
    wka_copy = copy(wk_hbm.at[:, 0:KSPLIT], wstage.at[0, :, 0:KSPLIT], 2)
    wkb_copy = copy(wk_hbm.at[:, KSPLIT:D], wstage.at[0, :, KSPLIT:D], 19)
    beta_copy = copy(beta_hbm, beta_ref, 6)
    wr_copy = copy(wr_hbm, wr_ref, 7)
    moe_copies = [copy(wg_hbm, wg, 8), copy(wu_hbm, wu, 9), copy(wd_hbm, wd, 10)]

    def out_copy(lo, hi, i):
        return copy(outb.at[:, lo:hi], out_hbm.at[:, lo:hi], 11 + i)

    half = D // 2
    emitted = set()

    def produced(*key):
        emitted.add(key)

    def require(*key):
        assert key in emitted, key

    def require_heads(s, j):
        for h in range(H):
            require('ot', s, h, j)

    fillers = []

    def fill(n):
        for _ in range(min(n, len(fillers))):
            fillers.pop(0)()

    clock = [0]
    ties = []

    def tile_cols(s, tt):
        return slice(s * L + tt * T, s * L + (tt + 1) * T)

    def local_cols(tt):
        return slice(tt * T, (tt + 1) * T)

    def col_sq_part(i, lo, hi):
        acc = None
        for r in range(lo, hi, 16):
            w = wstage[i, r:r + 16, :].astype(f32)
            w = w * w
            part = w[0:8] + w[8:16]
            acc = part if acc is None else acc + part
        return acc

    def col_sq_max(parts):
        acc = functools.reduce(lambda u, v: u + v, parts)
        return jnp.max(jnp.sum(acc, axis=0, keepdims=True), axis=1, keepdims=True)

    def tie_of(part):
        folded = functools.reduce(lambda u, v: u + v, [part[:, c:c + T] for c in range(0, 4 * T, T)])
        return _zero_after(folded[0:1, 0:1] + part[0:1, 4 * T:4 * T + 1])

    def transpose_weight(i):
        return _to_u32(wstage[i].T)

    def ln_stats(s, tt):
        return _layernorm_stats(xt[:, tile_cols(s, tt)])

    def normalize(s, tt, stats):
        cs = tile_cols(s, tt)
        xn[:, cs] = _layernorm_apply(xt[:, cs], stats)
        produced('xn', s, tt)

    def xn_tile(s, tt):
        require('xn', s, tt)
        return xn[:, tile_cols(s, tt)].astype(bf16)

    def keys_raw(s, tt, lo=0, hi=D):
        kt = _dot(_to_bf16(wt[lo // 2:hi // 2, :]), xn_tile(s, tt))
        fill(CFG['fill_proj'])
        return kt

    def keys_finish(s, tt, kt, tie=None):
        if tie is not None:
            kt = kt + tie
        words = jnp.take_along_axis(_pack_pairs(kt), _unpaired_index(_iota((half, T), 1)), axis=1)
        shift_rows = _iota((8, T), 0) >= 5
        for b in range(NQUAD):
            slab = words[QUAD_OFF[b] // 2:QUAD_OFF[b] // 2 + T // 2, :]
            if b == NQUAD - 1:
                ones = jnp.where(shift_rows, (slab[0:8] & jnp.uint32(0xFFFF0000)) | jnp.uint32(0x3F80), slab[0:8])
                slab = jnp.concatenate([ones, slab[8:]], axis=0)
            else:
                ones = jnp.where(shift_rows, (slab[56:64] & jnp.uint32(0xFFFF)) | jnp.uint32(0x3F800000), slab[56:64])
                slab = jnp.concatenate([slab[:56], ones], axis=0)
            kp[s % 2, b, tt * (T // 2):(tt + 1) * (T // 2), :] = _to_u32(_to_bf16(slab).T)
        produced('k', s, tt)
        return _phi(kt).astype(bf16)

    def project_k(s, tt):
        return keys_finish(s, tt, keys_raw(s, tt))

    def project_q(s, tt, tie=None):
        q = _dot(_to_bf16(wt[half:2 * half, :]), xn_tile(s, tt))
        fill(CFG['fill_proj'])
        qt[s % 2, :, local_cols(tt)] = _pack_pairs(q * (QSCALE if tie is None else QSCALE + tie))
        produced('q', s, tt)
        return _phi(q).astype(bf16)

    def require_segment_done(s):
        if s >= 0:
            for j in range(NT):
                require_heads(s, j)

    def project_v(s, tt):
        require_segment_done(s - 2)
        v = _dot(_to_bf16(wt[2 * half:3 * half, :]), xn_tile(s, tt))
        fill(CFG['fill_proj'])
        vt[s % 2, :, local_cols(tt)] = v
        produced('v', s, tt)

    def router_scores(lhs, s, tt):
        row = s * NT + tt
        rrow[row:row + 1, :] = _dot(lhs, xn_tile(s, tt))[0:1, :]
        produced('r', s, tt)

    def memory_read(s, tt, pq):
        require_segment_done(s - 2)
        for g in range(NGRP):
            require('mt', s - 1, g)
        for g in range(NGRP):
            num[s % 2, g, :, local_cols(tt)] = _dot(mt[g].astype(bf16), pq[SLAB * g:SLAB * g + T, :])
        produced('num', s, tt)

    def memory_update(s, g, pk):
        ones_row = 0 if g == NGRP - 1 else T - 1
        vs = jnp.where(_iota((T, L), 0) == ones_row, 1.0, vt[s % 2, SLAB * g:SLAB * g + T, :]).astype(bf16)
        m = _dot_nt(vs, jnp.concatenate([p[SLAB * g:SLAB * g + T, :] for p in pk], axis=1))
        hr = _head_of_slab_index(_iota((T, T), 0), g)
        hc = _head_of_slab_index(_iota((T, T), 1), g)
        keep = (hr == hc) & (hr >= GROUP_FIRST[g]) & (hr < GROUP_FIRST[g + 1])
        mm = jnp.where(keep, m, 0.0)
        z = m[ones_row:ones_row + 1, :]
        if s > 0:
            mm = mm + mt[g, 0:T, :]
            z = z + zt[g, 0:1, :]
        mt[g, 0:T, :] = mm
        zt[g, 0:1, :] = z
        zsel = _head_of_slab_index(_iota((16, T), 1), g) == _iota((16, T), 0) + GROUP_FIRST[g]
        mt[g, T:MROWS, :] = jnp.where(zsel, z, 0.0)
        produced('mt', s, g)

    def head_groups(b, a):
        f = DH * (4 * b + a) - QUAD_OFF[b]
        return f, (f // 16, f // 16 + 1)

    def build_query_masks():
        block = _iota((8, T), 1) // SUB
        for b in range(NQUAD):
            for a in range(4):
                f, groups = head_groups(b, a)
                for n, g in enumerate(groups):
                    qmask[b, 4 * a + 2 * n] = _pair_mask(16 * g, f, f + DH)
                    qmask[b, 4 * a + 2 * n + 1] = _pair_mask(16 * g, f, f + DH, block == a)

    def stack_groups(groups):
        return _to_bf16(jnp.concatenate(
            [groups.get(g, jnp.zeros((8, T), u32)) for g in range(T // 16)], axis=0))

    def quad_queries(s, b, j, tie):
        tile = s * NT + j
        last = b == NQUAD - 1
        shift_group = 0 if last else T // 16 - 1
        base = QUAD_OFF[b] // 2
        words = {}

        def group(g):
            if g not in words:
                words[g] = qt[s % 2, base + 8 * g:base + 8 * g + 8, local_cols(j)]
            return words[g]

        wide = []
        for a in range(4):
            _, groups = head_groups(b, a)
            parts = {g: group(g) & qmask[b, 4 * a + 2 * n] for n, g in enumerate(groups)}
            if j > 0:
                parts[shift_group] = mx[int(last) + shift_sel * (2 - int(last) + (4 * b + a) * (S // T) + tile)]
                wide.append(stack_groups(parts))
        packed = []
        for i in range(4):
            parts = {}
            for a in range(4):
                _, groups = head_groups(b, a)
                shift = (SUB * (a - i)) % T
                for n, g in enumerate(groups):
                    moved = group(g) if shift == 0 else pltpu.roll(group(g), shift, 1)
                    piece = moved & qmask[b, 4 * a + 2 * n + 1]
                    parts[g] = piece if g not in parts else parts[g] | piece
            rows = mxp[int(last) + shift_sel * (2 - int(last) + tile * H + 4 * b + i)]
            if tie is not None and i == 3:
                rows = rows | tie
            parts[shift_group] = rows
            packed.append(stack_groups(parts))
        return wide, packed

    def scores(s, b, j):
        require('q', s, j)
        for tt in range(j + 1):
            require('k', s, tt)
        tie = None
        unit = clock[0] = (s * NQUAD + b) * NT + j
        due = [z for when, z in ties if when <= unit]
        ties[:] = [(when, z) for when, z in ties if when > unit]
        if due:
            tie = functools.reduce(lambda u, v: u | v, due)
        wide, packed = quad_queries(s, b, j, tie)
        k0 = j * (T // 2)
        off = None
        if j > 0:
            logits = _dot(_to_bf16(kp[s % 2, b, 0:k0, :]), jnp.concatenate(wide, axis=1))
            fill(CFG['fill_qk'])
            off = jnp.exp2(logits)
        causal = _unpaired_index(_iota((SUB, T), 0)) <= (_iota((SUB, T), 1) & (SUB - 1))
        diag = [None] * 4
        for i in range(4):
            n = SUB * (i + 1)
            e = jnp.exp2(_dot(_to_bf16(kp[s % 2, b, k0:k0 + n // 2, :]), packed[i]))
            blocks = [e[r * SUB:(r + 1) * SUB, :] for r in range(i)]
            blocks.append(jnp.where(causal, e[i * SUB:, :], 0.0))
            diag[i] = blocks
        per_head = [[] for _ in range(4)]
        for r in range(4):
            outs = _block_transpose([diag[i][r] if i >= r else None for i in range(4)])
            for a in range(4):
                per_head[a].append(outs[a])
        ps = []
        for a in range(4):
            parts = ([off[:, a * T:(a + 1) * T]] if j > 0 else []) + per_head[a]
            ps.append(_pack_pairs(jnp.concatenate(parts, axis=0)))
        rows = [u[r:r + 8] for u in ps for r in range(0, u.shape[0], 8)]
        while len(rows) > 1:
            rows = [rows[i] | rows[i + 1] for i in range(0, len(rows) - 1, 2)] + rows[len(rows) & ~1:]
        ties.append((unit + CFG['tie_p'], _zero_bits_after(rows[0])))
        return [_to_bf16(u) for u in ps]

    def values(s, h, j, p):
        g = _group_of(h)
        w0 = min((DH * h // 16) * 16, D - 32)
        off = DH * h - w0
        ones_row = 31 if off < 14 else 0
        n = (j + 1) * T
        cs = local_cols(j)
        for tt in range(j + 1):
            require('v', s, tt)
        if s > 0:
            require('num', s, j)
        g0 = (ones_row // 8) * 8
        marked = jnp.where(_iota((8, n), 0) == ones_row - g0, 1.0, vt[s % 2, w0 + g0:w0 + g0 + 8, 0:n])
        rest = vt[s % 2, w0 + 8:w0 + 32, 0:n] if g0 == 0 else vt[s % 2, w0:w0 + 24, 0:n]
        vwin = jnp.concatenate([marked, rest] if g0 == 0 else [rest, marked], axis=0).astype(bf16)
        gate = gb[h:h + 1, :]
        acc = _dot(vwin, p)
        res = acc * ((1.0 - gate) / acc[ones_row:ones_row + 1, :])
        if s > 0:
            m0 = w0 - SLAB * g
            zr = T + h - GROUP_FIRST[g]
            den = num[s % 2, g, zr:zr + 1, cs] + 1e-6
            res = res + num[s % 2, g, m0:m0 + 32, cs] * (gate / den)
        else:
            folded = (res[0:8] + res[8:16]) + (res[16:24] + res[24:32])
            ties.append((clock[0] + CFG['tie_res'], _zero_bits_after(_to_u32(folded))))
        ot[s, DH * h:DH * h + DH, cs] = res[off:off + DH, :]
        produced('ot', s, h, j)

    def route():
        for s in range(NSEG):
            for tt in range(NT):
                require('r', s, tt)
        r = _round_bf16(rrow[...])
        idx = _iota((S // T, T), 0) * T + _iota((S // T, T), 1)
        m1 = jnp.max(r)
        i1 = jnp.min(jnp.where(r == m1, idx, S - 1))
        r2 = jnp.where(idx == i1, -jnp.inf, r)
        m2 = jnp.max(r2)
        i2 = jnp.min(jnp.where(r2 == m2, idx, S - 1))
        return (i1, i2), (m1, m2)

    def select_tokens(ids):
        sel = None
        for row, i in enumerate(ids):
            hit = (_iota((16, T), 0) == row) & (_iota((16, T), 1) == i % T)
            cs = pl.ds(pl.multiple_of((i // T) * T, T), T)
            part = _dot_nt(jnp.where(hit, 1.0, 0.0).astype(bf16), xn[:, cs].astype(bf16))
            sel = part if sel is None else sel + part
        return sel.astype(bf16)

    def queue_moe(xsel, state):
        ktiles = [(k, min(k + T, D)) for k in range(0, D, T)]
        pre, hid = {}, {}
        ycols = state['ycols'] = [None] * len(ktiles)

        def first(w, name, c, lo, hi):
            def fn():
                part = _dot(xsel[:, lo:hi], w[lo:hi, c * T:(c + 1) * T])
                pre[name, c] = part if lo == 0 else pre[name, c] + part
            return fn

        def down(c, n, lo, hi):
            def fn():
                if c not in hid:
                    gpre = _round_bf16(pre.pop(('g', c)))
                    gact = _round_bf16(gpre * _sigmoid(gpre))
                    hid[c] = (gact * _round_bf16(pre.pop(('u', c)))).astype(bf16)
                part = _dot_nt(hid[c], wd[lo:hi, c * T:(c + 1) * T])
                ycols[n] = part if ycols[n] is None else ycols[n] + part
            return fn

        delay = CFG['moe_delay']
        for c in range(NCHUNK + delay):
            if c < NCHUNK:
                for lo, hi in ktiles:
                    fillers.append(first(wg, 'g', c, lo, hi))
                    fillers.append(first(wu, 'u', c, lo, hi))
            if c >= delay:
                for n, (lo, hi) in enumerate(ktiles):
                    fillers.append(down(c - delay, n, lo, hi))

    def moe_result(sel_scores, y):
        row = _iota((16, D), 0)
        gate = jnp.where(row == 0, sel_scores[0], sel_scores[1])
        return (_round_bf16(y) * _sigmoid(gate)).astype(bf16)

    def patch_early(ids, y):
        for k, i in enumerate(ids):
            hit = (_iota((16, T), 0) == k) & (_iota((16, T), 1) == i % T) & (i < EARLY * L)
            cs = pl.ds(pl.multiple_of((jnp.minimum(i, EARLY * L - 1) // T) * T, T), T)
            patch = _dot_tn(y, jnp.where(hit, 1.0, 0.0).astype(bf16))
            outb[:, cs] = (outb[:, cs].astype(f32) + patch).astype(bf16)

    def out_lhs(ids, y):
        place = (_iota((16, T), 1) == _iota((16, T), 0) + 64) & (_iota((16, T), 0) < 2)
        ycols = _dot_tn(y, jnp.where(place, 1.0, 0.0).astype(bf16))
        last = _to_bf16(wot[:, 4 * T:5 * T]).astype(f32) + ycols
        for s in range(EARLY, NSEG):
            tok = _iota((64, L), 1) + s * L
            rows = _iota((64, L), 0)
            hit = ((rows == 0) & (tok == ids[0])) | ((rows == 1) & (tok == ids[1]))
            ot[s, D:D + 64, :] = jnp.where(hit, 1.0, 0.0)
        return jnp.concatenate([_to_bf16(wot[:, 0:4 * T]), last.astype(bf16)], axis=1)

    def out_project_early(s, tt):
        require_heads(s, tt)
        require('wot')
        cs = tile_cols(s, tt)
        attn = _dot(_to_bf16(wot[:, 0:D]), ot[s, 0:D, local_cols(tt)].astype(bf16))
        fill(CFG['fill_proj'])
        outb[:, cs] = (attn + xn[:, cs] + xt[:, cs].astype(f32)).astype(bf16)

    def out_project(lhs, s, tt):
        require_heads(s, tt)
        cs = tile_cols(s, tt)
        attn = _dot(lhs, ot[s, :, local_cols(tt)].astype(bf16))
        outb[:, cs] = (attn + xn[:, cs] + xt[:, cs].astype(f32)).astype(bf16)

    def row_maxima():
        def project_tile(tt, carry):
            cs = pl.ds(pl.multiple_of(tt * T, T), T)
            y = _layernorm_apply(xt[:, cs], _layernorm_stats(xt[:, cs])).astype(bf16)
            kall[:, cs] = _dot(_to_bf16(wt[0:half, :]), y).astype(bf16)
            qall[:, cs] = (_dot(_to_bf16(wt[half:2 * half, :]), y) * QSCALE).astype(bf16)
            return carry

        lax.fori_loop(0, S // T, project_tile, 0)

        def head_tile(i, carry):
            h = i // (S // T)
            tt = i % (S // T)
            cs = pl.ds(pl.multiple_of(tt * T, T), T)
            seg = pl.ds(pl.multiple_of((tt // NT) * L, L), L)
            rows = _iota((D, T), 0)
            qm = jnp.where((rows >= DH * h) & (rows < DH * h + DH), qall[:, cs].astype(f32), 0.0)
            logits = _dot_tn(kall[:, seg], qm.astype(bf16))
            seen = _iota((L, T), 0) <= _iota((L, T), 1) + (tt % NT) * T
            m = jnp.max(jnp.where(seen, logits, NEG_BIG), axis=0, keepdims=True)
            mrow[:, cs] = jnp.where(_iota((H, T), 0) == h, m, mrow[:, cs])
            wide_m = jnp.broadcast_to(m, (8, T))
            mx[2 + i] = jnp.where(h >= H - 4, _shift_words(wide_m, True), _shift_words(wide_m, False))
            return carry

        mrow[...] = jnp.zeros(mrow.shape, f32)
        lax.fori_loop(0, H * (S // T), head_tile, 0)

        def pack_tile(tt, carry):
            cs = pl.ds(pl.multiple_of(tt * T, T), T)
            m = mrow[:, cs]
            block = _iota((1, T), 1) // SUB
            for b in range(NQUAD):
                for i in range(4):
                    row = jnp.zeros((1, T), f32)
                    for a in range(4):
                        src = m[4 * b + a:4 * b + a + 1, :]
                        shift = (SUB * (a - i)) % T
                        row = jnp.where(block == a, src if shift == 0 else pltpu.roll(src, shift, 1), row)
                    mxp[2 + tt * H + 4 * b + i] = _shift_words(jnp.broadcast_to(row, (8, T)), b == NQUAD - 1)
            return carry

        lax.fori_loop(0, S // T, pack_tile, 0)

    for c in (xa_copy, wka_copy, xb_copy, wkb_copy, wq_copy, wv_copy):
        c.start()
    wot[:, 4 * T:5 * T] = jnp.zeros((half, T), u32)
    pk, pq = {}, {}
    sq = [[], []]

    def sq_tie(i, n, parts):
        rows = -(-D // (16 * parts)) * 16
        part = col_sq_part(i, n * rows, min(D, (n + 1) * rows))
        sq[i].append(part)
        return tie_of(part)

    build_query_masks()
    with _scope('p0_wait'):
        xa_copy.wait()
    with _scope('p0'):
        normalize(0, 0, ln_stats(0, 0))
    with _scope('p1_wait'):
        wka_copy.wait()
    with _scope('p1'):
        wt[0:KSPLIT // 2, :] = _to_u32(wstage[0, :, 0:KSPLIT].T)
        ka = [keys_raw(0, 0, 0, KSPLIT)]
    with _scope('p1b_wait'):
        xb_copy.wait()
    with _scope('p1b'):
        for tt in range(1, NT):
            normalize(0, tt, ln_stats(0, tt))
            if tt < NT - 1:
                ka.append(keys_raw(0, tt, 0, KSPLIT))
    with _scope('p1c_wait'):
        wkb_copy.wait()
    with _scope('p1c'):
        ka.append(keys_raw(0, NT - 1, 0, KSPLIT))
        wt[KSPLIT // 2:half, :] = _to_u32(wstage[0, :, KSPLIT:D].T)
        kb = []
        for tt in range(NT - 1):
            kb.append(keys_raw(0, tt, KSPLIT, D))
            if tt > 0:
                pk[0, tt - 1] = keys_finish(0, tt - 1, jnp.concatenate([ka[tt - 1], kb[tt - 1]], axis=0),
                                            sq_tie(0, tt - 1, 2))
    with _scope('p2_wait'):
        wq_copy.wait()
    for c in (xr_copy, beta_copy, wr_copy, wo_copy):
        c.start()
    with _scope('p2'):
        k2 = jnp.concatenate([ka[2], kb[2]], axis=0)
        k3 = jnp.concatenate([ka[3], keys_raw(0, 3, KSPLIT, D)], axis=0)
        wt[half:2 * half, :] = transpose_weight(1)
        pk[0, 2] = keys_finish(0, 2, k2)
        project_q(0, 0, sq_tie(1, 0, 3))
        pk[0, 3] = keys_finish(0, 3, k3)
        for tt in range(1, NT - 1):
            project_q(0, tt, sq_tie(1, tt, 3))
    with _scope('p3_wait'):
        wv_copy.wait()
    with _scope('p3'):
        wt[2 * half:3 * half, :] = transpose_weight(2)
        project_q(0, NT - 1)
        for tt in range(NT - 1):
            project_v(0, tt)
        csq = [col_sq_max(parts) for parts in sq]
        bound = (QSCALE * LN_NORM2 * DH) * jnp.sqrt(csq[0] * csq[1])
        for low in range(2):
            words = _shift_words(jnp.broadcast_to(bound, (8, T)), low == 1)
            mx[low] = words
            mxp[low] = words
        shift_sel = jnp.max(jnp.where(bound <= LOGIT_LIMIT, 0, 1))
        unsafe = shift_sel > 0
    for c in moe_copies:
        c.start()
    with _scope('p4_wait'):
        for c in (xr_copy, beta_copy, wr_copy, wo_copy):
            c.wait()

    @pl.when(unsafe)
    def _():
        row_maxima()

    project_v(0, NT - 1)
    gb[...] = _sigmoid(jnp.broadcast_to(beta_ref[...].astype(f32).reshape(1, H), (T, H)).T)

    slots = {}
    st = {}

    def at(s, b, j, fn):
        slots.setdefault((s, b, j), []).append(fn)

    def at_pos(s, pos, fn):
        at(s, pos // NT, pos % NT, fn)

    def wr_lhs():
        if 'wr' not in st:
            w = jnp.broadcast_to(wr_ref[...].astype(f32).reshape(1, D), (16, D))
            st['wr'] = jnp.where(_iota((16, D), 0) == 0, w, 0.0).astype(bf16)
        return st['wr']

    stats = {}

    def stats_task(s, tt):
        def fn():
            stats[s, tt] = ln_stats(s, tt)
            inv = jnp.broadcast_to(stats[s, tt][1], (8, T))
            ties.append((clock[0] + CFG['tie_ln'], _zero_bits_after(_to_u32(inv))))
        return fn

    def norm_task(s, tt):
        return lambda: normalize(s, tt, stats[s, tt])

    def score_task(s, tt):
        return lambda: router_scores(wr_lhs(), s, tt)

    for s in range(NSEG - 1):
        for g in range(NGRP):
            at_pos(s, CFG['upd_pos'][g], lambda s=s, g=g: memory_update(s, g, [pk[s, tt] for tt in range(NT)]))
        if s == 0:
            at_pos(0, 3, stats_task(1, 0))
            at_pos(0, 5, norm_task(1, 0))
        for tt in range(NT):
            p0 = 9 + 6 * tt
            if s == 0:
                at_pos(s, p0, stats_task(2, tt))
                if tt > 0:
                    at_pos(s, p0, norm_task(3, tt - 1))
            at_pos(s, p0, lambda s=s, tt=tt: pk.__setitem__((s + 1, tt), project_k(s + 1, tt)))
            if s == 0:
                if tt > 0:
                    at_pos(s, p0, score_task(3, tt - 1))
                at_pos(s, p0 + 2, norm_task(2, tt))
                if tt + 1 < NT:
                    at_pos(s, p0 + 2, stats_task(1, tt + 1))
            at_pos(s, p0 + 2, lambda s=s, tt=tt: pq.__setitem__((s + 1, tt), project_q(s + 1, tt)))
            if s == 0:
                at_pos(s, p0 + 2, score_task(2, tt))
                if tt + 1 < NT:
                    at_pos(s, p0 + 4, norm_task(1, tt + 1))
                at_pos(s, p0 + 4, stats_task(3, tt))
            at_pos(s, p0 + 4, lambda s=s, tt=tt: project_v(s + 1, tt))
            at_pos(s, p0 + CFG['read_off'], lambda s=s, tt=tt: memory_read(s + 1, tt, pq[s + 1, tt]))
    at_pos(1, 0, norm_task(3, NT - 1))
    for s in range(EARLY):
        for tt in range(NT):
            at_pos(s + 1, CFG['early_pos'][s][tt], lambda s=s, tt=tt: out_project_early(s, tt))
    at_pos(1, 1, score_task(3, NT - 1))
    for tt in range(NT):
        at_pos(0, 1 + 2 * tt, score_task(0, tt))
        at_pos(0, 10 + 6 * tt, score_task(1, tt))

    def set_out_weight():
        wot[:, 0:D] = transpose_weight(3)
        produced('wot')

    at_pos(0, 22, set_out_weight)

    at_pos(1, 2, lambda: st.update(zip(('ids', 'sel'), route())))
    at_pos(1, CFG['select_pos'], lambda: st.update(xsel=select_tokens(st['ids'])))

    def start_moe():
        with _scope('moe_wait'):
            for c in moe_copies:
                c.wait()
        queue_moe(st['xsel'], st)

    at(1, CFG['moe_quad'], -1, start_moe)

    def finish_moe():
        fill(len(fillers))
        y = moe_result(st['sel'], jnp.concatenate(st['ycols'], axis=1))
        patch_early(st['ids'], y)
        st['lhs'] = out_lhs(st['ids'], y)

    e0 = CFG['moe_end']
    at_pos(3, e0, finish_moe)
    for s in range(EARLY):
        at_pos(3, e0 + 1 + s, lambda s=s: out_copy(s * L, (s + 1) * L, s).start())
    for tt in range(NT):
        at_pos(3, e0 + 2 + CFG['op_gap'] * tt, lambda tt=tt: out_project(st['lhs'], 2, tt))
    at_pos(3, e0 + 3 + CFG['op_gap'] * (NT - 1), lambda: out_copy(2 * L, 3 * L, 2).start())

    def quad_values(s, b, j, ps):
        for a in range(4):
            values(s, 4 * b + a, j, ps[a])

    pending = []
    for s in range(NSEG):
        for b in range(NQUAD):
            for fn in slots.pop((s, b, -1), ()):
                fn()
            for j in range(NT):
                pending.append((s, b, j, scores(s, b, j)))
                for fn in slots.pop((s, b, j), ()):
                    fn()
                if len(pending) > CFG['lag']:
                    quad_values(*pending.pop(0))
    assert not slots, slots.keys()
    s = NSEG - 1

    def last_tile(tt):
        out_project(st['lhs'], s, tt)
        out_copy(s * L + tt * T, s * L + (tt + 1) * T, 3 + tt).start()

    done = 0
    for unit in pending:
        quad_values(*unit)
        while done < NT and unit[1] == NQUAD - 1 and done < unit[2]:
            last_tile(done)
            done += 1
    while done < NT:
        last_tile(done)
        done += 1
    with _scope('out_wait'):
        for k in range(NSEG - 1):
            out_copy(k * L, (k + 1) * L, k).wait()
        for tt in range(NT):
            out_copy(s * L + tt * T, s * L + (tt + 1) * T, 3 + tt).wait()


@jax.jit
def pallas_parallel_sum__memory_aug_infini_attn__moe_arch_mod__prompt_kernel(
    A_x: jax.Array,
    A_wq: jax.Array,
    A_wk: jax.Array,
    A_wv: jax.Array,
    A_wo: jax.Array,
    A_beta: jax.Array,
    B_x: jax.Array,
    B_w_r: jax.Array,
    B_w_gate: jax.Array,
    B_w_up: jax.Array,
    B_w_down: jax.Array,
):
    del B_x
    x_t = jnp.transpose(A_x, (0, 2, 1)).reshape(D, S)
    wd_t = B_w_down.T
    hbm = pl.BlockSpec(memory_space=pl.ANY)
    out_t = pl.pallas_call(
        _kernel,
        out_shape=jax.ShapeDtypeStruct((D, S), bf16),
        in_specs=[hbm] * 10,
        out_specs=hbm,
        scratch_shapes=[
            pltpu.VMEM((D, S), bf16),
            pltpu.VMEM((D, S), f32),
            pltpu.VMEM((4, D, D), bf16),
            pltpu.VMEM((3 * D // 2, D), u32),
            pltpu.VMEM((D // 2, 5 * T), u32),
            pltpu.VMEM((D, F), bf16),
            pltpu.VMEM((D, F), bf16),
            pltpu.VMEM((D, F), bf16),
            pltpu.VMEM((H,), bf16),
            pltpu.VMEM((D,), bf16),
            pltpu.VMEM((2, D // 2, L), u32),
            pltpu.VMEM((2, D, L), f32),
            pltpu.VMEM((2, NQUAD, L // 2, T), u32),
            pltpu.VMEM((2, NGRP, MROWS, L), f32),
            pltpu.VMEM((NGRP, MROWS, T), f32),
            pltpu.VMEM((NGRP, 8, T), f32),
            pltpu.VMEM((NSEG, 5 * T, L), f32),
            pltpu.VMEM((2 + H * S // T, 8, T), u32),
            pltpu.VMEM((2 + H * S // T, 8, T), u32),
            pltpu.VMEM((H, S), f32),
            pltpu.VMEM((NQUAD, 16, 8, T), u32),
            pltpu.VMEM((S // T, T), f32),
            pltpu.VMEM((D, S), bf16),
            pltpu.VMEM((H, T), f32),
            pltpu.VMEM((D, S), bf16),
            pltpu.VMEM((D, S), bf16),
            pltpu.SemaphoreType.DMA((20,)),
        ],
        compiler_params=pltpu.CompilerParams(vmem_limit_bytes=100 * 1024 * 1024),
        name="infini_moe",
    )(x_t, A_wq, A_wk, A_wv, A_wo, A_beta, B_w_r, B_w_gate, B_w_up, wd_t)
    return jnp.transpose(out_t.reshape(1, D, S), (0, 2, 1))
```

```python
import contextlib
import functools

import jax
import jax.numpy as jnp
from jax import lax
from jax.experimental import pallas as pl
from jax.experimental.pallas import tpu as pltpu

S, D, H, DH = 2048, 576, 32, 18
NSEG, L, F = 4, 512, 4608
T = 128
NT = L // T
NGRP = 5
SLAB = 112
GROUP_FIRST = (0, 7, 13, 19, 25, 32)
MROWS = 144
NCHUNK = F // T
NQUAD = H // 4
QUAD_OFF = (0, 64, 144, 208, 288, 352, 432, 448)
EARLY = 2
KSPLIT = 256
SUB = 32

bf16, f32, u32, i32 = jnp.bfloat16, jnp.float32, jnp.uint32, jnp.int32

LOG2E = 1.4426950408889634
QSCALE = (DH ** -0.5) * LOG2E
LN_NORM2 = 2.1 * D
LOGIT_LIMIT = 50.0
NEG_BIG = -1e30


PROFILE_SCOPES = False
CFG = dict(
    lag=5,
    tie_p=3,
    tie_res=3,
    tie_ln=1,
    fill_proj=10,
    fill_qk=8,
    select_pos=7,
    moe_quad=5,
    moe_end=8,
    op_gap=3,
    read_off=4,
    upd_pos=(0, 2, 4, 6, 8),
    early_pos=((8, 14, 20, 26), (3, 5, 7, 9)),
    moe_delay=2,
    tail_parts=(1, 1, 1, 9),
)


def _scope(name):
    return jax.named_scope(name) if PROFILE_SCOPES else contextlib.nullcontext()


def _group_of(h):
    for g in range(NGRP):
        if GROUP_FIRST[g] <= h < GROUP_FIRST[g + 1]:
            return g
    raise ValueError(h)


def _to_bf16(x):
    return pltpu.bitcast(x, bf16)


def _to_u32(x):
    return pltpu.bitcast(x, u32)


def _round_bf16(x):
    return x.astype(bf16).astype(f32)


def _iota(shape, dim):
    return lax.broadcasted_iota(i32, shape, dim)


def _dot(a, b):
    return jnp.dot(a, b, preferred_element_type=f32)


def _dot_nt(a, b):
    return lax.dot_general(a, b, (((1,), (1,)), ((), ())), preferred_element_type=f32)


def _dot_tn(a, b):
    return lax.dot_general(a, b, (((0,), (0,)), ((), ())), preferred_element_type=f32)


def _pack_pairs(x):
    lo = jnp.concatenate([x[r:r + 8] for r in range(0, x.shape[0], 16)], axis=0)
    hi = jnp.concatenate([x[r + 8:r + 16] for r in range(0, x.shape[0], 16)], axis=0)
    return pltpu.pack_elementwise([lo, hi], packed_dtype=bf16)


def _unpaired_index(r):
    x = r & 15
    return (r - x) + jnp.where(x < 8, 2 * x, 2 * (x - 8) + 1)


def _zero_bits_after(u):
    sixteen = jnp.full(u.shape, 16, u32)
    return lax.shift_right_logical(lax.shift_right_logical(u, sixteen), sixteen)


def _pair_mask(first, lo, hi, keep_lane=None):
    f = _iota((8, T), 0) + first
    low = (f >= lo) & (f < hi)
    high = (f + 8 >= lo) & (f + 8 < hi)
    if keep_lane is not None:
        low, high = low & keep_lane, high & keep_lane
    return jnp.where(low, jnp.uint32(0xFFFF), jnp.uint32(0)) | jnp.where(high, jnp.uint32(0xFFFF0000), jnp.uint32(0))


def _bf16_bits(x):
    return pltpu.bitcast(_round_bf16(x), u32)


def _shift_words(m, low_half):
    first = _round_bf16(-m)
    second = _round_bf16(-m - first)
    third = -m - first - second
    row = _iota((8, T), 0)
    val = jnp.where(row == 5, first, jnp.where(row == 6, second, jnp.where(row == 7, third, 0.0)))
    bits = _bf16_bits(val)
    return lax.shift_right_logical(bits, jnp.full(bits.shape, 16, u32)) if low_half else bits


def _phi(t):
    return jnp.where(t > 0, t + 1.0, jnp.exp(t))


def _sigmoid(t):
    return _round_bf16(1.0 / _round_bf16(1.0 + _round_bf16(jnp.exp(-t))))


def _layernorm_stats(xb):
    x0 = xb[0:1, :].astype(f32)
    acc1, acc2 = [None] * 4, [None] * 4
    for n, r in enumerate(range(0, D, 16)):
        c = xb[r:r + 16, :].astype(f32) - x0
        for part in range(2):
            k = (2 * n + part) % 4
            piece = c[8 * part:8 * part + 8, :]
            acc1[k] = piece if acc1[k] is None else acc1[k] + piece
            acc2[k] = piece * piece if acc2[k] is None else acc2[k] + piece * piece
    s1 = jnp.sum((acc1[0] + acc1[1]) + (acc1[2] + acc1[3]), axis=0, keepdims=True) / D
    s2 = jnp.sum((acc2[0] + acc2[1]) + (acc2[2] + acc2[3]), axis=0, keepdims=True) / D
    var = jnp.maximum(s2 - s1 * s1, 0.0)
    eps = _round_bf16(jnp.full((1, 1), 1e-5, f32))
    sd = _round_bf16(jnp.sqrt(_round_bf16(_round_bf16(var) + eps)))
    return _round_bf16(x0 + s1), 1.0 / sd


def _layernorm_apply(xb, stats):
    mean, inv = stats
    return _round_bf16(xb.astype(f32) - mean) * inv


def _block_transpose(xs):
    lane = _iota(next(x for x in xs if x is not None).shape, 1)

    def exchange(u, v, low, shift):
        def pick(p, q):
            if p is None and q is None:
                return None
            return jnp.where(low, 0.0 if p is None else p, 0.0 if q is None else q)
        ru = None if u is None else pltpu.roll(u, T - shift, 1)
        rv = None if v is None else pltpu.roll(v, shift, 1)
        return pick(u, rv), pick(ru, v)

    y0, y2 = exchange(xs[0], xs[2], lane < 64, 64)
    y1, y3 = exchange(xs[1], xs[3], lane < 64, 64)
    low = (lane & 32) == 0
    z0, z1 = exchange(y0, y1, low, 32)
    z2, z3 = exchange(y2, y3, low, 32)
    return [z0, z1, z2, z3]


def _head_of_slab_index(idx, g):
    return ((idx + SLAB * g) * 3641) >> 16


def _zero_after(x):
    sign = lax.shift_right_logical(pltpu.bitcast(x, i32), 31)
    return sign.astype(f32) * 0.0


def _kernel(x_hbm, wq_hbm, wk_hbm, wv_hbm, wo_hbm, beta_hbm, wr_hbm, wg_hbm, wu_hbm, wd_hbm,
            out_hbm,
            xt, xn, wstage, wt, wot, wg, wu, wd, beta_ref, wr_ref, qt, vt, kp, num, mt, zt, ot,
            mx, mxp, mrow, qmask, rrow, outb, gb, kall, qall, sems):
    def copy(src, dst, i):
        return pltpu.make_async_copy(src, dst, sems.at[i])

    xa_copy = copy(x_hbm.at[:, 0:T], xt.at[:, 0:T], 0)
    xb_copy = copy(x_hbm.at[:, T:L], xt.at[:, T:L], 18)
    xr_copy = copy(x_hbm.at[:, L:S], xt.at[:, L:S], 1)
    wq_copy, wv_copy, wo_copy = [
        copy(w, wstage.at[i], 2 + i) for i, w in ((1, wq_hbm), (2, wv_hbm), (3, wo_hbm))]
    wka_copy = copy(wk_hbm.at[:, 0:KSPLIT], wstage.at[0, :, 0:KSPLIT], 2)
    wkb_copy = copy(wk_hbm.at[:, KSPLIT:D], wstage.at[0, :, KSPLIT:D], 19)
    beta_copy = copy(beta_hbm, beta_ref, 6)
    wr_copy = copy(wr_hbm, wr_ref, 7)
    moe_copies = [copy(wg_hbm, wg, 8), copy(wu_hbm, wu, 9), copy(wd_hbm, wd, 10)]

    def out_copy(lo, hi, i):
        return copy(outb.at[:, lo:hi], out_hbm.at[:, lo:hi], 11 + i)

    half = D // 2
    emitted = set()

    def produced(*key):
        emitted.add(key)

    def require(*key):
        assert key in emitted, key

    def require_heads(s, j):
        for h in range(H):
            require('ot', s, h, j)

    fillers = []

    def fill(n):
        for _ in range(min(n, len(fillers))):
            fillers.pop(0)()

    clock = [0]
    ties = []

    def tile_cols(s, tt):
        return slice(s * L + tt * T, s * L + (tt + 1) * T)

    def local_cols(tt):
        return slice(tt * T, (tt + 1) * T)

    def col_sq_part(i, lo, hi):
        acc = None
        for r in range(lo, hi, 16):
            w = wstage[i, r:r + 16, :].astype(f32)
            w = w * w
            part = w[0:8] + w[8:16]
            acc = part if acc is None else acc + part
        return acc

    def col_sq_max(parts):
        acc = functools.reduce(lambda u, v: u + v, parts)
        return jnp.max(jnp.sum(acc, axis=0, keepdims=True), axis=1, keepdims=True)

    def tie_of(part):
        folded = functools.reduce(lambda u, v: u + v, [part[:, c:c + T] for c in range(0, 4 * T, T)])
        return _zero_after(folded[0:1, 0:1] + part[0:1, 4 * T:4 * T + 1])

    def transpose_weight(i):
        return _to_u32(wstage[i].T)

    def ln_stats(s, tt):
        return _layernorm_stats(xt[:, tile_cols(s, tt)])

    def normalize(s, tt, stats):
        cs = tile_cols(s, tt)
        xn[:, cs] = _layernorm_apply(xt[:, cs], stats)
        produced('xn', s, tt)

    def xn_tile(s, tt):
        require('xn', s, tt)
        return xn[:, tile_cols(s, tt)].astype(bf16)

    def keys_raw(s, tt, lo=0, hi=D):
        kt = _dot(_to_bf16(wt[lo // 2:hi // 2, :]), xn_tile(s, tt))
        fill(CFG['fill_proj'])
        return kt

    def keys_finish(s, tt, kt, tie=None):
        if tie is not None:
            kt = kt + tie
        words = jnp.take_along_axis(_pack_pairs(kt), _unpaired_index(_iota((half, T), 1)), axis=1)
        shift_rows = _iota((8, T), 0) >= 5
        for b in range(NQUAD):
            slab = words[QUAD_OFF[b] // 2:QUAD_OFF[b] // 2 + T // 2, :]
            if b == NQUAD - 1:
                ones = jnp.where(shift_rows, (slab[0:8] & jnp.uint32(0xFFFF0000)) | jnp.uint32(0x3F80), slab[0:8])
                slab = jnp.concatenate([ones, slab[8:]], axis=0)
            else:
                ones = jnp.where(shift_rows, (slab[56:64] & jnp.uint32(0xFFFF)) | jnp.uint32(0x3F800000), slab[56:64])
                slab = jnp.concatenate([slab[:56], ones], axis=0)
            kp[s % 2, b, tt * (T // 2):(tt + 1) * (T // 2), :] = _to_u32(_to_bf16(slab).T)
        produced('k', s, tt)
        return _phi(kt).astype(bf16)

    def project_k(s, tt):
        return keys_finish(s, tt, keys_raw(s, tt))

    def project_q(s, tt, tie=None):
        q = _dot(_to_bf16(wt[half:2 * half, :]), xn_tile(s, tt))
        fill(CFG['fill_proj'])
        qt[s % 2, :, local_cols(tt)] = _pack_pairs(q * (QSCALE if tie is None else QSCALE + tie))
        produced('q', s, tt)
        return _phi(q).astype(bf16)

    def require_segment_done(s):
        if s >= 0:
            for j in range(NT):
                require_heads(s, j)

    def project_v(s, tt):
        require_segment_done(s - 2)
        v = _dot(_to_bf16(wt[2 * half:3 * half, :]), xn_tile(s, tt))
        fill(CFG['fill_proj'])
        vt[s % 2, :, local_cols(tt)] = v
        produced('v', s, tt)

    def router_scores(lhs, s, tt):
        row = s * NT + tt
        rrow[row:row + 1, :] = _dot(lhs, xn_tile(s, tt))[0:1, :]
        produced('r', s, tt)

    def memory_read(s, tt, pq):
        require_segment_done(s - 2)
        for g in range(NGRP):
            require('mt', s - 1, g)
        for g in range(NGRP):
            num[s % 2, g, :, local_cols(tt)] = _dot(mt[g].astype(bf16), pq[SLAB * g:SLAB * g + T, :])
        produced('num', s, tt)

    def memory_update(s, g, pk):
        ones_row = 0 if g == NGRP - 1 else T - 1
        vs = jnp.where(_iota((T, L), 0) == ones_row, 1.0, vt[s % 2, SLAB * g:SLAB * g + T, :]).astype(bf16)
        m = _dot_nt(vs, jnp.concatenate([p[SLAB * g:SLAB * g + T, :] for p in pk], axis=1))
        hr = _head_of_slab_index(_iota((T, T), 0), g)
        hc = _head_of_slab_index(_iota((T, T), 1), g)
        keep = (hr == hc) & (hr >= GROUP_FIRST[g]) & (hr < GROUP_FIRST[g + 1])
        mm = jnp.where(keep, m, 0.0)
        z = m[ones_row:ones_row + 1, :]
        if s > 0:
            mm = mm + mt[g, 0:T, :]
            z = z + zt[g, 0:1, :]
        mt[g, 0:T, :] = mm
        zt[g, 0:1, :] = z
        zsel = _head_of_slab_index(_iota((16, T), 1), g) == _iota((16, T), 0) + GROUP_FIRST[g]
        mt[g, T:MROWS, :] = jnp.where(zsel, z, 0.0)
        produced('mt', s, g)

    def head_groups(b, a):
        f = DH * (4 * b + a) - QUAD_OFF[b]
        return f, (f // 16, f // 16 + 1)

    def build_query_masks():
        block = _iota((8, T), 1) // SUB
        for b in range(NQUAD):
            for a in range(4):
                f, groups = head_groups(b, a)
                for n, g in enumerate(groups):
                    qmask[b, 4 * a + 2 * n] = _pair_mask(16 * g, f, f + DH)
                    qmask[b, 4 * a + 2 * n + 1] = _pair_mask(16 * g, f, f + DH, block == a)

    def stack_groups(groups):
        return _to_bf16(jnp.concatenate(
            [groups.get(g, jnp.zeros((8, T), u32)) for g in range(T // 16)], axis=0))

    def quad_queries(s, b, j, tie):
        tile = s * NT + j
        last = b == NQUAD - 1
        shift_group = 0 if last else T // 16 - 1
        base = QUAD_OFF[b] // 2
        words = {}

        def group(g):
            if g not in words:
                words[g] = qt[s % 2, base + 8 * g:base + 8 * g + 8, local_cols(j)]
            return words[g]

        wide = []
        for a in range(4):
            _, groups = head_groups(b, a)
            parts = {g: group(g) & qmask[b, 4 * a + 2 * n] for n, g in enumerate(groups)}
            if j > 0:
                parts[shift_group] = mx[int(last) + shift_sel * (2 - int(last) + (4 * b + a) * (S // T) + tile)]
                wide.append(stack_groups(parts))
        packed = []
        for i in range(4):
            parts = {}
            for a in range(4):
                _, groups = head_groups(b, a)
                shift = (SUB * (a - i)) % T
                for n, g in enumerate(groups):
                    moved = group(g) if shift == 0 else pltpu.roll(group(g), shift, 1)
                    piece = moved & qmask[b, 4 * a + 2 * n + 1]
                    parts[g] = piece if g not in parts else parts[g] | piece
            rows = mxp[int(last) + shift_sel * (2 - int(last) + tile * H + 4 * b + i)]
            if tie is not None and i == 3:
                rows = rows | tie
            parts[shift_group] = rows
            packed.append(stack_groups(parts))
        return wide, packed

    def scores(s, b, j):
        require('q', s, j)
        for tt in range(j + 1):
            require('k', s, tt)
        tie = None
        unit = clock[0] = (s * NQUAD + b) * NT + j
        due = [z for when, z in ties if when <= unit]
        ties[:] = [(when, z) for when, z in ties if when > unit]
        if due:
            tie = functools.reduce(lambda u, v: u | v, due)
        wide, packed = quad_queries(s, b, j, tie)
        k0 = j * (T // 2)
        off = None
        if j > 0:
            logits = _dot(_to_bf16(kp[s % 2, b, 0:k0, :]), jnp.concatenate(wide, axis=1))
            fill(CFG['fill_qk'])
            off = jnp.exp2(logits)
        causal = _unpaired_index(_iota((SUB, T), 0)) <= (_iota((SUB, T), 1) & (SUB - 1))
        diag = [None] * 4
        for i in range(4):
            n = SUB * (i + 1)
            e = jnp.exp2(_dot(_to_bf16(kp[s % 2, b, k0:k0 + n // 2, :]), packed[i]))
            blocks = [e[r * SUB:(r + 1) * SUB, :] for r in range(i)]
            blocks.append(jnp.where(causal, e[i * SUB:, :], 0.0))
            diag[i] = blocks
        per_head = [[] for _ in range(4)]
        for r in range(4):
            outs = _block_transpose([diag[i][r] if i >= r else None for i in range(4)])
            for a in range(4):
                per_head[a].append(outs[a])
        ps = []
        for a in range(4):
            parts = ([off[:, a * T:(a + 1) * T]] if j > 0 else []) + per_head[a]
            ps.append(_pack_pairs(jnp.concatenate(parts, axis=0)))
        rows = [u[r:r + 8] for u in ps for r in range(0, u.shape[0], 8)]
        while len(rows) > 1:
            rows = [rows[i] | rows[i + 1] for i in range(0, len(rows) - 1, 2)] + rows[len(rows) & ~1:]
        ties.append((unit + CFG['tie_p'], _zero_bits_after(rows[0])))
        return [_to_bf16(u) for u in ps]

    def values(s, h, j, p):
        g = _group_of(h)
        w0 = min((DH * h // 16) * 16, D - 32)
        off = DH * h - w0
        ones_row = 31 if off < 14 else 0
        n = (j + 1) * T
        cs = local_cols(j)
        for tt in range(j + 1):
            require('v', s, tt)
        if s > 0:
            require('num', s, j)
        g0 = (ones_row // 8) * 8
        marked = jnp.where(_iota((8, n), 0) == ones_row - g0, 1.0, vt[s % 2, w0 + g0:w0 + g0 + 8, 0:n])
        rest = vt[s % 2, w0 + 8:w0 + 32, 0:n] if g0 == 0 else vt[s % 2, w0:w0 + 24, 0:n]
        vwin = jnp.concatenate([marked, rest] if g0 == 0 else [rest, marked], axis=0).astype(bf16)
        gate = gb[h:h + 1, :]
        acc = _dot(vwin, p)
        res = acc * ((1.0 - gate) / acc[ones_row:ones_row + 1, :])
        if s > 0:
            m0 = w0 - SLAB * g
            zr = T + h - GROUP_FIRST[g]
            den = num[s % 2, g, zr:zr + 1, cs] + 1e-6
            res = res + num[s % 2, g, m0:m0 + 32, cs] * (gate / den)
        else:
            folded = (res[0:8] + res[8:16]) + (res[16:24] + res[24:32])
            ties.append((clock[0] + CFG['tie_res'], _zero_bits_after(_to_u32(folded))))
        ot[s, DH * h:DH * h + DH, cs] = res[off:off + DH, :]
        produced('ot', s, h, j)

    def route():
        for s in range(NSEG):
            for tt in range(NT):
                require('r', s, tt)
        r = _round_bf16(rrow[...])
        idx = _iota((S // T, T), 0) * T + _iota((S // T, T), 1)
        m1 = jnp.max(r)
        i1 = jnp.min(jnp.where(r == m1, idx, S - 1))
        r2 = jnp.where(idx == i1, -jnp.inf, r)
        m2 = jnp.max(r2)
        i2 = jnp.min(jnp.where(r2 == m2, idx, S - 1))
        return (i1, i2), (m1, m2)

    def select_tokens(ids):
        sel = None
        for row, i in enumerate(ids):
            hit = (_iota((16, T), 0) == row) & (_iota((16, T), 1) == i % T)
            cs = pl.ds(pl.multiple_of((i // T) * T, T), T)
            part = _dot_nt(jnp.where(hit, 1.0, 0.0).astype(bf16), xn[:, cs].astype(bf16))
            sel = part if sel is None else sel + part
        return sel.astype(bf16)

    def queue_moe(xsel, state):
        ktiles = [(k, min(k + T, D)) for k in range(0, D, T)]
        pre, hid = {}, {}
        ycols = state['ycols'] = [None] * len(ktiles)

        def first(w, name, c, lo, hi):
            def fn():
                part = _dot(xsel[:, lo:hi], w[lo:hi, c * T:(c + 1) * T])
                pre[name, c] = part if lo == 0 else pre[name, c] + part
            return fn

        def down(c, n, lo, hi):
            def fn():
                if c not in hid:
                    gpre = _round_bf16(pre.pop(('g', c)))
                    gact = _round_bf16(gpre * _sigmoid(gpre))
                    hid[c] = (gact * _round_bf16(pre.pop(('u', c)))).astype(bf16)
                part = _dot_nt(hid[c], wd[lo:hi, c * T:(c + 1) * T])
                ycols[n] = part if ycols[n] is None else ycols[n] + part
            return fn

        delay = CFG['moe_delay']
        for c in range(NCHUNK + delay):
            if c < NCHUNK:
                for lo, hi in ktiles:
                    fillers.append(first(wg, 'g', c, lo, hi))
                    fillers.append(first(wu, 'u', c, lo, hi))
            if c >= delay:
                for n, (lo, hi) in enumerate(ktiles):
                    fillers.append(down(c - delay, n, lo, hi))

    def moe_result(sel_scores, y):
        row = _iota((16, D), 0)
        gate = jnp.where(row == 0, sel_scores[0], sel_scores[1])
        return (_round_bf16(y) * _sigmoid(gate)).astype(bf16)

    def patch_early(ids, y):
        for k, i in enumerate(ids):
            hit = (_iota((16, T), 0) == k) & (_iota((16, T), 1) == i % T) & (i < EARLY * L)
            cs = pl.ds(pl.multiple_of((jnp.minimum(i, EARLY * L - 1) // T) * T, T), T)
            patch = _dot_tn(y, jnp.where(hit, 1.0, 0.0).astype(bf16))
            outb[:, cs] = (outb[:, cs].astype(f32) + patch).astype(bf16)

    def out_lhs(ids, y):
        place = (_iota((16, T), 1) == _iota((16, T), 0) + 64) & (_iota((16, T), 0) < 2)
        ycols = _dot_tn(y, jnp.where(place, 1.0, 0.0).astype(bf16))
        last = _to_bf16(wot[:, 4 * T:5 * T]).astype(f32) + ycols
        for s in range(EARLY, NSEG):
            tok = _iota((64, L), 1) + s * L
            rows = _iota((64, L), 0)
            hit = ((rows == 0) & (tok == ids[0])) | ((rows == 1) & (tok == ids[1]))
            ot[s, D:D + 64, :] = jnp.where(hit, 1.0, 0.0)
        return jnp.concatenate([_to_bf16(wot[:, 0:4 * T]), last.astype(bf16)], axis=1)

    def out_project_early(s, tt):
        require_heads(s, tt)
        require('wot')
        cs = tile_cols(s, tt)
        attn = _dot(_to_bf16(wot[:, 0:D]), ot[s, 0:D, local_cols(tt)].astype(bf16))
        fill(CFG['fill_proj'])
        outb[:, cs] = (attn + xn[:, cs] + xt[:, cs].astype(f32)).astype(bf16)

    def out_project(lhs, s, tt, parts=1):
        require_heads(s, tt)
        cs = tile_cols(s, tt)
        rhs = ot[s, :, local_cols(tt)].astype(bf16)
        for r in range(0, D, D // parts):
            rows = slice(r, r + D // parts)
            attn = _dot(lhs[rows, :], rhs)
            outb[rows, cs] = (attn + xn[rows, cs] + xt[rows, cs].astype(f32)).astype(bf16)

    def row_maxima():
        def project_tile(tt, carry):
            cs = pl.ds(pl.multiple_of(tt * T, T), T)
            y = _layernorm_apply(xt[:, cs], _layernorm_stats(xt[:, cs])).astype(bf16)
            kall[:, cs] = _dot(_to_bf16(wt[0:half, :]), y).astype(bf16)
            qall[:, cs] = (_dot(_to_bf16(wt[half:2 * half, :]), y) * QSCALE).astype(bf16)
            return carry

        lax.fori_loop(0, S // T, project_tile, 0)

        def head_tile(i, carry):
            h = i // (S // T)
            tt = i % (S // T)
            cs = pl.ds(pl.multiple_of(tt * T, T), T)
            seg = pl.ds(pl.multiple_of((tt // NT) * L, L), L)
            rows = _iota((D, T), 0)
            qm = jnp.where((rows >= DH * h) & (rows < DH * h + DH), qall[:, cs].astype(f32), 0.0)
            logits = _dot_tn(kall[:, seg], qm.astype(bf16))
            seen = _iota((L, T), 0) <= _iota((L, T), 1) + (tt % NT) * T
            m = jnp.max(jnp.where(seen, logits, NEG_BIG), axis=0, keepdims=True)
            mrow[:, cs] = jnp.where(_iota((H, T), 0) == h, m, mrow[:, cs])
            wide_m = jnp.broadcast_to(m, (8, T))
            mx[2 + i] = jnp.where(h >= H - 4, _shift_words(wide_m, True), _shift_words(wide_m, False))
            return carry

        mrow[...] = jnp.zeros(mrow.shape, f32)
        lax.fori_loop(0, H * (S // T), head_tile, 0)

        def pack_tile(tt, carry):
            cs = pl.ds(pl.multiple_of(tt * T, T), T)
            m = mrow[:, cs]
            block = _iota((1, T), 1) // SUB
            for b in range(NQUAD):
                for i in range(4):
                    row = jnp.zeros((1, T), f32)
                    for a in range(4):
                        src = m[4 * b + a:4 * b + a + 1, :]
                        shift = (SUB * (a - i)) % T
                        row = jnp.where(block == a, src if shift == 0 else pltpu.roll(src, shift, 1), row)
                    mxp[2 + tt * H + 4 * b + i] = _shift_words(jnp.broadcast_to(row, (8, T)), b == NQUAD - 1)
            return carry

        lax.fori_loop(0, S // T, pack_tile, 0)

    for c in (xa_copy, wka_copy, xb_copy, wkb_copy, wq_copy, wv_copy):
        c.start()
    wot[:, 4 * T:5 * T] = jnp.zeros((half, T), u32)
    pk, pq = {}, {}
    sq = [[], []]

    def sq_tie(i, n, parts):
        rows = -(-D // (16 * parts)) * 16
        part = col_sq_part(i, n * rows, min(D, (n + 1) * rows))
        sq[i].append(part)
        return tie_of(part)

    build_query_masks()
    with _scope('p0_wait'):
        xa_copy.wait()
    with _scope('p0'):
        normalize(0, 0, ln_stats(0, 0))
    with _scope('p1_wait'):
        wka_copy.wait()
    with _scope('p1'):
        wt[0:KSPLIT // 2, :] = _to_u32(wstage[0, :, 0:KSPLIT].T)
        ka = [keys_raw(0, 0, 0, KSPLIT)]
    with _scope('p1b_wait'):
        xb_copy.wait()
    with _scope('p1b'):
        for tt in range(1, NT):
            normalize(0, tt, ln_stats(0, tt))
            if tt < NT - 1:
                ka.append(keys_raw(0, tt, 0, KSPLIT))
    with _scope('p1c_wait'):
        wkb_copy.wait()
    with _scope('p1c'):
        ka.append(keys_raw(0, NT - 1, 0, KSPLIT))
        wt[KSPLIT // 2:half, :] = _to_u32(wstage[0, :, KSPLIT:D].T)
        kb = []
        for tt in range(NT - 1):
            kb.append(keys_raw(0, tt, KSPLIT, D))
            if tt > 0:
                pk[0, tt - 1] = keys_finish(0, tt - 1, jnp.concatenate([ka[tt - 1], kb[tt - 1]], axis=0),
                                            sq_tie(0, tt - 1, 2))
    with _scope('p2_wait'):
        wq_copy.wait()
    for c in (xr_copy, beta_copy, wr_copy, wo_copy):
        c.start()
    with _scope('p2'):
        k2 = jnp.concatenate([ka[2], kb[2]], axis=0)
        k3 = jnp.concatenate([ka[3], keys_raw(0, 3, KSPLIT, D)], axis=0)
        wt[half:2 * half, :] = transpose_weight(1)
        pk[0, 2] = keys_finish(0, 2, k2)
        project_q(0, 0, sq_tie(1, 0, 3))
        pk[0, 3] = keys_finish(0, 3, k3)
        for tt in range(1, NT - 1):
            project_q(0, tt, sq_tie(1, tt, 3))
    with _scope('p3_wait'):
        wv_copy.wait()
    with _scope('p3'):
        wt[2 * half:3 * half, :] = transpose_weight(2)
        project_q(0, NT - 1)
        for tt in range(NT - 1):
            project_v(0, tt)
        csq = [col_sq_max(parts) for parts in sq]
        bound = (QSCALE * LN_NORM2 * DH) * jnp.sqrt(csq[0] * csq[1])
        for low in range(2):
            words = _shift_words(jnp.broadcast_to(bound, (8, T)), low == 1)
            mx[low] = words
            mxp[low] = words
        shift_sel = jnp.max(jnp.where(bound <= LOGIT_LIMIT, 0, 1))
        unsafe = shift_sel > 0
    for c in moe_copies:
        c.start()
    with _scope('p4_wait'):
        for c in (xr_copy, beta_copy, wr_copy, wo_copy):
            c.wait()

    @pl.when(unsafe)
    def _():
        row_maxima()

    project_v(0, NT - 1)
    gb[...] = _sigmoid(jnp.broadcast_to(beta_ref[...].astype(f32).reshape(1, H), (T, H)).T)

    slots = {}
    st = {}

    def at(s, b, j, fn):
        slots.setdefault((s, b, j), []).append(fn)

    def at_pos(s, pos, fn):
        at(s, pos // NT, pos % NT, fn)

    def wr_lhs():
        if 'wr' not in st:
            w = jnp.broadcast_to(wr_ref[...].astype(f32).reshape(1, D), (16, D))
            st['wr'] = jnp.where(_iota((16, D), 0) == 0, w, 0.0).astype(bf16)
        return st['wr']

    stats = {}

    def stats_task(s, tt):
        def fn():
            stats[s, tt] = ln_stats(s, tt)
            inv = jnp.broadcast_to(stats[s, tt][1], (8, T))
            ties.append((clock[0] + CFG['tie_ln'], _zero_bits_after(_to_u32(inv))))
        return fn

    def norm_task(s, tt):
        return lambda: normalize(s, tt, stats[s, tt])

    def score_task(s, tt):
        return lambda: router_scores(wr_lhs(), s, tt)

    for s in range(NSEG - 1):
        for g in range(NGRP):
            at_pos(s, CFG['upd_pos'][g], lambda s=s, g=g: memory_update(s, g, [pk[s, tt] for tt in range(NT)]))
        if s == 0:
            at_pos(0, 3, stats_task(1, 0))
            at_pos(0, 5, norm_task(1, 0))
        for tt in range(NT):
            p0 = 9 + 6 * tt
            if s == 0:
                at_pos(s, p0, stats_task(2, tt))
                if tt > 0:
                    at_pos(s, p0, norm_task(3, tt - 1))
            at_pos(s, p0, lambda s=s, tt=tt: pk.__setitem__((s + 1, tt), project_k(s + 1, tt)))
            if s == 0:
                if tt > 0:
                    at_pos(s, p0, score_task(3, tt - 1))
                at_pos(s, p0 + 2, norm_task(2, tt))
                if tt + 1 < NT:
                    at_pos(s, p0 + 2, stats_task(1, tt + 1))
            at_pos(s, p0 + 2, lambda s=s, tt=tt: pq.__setitem__((s + 1, tt), project_q(s + 1, tt)))
            if s == 0:
                at_pos(s, p0 + 2, score_task(2, tt))
                if tt + 1 < NT:
                    at_pos(s, p0 + 4, norm_task(1, tt + 1))
                at_pos(s, p0 + 4, stats_task(3, tt))
            at_pos(s, p0 + 4, lambda s=s, tt=tt: project_v(s + 1, tt))
            at_pos(s, p0 + CFG['read_off'], lambda s=s, tt=tt: memory_read(s + 1, tt, pq[s + 1, tt]))
    at_pos(1, 0, norm_task(3, NT - 1))
    for s in range(EARLY):
        for tt in range(NT):
            at_pos(s + 1, CFG['early_pos'][s][tt], lambda s=s, tt=tt: out_project_early(s, tt))
    at_pos(1, 1, score_task(3, NT - 1))
    for tt in range(NT):
        at_pos(0, 1 + 2 * tt, score_task(0, tt))
        at_pos(0, 10 + 6 * tt, score_task(1, tt))

    def set_out_weight():
        wot[:, 0:D] = transpose_weight(3)
        produced('wot')

    at_pos(0, 22, set_out_weight)

    at_pos(1, 2, lambda: st.update(zip(('ids', 'sel'), route())))
    at_pos(1, CFG['select_pos'], lambda: st.update(xsel=select_tokens(st['ids'])))

    def start_moe():
        with _scope('moe_wait'):
            for c in moe_copies:
                c.wait()
        queue_moe(st['xsel'], st)

    at(1, CFG['moe_quad'], -1, start_moe)

    def finish_moe():
        fill(len(fillers))
        y = moe_result(st['sel'], jnp.concatenate(st['ycols'], axis=1))
        patch_early(st['ids'], y)
        st['lhs'] = out_lhs(st['ids'], y)

    e0 = CFG['moe_end']
    at_pos(3, e0, finish_moe)
    for s in range(EARLY):
        at_pos(3, e0 + 1 + s, lambda s=s: out_copy(s * L, (s + 1) * L, s).start())
    for tt in range(NT):
        at_pos(3, e0 + 2 + CFG['op_gap'] * tt, lambda tt=tt: out_project(st['lhs'], 2, tt))
    at_pos(3, e0 + 3 + CFG['op_gap'] * (NT - 1), lambda: out_copy(2 * L, 3 * L, 2).start())

    def quad_values(s, b, j, ps):
        for a in range(4):
            values(s, 4 * b + a, j, ps[a])

    pending = []
    for s in range(NSEG):
        for b in range(NQUAD):
            for fn in slots.pop((s, b, -1), ()):
                fn()
            for j in range(NT):
                pending.append((s, b, j, scores(s, b, j)))
                for fn in slots.pop((s, b, j), ()):
                    fn()
                if len(pending) > CFG['lag']:
                    quad_values(*pending.pop(0))
    assert not slots, slots.keys()
    s = NSEG - 1

    def last_tile(tt):
        out_project(st['lhs'], s, tt, CFG['tail_parts'][tt])
        out_copy(s * L + tt * T, s * L + (tt + 1) * T, 3 + tt).start()

    done = 0
    for unit in pending:
        quad_values(*unit)
        while done < NT and unit[1] == NQUAD - 1 and done < unit[2]:
            last_tile(done)
            done += 1
    while done < NT:
        last_tile(done)
        done += 1
    with _scope('out_wait'):
        for k in range(NSEG - 1):
            out_copy(k * L, (k + 1) * L, k).wait()
        for tt in range(NT):
            out_copy(s * L + tt * T, s * L + (tt + 1) * T, 3 + tt).wait()


@jax.jit
def pallas_parallel_sum__memory_aug_infini_attn__moe_arch_mod__prompt_kernel(
    A_x: jax.Array,
    A_wq: jax.Array,
    A_wk: jax.Array,
    A_wv: jax.Array,
    A_wo: jax.Array,
    A_beta: jax.Array,
    B_x: jax.Array,
    B_w_r: jax.Array,
    B_w_gate: jax.Array,
    B_w_up: jax.Array,
    B_w_down: jax.Array,
):
    del B_x
    x_t = jnp.transpose(A_x, (0, 2, 1)).reshape(D, S)
    wd_t = B_w_down.T
    hbm = pl.BlockSpec(memory_space=pl.ANY)
    out_t = pl.pallas_call(
        _kernel,
        out_shape=jax.ShapeDtypeStruct((D, S), bf16),
        in_specs=[hbm] * 10,
        out_specs=hbm,
        scratch_shapes=[
            pltpu.VMEM((D, S), bf16),
            pltpu.VMEM((D, S), f32),
            pltpu.VMEM((4, D, D), bf16),
            pltpu.VMEM((3 * D // 2, D), u32),
            pltpu.VMEM((D // 2, 5 * T), u32),
            pltpu.VMEM((D, F), bf16),
            pltpu.VMEM((D, F), bf16),
            pltpu.VMEM((D, F), bf16),
            pltpu.VMEM((H,), bf16),
            pltpu.VMEM((D,), bf16),
            pltpu.VMEM((2, D // 2, L), u32),
            pltpu.VMEM((2, D, L), f32),
            pltpu.VMEM((2, NQUAD, L // 2, T), u32),
            pltpu.VMEM((2, NGRP, MROWS, L), f32),
            pltpu.VMEM((NGRP, MROWS, T), f32),
            pltpu.VMEM((NGRP, 8, T), f32),
            pltpu.VMEM((NSEG, 5 * T, L), f32),
            pltpu.VMEM((2 + H * S // T, 8, T), u32),
            pltpu.VMEM((2 + H * S // T, 8, T), u32),
            pltpu.VMEM((H, S), f32),
            pltpu.VMEM((NQUAD, 16, 8, T), u32),
            pltpu.VMEM((S // T, T), f32),
            pltpu.VMEM((D, S), bf16),
            pltpu.VMEM((H, T), f32),
            pltpu.VMEM((D, S), bf16),
            pltpu.VMEM((D, S), bf16),
            pltpu.SemaphoreType.DMA((20,)),
        ],
        compiler_params=pltpu.CompilerParams(vmem_limit_bytes=100 * 1024 * 1024),
        name="infini_moe",
    )(x_t, A_wq, A_wk, A_wv, A_wo, A_beta, B_w_r, B_w_gate, B_w_up, wd_t)
    return jnp.transpose(out_t.reshape(1, D, S), (0, 2, 1))
```

```python
import contextlib
import functools

import jax
import jax.numpy as jnp
from jax import lax
from jax.experimental import pallas as pl
from jax.experimental.pallas import tpu as pltpu

S, D, H, DH = 2048, 576, 32, 18
NSEG, L, F = 4, 512, 4608
T = 128
NT = L // T
NGRP = 5
SLAB = 112
GROUP_FIRST = (0, 7, 13, 19, 25, 32)
MROWS = 144
NCHUNK = F // T
NQUAD = H // 4
QUAD_OFF = (0, 64, 144, 208, 288, 352, 432, 448)
EARLY = 2
KSPLIT = 256
SUB = 32

bf16, f32, u32, i32 = jnp.bfloat16, jnp.float32, jnp.uint32, jnp.int32

LOG2E = 1.4426950408889634
QSCALE = (DH ** -0.5) * LOG2E
LN_NORM2 = 2.1 * D
LOGIT_LIMIT = 50.0
NEG_BIG = -1e30


PROFILE_SCOPES = False
CFG = dict(
    lag=5,
    tie_p=3,
    tie_res=3,
    tie_ln=1,
    fill_proj=10,
    fill_qk=8,
    select_pos=7,
    moe_quad=5,
    moe_end=8,
    op_gap=3,
    read_off=4,
    upd_pos=(0, 2, 4, 6, 8),
    early_pos=(((1, 8), (1, 14), (1, 20), (1, 26)), ((2, 3), (2, 5), (2, 7), (2, 9))),
    wot_pos=(0, 22),
    moe_delay=2,
    splits={('q', 0, 2, 0): 4, ('v', 0, 2, 0): 4, ('k', 0, 2, 256): 4, ('k', 0, 2, 0): 4, ('k', 0, 0, 0): 4},
    tail_parts=(1, 1, 1, 9),
)


def _scope(name):
    return jax.named_scope(name) if PROFILE_SCOPES else contextlib.nullcontext()


def _group_of(h):
    for g in range(NGRP):
        if GROUP_FIRST[g] <= h < GROUP_FIRST[g + 1]:
            return g
    raise ValueError(h)


def _to_bf16(x):
    return pltpu.bitcast(x, bf16)


def _to_u32(x):
    return pltpu.bitcast(x, u32)


def _round_bf16(x):
    return x.astype(bf16).astype(f32)


def _iota(shape, dim):
    return lax.broadcasted_iota(i32, shape, dim)


def _dot(a, b):
    return jnp.dot(a, b, preferred_element_type=f32)


def _dot_nt(a, b):
    return lax.dot_general(a, b, (((1,), (1,)), ((), ())), preferred_element_type=f32)


def _dot_tn(a, b):
    return lax.dot_general(a, b, (((0,), (0,)), ((), ())), preferred_element_type=f32)


def _pack_pairs(x):
    lo = jnp.concatenate([x[r:r + 8] for r in range(0, x.shape[0], 16)], axis=0)
    hi = jnp.concatenate([x[r + 8:r + 16] for r in range(0, x.shape[0], 16)], axis=0)
    return pltpu.pack_elementwise([lo, hi], packed_dtype=bf16)


def _unpaired_index(r):
    x = r & 15
    return (r - x) + jnp.where(x < 8, 2 * x, 2 * (x - 8) + 1)


def _zero_bits_after(u):
    sixteen = jnp.full(u.shape, 16, u32)
    return lax.shift_right_logical(lax.shift_right_logical(u, sixteen), sixteen)


def _pair_mask(first, lo, hi, keep_lane=None):
    f = _iota((8, T), 0) + first
    low = (f >= lo) & (f < hi)
    high = (f + 8 >= lo) & (f + 8 < hi)
    if keep_lane is not None:
        low, high = low & keep_lane, high & keep_lane
    return jnp.where(low, jnp.uint32(0xFFFF), jnp.uint32(0)) | jnp.where(high, jnp.uint32(0xFFFF0000), jnp.uint32(0))


def _bf16_bits(x):
    return pltpu.bitcast(_round_bf16(x), u32)


def _shift_words(m, low_half):
    first = _round_bf16(-m)
    second = _round_bf16(-m - first)
    third = -m - first - second
    row = _iota((8, T), 0)
    val = jnp.where(row == 5, first, jnp.where(row == 6, second, jnp.where(row == 7, third, 0.0)))
    bits = _bf16_bits(val)
    return lax.shift_right_logical(bits, jnp.full(bits.shape, 16, u32)) if low_half else bits


def _phi(t):
    return jnp.where(t > 0, t + 1.0, jnp.exp(t))


def _sigmoid(t):
    return _round_bf16(1.0 / _round_bf16(1.0 + _round_bf16(jnp.exp(-t))))


def _layernorm_stats(xb):
    x0 = xb[0:1, :].astype(f32)
    acc1, acc2 = [None] * 4, [None] * 4
    for n, r in enumerate(range(0, D, 16)):
        c = xb[r:r + 16, :].astype(f32) - x0
        for part in range(2):
            k = (2 * n + part) % 4
            piece = c[8 * part:8 * part + 8, :]
            acc1[k] = piece if acc1[k] is None else acc1[k] + piece
            acc2[k] = piece * piece if acc2[k] is None else acc2[k] + piece * piece
    s1 = jnp.sum((acc1[0] + acc1[1]) + (acc1[2] + acc1[3]), axis=0, keepdims=True) / D
    s2 = jnp.sum((acc2[0] + acc2[1]) + (acc2[2] + acc2[3]), axis=0, keepdims=True) / D
    var = jnp.maximum(s2 - s1 * s1, 0.0)
    eps = _round_bf16(jnp.full((1, 1), 1e-5, f32))
    sd = _round_bf16(jnp.sqrt(_round_bf16(_round_bf16(var) + eps)))
    return _round_bf16(x0 + s1), 1.0 / sd


def _layernorm_apply(xb, stats):
    mean, inv = stats
    return _round_bf16(xb.astype(f32) - mean) * inv


def _block_transpose(xs):
    lane = _iota(next(x for x in xs if x is not None).shape, 1)

    def exchange(u, v, low, shift):
        def pick(p, q):
            if p is None and q is None:
                return None
            return jnp.where(low, 0.0 if p is None else p, 0.0 if q is None else q)
        ru = None if u is None else pltpu.roll(u, T - shift, 1)
        rv = None if v is None else pltpu.roll(v, shift, 1)
        return pick(u, rv), pick(ru, v)

    y0, y2 = exchange(xs[0], xs[2], lane < 64, 64)
    y1, y3 = exchange(xs[1], xs[3], lane < 64, 64)
    low = (lane & 32) == 0
    z0, z1 = exchange(y0, y1, low, 32)
    z2, z3 = exchange(y2, y3, low, 32)
    return [z0, z1, z2, z3]


def _head_of_slab_index(idx, g):
    return ((idx + SLAB * g) * 3641) >> 16


def _zero_after(x):
    sign = lax.shift_right_logical(pltpu.bitcast(x, i32), 31)
    return sign.astype(f32) * 0.0


def _kernel(x_hbm, wq_hbm, wk_hbm, wv_hbm, wo_hbm, beta_hbm, wr_hbm, wg_hbm, wu_hbm, wd_hbm,
            out_hbm,
            xt, xn, wstage, wt, wot, wg, wu, wd, beta_ref, wr_ref, qt, vt, kp, num, mt, zt, ot,
            mx, mxp, mrow, qmask, rrow, outb, gb, kall, qall, sems):
    def copy(src, dst, i):
        return pltpu.make_async_copy(src, dst, sems.at[i])

    xa_copy = copy(x_hbm.at[:, 0:T], xt.at[:, 0:T], 0)
    xb_copy = copy(x_hbm.at[:, T:L], xt.at[:, T:L], 18)
    xr_copy = copy(x_hbm.at[:, L:S], xt.at[:, L:S], 1)
    wq_copy, wv_copy, wo_copy = [
        copy(w, wstage.at[i], 2 + i) for i, w in ((1, wq_hbm), (2, wv_hbm), (3, wo_hbm))]
    wka_copy = copy(wk_hbm.at[:, 0:KSPLIT], wstage.at[0, :, 0:KSPLIT], 2)
    wkb_copy = copy(wk_hbm.at[:, KSPLIT:D], wstage.at[0, :, KSPLIT:D], 19)
    beta_copy = copy(beta_hbm, beta_ref, 6)
    wr_copy = copy(wr_hbm, wr_ref, 7)
    moe_copies = [copy(wg_hbm, wg, 8), copy(wu_hbm, wu, 9), copy(wd_hbm, wd, 10)]

    def out_copy(lo, hi, i):
        return copy(outb.at[:, lo:hi], out_hbm.at[:, lo:hi], 11 + i)

    half = D // 2
    emitted = set()

    def produced(*key):
        emitted.add(key)

    def require(*key):
        assert key in emitted, key

    def require_heads(s, j):
        for h in range(H):
            require('ot', s, h, j)

    fillers = []

    def fill(n):
        for _ in range(min(n, len(fillers))):
            fillers.pop(0)()

    clock = [0]
    ties = []

    def tile_cols(s, tt):
        return slice(s * L + tt * T, s * L + (tt + 1) * T)

    def local_cols(tt):
        return slice(tt * T, (tt + 1) * T)

    def col_sq_part(i, lo, hi):
        acc = None
        for r in range(lo, hi, 16):
            w = wstage[i, r:r + 16, :].astype(f32)
            w = w * w
            part = w[0:8] + w[8:16]
            acc = part if acc is None else acc + part
        return acc

    def col_sq_max(parts):
        acc = functools.reduce(lambda u, v: u + v, parts)
        return jnp.max(jnp.sum(acc, axis=0, keepdims=True), axis=1, keepdims=True)

    def tie_of(part):
        folded = functools.reduce(lambda u, v: u + v, [part[:, c:c + T] for c in range(0, 4 * T, T)])
        return _zero_after(folded[0:1, 0:1] + part[0:1, 4 * T:4 * T + 1])

    def transpose_weight(i):
        return _to_u32(wstage[i].T)

    def ln_stats(s, tt):
        return _layernorm_stats(xt[:, tile_cols(s, tt)])

    def normalize(s, tt, stats):
        cs = tile_cols(s, tt)
        xn[:, cs] = _layernorm_apply(xt[:, cs], stats)
        produced('xn', s, tt)

    def xn_tile(s, tt):
        require('xn', s, tt)
        return xn[:, tile_cols(s, tt)].astype(bf16)

    def project(base, lo, hi, name, s, tt):
        rhs = xn_tile(s, tt)
        parts = CFG['splits'].get((name, s, tt, lo), 1)
        step = (hi - lo) // parts
        out = [_dot(_to_bf16(wt[(base + r) // 2:(base + r + step) // 2, :]), rhs) for r in range(lo, hi, step)]
        fill(CFG['fill_proj'])
        return out[0] if parts == 1 else jnp.concatenate(out, axis=0)

    def keys_raw(s, tt, lo=0, hi=D):
        return project(0, lo, hi, 'k', s, tt)

    def keys_finish(s, tt, kt, tie=None):
        if tie is not None:
            kt = kt + tie
        words = jnp.take_along_axis(_pack_pairs(kt), _unpaired_index(_iota((half, T), 1)), axis=1)
        shift_rows = _iota((8, T), 0) >= 5
        for b in range(NQUAD):
            slab = words[QUAD_OFF[b] // 2:QUAD_OFF[b] // 2 + T // 2, :]
            if b == NQUAD - 1:
                ones = jnp.where(shift_rows, (slab[0:8] & jnp.uint32(0xFFFF0000)) | jnp.uint32(0x3F80), slab[0:8])
                slab = jnp.concatenate([ones, slab[8:]], axis=0)
            else:
                ones = jnp.where(shift_rows, (slab[56:64] & jnp.uint32(0xFFFF)) | jnp.uint32(0x3F800000), slab[56:64])
                slab = jnp.concatenate([slab[:56], ones], axis=0)
            kp[s % 2, b, tt * (T // 2):(tt + 1) * (T // 2), :] = _to_u32(_to_bf16(slab).T)
        produced('k', s, tt)
        return _phi(kt).astype(bf16)

    def project_k(s, tt):
        return keys_finish(s, tt, keys_raw(s, tt))

    def project_q(s, tt, tie=None):
        q = project(D, 0, D, 'q', s, tt)
        qt[s % 2, :, local_cols(tt)] = _pack_pairs(q * (QSCALE if tie is None else QSCALE + tie))
        produced('q', s, tt)
        return _phi(q).astype(bf16)

    def require_segment_done(s):
        if s >= 0:
            for j in range(NT):
                require_heads(s, j)

    def project_v(s, tt):
        require_segment_done(s - 2)
        v = project(2 * D, 0, D, 'v', s, tt)
        vt[s % 2, :, local_cols(tt)] = v
        produced('v', s, tt)

    def router_scores(lhs, s, tt):
        row = s * NT + tt
        rrow[row:row + 1, :] = _dot(lhs, xn_tile(s, tt))[0:1, :]
        produced('r', s, tt)

    def memory_read(s, tt, pq):
        require_segment_done(s - 2)
        for g in range(NGRP):
            require('mt', s - 1, g)
        for g in range(NGRP):
            num[s % 2, g, :, local_cols(tt)] = _dot(mt[g].astype(bf16), pq[SLAB * g:SLAB * g + T, :])
        produced('num', s, tt)

    def memory_update(s, g, pk):
        ones_row = 0 if g == NGRP - 1 else T - 1
        vs = jnp.where(_iota((T, L), 0) == ones_row, 1.0, vt[s % 2, SLAB * g:SLAB * g + T, :]).astype(bf16)
        m = _dot_nt(vs, jnp.concatenate([p[SLAB * g:SLAB * g + T, :] for p in pk], axis=1))
        hr = _head_of_slab_index(_iota((T, T), 0), g)
        hc = _head_of_slab_index(_iota((T, T), 1), g)
        keep = (hr == hc) & (hr >= GROUP_FIRST[g]) & (hr < GROUP_FIRST[g + 1])
        mm = jnp.where(keep, m, 0.0)
        z = m[ones_row:ones_row + 1, :]
        if s > 0:
            mm = mm + mt[g, 0:T, :]
            z = z + zt[g, 0:1, :]
        mt[g, 0:T, :] = mm
        zt[g, 0:1, :] = z
        zsel = _head_of_slab_index(_iota((16, T), 1), g) == _iota((16, T), 0) + GROUP_FIRST[g]
        mt[g, T:MROWS, :] = jnp.where(zsel, z, 0.0)
        produced('mt', s, g)

    def head_groups(b, a):
        f = DH * (4 * b + a) - QUAD_OFF[b]
        return f, (f // 16, f // 16 + 1)

    def build_query_masks():
        block = _iota((8, T), 1) // SUB
        for b in range(NQUAD):
            for a in range(4):
                f, groups = head_groups(b, a)
                for n, g in enumerate(groups):
                    qmask[b, 4 * a + 2 * n] = _pair_mask(16 * g, f, f + DH)
                    qmask[b, 4 * a + 2 * n + 1] = _pair_mask(16 * g, f, f + DH, block == a)

    def stack_groups(groups):
        return _to_bf16(jnp.concatenate(
            [groups.get(g, jnp.zeros((8, T), u32)) for g in range(T // 16)], axis=0))

    def quad_queries(s, b, j, tie):
        tile = s * NT + j
        last = b == NQUAD - 1
        shift_group = 0 if last else T // 16 - 1
        base = QUAD_OFF[b] // 2
        words = {}

        def group(g):
            if g not in words:
                words[g] = qt[s % 2, base + 8 * g:base + 8 * g + 8, local_cols(j)]
            return words[g]

        wide = []
        for a in range(4):
            _, groups = head_groups(b, a)
            parts = {g: group(g) & qmask[b, 4 * a + 2 * n] for n, g in enumerate(groups)}
            if j > 0:
                parts[shift_group] = mx[int(last) + shift_sel * (2 - int(last) + (4 * b + a) * (S // T) + tile)]
                wide.append(stack_groups(parts))
        packed = []
        for i in range(4):
            parts = {}
            for a in range(4):
                _, groups = head_groups(b, a)
                shift = (SUB * (a - i)) % T
                for n, g in enumerate(groups):
                    moved = group(g) if shift == 0 else pltpu.roll(group(g), shift, 1)
                    piece = moved & qmask[b, 4 * a + 2 * n + 1]
                    parts[g] = piece if g not in parts else parts[g] | piece
            rows = mxp[int(last) + shift_sel * (2 - int(last) + tile * H + 4 * b + i)]
            if tie is not None and i == 3:
                rows = rows | tie
            parts[shift_group] = rows
            packed.append(stack_groups(parts))
        return wide, packed

    def scores(s, b, j):
        require('q', s, j)
        for tt in range(j + 1):
            require('k', s, tt)
        tie = None
        unit = clock[0] = (s * NQUAD + b) * NT + j
        due = [z for when, z in ties if when <= unit]
        ties[:] = [(when, z) for when, z in ties if when > unit]
        if due:
            tie = functools.reduce(lambda u, v: u | v, due)
        wide, packed = quad_queries(s, b, j, tie)
        k0 = j * (T // 2)
        off = None
        if j > 0:
            logits = _dot(_to_bf16(kp[s % 2, b, 0:k0, :]), jnp.concatenate(wide, axis=1))
            fill(CFG['fill_qk'])
            off = jnp.exp2(logits)
        causal = _unpaired_index(_iota((SUB, T), 0)) <= (_iota((SUB, T), 1) & (SUB - 1))
        diag = [None] * 4
        for i in range(4):
            n = SUB * (i + 1)
            e = jnp.exp2(_dot(_to_bf16(kp[s % 2, b, k0:k0 + n // 2, :]), packed[i]))
            blocks = [e[r * SUB:(r + 1) * SUB, :] for r in range(i)]
            blocks.append(jnp.where(causal, e[i * SUB:, :], 0.0))
            diag[i] = blocks
        per_head = [[] for _ in range(4)]
        for r in range(4):
            outs = _block_transpose([diag[i][r] if i >= r else None for i in range(4)])
            for a in range(4):
                per_head[a].append(outs[a])
        ps = []
        for a in range(4):
            parts = ([off[:, a * T:(a + 1) * T]] if j > 0 else []) + per_head[a]
            ps.append(_pack_pairs(jnp.concatenate(parts, axis=0)))
        rows = [u[r:r + 8] for u in ps for r in range(0, u.shape[0], 8)]
        while len(rows) > 1:
            rows = [rows[i] | rows[i + 1] for i in range(0, len(rows) - 1, 2)] + rows[len(rows) & ~1:]
        ties.append((unit + CFG['tie_p'], _zero_bits_after(rows[0])))
        return [_to_bf16(u) for u in ps]

    def values(s, h, j, p):
        g = _group_of(h)
        w0 = min((DH * h // 16) * 16, D - 32)
        off = DH * h - w0
        ones_row = 31 if off < 14 else 0
        n = (j + 1) * T
        cs = local_cols(j)
        for tt in range(j + 1):
            require('v', s, tt)
        if s > 0:
            require('num', s, j)
        g0 = (ones_row // 8) * 8
        marked = jnp.where(_iota((8, n), 0) == ones_row - g0, 1.0, vt[s % 2, w0 + g0:w0 + g0 + 8, 0:n])
        rest = vt[s % 2, w0 + 8:w0 + 32, 0:n] if g0 == 0 else vt[s % 2, w0:w0 + 24, 0:n]
        vwin = jnp.concatenate([marked, rest] if g0 == 0 else [rest, marked], axis=0).astype(bf16)
        gate = gb[h:h + 1, :]
        acc = _dot(vwin, p)
        res = acc * ((1.0 - gate) / acc[ones_row:ones_row + 1, :])
        if s > 0:
            m0 = w0 - SLAB * g
            zr = T + h - GROUP_FIRST[g]
            den = num[s % 2, g, zr:zr + 1, cs] + 1e-6
            res = res + num[s % 2, g, m0:m0 + 32, cs] * (gate / den)
        else:
            folded = (res[0:8] + res[8:16]) + (res[16:24] + res[24:32])
            ties.append((clock[0] + CFG['tie_res'], _zero_bits_after(_to_u32(folded))))
        ot[s, DH * h:DH * h + DH, cs] = res[off:off + DH, :]
        produced('ot', s, h, j)

    def route():
        for s in range(NSEG):
            for tt in range(NT):
                require('r', s, tt)
        r = _round_bf16(rrow[...])
        idx = _iota((S // T, T), 0) * T + _iota((S // T, T), 1)
        m1 = jnp.max(r)
        i1 = jnp.min(jnp.where(r == m1, idx, S - 1))
        r2 = jnp.where(idx == i1, -jnp.inf, r)
        m2 = jnp.max(r2)
        i2 = jnp.min(jnp.where(r2 == m2, idx, S - 1))
        return (i1, i2), (m1, m2)

    def select_tokens(ids):
        sel = None
        for row, i in enumerate(ids):
            hit = (_iota((16, T), 0) == row) & (_iota((16, T), 1) == i % T)
            cs = pl.ds(pl.multiple_of((i // T) * T, T), T)
            part = _dot_nt(jnp.where(hit, 1.0, 0.0).astype(bf16), xn[:, cs].astype(bf16))
            sel = part if sel is None else sel + part
        return sel.astype(bf16)

    def queue_moe(xsel, state):
        ktiles = [(k, min(k + T, D)) for k in range(0, D, T)]
        pre, hid = {}, {}
        ycols = state['ycols'] = [None] * len(ktiles)

        def first(w, name, c, lo, hi):
            def fn():
                part = _dot(xsel[:, lo:hi], w[lo:hi, c * T:(c + 1) * T])
                pre[name, c] = part if lo == 0 else pre[name, c] + part
            return fn

        def down(c, n, lo, hi):
            def fn():
                if c not in hid:
                    gpre = _round_bf16(pre.pop(('g', c)))
                    gact = _round_bf16(gpre * _sigmoid(gpre))
                    hid[c] = (gact * _round_bf16(pre.pop(('u', c)))).astype(bf16)
                part = _dot_nt(hid[c], wd[lo:hi, c * T:(c + 1) * T])
                ycols[n] = part if ycols[n] is None else ycols[n] + part
            return fn

        delay = CFG['moe_delay']
        for c in range(NCHUNK + delay):
            if c < NCHUNK:
                for lo, hi in ktiles:
                    fillers.append(first(wg, 'g', c, lo, hi))
                    fillers.append(first(wu, 'u', c, lo, hi))
            if c >= delay:
                for n, (lo, hi) in enumerate(ktiles):
                    fillers.append(down(c - delay, n, lo, hi))

    def moe_result(sel_scores, y):
        row = _iota((16, D), 0)
        gate = jnp.where(row == 0, sel_scores[0], sel_scores[1])
        return (_round_bf16(y) * _sigmoid(gate)).astype(bf16)

    def patch_early(ids, y):
        for k, i in enumerate(ids):
            hit = (_iota((16, T), 0) == k) & (_iota((16, T), 1) == i % T) & (i < EARLY * L)
            cs = pl.ds(pl.multiple_of((jnp.minimum(i, EARLY * L - 1) // T) * T, T), T)
            patch = _dot_tn(y, jnp.where(hit, 1.0, 0.0).astype(bf16))
            outb[:, cs] = (outb[:, cs].astype(f32) + patch).astype(bf16)

    def out_lhs(ids, y):
        place = (_iota((16, T), 1) == _iota((16, T), 0) + 64) & (_iota((16, T), 0) < 2)
        ycols = _dot_tn(y, jnp.where(place, 1.0, 0.0).astype(bf16))
        last = _to_bf16(wot[:, 4 * T:5 * T]).astype(f32) + ycols
        for s in range(EARLY, NSEG):
            tok = _iota((64, L), 1) + s * L
            rows = _iota((64, L), 0)
            hit = ((rows == 0) & (tok == ids[0])) | ((rows == 1) & (tok == ids[1]))
            ot[s, D:D + 64, :] = jnp.where(hit, 1.0, 0.0)
        return jnp.concatenate([_to_bf16(wot[:, 0:4 * T]), last.astype(bf16)], axis=1)

    def out_project_early(s, tt):
        require_heads(s, tt)
        require('wot')
        cs = tile_cols(s, tt)
        attn = _dot(_to_bf16(wot[:, 0:D]), ot[s, 0:D, local_cols(tt)].astype(bf16))
        fill(CFG['fill_proj'])
        outb[:, cs] = (attn + xn[:, cs] + xt[:, cs].astype(f32)).astype(bf16)

    def out_project(lhs, s, tt, parts=1):
        require_heads(s, tt)
        cs = tile_cols(s, tt)
        rhs = ot[s, :, local_cols(tt)].astype(bf16)
        for r in range(0, D, D // parts):
            rows = slice(r, r + D // parts)
            attn = _dot(lhs[rows, :], rhs)
            outb[rows, cs] = (attn + xn[rows, cs] + xt[rows, cs].astype(f32)).astype(bf16)

    def row_maxima():
        def project_tile(tt, carry):
            cs = pl.ds(pl.multiple_of(tt * T, T), T)
            y = _layernorm_apply(xt[:, cs], _layernorm_stats(xt[:, cs])).astype(bf16)
            kall[:, cs] = _dot(_to_bf16(wt[0:half, :]), y).astype(bf16)
            qall[:, cs] = (_dot(_to_bf16(wt[half:2 * half, :]), y) * QSCALE).astype(bf16)
            return carry

        lax.fori_loop(0, S // T, project_tile, 0)

        def head_tile(i, carry):
            h = i // (S // T)
            tt = i % (S // T)
            cs = pl.ds(pl.multiple_of(tt * T, T), T)
            seg = pl.ds(pl.multiple_of((tt // NT) * L, L), L)
            rows = _iota((D, T), 0)
            qm = jnp.where((rows >= DH * h) & (rows < DH * h + DH), qall[:, cs].astype(f32), 0.0)
            logits = _dot_tn(kall[:, seg], qm.astype(bf16))
            seen = _iota((L, T), 0) <= _iota((L, T), 1) + (tt % NT) * T
            m = jnp.max(jnp.where(seen, logits, NEG_BIG), axis=0, keepdims=True)
            mrow[:, cs] = jnp.where(_iota((H, T), 0) == h, m, mrow[:, cs])
            wide_m = jnp.broadcast_to(m, (8, T))
            mx[2 + i] = jnp.where(h >= H - 4, _shift_words(wide_m, True), _shift_words(wide_m, False))
            return carry

        mrow[...] = jnp.zeros(mrow.shape, f32)
        lax.fori_loop(0, H * (S // T), head_tile, 0)

        def pack_tile(tt, carry):
            cs = pl.ds(pl.multiple_of(tt * T, T), T)
            m = mrow[:, cs]
            block = _iota((1, T), 1) // SUB
            for b in range(NQUAD):
                for i in range(4):
                    row = jnp.zeros((1, T), f32)
                    for a in range(4):
                        src = m[4 * b + a:4 * b + a + 1, :]
                        shift = (SUB * (a - i)) % T
                        row = jnp.where(block == a, src if shift == 0 else pltpu.roll(src, shift, 1), row)
                    mxp[2 + tt * H + 4 * b + i] = _shift_words(jnp.broadcast_to(row, (8, T)), b == NQUAD - 1)
            return carry

        lax.fori_loop(0, S // T, pack_tile, 0)

    for c in (xa_copy, wka_copy, xb_copy, wkb_copy, wq_copy, wv_copy):
        c.start()
    wot[:, 4 * T:5 * T] = jnp.zeros((half, T), u32)
    pk, pq = {}, {}
    sq = [[], []]

    def sq_tie(i, n, parts):
        rows = -(-D // (16 * parts)) * 16
        part = col_sq_part(i, n * rows, min(D, (n + 1) * rows))
        sq[i].append(part)
        return tie_of(part)

    build_query_masks()
    with _scope('p0_wait'):
        xa_copy.wait()
    with _scope('p0'):
        normalize(0, 0, ln_stats(0, 0))
    with _scope('p1_wait'):
        wka_copy.wait()
    with _scope('p1'):
        wt[0:KSPLIT // 2, :] = _to_u32(wstage[0, :, 0:KSPLIT].T)
        ka = [keys_raw(0, 0, 0, KSPLIT)]
    with _scope('p1b_wait'):
        xb_copy.wait()
    with _scope('p1b'):
        for tt in range(1, NT):
            normalize(0, tt, ln_stats(0, tt))
            if tt < NT - 1:
                ka.append(keys_raw(0, tt, 0, KSPLIT))
    with _scope('p1c_wait'):
        wkb_copy.wait()
    with _scope('p1c'):
        ka.append(keys_raw(0, NT - 1, 0, KSPLIT))
        wt[KSPLIT // 2:half, :] = _to_u32(wstage[0, :, KSPLIT:D].T)
        kb = []
        for tt in range(NT - 1):
            kb.append(keys_raw(0, tt, KSPLIT, D))
            if tt > 0:
                pk[0, tt - 1] = keys_finish(0, tt - 1, jnp.concatenate([ka[tt - 1], kb[tt - 1]], axis=0),
                                            sq_tie(0, tt - 1, 2))
    with _scope('p2_wait'):
        wq_copy.wait()
    for c in (xr_copy, beta_copy, wr_copy, wo_copy):
        c.start()
    with _scope('p2'):
        k2 = jnp.concatenate([ka[2], kb[2]], axis=0)
        k3 = jnp.concatenate([ka[3], keys_raw(0, 3, KSPLIT, D)], axis=0)
        wt[half:2 * half, :] = transpose_weight(1)
        pk[0, 2] = keys_finish(0, 2, k2)
        project_q(0, 0, sq_tie(1, 0, 3))
        pk[0, 3] = keys_finish(0, 3, k3)
        for tt in range(1, NT - 1):
            project_q(0, tt, sq_tie(1, tt, 3))
    with _scope('p3_wait'):
        wv_copy.wait()
    with _scope('p3'):
        wt[2 * half:3 * half, :] = transpose_weight(2)
        project_q(0, NT - 1)
        for tt in range(NT - 1):
            project_v(0, tt)
        csq = [col_sq_max(parts) for parts in sq]
        bound = (QSCALE * LN_NORM2 * DH) * jnp.sqrt(csq[0] * csq[1])
        for low in range(2):
            words = _shift_words(jnp.broadcast_to(bound, (8, T)), low == 1)
            mx[low] = words
            mxp[low] = words
        shift_sel = jnp.max(jnp.where(bound <= LOGIT_LIMIT, 0, 1))
        unsafe = shift_sel > 0
    for c in moe_copies:
        c.start()
    with _scope('p4_wait'):
        for c in (xr_copy, beta_copy, wr_copy, wo_copy):
            c.wait()

    @pl.when(unsafe)
    def _():
        row_maxima()

    project_v(0, NT - 1)
    gb[...] = _sigmoid(jnp.broadcast_to(beta_ref[...].astype(f32).reshape(1, H), (T, H)).T)

    slots = {}
    st = {}

    def at(s, b, j, fn):
        slots.setdefault((s, b, j), []).append(fn)

    def at_pos(s, pos, fn):
        at(s, pos // NT, pos % NT, fn)

    def wr_lhs():
        if 'wr' not in st:
            w = jnp.broadcast_to(wr_ref[...].astype(f32).reshape(1, D), (16, D))
            st['wr'] = jnp.where(_iota((16, D), 0) == 0, w, 0.0).astype(bf16)
        return st['wr']

    stats = {}

    def stats_task(s, tt):
        def fn():
            stats[s, tt] = ln_stats(s, tt)
            inv = jnp.broadcast_to(stats[s, tt][1], (8, T))
            ties.append((clock[0] + CFG['tie_ln'], _zero_bits_after(_to_u32(inv))))
        return fn

    def norm_task(s, tt):
        return lambda: normalize(s, tt, stats[s, tt])

    def score_task(s, tt):
        return lambda: router_scores(wr_lhs(), s, tt)

    for s in range(NSEG - 1):
        for g in range(NGRP):
            at_pos(s, CFG['upd_pos'][g], lambda s=s, g=g: memory_update(s, g, [pk[s, tt] for tt in range(NT)]))
        if s == 0:
            at_pos(0, 3, stats_task(1, 0))
            at_pos(0, 5, norm_task(1, 0))
        for tt in range(NT):
            p0 = 9 + 6 * tt
            if s == 0:
                at_pos(s, p0, stats_task(2, tt))
                if tt > 0:
                    at_pos(s, p0, norm_task(3, tt - 1))
            at_pos(s, p0, lambda s=s, tt=tt: pk.__setitem__((s + 1, tt), project_k(s + 1, tt)))
            if s == 0:
                if tt > 0:
                    at_pos(s, p0, score_task(3, tt - 1))
                at_pos(s, p0 + 2, norm_task(2, tt))
                if tt + 1 < NT:
                    at_pos(s, p0 + 2, stats_task(1, tt + 1))
            at_pos(s, p0 + 2, lambda s=s, tt=tt: pq.__setitem__((s + 1, tt), project_q(s + 1, tt)))
            if s == 0:
                at_pos(s, p0 + 2, score_task(2, tt))
                if tt + 1 < NT:
                    at_pos(s, p0 + 4, norm_task(1, tt + 1))
                at_pos(s, p0 + 4, stats_task(3, tt))
            at_pos(s, p0 + 4, lambda s=s, tt=tt: project_v(s + 1, tt))
            at_pos(s, p0 + CFG['read_off'], lambda s=s, tt=tt: memory_read(s + 1, tt, pq[s + 1, tt]))
    at_pos(1, 0, norm_task(3, NT - 1))
    for s in range(EARLY):
        for tt in range(NT):
            at_pos(*CFG['early_pos'][s][tt], lambda s=s, tt=tt: out_project_early(s, tt))
    at_pos(1, 1, score_task(3, NT - 1))
    for tt in range(NT):
        at_pos(0, 1 + 2 * tt, score_task(0, tt))
        at_pos(0, 10 + 6 * tt, score_task(1, tt))

    def set_out_weight():
        wot[:, 0:D] = transpose_weight(3)
        produced('wot')

    at_pos(*CFG['wot_pos'], set_out_weight)

    at_pos(1, 2, lambda: st.update(zip(('ids', 'sel'), route())))
    at_pos(1, CFG['select_pos'], lambda: st.update(xsel=select_tokens(st['ids'])))

    def start_moe():
        with _scope('moe_wait'):
            for c in moe_copies:
                c.wait()
        queue_moe(st['xsel'], st)

    at(1, CFG['moe_quad'], -1, start_moe)

    def finish_moe():
        fill(len(fillers))
        y = moe_result(st['sel'], jnp.concatenate(st['ycols'], axis=1))
        patch_early(st['ids'], y)
        st['lhs'] = out_lhs(st['ids'], y)

    e0 = CFG['moe_end']
    at_pos(3, e0, finish_moe)
    for s in range(EARLY):
        at_pos(3, e0 + 1 + s, lambda s=s: out_copy(s * L, (s + 1) * L, s).start())
    for tt in range(NT):
        at_pos(3, e0 + 2 + CFG['op_gap'] * tt, lambda tt=tt: out_project(st['lhs'], 2, tt))
    at_pos(3, e0 + 3 + CFG['op_gap'] * (NT - 1), lambda: out_copy(2 * L, 3 * L, 2).start())

    def quad_values(s, b, j, ps):
        for a in range(4):
            values(s, 4 * b + a, j, ps[a])

    pending = []
    for s in range(NSEG):
        for b in range(NQUAD):
            for fn in slots.pop((s, b, -1), ()):
                fn()
            for j in range(NT):
                pending.append((s, b, j, scores(s, b, j)))
                for fn in slots.pop((s, b, j), ()):
                    fn()
                if len(pending) > CFG['lag']:
                    quad_values(*pending.pop(0))
    assert not slots, slots.keys()
    s = NSEG - 1

    def last_tile(tt):
        out_project(st['lhs'], s, tt, CFG['tail_parts'][tt])
        out_copy(s * L + tt * T, s * L + (tt + 1) * T, 3 + tt).start()

    done = 0
    for unit in pending:
        quad_values(*unit)
        while done < NT and unit[1] == NQUAD - 1 and done < unit[2]:
            last_tile(done)
            done += 1
    while done < NT:
        last_tile(done)
        done += 1
    with _scope('out_wait'):
        for k in range(NSEG - 1):
            out_copy(k * L, (k + 1) * L, k).wait()
        for tt in range(NT):
            out_copy(s * L + tt * T, s * L + (tt + 1) * T, 3 + tt).wait()


@jax.jit
def pallas_parallel_sum__memory_aug_infini_attn__moe_arch_mod__prompt_kernel(
    A_x: jax.Array,
    A_wq: jax.Array,
    A_wk: jax.Array,
    A_wv: jax.Array,
    A_wo: jax.Array,
    A_beta: jax.Array,
    B_x: jax.Array,
    B_w_r: jax.Array,
    B_w_gate: jax.Array,
    B_w_up: jax.Array,
    B_w_down: jax.Array,
):
    del B_x
    x_t = jnp.transpose(A_x, (0, 2, 1)).reshape(D, S)
    wd_t = B_w_down.T
    hbm = pl.BlockSpec(memory_space=pl.ANY)
    out_t = pl.pallas_call(
        _kernel,
        out_shape=jax.ShapeDtypeStruct((D, S), bf16),
        in_specs=[hbm] * 10,
        out_specs=hbm,
        scratch_shapes=[
            pltpu.VMEM((D, S), bf16),
            pltpu.VMEM((D, S), f32),
            pltpu.VMEM((4, D, D), bf16),
            pltpu.VMEM((3 * D // 2, D), u32),
            pltpu.VMEM((D // 2, 5 * T), u32),
            pltpu.VMEM((D, F), bf16),
            pltpu.VMEM((D, F), bf16),
            pltpu.VMEM((D, F), bf16),
            pltpu.VMEM((H,), bf16),
            pltpu.VMEM((D,), bf16),
            pltpu.VMEM((2, D // 2, L), u32),
            pltpu.VMEM((2, D, L), f32),
            pltpu.VMEM((2, NQUAD, L // 2, T), u32),
            pltpu.VMEM((2, NGRP, MROWS, L), f32),
            pltpu.VMEM((NGRP, MROWS, T), f32),
            pltpu.VMEM((NGRP, 8, T), f32),
            pltpu.VMEM((NSEG, 5 * T, L), f32),
            pltpu.VMEM((2 + H * S // T, 8, T), u32),
            pltpu.VMEM((2 + H * S // T, 8, T), u32),
            pltpu.VMEM((H, S), f32),
            pltpu.VMEM((NQUAD, 16, 8, T), u32),
            pltpu.VMEM((S // T, T), f32),
            pltpu.VMEM((D, S), bf16),
            pltpu.VMEM((H, T), f32),
            pltpu.VMEM((D, S), bf16),
            pltpu.VMEM((D, S), bf16),
            pltpu.SemaphoreType.DMA((20,)),
        ],
        compiler_params=pltpu.CompilerParams(vmem_limit_bytes=100 * 1024 * 1024),
        name="infini_moe",
    )(x_t, A_wq, A_wk, A_wv, A_wo, A_beta, B_w_r, B_w_gate, B_w_up, wd_t)
    return jnp.transpose(out_t.reshape(1, D, S), (0, 2, 1))
```

```python
import contextlib
import functools

import jax
import jax.numpy as jnp
from jax import lax
from jax.experimental import pallas as pl
from jax.experimental.pallas import tpu as pltpu

S, D, H, DH = 2048, 576, 32, 18
NSEG, L, F = 4, 512, 4608
T = 128
NT = L // T
NGRP = 5
SLAB = 112
GROUP_FIRST = (0, 7, 13, 19, 25, 32)
MROWS = 144
NCHUNK = F // T
NQUAD = H // 4
QUAD_OFF = (0, 64, 144, 208, 288, 352, 432, 448)
EARLY = 2
KSPLIT = 256
SUB = 32

bf16, f32, u32, i32 = jnp.bfloat16, jnp.float32, jnp.uint32, jnp.int32

LOG2E = 1.4426950408889634
QSCALE = (DH ** -0.5) * LOG2E
LN_NORM2 = 2.1 * D
LOGIT_LIMIT = 50.0
NEG_BIG = -1e30


PROFILE_SCOPES = False
CFG = dict(
    lag=5,
    tie_p=3,
    tie_res=3,
    tie_ln=1,
    fill_proj=10,
    fill_qk=8,
    select_pos=7,
    moe_quad=5,
    moe_end=8,
    op_gap=3,
    read_off=4,
    upd_pos=(0, 2, 4, 6, 8),
    early_pos=(((1, 8), (1, 14), (1, 20), (1, 26)), ((2, 3), (2, 5), (2, 7), (2, 9))),
    wot_pos=(0, 22),
    moe_delay=2,
    splits={('q', 0, 2, 0): 4, ('v', 0, 2, 0): 4, ('k', 0, 2, 256): 4, ('k', 0, 2, 0): 4, ('k', 0, 0, 0): 4},
    tail_parts=(1, 1, 1, 9),
)


def _scope(name):
    return jax.named_scope(name) if PROFILE_SCOPES else contextlib.nullcontext()


def _group_of(h):
    for g in range(NGRP):
        if GROUP_FIRST[g] <= h < GROUP_FIRST[g + 1]:
            return g
    raise ValueError(h)


def _to_bf16(x):
    return pltpu.bitcast(x, bf16)


def _to_u32(x):
    return pltpu.bitcast(x, u32)


def _round_bf16(x):
    return x.astype(bf16).astype(f32)


def _iota(shape, dim):
    return lax.broadcasted_iota(i32, shape, dim)


def _dot(a, b):
    return jnp.dot(a, b, preferred_element_type=f32)


def _dot_nt(a, b):
    return lax.dot_general(a, b, (((1,), (1,)), ((), ())), preferred_element_type=f32)


def _dot_tn(a, b):
    return lax.dot_general(a, b, (((0,), (0,)), ((), ())), preferred_element_type=f32)


def _pack_pairs(x):
    lo = jnp.concatenate([x[r:r + 8] for r in range(0, x.shape[0], 16)], axis=0)
    hi = jnp.concatenate([x[r + 8:r + 16] for r in range(0, x.shape[0], 16)], axis=0)
    return pltpu.pack_elementwise([lo, hi], packed_dtype=bf16)


def _unpaired_index(r):
    x = r & 15
    return (r - x) + jnp.where(x < 8, 2 * x, 2 * (x - 8) + 1)


def _zero_bits_after(u):
    sixteen = jnp.full(u.shape, 16, u32)
    return lax.shift_right_logical(lax.shift_right_logical(u, sixteen), sixteen)


def _pair_mask(first, lo, hi, keep_lane=None):
    f = _iota((8, T), 0) + first
    low = (f >= lo) & (f < hi)
    high = (f + 8 >= lo) & (f + 8 < hi)
    if keep_lane is not None:
        low, high = low & keep_lane, high & keep_lane
    return jnp.where(low, jnp.uint32(0xFFFF), jnp.uint32(0)) | jnp.where(high, jnp.uint32(0xFFFF0000), jnp.uint32(0))


def _bf16_bits(x):
    return pltpu.bitcast(_round_bf16(x), u32)


def _shift_words(m, low_half):
    first = _round_bf16(-m)
    second = _round_bf16(-m - first)
    third = -m - first - second
    row = _iota((8, T), 0)
    val = jnp.where(row == 5, first, jnp.where(row == 6, second, jnp.where(row == 7, third, 0.0)))
    bits = _bf16_bits(val)
    return lax.shift_right_logical(bits, jnp.full(bits.shape, 16, u32)) if low_half else bits


def _phi(t):
    return jnp.where(t > 0, t + 1.0, jnp.exp(t))


def _sigmoid(t):
    return _round_bf16(1.0 / _round_bf16(1.0 + _round_bf16(jnp.exp(-t))))


def _finish_stats(x0, sum1, sum2):
    s1 = sum1 / D
    var = jnp.maximum(sum2 / D - s1 * s1, 0.0)
    eps = _round_bf16(jnp.full((1, 1), 1e-5, f32))
    sd = _round_bf16(jnp.sqrt(_round_bf16(_round_bf16(var) + eps)))
    return _round_bf16(x0 + s1), 1.0 / sd


def _layernorm_stats(xb):
    x0 = xb[0:1, :].astype(f32)
    acc1, acc2 = [None] * 4, [None] * 4
    for n, r in enumerate(range(0, D, 16)):
        c = xb[r:r + 16, :].astype(f32) - x0
        for part in range(2):
            k = (2 * n + part) % 4
            piece = c[8 * part:8 * part + 8, :]
            acc1[k] = piece if acc1[k] is None else acc1[k] + piece
            acc2[k] = piece * piece if acc2[k] is None else acc2[k] + piece * piece
    return _finish_stats(x0, jnp.sum((acc1[0] + acc1[1]) + (acc1[2] + acc1[3]), axis=0, keepdims=True),
                         jnp.sum((acc2[0] + acc2[1]) + (acc2[2] + acc2[3]), axis=0, keepdims=True))


def _layernorm_apply(xb, stats):
    mean, inv = stats
    return _round_bf16(xb.astype(f32) - mean) * inv


def _block_transpose(xs):
    lane = _iota(next(x for x in xs if x is not None).shape, 1)

    def exchange(u, v, low, shift):
        def pick(p, q):
            if p is None and q is None:
                return None
            return jnp.where(low, 0.0 if p is None else p, 0.0 if q is None else q)
        ru = None if u is None else pltpu.roll(u, T - shift, 1)
        rv = None if v is None else pltpu.roll(v, shift, 1)
        return pick(u, rv), pick(ru, v)

    y0, y2 = exchange(xs[0], xs[2], lane < 64, 64)
    y1, y3 = exchange(xs[1], xs[3], lane < 64, 64)
    low = (lane & 32) == 0
    z0, z1 = exchange(y0, y1, low, 32)
    z2, z3 = exchange(y2, y3, low, 32)
    return [z0, z1, z2, z3]


def _head_of_slab_index(idx, g):
    return ((idx + SLAB * g) * 3641) >> 16


def _zero_after(x):
    sign = lax.shift_right_logical(pltpu.bitcast(x, i32), 31)
    return sign.astype(f32) * 0.0


def _kernel(x_hbm, wq_hbm, wk_hbm, wv_hbm, wo_hbm, beta_hbm, wr_hbm, wg_hbm, wu_hbm, wd_hbm,
            out_hbm,
            xt, xn, wstage, wt, wot, wg, wu, wd, beta_ref, wr_ref, qt, vt, kp, num, mt, zt, ot,
            mx, mxp, mrow, qmask, rrow, outb, gb, ybuf, kq, sems):
    def copy(src, dst, i):
        return pltpu.make_async_copy(src, dst, sems.at[i])

    xa_copy = copy(x_hbm.at[:, 0:T], xt.at[:, 0:T], 0)
    xb_copy = copy(x_hbm.at[:, T:L], xt.at[:, T:L], 18)
    xr_copy = copy(x_hbm.at[:, L:S], xt.at[:, L:S], 1)
    wq_copy, wv_copy, wo_copy = [
        copy(w, wstage.at[i], 2 + i) for i, w in ((1, wq_hbm), (2, wv_hbm), (3, wo_hbm))]
    wka_copy = copy(wk_hbm.at[:, 0:KSPLIT], wstage.at[0, :, 0:KSPLIT], 2)
    wkb_copy = copy(wk_hbm.at[:, KSPLIT:D], wstage.at[0, :, KSPLIT:D], 19)
    beta_copy = copy(beta_hbm, beta_ref, 6)
    wr_copy = copy(wr_hbm, wr_ref, 7)
    moe_copies = [copy(wg_hbm, wg, 8), copy(wu_hbm, wu, 9), copy(wd_hbm, wd, 10)]

    def out_copy(lo, hi, i):
        return copy(outb.at[:, lo:hi], out_hbm.at[:, lo:hi], 11 + i)

    half = D // 2
    emitted = set()

    def produced(*key):
        emitted.add(key)

    def require(*key):
        assert key in emitted, key

    def require_heads(s, j):
        for h in range(H):
            require('ot', s, h, j)

    fillers = []

    def fill(n):
        for _ in range(min(n, len(fillers))):
            fillers.pop(0)()

    clock = [0]
    ties = []

    def tile_cols(s, tt):
        return slice(s * L + tt * T, s * L + (tt + 1) * T)

    def local_cols(tt):
        return slice(tt * T, (tt + 1) * T)

    def col_sq_part(i, lo, hi):
        acc = None
        for r in range(lo, hi, 16):
            w = wstage[i, r:r + 16, :].astype(f32)
            w = w * w
            part = w[0:8] + w[8:16]
            acc = part if acc is None else acc + part
        return acc

    def col_sq_max(parts):
        acc = functools.reduce(lambda u, v: u + v, parts)
        return jnp.max(jnp.sum(acc, axis=0, keepdims=True), axis=1, keepdims=True)

    def tie_of(part):
        folded = functools.reduce(lambda u, v: u + v, [part[:, c:c + T] for c in range(0, 4 * T, T)])
        return _zero_after(folded[0:1, 0:1] + part[0:1, 4 * T:4 * T + 1])

    def transpose_weight(i):
        return _to_u32(wstage[i].T)

    def ln_stats(s, tt):
        return _layernorm_stats(xt[:, tile_cols(s, tt)])

    def normalize(s, tt, stats):
        cs = tile_cols(s, tt)
        xn[:, cs] = _layernorm_apply(xt[:, cs], stats)
        produced('xn', s, tt)

    def xn_tile(s, tt):
        require('xn', s, tt)
        return xn[:, tile_cols(s, tt)].astype(bf16)

    def project(base, lo, hi, name, s, tt):
        rhs = xn_tile(s, tt)
        parts = CFG['splits'].get((name, s, tt, lo), 1)
        step = (hi - lo) // parts
        out = [_dot(_to_bf16(wt[(base + r) // 2:(base + r + step) // 2, :]), rhs) for r in range(lo, hi, step)]
        fill(CFG['fill_proj'])
        return out[0] if parts == 1 else jnp.concatenate(out, axis=0)

    def keys_raw(s, tt, lo=0, hi=D):
        return project(0, lo, hi, 'k', s, tt)

    def keys_finish(s, tt, kt, tie=None):
        if tie is not None:
            kt = kt + tie
        words = jnp.take_along_axis(_pack_pairs(kt), _unpaired_index(_iota((half, T), 1)), axis=1)
        shift_rows = _iota((8, T), 0) >= 5
        for b in range(NQUAD):
            slab = words[QUAD_OFF[b] // 2:QUAD_OFF[b] // 2 + T // 2, :]
            if b == NQUAD - 1:
                ones = jnp.where(shift_rows, (slab[0:8] & jnp.uint32(0xFFFF0000)) | jnp.uint32(0x3F80), slab[0:8])
                slab = jnp.concatenate([ones, slab[8:]], axis=0)
            else:
                ones = jnp.where(shift_rows, (slab[56:64] & jnp.uint32(0xFFFF)) | jnp.uint32(0x3F800000), slab[56:64])
                slab = jnp.concatenate([slab[:56], ones], axis=0)
            kp[s % 2, b, tt * (T // 2):(tt + 1) * (T // 2), :] = _to_u32(_to_bf16(slab).T)
        produced('k', s, tt)
        return _phi(kt).astype(bf16)

    def project_k(s, tt):
        return keys_finish(s, tt, keys_raw(s, tt))

    def project_q(s, tt, tie=None):
        q = project(D, 0, D, 'q', s, tt)
        qt[s % 2, :, local_cols(tt)] = _pack_pairs(q * (QSCALE if tie is None else QSCALE + tie))
        produced('q', s, tt)
        return _phi(q).astype(bf16)

    def require_segment_done(s):
        if s >= 0:
            for j in range(NT):
                require_heads(s, j)

    def project_v(s, tt):
        require_segment_done(s - 2)
        v = project(2 * D, 0, D, 'v', s, tt)
        vt[s % 2, :, local_cols(tt)] = v
        produced('v', s, tt)

    def router_scores(lhs, s, tt):
        row = s * NT + tt
        rrow[row:row + 1, :] = _dot(lhs, xn_tile(s, tt))[0:1, :]
        produced('r', s, tt)

    def memory_read(s, tt, pq):
        require_segment_done(s - 2)
        for g in range(NGRP):
            require('mt', s - 1, g)
        for g in range(NGRP):
            num[s % 2, g, :, local_cols(tt)] = _dot(mt[g].astype(bf16), pq[SLAB * g:SLAB * g + T, :])
        produced('num', s, tt)

    def memory_update(s, g, pk):
        ones_row = 0 if g == NGRP - 1 else T - 1
        vs = jnp.where(_iota((T, L), 0) == ones_row, 1.0, vt[s % 2, SLAB * g:SLAB * g + T, :]).astype(bf16)
        m = _dot_nt(vs, jnp.concatenate([p[SLAB * g:SLAB * g + T, :] for p in pk], axis=1))
        hr = _head_of_slab_index(_iota((T, T), 0), g)
        hc = _head_of_slab_index(_iota((T, T), 1), g)
        keep = (hr == hc) & (hr >= GROUP_FIRST[g]) & (hr < GROUP_FIRST[g + 1])
        mm = jnp.where(keep, m, 0.0)
        z = m[ones_row:ones_row + 1, :]
        if s > 0:
            mm = mm + mt[g, 0:T, :]
            z = z + zt[g, 0:1, :]
        mt[g, 0:T, :] = mm
        zt[g, 0:1, :] = z
        zsel = _head_of_slab_index(_iota((16, T), 1), g) == _iota((16, T), 0) + GROUP_FIRST[g]
        mt[g, T:MROWS, :] = jnp.where(zsel, z, 0.0)
        produced('mt', s, g)

    def head_groups(b, a):
        f = DH * (4 * b + a) - QUAD_OFF[b]
        return f, (f // 16, f // 16 + 1)

    def build_query_masks():
        block = _iota((8, T), 1) // SUB
        for b in range(NQUAD):
            for a in range(4):
                f, groups = head_groups(b, a)
                for n, g in enumerate(groups):
                    qmask[b, 4 * a + 2 * n] = _pair_mask(16 * g, f, f + DH)
                    qmask[b, 4 * a + 2 * n + 1] = _pair_mask(16 * g, f, f + DH, block == a)

    def stack_groups(groups):
        return _to_bf16(jnp.concatenate(
            [groups.get(g, jnp.zeros((8, T), u32)) for g in range(T // 16)], axis=0))

    def quad_queries(s, b, j, tie):
        tile = s * NT + j
        last = b == NQUAD - 1
        shift_group = 0 if last else T // 16 - 1
        base = QUAD_OFF[b] // 2
        words = {}

        def group(g):
            if g not in words:
                words[g] = qt[s % 2, base + 8 * g:base + 8 * g + 8, local_cols(j)]
            return words[g]

        wide = []
        for a in range(4):
            _, groups = head_groups(b, a)
            parts = {g: group(g) & qmask[b, 4 * a + 2 * n] for n, g in enumerate(groups)}
            if j > 0:
                parts[shift_group] = mx[int(last) + shift_sel * (2 - int(last) + (4 * b + a) * (S // T) + tile)]
                wide.append(stack_groups(parts))
        packed = []
        for i in range(4):
            parts = {}
            for a in range(4):
                _, groups = head_groups(b, a)
                shift = (SUB * (a - i)) % T
                for n, g in enumerate(groups):
                    moved = group(g) if shift == 0 else pltpu.roll(group(g), shift, 1)
                    piece = moved & qmask[b, 4 * a + 2 * n + 1]
                    parts[g] = piece if g not in parts else parts[g] | piece
            rows = mxp[int(last) + shift_sel * (2 - int(last) + tile * H + 4 * b + i)]
            if tie is not None and i == 3:
                rows = rows | tie
            parts[shift_group] = rows
            packed.append(stack_groups(parts))
        return wide, packed

    def scores(s, b, j):
        require('q', s, j)
        for tt in range(j + 1):
            require('k', s, tt)
        tie = None
        unit = clock[0] = (s * NQUAD + b) * NT + j
        due = [z for when, z in ties if when <= unit]
        ties[:] = [(when, z) for when, z in ties if when > unit]
        if due:
            tie = functools.reduce(lambda u, v: u | v, due)
        wide, packed = quad_queries(s, b, j, tie)
        k0 = j * (T // 2)
        off = None
        if j > 0:
            logits = _dot(_to_bf16(kp[s % 2, b, 0:k0, :]), jnp.concatenate(wide, axis=1))
            fill(CFG['fill_qk'])
            off = jnp.exp2(logits)
        causal = _unpaired_index(_iota((SUB, T), 0)) <= (_iota((SUB, T), 1) & (SUB - 1))
        diag = [None] * 4
        for i in range(4):
            n = SUB * (i + 1)
            e = jnp.exp2(_dot(_to_bf16(kp[s % 2, b, k0:k0 + n // 2, :]), packed[i]))
            blocks = [e[r * SUB:(r + 1) * SUB, :] for r in range(i)]
            blocks.append(jnp.where(causal, e[i * SUB:, :], 0.0))
            diag[i] = blocks
        per_head = [[] for _ in range(4)]
        for r in range(4):
            outs = _block_transpose([diag[i][r] if i >= r else None for i in range(4)])
            for a in range(4):
                per_head[a].append(outs[a])
        ps = []
        for a in range(4):
            parts = ([off[:, a * T:(a + 1) * T]] if j > 0 else []) + per_head[a]
            ps.append(_pack_pairs(jnp.concatenate(parts, axis=0)))
        rows = [u[r:r + 8] for u in ps for r in range(0, u.shape[0], 8)]
        while len(rows) > 1:
            rows = [rows[i] | rows[i + 1] for i in range(0, len(rows) - 1, 2)] + rows[len(rows) & ~1:]
        ties.append((unit + CFG['tie_p'], _zero_bits_after(rows[0])))
        return [_to_bf16(u) for u in ps]

    def values(s, h, j, p):
        g = _group_of(h)
        w0 = min((DH * h // 16) * 16, D - 32)
        off = DH * h - w0
        ones_row = 31 if off < 14 else 0
        n = (j + 1) * T
        cs = local_cols(j)
        for tt in range(j + 1):
            require('v', s, tt)
        if s > 0:
            require('num', s, j)
        g0 = (ones_row // 8) * 8
        marked = jnp.where(_iota((8, n), 0) == ones_row - g0, 1.0, vt[s % 2, w0 + g0:w0 + g0 + 8, 0:n])
        rest = vt[s % 2, w0 + 8:w0 + 32, 0:n] if g0 == 0 else vt[s % 2, w0:w0 + 24, 0:n]
        vwin = jnp.concatenate([marked, rest] if g0 == 0 else [rest, marked], axis=0).astype(bf16)
        gate = gb[h:h + 1, :]
        acc = _dot(vwin, p)
        res = acc * ((1.0 - gate) / acc[ones_row:ones_row + 1, :])
        if s > 0:
            m0 = w0 - SLAB * g
            zr = T + h - GROUP_FIRST[g]
            den = num[s % 2, g, zr:zr + 1, cs] + 1e-6
            res = res + num[s % 2, g, m0:m0 + 32, cs] * (gate / den)
        else:
            folded = (res[0:8] + res[8:16]) + (res[16:24] + res[24:32])
            ties.append((clock[0] + CFG['tie_res'], _zero_bits_after(_to_u32(folded))))
        ot[s, DH * h:DH * h + DH, cs] = res[off:off + DH, :]
        produced('ot', s, h, j)

    def route():
        for s in range(NSEG):
            for tt in range(NT):
                require('r', s, tt)
        r = _round_bf16(rrow[...])
        idx = _iota((S // T, T), 0) * T + _iota((S // T, T), 1)
        m1 = jnp.max(r)
        i1 = jnp.min(jnp.where(r == m1, idx, S - 1))
        r2 = jnp.where(idx == i1, -jnp.inf, r)
        m2 = jnp.max(r2)
        i2 = jnp.min(jnp.where(r2 == m2, idx, S - 1))
        return (i1, i2), (m1, m2)

    def select_tokens(ids):
        sel = None
        for row, i in enumerate(ids):
            hit = (_iota((16, T), 0) == row) & (_iota((16, T), 1) == i % T)
            cs = pl.ds(pl.multiple_of((i // T) * T, T), T)
            part = _dot_nt(jnp.where(hit, 1.0, 0.0).astype(bf16), xn[:, cs].astype(bf16))
            sel = part if sel is None else sel + part
        return sel.astype(bf16)

    def queue_moe(xsel, state):
        ktiles = [(k, min(k + T, D)) for k in range(0, D, T)]
        pre, hid = {}, {}
        ycols = state['ycols'] = [None] * len(ktiles)

        def first(w, name, c, lo, hi):
            def fn():
                part = _dot(xsel[:, lo:hi], w[lo:hi, c * T:(c + 1) * T])
                pre[name, c] = part if lo == 0 else pre[name, c] + part
            return fn

        def down(c, n, lo, hi):
            def fn():
                if c not in hid:
                    gpre = _round_bf16(pre.pop(('g', c)))
                    gact = _round_bf16(gpre * _sigmoid(gpre))
                    hid[c] = (gact * _round_bf16(pre.pop(('u', c)))).astype(bf16)
                part = _dot_nt(hid[c], wd[lo:hi, c * T:(c + 1) * T])
                ycols[n] = part if ycols[n] is None else ycols[n] + part
            return fn

        delay = CFG['moe_delay']
        for c in range(NCHUNK + delay):
            if c < NCHUNK:
                for lo, hi in ktiles:
                    fillers.append(first(wg, 'g', c, lo, hi))
                    fillers.append(first(wu, 'u', c, lo, hi))
            if c >= delay:
                for n, (lo, hi) in enumerate(ktiles):
                    fillers.append(down(c - delay, n, lo, hi))

    def moe_result(sel_scores, y):
        row = _iota((16, D), 0)
        gate = jnp.where(row == 0, sel_scores[0], sel_scores[1])
        return (_round_bf16(y) * _sigmoid(gate)).astype(bf16)

    def patch_early(ids, y):
        for k, i in enumerate(ids):
            hit = (_iota((16, T), 0) == k) & (_iota((16, T), 1) == i % T) & (i < EARLY * L)
            cs = pl.ds(pl.multiple_of((jnp.minimum(i, EARLY * L - 1) // T) * T, T), T)
            patch = _dot_tn(y, jnp.where(hit, 1.0, 0.0).astype(bf16))
            outb[:, cs] = (outb[:, cs].astype(f32) + patch).astype(bf16)

    def out_lhs(ids, y):
        place = (_iota((16, T), 1) == _iota((16, T), 0) + 64) & (_iota((16, T), 0) < 2)
        ycols = _dot_tn(y, jnp.where(place, 1.0, 0.0).astype(bf16))
        last = _to_bf16(wot[:, 4 * T:5 * T]).astype(f32) + ycols
        for s in range(EARLY, NSEG):
            tok = _iota((64, L), 1) + s * L
            rows = _iota((64, L), 0)
            hit = ((rows == 0) & (tok == ids[0])) | ((rows == 1) & (tok == ids[1]))
            ot[s, D:D + 64, :] = jnp.where(hit, 1.0, 0.0)
        return jnp.concatenate([_to_bf16(wot[:, 0:4 * T]), last.astype(bf16)], axis=1)

    def out_project_early(s, tt):
        require_heads(s, tt)
        require('wot')
        cs = tile_cols(s, tt)
        attn = _dot(_to_bf16(wot[:, 0:D]), ot[s, 0:D, local_cols(tt)].astype(bf16))
        fill(CFG['fill_proj'])
        outb[:, cs] = (attn + xn[:, cs] + xt[:, cs].astype(f32)).astype(bf16)

    def out_project(lhs, s, tt, parts=1):
        require_heads(s, tt)
        cs = tile_cols(s, tt)
        rhs = ot[s, :, local_cols(tt)].astype(bf16)
        for r in range(0, D, D // parts):
            rows = slice(r, r + D // parts)
            attn = _dot(lhs[rows, :], rhs)
            outb[rows, cs] = (attn + xn[rows, cs] + xt[rows, cs].astype(f32)).astype(bf16)

    def row_maxima():
        def lanes(tt):
            return pl.ds(pl.multiple_of(tt * T, T), T)

        def normalize_tile(tt, carry):
            cs = lanes(tt)
            x0 = xt[0:16, cs].astype(f32)[0:1, :]

            def block(n):
                return pl.ds(pl.multiple_of(n * 16, 16), 16)

            def moments(n, acc):
                c = xt[block(n), cs].astype(f32) - x0
                return acc[0] + c, acc[1] + c * c

            zero = jnp.zeros((16, T), f32)
            a1, a2 = lax.fori_loop(0, D // 16, moments, (zero, zero))
            mean, inv = _finish_stats(x0, jnp.sum(a1, axis=0, keepdims=True), jnp.sum(a2, axis=0, keepdims=True))

            def apply(n, c):
                ybuf[block(n), cs] = _layernorm_apply(xt[block(n), cs], (mean, inv)).astype(bf16)
                return c

            return lax.fori_loop(0, D // 16, apply, carry)

        lax.fori_loop(0, S // T, normalize_tile, 0)

        def project_block(i, carry):
            cs = lanes(i // 9)
            rb = i % 9
            w = wt[pl.ds(pl.multiple_of(rb * (T // 2), T // 2), T // 2), :]
            scale = jnp.where(_iota((T, T), 0) + rb * T >= D, QSCALE, 1.0)
            kq[pl.ds(pl.multiple_of(rb * T, T), T), cs] = (_dot(_to_bf16(w), ybuf[:, cs]) * scale).astype(bf16)
            return carry

        lax.fori_loop(0, 9 * (S // T), project_block, 0)

        def head_tile(i, carry):
            h = i // (S // T)
            tt = i % (S // T)
            first = jnp.minimum((72 * (h // 4) // 16) * 16, D - T)
            rows = _iota((T, T), 0) + first
            q = kq[pl.ds(pl.multiple_of(D + first, 16), T), lanes(tt)].astype(f32)
            qm = jnp.where((rows >= DH * h) & (rows < DH * h + DH), q, 0.0).astype(bf16)

            def key_tile(kt, m):
                k = kq[pl.ds(pl.multiple_of(first, 16), T), lanes((tt // NT) * NT + kt)]
                seen = _iota((T, T), 0) + kt * T <= _iota((T, T), 1) + (tt % NT) * T
                best = jnp.max(jnp.where(seen, _dot_tn(k, qm), NEG_BIG), axis=0, keepdims=True)
                return jnp.maximum(m, best)

            m = lax.fori_loop(0, tt % NT + 1, key_tile, jnp.full((1, T), NEG_BIG, f32))
            mrow[:, lanes(tt)] = jnp.where(_iota((H, T), 0) == h, m, mrow[:, lanes(tt)])
            wide_m = jnp.broadcast_to(m, (8, T))
            mx[2 + i] = jnp.where(h >= H - 4, _shift_words(wide_m, True), _shift_words(wide_m, False))
            return carry

        mrow[...] = jnp.zeros(mrow.shape, f32)
        lax.fori_loop(0, H * (S // T), head_tile, 0)

        def pack_tile(n, carry):
            tt = n // H
            b = (n % H) // 4
            i = n % 4
            m = mrow[:, lanes(tt)]
            block = _iota((1, T), 1) // SUB
            row = jnp.zeros((1, T), f32)
            for a in range(4):
                src = jnp.sum(jnp.where(_iota((H, T), 0) == 4 * b + a, m, 0.0), axis=0, keepdims=True)
                moved = pltpu.roll(src, (SUB * (a - i) + T) % T, 1)
                row = jnp.where(block == a, moved, row)
            wide_m = jnp.broadcast_to(row, (8, T))
            mxp[2 + n] = jnp.where(b == NQUAD - 1, _shift_words(wide_m, True), _shift_words(wide_m, False))
            return carry

        lax.fori_loop(0, H * (S // T), pack_tile, 0)

    for c in (xa_copy, wka_copy, xb_copy, wkb_copy, wq_copy, wv_copy):
        c.start()
    wot[:, 4 * T:5 * T] = jnp.zeros((half, T), u32)
    pk, pq = {}, {}
    sq = [[], []]

    def sq_tie(i, n, parts):
        rows = -(-D // (16 * parts)) * 16
        part = col_sq_part(i, n * rows, min(D, (n + 1) * rows))
        sq[i].append(part)
        return tie_of(part)

    build_query_masks()
    with _scope('p0_wait'):
        xa_copy.wait()
    with _scope('p0'):
        normalize(0, 0, ln_stats(0, 0))
    with _scope('p1_wait'):
        wka_copy.wait()
    with _scope('p1'):
        wt[0:KSPLIT // 2, :] = _to_u32(wstage[0, :, 0:KSPLIT].T)
        ka = [keys_raw(0, 0, 0, KSPLIT)]
    with _scope('p1b_wait'):
        xb_copy.wait()
    with _scope('p1b'):
        for tt in range(1, NT):
            normalize(0, tt, ln_stats(0, tt))
            if tt < NT - 1:
                ka.append(keys_raw(0, tt, 0, KSPLIT))
    with _scope('p1c_wait'):
        wkb_copy.wait()
    with _scope('p1c'):
        ka.append(keys_raw(0, NT - 1, 0, KSPLIT))
        wt[KSPLIT // 2:half, :] = _to_u32(wstage[0, :, KSPLIT:D].T)
        kb = []
        for tt in range(NT - 1):
            kb.append(keys_raw(0, tt, KSPLIT, D))
            if tt > 0:
                pk[0, tt - 1] = keys_finish(0, tt - 1, jnp.concatenate([ka[tt - 1], kb[tt - 1]], axis=0),
                                            sq_tie(0, tt - 1, 2))
    with _scope('p2_wait'):
        wq_copy.wait()
    for c in (xr_copy, beta_copy, wr_copy, wo_copy):
        c.start()
    with _scope('p2'):
        k2 = jnp.concatenate([ka[2], kb[2]], axis=0)
        k3 = jnp.concatenate([ka[3], keys_raw(0, 3, KSPLIT, D)], axis=0)
        wt[half:2 * half, :] = transpose_weight(1)
        pk[0, 2] = keys_finish(0, 2, k2)
        project_q(0, 0, sq_tie(1, 0, 3))
        pk[0, 3] = keys_finish(0, 3, k3)
        for tt in range(1, NT - 1):
            project_q(0, tt, sq_tie(1, tt, 3))
    with _scope('p3_wait'):
        wv_copy.wait()
    with _scope('p3'):
        wt[2 * half:3 * half, :] = transpose_weight(2)
        project_q(0, NT - 1)
        for tt in range(NT - 1):
            project_v(0, tt)
        csq = [col_sq_max(parts) for parts in sq]
        bound = (QSCALE * LN_NORM2 * DH) * jnp.sqrt(csq[0] * csq[1])
        for low in range(2):
            words = _shift_words(jnp.broadcast_to(bound, (8, T)), low == 1)
            mx[low] = words
            mxp[low] = words
        shift_sel = jnp.max(jnp.where(bound <= LOGIT_LIMIT, 0, 1))
        unsafe = shift_sel > 0
    for c in moe_copies:
        c.start()

    @pl.when(unsafe)
    def _():
        xr_copy.wait()
        row_maxima()
        xr_copy.start()

    with _scope('p4_wait'):
        for c in (xr_copy, beta_copy, wr_copy, wo_copy):
            c.wait()

    project_v(0, NT - 1)
    gb[...] = _sigmoid(jnp.broadcast_to(beta_ref[...].astype(f32).reshape(1, H), (T, H)).T)

    slots = {}
    st = {}

    def at(s, b, j, fn):
        slots.setdefault((s, b, j), []).append(fn)

    def at_pos(s, pos, fn):
        at(s, pos // NT, pos % NT, fn)

    def wr_lhs():
        if 'wr' not in st:
            w = jnp.broadcast_to(wr_ref[...].astype(f32).reshape(1, D), (16, D))
            st['wr'] = jnp.where(_iota((16, D), 0) == 0, w, 0.0).astype(bf16)
        return st['wr']

    stats = {}

    def stats_task(s, tt):
        def fn():
            stats[s, tt] = ln_stats(s, tt)
            inv = jnp.broadcast_to(stats[s, tt][1], (8, T))
            ties.append((clock[0] + CFG['tie_ln'], _zero_bits_after(_to_u32(inv))))
        return fn

    def norm_task(s, tt):
        return lambda: normalize(s, tt, stats[s, tt])

    def score_task(s, tt):
        return lambda: router_scores(wr_lhs(), s, tt)

    for s in range(NSEG - 1):
        for g in range(NGRP):
            at_pos(s, CFG['upd_pos'][g], lambda s=s, g=g: memory_update(s, g, [pk[s, tt] for tt in range(NT)]))
        if s == 0:
            at_pos(0, 3, stats_task(1, 0))
            at_pos(0, 5, norm_task(1, 0))
        for tt in range(NT):
            p0 = 9 + 6 * tt
            if s == 0:
                at_pos(s, p0, stats_task(2, tt))
                if tt > 0:
                    at_pos(s, p0, norm_task(3, tt - 1))
            at_pos(s, p0, lambda s=s, tt=tt: pk.__setitem__((s + 1, tt), project_k(s + 1, tt)))
            if s == 0:
                if tt > 0:
                    at_pos(s, p0, score_task(3, tt - 1))
                at_pos(s, p0 + 2, norm_task(2, tt))
                if tt + 1 < NT:
                    at_pos(s, p0 + 2, stats_task(1, tt + 1))
            at_pos(s, p0 + 2, lambda s=s, tt=tt: pq.__setitem__((s + 1, tt), project_q(s + 1, tt)))
            if s == 0:
                at_pos(s, p0 + 2, score_task(2, tt))
                if tt + 1 < NT:
                    at_pos(s, p0 + 4, norm_task(1, tt + 1))
                at_pos(s, p0 + 4, stats_task(3, tt))
            at_pos(s, p0 + 4, lambda s=s, tt=tt: project_v(s + 1, tt))
            at_pos(s, p0 + CFG['read_off'], lambda s=s, tt=tt: memory_read(s + 1, tt, pq[s + 1, tt]))
    at_pos(1, 0, norm_task(3, NT - 1))
    for s in range(EARLY):
        for tt in range(NT):
            at_pos(*CFG['early_pos'][s][tt], lambda s=s, tt=tt: out_project_early(s, tt))
    at_pos(1, 1, score_task(3, NT - 1))
    for tt in range(NT):
        at_pos(0, 1 + 2 * tt, score_task(0, tt))
        at_pos(0, 10 + 6 * tt, score_task(1, tt))

    def set_out_weight():
        wot[:, 0:D] = transpose_weight(3)
        produced('wot')

    at_pos(*CFG['wot_pos'], set_out_weight)

    at_pos(1, 2, lambda: st.update(zip(('ids', 'sel'), route())))
    at_pos(1, CFG['select_pos'], lambda: st.update(xsel=select_tokens(st['ids'])))

    def start_moe():
        with _scope('moe_wait'):
            for c in moe_copies:
                c.wait()
        queue_moe(st['xsel'], st)

    at(1, CFG['moe_quad'], -1, start_moe)

    def finish_moe():
        fill(len(fillers))
        y = moe_result(st['sel'], jnp.concatenate(st['ycols'], axis=1))
        patch_early(st['ids'], y)
        st['lhs'] = out_lhs(st['ids'], y)

    e0 = CFG['moe_end']
    at_pos(3, e0, finish_moe)
    for s in range(EARLY):
        at_pos(3, e0 + 1 + s, lambda s=s: out_copy(s * L, (s + 1) * L, s).start())
    for tt in range(NT):
        at_pos(3, e0 + 2 + CFG['op_gap'] * tt, lambda tt=tt: out_project(st['lhs'], 2, tt))
    at_pos(3, e0 + 3 + CFG['op_gap'] * (NT - 1), lambda: out_copy(2 * L, 3 * L, 2).start())

    def quad_values(s, b, j, ps):
        for a in range(4):
            values(s, 4 * b + a, j, ps[a])

    pending = []
    for s in range(NSEG):
        for b in range(NQUAD):
            for fn in slots.pop((s, b, -1), ()):
                fn()
            for j in range(NT):
                pending.append((s, b, j, scores(s, b, j)))
                for fn in slots.pop((s, b, j), ()):
                    fn()
                if len(pending) > CFG['lag']:
                    quad_values(*pending.pop(0))
    assert not slots, slots.keys()
    s = NSEG - 1

    def last_tile(tt):
        out_project(st['lhs'], s, tt, CFG['tail_parts'][tt])
        out_copy(s * L + tt * T, s * L + (tt + 1) * T, 3 + tt).start()

    done = 0
    for unit in pending:
        quad_values(*unit)
        while done < NT and unit[1] == NQUAD - 1 and done < unit[2]:
            last_tile(done)
            done += 1
    while done < NT:
        last_tile(done)
        done += 1
    with _scope('out_wait'):
        for k in range(NSEG - 1):
            out_copy(k * L, (k + 1) * L, k).wait()
        for tt in range(NT):
            out_copy(s * L + tt * T, s * L + (tt + 1) * T, 3 + tt).wait()


@jax.jit
def pallas_parallel_sum__memory_aug_infini_attn__moe_arch_mod__prompt_kernel(
    A_x: jax.Array,
    A_wq: jax.Array,
    A_wk: jax.Array,
    A_wv: jax.Array,
    A_wo: jax.Array,
    A_beta: jax.Array,
    B_x: jax.Array,
    B_w_r: jax.Array,
    B_w_gate: jax.Array,
    B_w_up: jax.Array,
    B_w_down: jax.Array,
):
    del B_x
    x_t = jnp.transpose(A_x, (0, 2, 1)).reshape(D, S)
    wd_t = B_w_down.T
    hbm = pl.BlockSpec(memory_space=pl.ANY)
    out_t = pl.pallas_call(
        _kernel,
        out_shape=jax.ShapeDtypeStruct((D, S), bf16),
        in_specs=[hbm] * 10,
        out_specs=hbm,
        scratch_shapes=[
            pltpu.VMEM((D, S), bf16),
            pltpu.VMEM((D, S), f32),
            pltpu.VMEM((4, D, D), bf16),
            pltpu.VMEM((3 * D // 2, D), u32),
            pltpu.VMEM((D // 2, 5 * T), u32),
            pltpu.VMEM((D, F), bf16),
            pltpu.VMEM((D, F), bf16),
            pltpu.VMEM((D, F), bf16),
            pltpu.VMEM((H,), bf16),
            pltpu.VMEM((D,), bf16),
            pltpu.VMEM((2, D // 2, L), u32),
            pltpu.VMEM((2, D, L), f32),
            pltpu.VMEM((2, NQUAD, L // 2, T), u32),
            pltpu.VMEM((2, NGRP, MROWS, L), f32),
            pltpu.VMEM((NGRP, MROWS, T), f32),
            pltpu.VMEM((NGRP, 8, T), f32),
            pltpu.VMEM((NSEG, 5 * T, L), f32),
            pltpu.VMEM((2 + H * S // T, 8, T), u32),
            pltpu.VMEM((2 + H * S // T, 8, T), u32),
            pltpu.VMEM((H, S), f32),
            pltpu.VMEM((NQUAD, 16, 8, T), u32),
            pltpu.VMEM((S // T, T), f32),
            pltpu.VMEM((D, S), bf16),
            pltpu.VMEM((H, T), f32),
            pltpu.VMEM((D, S), bf16),
            pltpu.VMEM((2 * D, S), bf16),
            pltpu.SemaphoreType.DMA((20,)),
        ],
        compiler_params=pltpu.CompilerParams(vmem_limit_bytes=100 * 1024 * 1024),
        name="infini_moe",
    )(x_t, A_wq, A_wk, A_wv, A_wo, A_beta, B_w_r, B_w_gate, B_w_up, wd_t)
    return jnp.transpose(out_t.reshape(1, D, S), (0, 2, 1))
```
